```python
import jax
import jax.numpy as jnp

def _softmax(x, axis=-1):
    return jax.nn.softmax(x, axis=axis)

def _gelu(x):
    return jax.nn.gelu(x, approximate=True)

def _silu(x):
    return jax.nn.silu(x)

def _sigmoid(x):
    return jax.nn.sigmoid(x)

def _layernorm(x, axis=-1, eps=1e-05):
    m = jnp.mean(x, axis=axis, keepdims=True)
    v = jnp.var(x, axis=axis, keepdims=True)
    return (x - m) / jnp.sqrt(v + eps)

def _scatter_add(tgt, idx, src, axis=0):
    return tgt.at[idx].add(src)

def _segment_sum(src, seg, n):
    return jax.ops.segment_sum(src, seg, n)

class _Rng:

    def __init__(self, key):
        self._k = key

    def _next(self):
        self._k, sub = jax.random.split(self._k)
        return sub

    def normal(self, shape):
        return jax.random.normal(self._next(), shape, dtype=jnp.bfloat16)

    def randint(self, lo, hi, shape):
        return jax.random.randint(self._next(), shape, lo, hi, dtype=jnp.int32)

    def uniform(self, shape, lo=0.0, hi=1.0):
        return jax.random.uniform(self._next(), shape, jnp.bfloat16, lo, hi)

    def permutation(self, n):
        return jax.random.permutation(self._next(), n)
kernel_name = 'concat_heads__sliding_local_dilated__memory_aug_recurrent_mem_tr__prompt'

def setup_inputs():
    _rng = _Rng(jax.random.key(int.from_bytes(__import__("os").urandom(4), "little")))
    _w = lambda a: (lambda t: t.astype(jnp.bfloat16) if jnp.issubdtype(t.dtype, jnp.floating) else t)(jnp.asarray(a))

    def _A_setup():
        B, S, D = (1, 2048, 640)
        return {'x': _w((lambda *s: _rng.normal(s) * 0.05)(B, S, D)), 'wqkv': _w((lambda *s: _rng.normal(s) * 0.05)(D, 3 * D)), 'wo': _w((lambda *s: _rng.normal(s) * 0.05)(D, D))}
    _A_in = _A_setup()

    def _B_setup():
        B, S, Dm = (1, 2048, 640)
        H, Dh = (32, 192)
        M, seg = (8, 32)
        seg = min(seg, S)
        S = S // seg * seg
        return {'x': _w((lambda *s: _rng.normal(s) * 0.05)(B, S, Dm)), 'mem0': _w((lambda *s: _rng.normal(s) * 0.05)(B, M, Dm)), 'Wq': _w((lambda *s: _rng.normal(s) * 0.05)(Dm, H, Dh) * Dm ** (-0.5)), 'Wk': _w((lambda *s: _rng.normal(s) * 0.05)(Dm, H, Dh) * Dm ** (-0.5)), 'Wv': _w((lambda *s: _rng.normal(s) * 0.05)(Dm, H, Dh) * Dm ** (-0.5)), 'Wo': _w((lambda *s: _rng.normal(s) * 0.05)(H, Dh, Dm) * (H * Dh) ** (-0.5)), 'seg_len': seg}
    _B_in = _B_setup()
    return {'A_x': _A_in['x'], 'A_wqkv': _A_in['wqkv'], 'A_wo': _A_in['wo'], 'B_x': _B_in['x'], 'B_mem0': _B_in['mem0'], 'B_Wq': _B_in['Wq'], 'B_Wk': _B_in['Wk'], 'B_Wv': _B_in['Wv'], 'B_Wo': _B_in['Wo'], 'B_seg_len': _B_in['seg_len']}

def reference(A_x, A_wqkv, A_wo, B_x, B_mem0, B_Wq, B_Wk, B_Wv, B_Wo, B_seg_len):

    def _A_ref(x, wqkv, wo):
        B, S, D = x.shape
        H = 32
        Dh = D // H
        W, dil = (8, 2)
        qkv = (lambda x, *d: x.transpose(*d))((x @ wqkv).reshape(B, S, 3, H, Dh), 2, 0, 3, 1, 4)
        q, k, v = (qkv[0], qkv[1], qkv[2])
        scale = Dh ** (-0.5)
        pos = jnp.arange(S)
        off = jnp.arange(W) * dil
        idx = pos[:, None] - off[None, :]
        mask = idx >= 0
        idx_c = jnp.where(mask, idx, 0).reshape(-1)
        kg = k[:, :, idx_c, :].reshape(B, H, S, W, Dh)
        vg = v[:, :, idx_c, :].reshape(B, H, S, W, Dh)
        logits = jnp.einsum('bhsd,bhswd->bhsw', q, kg) * scale
        logits = jnp.where(mask[None, None, :, :], logits, -1000000000.0)
        attn = _softmax(logits, axis=-1)
        o = jnp.einsum('bhsw,bhswd->bhsd', attn, vg)
        return (lambda x, *d: x.transpose(*d))(o, 0, 2, 1, 3).reshape(B, S, D) @ wo

    def _B_ref(x, mem0, Wq, Wk, Wv, Wo, seg_len):
        B, S, Dm = x.shape
        H, Dh = (Wq.shape[1], Wq.shape[2])
        M = mem0.shape[1]
        scale = Dh ** (-0.5)
        n_seg = S // seg_len
        L = M + seg_len
        idx = jnp.arange(L)
        mask = (idx[:, None] < M) | (idx[:, None] >= idx[None, :])
        mem = mem0
        outs = []
        for s in range(n_seg):
            xs = x[:, s * seg_len:(s + 1) * seg_len, :].copy()
            h = jnp.concatenate([mem, xs], axis=1)
            q = jnp.einsum('btd,dhe->bhte', h, Wq)
            k = jnp.einsum('btd,dhe->bhte', h, Wk)
            v = jnp.einsum('btd,dhe->bhte', h, Wv)
            scores = jnp.einsum('bhqe,bhke->bhqk', q, k) * scale
            scores = jnp.where(mask[None, None], scores, -1000000000.0)
            p = _softmax(scores, axis=-1)
            o = jnp.einsum('bhqk,bhke->bhqe', p, v)
            o = jnp.einsum('bhte,hed->btd', o, Wo)
            mem = o[:, :M, :].copy()
            outs.append(o[:, M:, :])
        return jnp.concatenate(outs, axis=1)
    a = _A_ref(A_x, A_wqkv, A_wo)
    b = _B_ref(B_x, B_mem0, B_Wq, B_Wk, B_Wv, B_Wo, B_seg_len)
    return jnp.concatenate([a, b], axis=-1)
```

```python
import functools

import jax
import jax.numpy as jnp
import jax.experimental.pallas as pl
import jax.experimental.pallas.tpu as pltpu

F32 = jnp.float32
BF16 = jnp.bfloat16
U32 = jnp.uint32

S = 2048
D = 640
LT = D // 128

A_H = 32
A_DH = 20
A_W = 8
A_DIL = 2
A_PAD = 16
A_CH = 256
A_NCH = S // A_CH
A_SUB = 16

B_H = 32
B_DH = 192
B_F = B_H * B_DH
B_M = 8
B_SEG = 32
B_L = B_M + B_SEG
PAIR = 2 * B_DH
NPAIR = B_H // 2
W_NCH = 8
W_ROWS = B_F // W_NCH

NEG = -1000000000.0


def _nt(a, b):
    return jax.lax.dot_general(a, b, (((1,), (1,)), ((), ())), preferred_element_type=F32)


def _nn(a, b):
    return jnp.dot(a, b, preferred_element_type=F32)


def _kernel(ax_h, wqkv_h, woa_h, bx_h, mem0_h, wq_h, wk_h, wv_h, wo_h, out_h,
            ax_v, wqkv_v, woa_v, bx_v, mem0_v, wraw_v,
            tmp_v, wqkvp_v, woap_v, slab_v, outa_v,
            wb_v, wob_v, carry_v, ocarry_v, outb_v,
            sem_in, sem_w, sem_out):
    cp_wqkv = pltpu.make_async_copy(wqkv_h, wqkv_v, sem_in.at[0])
    cp_ax = pltpu.make_async_copy(ax_h, ax_v, sem_in.at[1])
    cp_woa = pltpu.make_async_copy(woa_h, woa_v, sem_in.at[2])
    cp_mem = pltpu.make_async_copy(mem0_h, mem0_v, sem_in.at[3])
    cp_bx = pltpu.make_async_copy(bx_h, bx_v, sem_in.at[4])
    w_hs = (wq_h, wk_h, wv_h, wo_h)

    def w_copy(m, c):
        return pltpu.make_async_copy(
            w_hs[m].at[pl.ds(c * W_ROWS, W_ROWS)],
            wraw_v.at[m, pl.ds(c * W_ROWS, W_ROWS)],
            sem_w.at[m * W_NCH + c])

    cp_wqkv.start()
    cp_ax.start()
    cp_woa.start()
    cp_mem.start()
    for c in range(W_NCH):
        for m in range(4):
            w_copy(m, c).start()
    cp_bx.start()

    for t in range(3 * LT):
        slab_v[t, 0:A_PAD, :] = jnp.zeros((A_PAD, 128), F32)

    cp_wqkv.wait()
    for b in range(3 * LT):
        blk = wqkv_v[:, b * 128:(b + 1) * 128].T.astype(F32)
        for t in range(LT):
            tmp_v[t, b * 128:(b + 1) * 128, :] = blk[:, t * 128:(t + 1) * 128]
    for p in range(3):
        for d in range(A_DH):
            r = p * D + d * A_H
            for t in range(LT):
                v = tmp_v[t, pl.ds(p * D + d, A_H, stride=A_DH), :]
                wqkvp_v[r // 2:(r + A_H) // 2, t * 128:(t + 1) * 128] = pltpu.bitcast(
                    v.astype(BF16), U32)

    def a_qkv(c):
        r0 = pl.multiple_of(c * A_CH, A_CH)
        x = ax_v[pl.ds(r0, A_CH), :]
        for b in range(3 * LT):
            w = pltpu.bitcast(wqkvp_v[b * 64:(b + 1) * 64, :], BF16)
            slab_v[b, pl.ds(r0 + A_PAD, A_CH), :] = _nt(x, w)

    cp_ax.wait()
    a_qkv(0)

    cp_woa.wait()
    for t in range(LT):
        tmp_v[t, 0:D, :] = woa_v[:, t * 128:(t + 1) * 128].astype(F32)
    for d in range(A_DH):
        r = d * A_H
        for t in range(LT):
            v = tmp_v[t, pl.ds(d, A_H, stride=A_DH), :]
            woap_v[r // 2:(r + A_H) // 2, t * 128:(t + 1) * 128] = pltpu.bitcast(
                v.astype(BF16), U32)

    a_scale = A_DH ** (-0.5)

    def a_attn(c, masked):
        r0 = pl.multiple_of(c * A_CH, A_CH)
        outs = []
        for sb in range(A_CH // A_SUB):
            base = r0 + (A_PAD + sb * A_SUB)
            q = [slab_v[t, pl.ds(base, A_SUB), :] for t in range(LT)]
            logits = []
            for w in range(A_W):
                acc = None
                for t in range(LT):
                    pr = q[t] * slab_v[LT + t, pl.ds(base - A_DIL * w, A_SUB), :]
                    acc = pr if acc is None else acc + pr
                acc = acc + pltpu.roll(acc, 64, 1)
                acc = acc + pltpu.roll(acc, 32, 1)
                acc = acc * a_scale
                if masked and sb == 0 and w > 0:
                    row = jax.lax.broadcasted_iota(jnp.int32, (A_SUB, 128), 0)
                    acc = jnp.where(row >= A_DIL * w, acc, NEG)
                logits.append(acc)
            m = logits[0]
            for w in range(1, A_W):
                m = jnp.maximum(m, logits[w])
            ps = [jnp.exp(l - m) for l in logits]
            den = ps[0]
            for w in range(1, A_W):
                den = den + ps[w]
            inv = 1.0 / den
            o = []
            for t in range(LT):
                acc = None
                for w in range(A_W):
                    pr = ps[w] * slab_v[2 * LT + t, pl.ds(base - A_DIL * w, A_SUB), :]
                    acc = pr if acc is None else acc + pr
                o.append((acc * inv).astype(BF16))
            outs.append(jnp.concatenate(o, axis=1))
        o_all = jnp.concatenate(outs, axis=0)
        res = _nn(o_all, pltpu.bitcast(woap_v[...], BF16))
        outa_v[pl.ds(r0, A_CH), :] = res.astype(BF16)

    def outa_copy(c):
        r0 = pl.multiple_of(c * A_CH, A_CH)
        return pltpu.make_async_copy(
            outa_v.at[pl.ds(r0, A_CH)], out_h.at[pl.ds(r0, A_CH), pl.ds(0, D)], sem_out.at[0])

    def b_relayout(c):
        for jj in range(W_ROWS // PAIR):
            row0 = pl.multiple_of(c * W_ROWS + jj * PAIR, PAIR)
            j = c * (W_ROWS // PAIR) + jj
            for m in range(3):
                blk = wraw_v[m, pl.ds(row0, PAIR), :]
                wb_v[j, :, m * PAIR:(m + 1) * PAIR] = pltpu.bitcast(blk.T, U32)
            wob_v[j] = pltpu.bitcast(wraw_v[3, pl.ds(row0, PAIR), :], U32)

    def w_wait(c):
        for m in range(4):
            w_copy(m, c).wait()

    a_qkv(1)
    a_attn(0, True)
    outa_copy(0).start()

    def a_body(c, carry):
        w_wait(c - 1)
        b_relayout(c - 1)
        a_qkv(c + 1)
        a_attn(c, False)
        outa_copy(c).start()
        return carry

    jax.lax.fori_loop(1, A_NCH - 1, a_body, 0)
    w_wait(A_NCH - 2)
    b_relayout(A_NCH - 2)
    a_attn(A_NCH - 1, False)
    outa_copy(A_NCH - 1).start()
    w_wait(A_NCH - 1)
    b_relayout(A_NCH - 1)
    cp_mem.wait()
    cp_bx.wait()

    b_scale = B_DH ** (-0.5)
    qrow = jax.lax.broadcasted_iota(jnp.int32, (B_L, 2 * B_L), 0)
    lane = jax.lax.broadcasted_iota(jnp.int32, (B_L, 2 * B_L), 1)
    first = lane < B_L
    kcol = jnp.where(first, lane, lane - B_L)
    allowed = (qrow >= B_SEG) | (kcol >= B_SEG) | (qrow >= kcol)
    flane = jax.lax.broadcasted_iota(jnp.int32, (B_L, 128), 1)
    left = flane < 64

    def blockdiag(t):
        z = jnp.zeros((B_L, 128), F32)
        mid = t[:, 128:256]
        top = jnp.concatenate([t[:, 0:128], jnp.where(left, mid, 0.0), z], axis=1)
        bot = jnp.concatenate([z, jnp.where(left, 0.0, mid), t[:, 256:384]], axis=1)
        return jnp.concatenate([top, bot], axis=0).astype(BF16)

    def attn(seg):
        q = seg[:, 0:PAIR].astype(BF16)
        kb = blockdiag(seg[:, PAIR:2 * PAIR])
        vb = blockdiag(seg[:, 2 * PAIR:3 * PAIR])
        s = _nt(q, kb) * b_scale
        s = jnp.where(allowed, s, NEG)
        ma = jnp.max(jnp.where(first, s, -jnp.inf), axis=1, keepdims=True)
        mb = jnp.max(jnp.where(first, -jnp.inf, s), axis=1, keepdims=True)
        p = jnp.exp(s - jnp.where(first, ma, mb))
        la = jnp.sum(jnp.where(first, p, 0.0), axis=1, keepdims=True)
        lb = jnp.sum(jnp.where(first, 0.0, p), axis=1, keepdims=True)
        p = p * jnp.where(first, 1.0 / la, 1.0 / lb)
        return _nn(p.astype(BF16), vb)

    def b_body(i, mem):
        r0 = pl.multiple_of(i * 64, 64)
        x = bx_v[pl.ds(r0, 64), :].astype(F32)
        h = jnp.concatenate([x[0:40], mem], axis=0).astype(BF16)
        acc = None
        for j in range(NPAIR):
            r = _nn(h, pltpu.bitcast(wb_v[j], BF16))
            carry_v[j] = r[32:40]
            o = attn(jnp.concatenate([r[0:32], r[40:48]], axis=0))
            ocarry_v[j] = o[24:32]
            lhs = jnp.concatenate([o[0:24], o[32:40]], axis=0).astype(BF16)
            d = _nn(lhs, pltpu.bitcast(wob_v[j], BF16))
            acc = d if acc is None else acc + d
        out_e = acc[0:24]
        mem = acc[24:32].astype(BF16).astype(F32)
        h = jnp.concatenate([x[40:64], mem], axis=0).astype(BF16)
        acc = None
        for j in range(NPAIR):
            r = _nn(h, pltpu.bitcast(wb_v[j], BF16))
            o = attn(jnp.concatenate([carry_v[j], r], axis=0))
            lhs = jnp.concatenate([o[0:32], ocarry_v[j], o[32:40]], axis=0).astype(BF16)
            d = _nn(lhs, pltpu.bitcast(wob_v[j], BF16))
            acc = d if acc is None else acc + d
        out = jnp.concatenate([out_e, acc[32:40], acc[0:32]], axis=0)
        outb_v[pl.ds(r0, 64), :] = out.astype(BF16)
        pltpu.make_async_copy(
            outb_v.at[pl.ds(r0, 64)], out_h.at[pl.ds(r0, 64), pl.ds(D, D)], sem_out.at[1]).start()
        return acc[40:48].astype(BF16).astype(F32)

    jax.lax.fori_loop(0, S // 64, b_body, mem0_v[...].astype(F32))

    pltpu.make_async_copy(outa_v, out_h.at[:, pl.ds(0, D)], sem_out.at[0]).wait()
    pltpu.make_async_copy(outb_v, out_h.at[:, pl.ds(D, D)], sem_out.at[1]).wait()


@functools.partial(jax.jit, static_argnames=("B_seg_len",))
def pallas_concat_heads__sliding_local_dilated__memory_aug_recurrent_mem_tr__prompt_kernel(
    A_x: jax.Array,
    A_wqkv: jax.Array,
    A_wo: jax.Array,
    B_x: jax.Array,
    B_mem0: jax.Array,
    B_Wq: jax.Array,
    B_Wk: jax.Array,
    B_Wv: jax.Array,
    B_Wo: jax.Array,
    B_seg_len: int,
):
    assert A_x.shape == (1, S, D) and B_x.shape == (1, S, D)
    assert B_seg_len == B_SEG and B_mem0.shape == (1, B_M, D)
    assert B_Wq.shape == (D, B_H, B_DH) and B_Wo.shape == (B_H, B_DH, D)

    def feat_major(w):
        return jnp.transpose(w, (1, 2, 0)).reshape(B_F, D)

    any_spec = pl.BlockSpec(memory_space=pl.ANY)
    out = pl.pallas_call(
        _kernel,
        out_shape=jax.ShapeDtypeStruct((S, 2 * D), BF16),
        in_specs=[any_spec] * 9,
        out_specs=any_spec,
        scratch_shapes=[
            pltpu.VMEM((S, D), BF16),
            pltpu.VMEM((D, 3 * D), BF16),
            pltpu.VMEM((D, D), BF16),
            pltpu.VMEM((S, D), BF16),
            pltpu.VMEM((B_M, D), BF16),
            pltpu.VMEM((4, B_F, D), BF16),
            pltpu.VMEM((LT, 3 * D, 128), F32),
            pltpu.VMEM((3 * D // 2, D), U32),
            pltpu.VMEM((D // 2, D), U32),
            pltpu.VMEM((3 * LT, A_PAD + S, 128), F32),
            pltpu.VMEM((S, D), BF16),
            pltpu.VMEM((NPAIR, D // 2, 3 * PAIR), U32),
            pltpu.VMEM((NPAIR, PAIR // 2, D), U32),
            pltpu.VMEM((NPAIR, 8, 3 * PAIR), F32),
            pltpu.VMEM((NPAIR, 8, PAIR), F32),
            pltpu.VMEM((S, D), BF16),
            pltpu.SemaphoreType.DMA((5,)),
            pltpu.SemaphoreType.DMA((4 * W_NCH,)),
            pltpu.SemaphoreType.DMA((2,)),
        ],
        compiler_params=pltpu.CompilerParams(vmem_limit_bytes=120 * 1024 * 1024),
    )(
        A_x.reshape(S, D), A_wqkv, A_wo, B_x.reshape(S, D), B_mem0.reshape(B_M, D),
        feat_major(B_Wq), feat_major(B_Wk), feat_major(B_Wv), B_Wo.reshape(B_F, D),
    )
    return out.reshape(1, S, 2 * D)
```

```python
import functools

import jax
import jax.numpy as jnp
import jax.experimental.pallas as pl
import jax.experimental.pallas.tpu as pltpu

F32 = jnp.float32
BF16 = jnp.bfloat16
U32 = jnp.uint32

S = 2048
D = 640
LT = D // 128

A_H = 32
A_DH = 20
A_W = 8
A_DIL = 2
A_PAD = 16
A_CH = 256
A_NCH = S // A_CH
A_SUB = 16

B_H = 32
B_DH = 192
B_F = B_H * B_DH
B_M = 8
B_SEG = 32
B_L = B_M + B_SEG
PAIR = 2 * B_DH
NPAIR = B_H // 2
W_NCH = 8
W_ROWS = B_F // W_NCH

NEG = -1000000000.0
LAG_S, LAG_V, LAG_O = 1, 2, 4


def _nt(a, b):
    return jax.lax.dot_general(a, b, (((1,), (1,)), ((), ())), preferred_element_type=F32)


def _nn(a, b):
    return jnp.dot(a, b, preferred_element_type=F32)


def _kernel(ax_h, wqkv_h, woa_h, bx_h, mem0_h, wq_h, wk_h, wv_h, wo_h, out_h,
            ax_v, wqkv_v, woa_v, bx_v, mem0_v, wraw_v,
            tmp_v, wqkvp_v, woap_v, slab_v, outa_v,
            wb_v, wob_v, carry_v, ocarry_v, outb_v,
            sem_in, sem_w, sem_out):
    cp_wqkv = pltpu.make_async_copy(wqkv_h, wqkv_v, sem_in.at[0])
    cp_ax = pltpu.make_async_copy(ax_h, ax_v, sem_in.at[1])
    cp_woa = pltpu.make_async_copy(woa_h, woa_v, sem_in.at[2])
    cp_mem = pltpu.make_async_copy(mem0_h, mem0_v, sem_in.at[3])
    cp_bx = pltpu.make_async_copy(bx_h, bx_v, sem_in.at[4])
    w_hs = (wq_h, wk_h, wv_h, wo_h)

    def w_copy(m, c):
        return pltpu.make_async_copy(
            w_hs[m].at[pl.ds(c * W_ROWS, W_ROWS)],
            wraw_v.at[m, pl.ds(c * W_ROWS, W_ROWS)],
            sem_w.at[m * W_NCH + c])

    cp_wqkv.start()
    cp_ax.start()
    cp_woa.start()
    cp_mem.start()
    for c in range(W_NCH):
        for m in range(4):
            w_copy(m, c).start()
    cp_bx.start()

    for t in range(3 * LT):
        slab_v[t, 0:A_PAD, :] = jnp.zeros((A_PAD, 128), F32)

    cp_wqkv.wait()
    for b in range(3 * LT):
        blk = wqkv_v[:, b * 128:(b + 1) * 128].T.astype(F32)
        for t in range(LT):
            tmp_v[t, b * 128:(b + 1) * 128, :] = blk[:, t * 128:(t + 1) * 128]
    for p in range(3):
        for d in range(A_DH):
            r = p * D + d * A_H
            for t in range(LT):
                v = tmp_v[t, pl.ds(p * D + d, A_H, stride=A_DH), :]
                wqkvp_v[r // 2:(r + A_H) // 2, t * 128:(t + 1) * 128] = pltpu.bitcast(
                    v.astype(BF16), U32)

    def a_qkv(c):
        r0 = pl.multiple_of(c * A_CH, A_CH)
        x = ax_v[pl.ds(r0, A_CH), :]
        for b in range(3 * LT):
            w = pltpu.bitcast(wqkvp_v[b * 64:(b + 1) * 64, :], BF16)
            slab_v[b, pl.ds(r0 + A_PAD, A_CH), :] = _nt(x, w)

    cp_ax.wait()
    a_qkv(0)

    cp_woa.wait()
    for t in range(LT):
        tmp_v[t, 0:D, :] = woa_v[:, t * 128:(t + 1) * 128].astype(F32)
    for d in range(A_DH):
        r = d * A_H
        for t in range(LT):
            v = tmp_v[t, pl.ds(d, A_H, stride=A_DH), :]
            woap_v[r // 2:(r + A_H) // 2, t * 128:(t + 1) * 128] = pltpu.bitcast(
                v.astype(BF16), U32)

    a_scale = A_DH ** (-0.5)

    def a_attn(c, masked):
        r0 = pl.multiple_of(c * A_CH, A_CH)
        outs = []
        for sb in range(A_CH // A_SUB):
            base = r0 + (A_PAD + sb * A_SUB)
            q = [slab_v[t, pl.ds(base, A_SUB), :] for t in range(LT)]
            logits = []
            for w in range(A_W):
                acc = None
                for t in range(LT):
                    pr = q[t] * slab_v[LT + t, pl.ds(base - A_DIL * w, A_SUB), :]
                    acc = pr if acc is None else acc + pr
                acc = acc + pltpu.roll(acc, 64, 1)
                acc = acc + pltpu.roll(acc, 32, 1)
                acc = acc * a_scale
                if masked and sb == 0 and w > 0:
                    row = jax.lax.broadcasted_iota(jnp.int32, (A_SUB, 128), 0)
                    acc = jnp.where(row >= A_DIL * w, acc, NEG)
                logits.append(acc)
            m = logits[0]
            for w in range(1, A_W):
                m = jnp.maximum(m, logits[w])
            ps = [jnp.exp(l - m) for l in logits]
            den = ps[0]
            for w in range(1, A_W):
                den = den + ps[w]
            inv = 1.0 / den
            o = []
            for t in range(LT):
                acc = None
                for w in range(A_W):
                    pr = ps[w] * slab_v[2 * LT + t, pl.ds(base - A_DIL * w, A_SUB), :]
                    acc = pr if acc is None else acc + pr
                o.append((acc * inv).astype(BF16))
            outs.append(jnp.concatenate(o, axis=1))
        o_all = jnp.concatenate(outs, axis=0)
        res = _nn(o_all, pltpu.bitcast(woap_v[...], BF16))
        outa_v[pl.ds(r0, A_CH), :] = res.astype(BF16)

    def outa_copy(c):
        r0 = pl.multiple_of(c * A_CH, A_CH)
        return pltpu.make_async_copy(
            outa_v.at[pl.ds(r0, A_CH)], out_h.at[pl.ds(r0, A_CH), pl.ds(0, D)], sem_out.at[0])

    def b_relayout(c):
        for jj in range(W_ROWS // PAIR):
            row0 = pl.multiple_of(c * W_ROWS + jj * PAIR, PAIR)
            j = c * (W_ROWS // PAIR) + jj
            for m in range(3):
                blk = wraw_v[m, pl.ds(row0, PAIR), :]
                wb_v[j, :, m * PAIR:(m + 1) * PAIR] = pltpu.bitcast(blk.T, U32)
            wob_v[j] = pltpu.bitcast(wraw_v[3, pl.ds(row0, PAIR), :], U32)

    def w_wait(c):
        for m in range(4):
            w_copy(m, c).wait()

    a_qkv(1)
    a_attn(0, True)
    outa_copy(0).start()

    def a_body(c, carry):
        w_wait(c - 1)
        b_relayout(c - 1)
        a_qkv(c + 1)
        a_attn(c, False)
        outa_copy(c).start()
        return carry

    jax.lax.fori_loop(1, A_NCH - 1, a_body, 0)
    w_wait(A_NCH - 2)
    b_relayout(A_NCH - 2)
    a_attn(A_NCH - 1, False)
    outa_copy(A_NCH - 1).start()
    w_wait(A_NCH - 1)
    b_relayout(A_NCH - 1)
    cp_mem.wait()
    cp_bx.wait()

    b_scale = B_DH ** (-0.5)
    qrow = jax.lax.broadcasted_iota(jnp.int32, (B_L, 2 * B_L), 0)
    lane = jax.lax.broadcasted_iota(jnp.int32, (B_L, 2 * B_L), 1)
    first = lane < B_L
    kcol = jnp.where(first, lane, lane - B_L)
    allowed = (qrow >= B_SEG) | (kcol >= B_SEG) | (qrow >= kcol)
    flane = jax.lax.broadcasted_iota(jnp.int32, (B_L, 128), 1)
    left = flane < 64

    def blockdiag(t):
        z = jnp.zeros((B_L, 128), F32)
        mid = t[:, 128:256]
        top = jnp.concatenate([t[:, 0:128], jnp.where(left, mid, 0.0), z], axis=1)
        bot = jnp.concatenate([z, jnp.where(left, 0.0, mid), t[:, 256:384]], axis=1)
        return jnp.concatenate([top, bot], axis=0).astype(BF16)

    def softmax(s):
        s = jnp.where(allowed, s * b_scale, NEG)
        ma = jnp.max(jnp.where(first, s, -jnp.inf), axis=1, keepdims=True)
        mb = jnp.max(jnp.where(first, -jnp.inf, s), axis=1, keepdims=True)
        p = jnp.exp(s - jnp.where(first, ma, mb))
        la = jnp.sum(jnp.where(first, p, 0.0), axis=1, keepdims=True)
        lb = jnp.sum(jnp.where(first, 0.0, p), axis=1, keepdims=True)
        l = jnp.where(first, la, lb)
        r = pl.reciprocal(l, approx=True)
        r = r * (2.0 - l * r)
        return (p * r).astype(BF16)

    def segment(h, even):
        qkv, prob, att = {}, {}, {}
        acc = [None]

        def proj(j):
            r = _nn(h, pltpu.bitcast(wb_v[j], BF16))
            if even:
                carry_v[j] = r[32:40]
                seg = jnp.concatenate([r[0:32], r[40:48]], axis=0)
            else:
                seg = jnp.concatenate([carry_v[j], r], axis=0)
            qkv[j] = (seg[:, 0:PAIR].astype(BF16), blockdiag(seg[:, PAIR:2 * PAIR]),
                      blockdiag(seg[:, 2 * PAIR:3 * PAIR]))

        def scores(j):
            prob[j] = softmax(_nt(qkv[j][0], qkv[j][1]))

        def values(j):
            o = _nn(prob[j], qkv[j][2])
            if even:
                ocarry_v[j] = o[24:32]
                lhs = jnp.concatenate([o[0:24], o[32:40]], axis=0)
            else:
                lhs = jnp.concatenate([o[0:32], ocarry_v[j], o[32:40]], axis=0)
            att[j] = lhs.astype(BF16)

        def outp(j):
            d = _nn(att[j], pltpu.bitcast(wob_v[j], BF16))
            acc[0] = d if acc[0] is None else acc[0] + d

        stages = ((proj, 0), (scores, LAG_S), (values, LAG_V), (outp, LAG_O))
        for t in range(NPAIR + LAG_O):
            for fn, lag in stages:
                if 0 <= t - lag < NPAIR:
                    fn(t - lag)
        return acc[0]

    def b_body(i, mem):
        r0 = pl.multiple_of(i * 64, 64)
        x = bx_v[pl.ds(r0, 64), :].astype(F32)
        acc = segment(jnp.concatenate([x[0:40], mem], axis=0).astype(BF16), True)
        out_e = acc[0:24]
        mem = acc[24:32].astype(BF16).astype(F32)
        acc = segment(jnp.concatenate([x[40:64], mem], axis=0).astype(BF16), False)
        out = jnp.concatenate([out_e, acc[32:40], acc[0:32]], axis=0)
        outb_v[pl.ds(r0, 64), :] = out.astype(BF16)
        pltpu.make_async_copy(
            outb_v.at[pl.ds(r0, 64)], out_h.at[pl.ds(r0, 64), pl.ds(D, D)], sem_out.at[1]).start()
        return acc[40:48].astype(BF16).astype(F32)

    jax.lax.fori_loop(0, S // 64, b_body, mem0_v[...].astype(F32))

    pltpu.make_async_copy(outa_v, out_h.at[:, pl.ds(0, D)], sem_out.at[0]).wait()
    pltpu.make_async_copy(outb_v, out_h.at[:, pl.ds(D, D)], sem_out.at[1]).wait()


@functools.partial(jax.jit, static_argnames=("B_seg_len",))
def pallas_concat_heads__sliding_local_dilated__memory_aug_recurrent_mem_tr__prompt_kernel(
    A_x: jax.Array,
    A_wqkv: jax.Array,
    A_wo: jax.Array,
    B_x: jax.Array,
    B_mem0: jax.Array,
    B_Wq: jax.Array,
    B_Wk: jax.Array,
    B_Wv: jax.Array,
    B_Wo: jax.Array,
    B_seg_len: int,
):
    assert A_x.shape == (1, S, D) and B_x.shape == (1, S, D)
    assert B_seg_len == B_SEG and B_mem0.shape == (1, B_M, D)
    assert B_Wq.shape == (D, B_H, B_DH) and B_Wo.shape == (B_H, B_DH, D)

    def feat_major(w):
        return jnp.transpose(w, (1, 2, 0)).reshape(B_F, D)

    any_spec = pl.BlockSpec(memory_space=pl.ANY)
    out = pl.pallas_call(
        _kernel,
        out_shape=jax.ShapeDtypeStruct((S, 2 * D), BF16),
        in_specs=[any_spec] * 9,
        out_specs=any_spec,
        scratch_shapes=[
            pltpu.VMEM((S, D), BF16),
            pltpu.VMEM((D, 3 * D), BF16),
            pltpu.VMEM((D, D), BF16),
            pltpu.VMEM((S, D), BF16),
            pltpu.VMEM((B_M, D), BF16),
            pltpu.VMEM((4, B_F, D), BF16),
            pltpu.VMEM((LT, 3 * D, 128), F32),
            pltpu.VMEM((3 * D // 2, D), U32),
            pltpu.VMEM((D // 2, D), U32),
            pltpu.VMEM((3 * LT, A_PAD + S, 128), F32),
            pltpu.VMEM((S, D), BF16),
            pltpu.VMEM((NPAIR, D // 2, 3 * PAIR), U32),
            pltpu.VMEM((NPAIR, PAIR // 2, D), U32),
            pltpu.VMEM((NPAIR, 8, 3 * PAIR), F32),
            pltpu.VMEM((NPAIR, 8, PAIR), F32),
            pltpu.VMEM((S, D), BF16),
            pltpu.SemaphoreType.DMA((5,)),
            pltpu.SemaphoreType.DMA((4 * W_NCH,)),
            pltpu.SemaphoreType.DMA((2,)),
        ],
        compiler_params=pltpu.CompilerParams(vmem_limit_bytes=120 * 1024 * 1024),
    )(
        A_x.reshape(S, D), A_wqkv, A_wo, B_x.reshape(S, D), B_mem0.reshape(B_M, D),
        feat_major(B_Wq), feat_major(B_Wk), feat_major(B_Wv), B_Wo.reshape(B_F, D),
    )
    return out.reshape(1, S, 2 * D)
```

```python
import functools

import jax
import jax.numpy as jnp
import jax.experimental.pallas as pl
import jax.experimental.pallas.tpu as pltpu

F32 = jnp.float32
BF16 = jnp.bfloat16
U32 = jnp.uint32

S = 2048
D = 640
LT = D // 128

A_H = 32
A_DH = 20
A_W = 8
A_DIL = 2
A_PAD = 16
A_CH = 256
A_NCH = S // A_CH
A_SUB = 16

B_H = 32
B_DH = 192
B_F = B_H * B_DH
B_M = 8
B_SEG = 32
B_L = B_M + B_SEG
PAIR = 2 * B_DH
NPAIR = B_H // 2
W_NCH = 8
W_ROWS = B_F // W_NCH

NEG = -1000000000.0
LAG_S, LAG_V, LAG_O = 1, 2, 4


def _nt(a, b):
    return jax.lax.dot_general(a, b, (((1,), (1,)), ((), ())), preferred_element_type=F32)


def _nn(a, b):
    return jnp.dot(a, b, preferred_element_type=F32)


def _kernel(ax_h, wqkv_h, woa_h, bx_h, mem0_h, wq_h, wk_h, wv_h, wo_h, out_h,
            ax_v, wqkv_v, woa_v, bx_v, mem0_v, wraw_v,
            tmp_v, wqkvp_v, woap_v, slab_v, outa_v,
            wb_v, wob_v, carry_v, ocarry_v, outb_v,
            sem_in, sem_out):
    cp_wqkv = pltpu.make_async_copy(wqkv_h, wqkv_v, sem_in.at[0])
    cp_ax = pltpu.make_async_copy(ax_h, ax_v, sem_in.at[1])
    cp_woa = pltpu.make_async_copy(woa_h, woa_v, sem_in.at[2])
    cp_mem = pltpu.make_async_copy(mem0_h, mem0_v, sem_in.at[3])
    cp_bx = pltpu.make_async_copy(bx_h, bx_v, sem_in.at[4])
    w_hs = (wq_h, wk_h, wv_h, wo_h)

    def w_copy(m, c):
        return pltpu.make_async_copy(
            w_hs[m].at[pl.ds(c * W_ROWS, W_ROWS)],
            wraw_v.at[m, pl.ds(c * W_ROWS, W_ROWS)],
            sem_in.at[5 + m * W_NCH + c])

    cp_wqkv.start()
    cp_ax.start()
    cp_woa.start()
    cp_mem.start()
    for c in range(W_NCH):
        for m in range(4):
            w_copy(m, c).start()
    cp_bx.start()

    for t in range(3 * LT):
        slab_v[t, 0:A_PAD, :] = jnp.zeros((A_PAD, 128), F32)

    cp_wqkv.wait()
    for b in range(3 * LT):
        blk = wqkv_v[:, b * 128:(b + 1) * 128].T.astype(F32)
        for t in range(LT):
            tmp_v[t, b * 128:(b + 1) * 128, :] = blk[:, t * 128:(t + 1) * 128]
    for p in range(3):
        for d in range(A_DH):
            r = p * D + d * A_H
            for t in range(LT):
                v = tmp_v[t, pl.ds(p * D + d, A_H, stride=A_DH), :]
                wqkvp_v[r // 2:(r + A_H) // 2, t * 128:(t + 1) * 128] = pltpu.bitcast(
                    v.astype(BF16), U32)

    def a_qkv(c):
        r0 = pl.multiple_of(c * A_CH, A_CH)
        x = ax_v[pl.ds(r0, A_CH), :]
        for b in range(3 * LT):
            w = pltpu.bitcast(wqkvp_v[b * 64:(b + 1) * 64, :], BF16)
            slab_v[b, pl.ds(r0 + A_PAD, A_CH), :] = _nt(x, w)

    cp_ax.wait()
    a_qkv(0)

    cp_woa.wait()
    for t in range(LT):
        tmp_v[t, 0:D, :] = woa_v[:, t * 128:(t + 1) * 128].astype(F32)
    for d in range(A_DH):
        r = d * A_H
        for t in range(LT):
            v = tmp_v[t, pl.ds(d, A_H, stride=A_DH), :]
            woap_v[r // 2:(r + A_H) // 2, t * 128:(t + 1) * 128] = pltpu.bitcast(
                v.astype(BF16), U32)

    a_scale = A_DH ** (-0.5)

    def a_attn(c, masked):
        r0 = pl.multiple_of(c * A_CH, A_CH)
        outs = []
        for sb in range(A_CH // A_SUB):
            base = r0 + (A_PAD + sb * A_SUB)
            q = [slab_v[t, pl.ds(base, A_SUB), :] for t in range(LT)]
            logits = []
            for w in range(A_W):
                acc = None
                for t in range(LT):
                    pr = q[t] * slab_v[LT + t, pl.ds(base - A_DIL * w, A_SUB), :]
                    acc = pr if acc is None else acc + pr
                acc = acc + pltpu.roll(acc, 64, 1)
                acc = acc + pltpu.roll(acc, 32, 1)
                acc = acc * a_scale
                if masked and sb == 0 and w > 0:
                    row = jax.lax.broadcasted_iota(jnp.int32, (A_SUB, 128), 0)
                    acc = jnp.where(row >= A_DIL * w, acc, NEG)
                logits.append(acc)
            m = logits[0]
            for w in range(1, A_W):
                m = jnp.maximum(m, logits[w])
            ps = [jnp.exp(l - m) for l in logits]
            den = ps[0]
            for w in range(1, A_W):
                den = den + ps[w]
            inv = 1.0 / den
            o = []
            for t in range(LT):
                acc = None
                for w in range(A_W):
                    pr = ps[w] * slab_v[2 * LT + t, pl.ds(base - A_DIL * w, A_SUB), :]
                    acc = pr if acc is None else acc + pr
                o.append((acc * inv).astype(BF16))
            outs.append(jnp.concatenate(o, axis=1))
        o_all = jnp.concatenate(outs, axis=0)
        res = _nn(o_all, pltpu.bitcast(woap_v[...], BF16))
        outa_v[pl.ds(r0, A_CH), :] = res.astype(BF16)

    def outa_copy(c):
        r0 = pl.multiple_of(c * A_CH, A_CH)
        return pltpu.make_async_copy(
            outa_v.at[pl.ds(r0, A_CH)], out_h.at[pl.ds(r0, A_CH), pl.ds(0, D)], sem_out.at[0])

    def b_relayout(c):
        for jj in range(W_ROWS // PAIR):
            row0 = pl.multiple_of(c * W_ROWS + jj * PAIR, PAIR)
            j = c * (W_ROWS // PAIR) + jj
            for m in range(3):
                blk = wraw_v[m, pl.ds(row0, PAIR), :]
                wb_v[j, :, m * PAIR:(m + 1) * PAIR] = pltpu.bitcast(blk.T, U32)
            wob_v[j] = pltpu.bitcast(wraw_v[3, pl.ds(row0, PAIR), :], U32)

    def w_wait(c):
        for m in range(4):
            w_copy(m, c).wait()

    a_qkv(1)
    a_attn(0, True)
    outa_copy(0).start()

    def a_body(c, carry):
        w_wait(c - 1)
        b_relayout(c - 1)
        a_qkv(c + 1)
        a_attn(c, False)
        outa_copy(c).start()
        return carry

    jax.lax.fori_loop(1, A_NCH - 1, a_body, 0)
    w_wait(A_NCH - 2)
    b_relayout(A_NCH - 2)
    a_attn(A_NCH - 1, False)
    outa_copy(A_NCH - 1).start()
    w_wait(A_NCH - 1)
    b_relayout(A_NCH - 1)
    cp_mem.wait()
    cp_bx.wait()

    b_scale = B_DH ** (-0.5)
    qrow = jax.lax.broadcasted_iota(jnp.int32, (B_L, 2 * B_L), 0)
    lane = jax.lax.broadcasted_iota(jnp.int32, (B_L, 2 * B_L), 1)
    first = lane < B_L
    kcol = jnp.where(first, lane, lane - B_L)
    allowed = (qrow >= B_SEG) | (kcol >= B_SEG) | (qrow >= kcol)
    flane = jax.lax.broadcasted_iota(jnp.int32, (B_L, 128), 1)
    left = flane < 64

    def blockdiag(t):
        z = jnp.zeros((B_L, 128), F32)
        mid = t[:, 128:256]
        top = jnp.concatenate([t[:, 0:128], jnp.where(left, mid, 0.0), z], axis=1)
        bot = jnp.concatenate([z, jnp.where(left, 0.0, mid), t[:, 256:384]], axis=1)
        return jnp.concatenate([top, bot], axis=0).astype(BF16)

    def softmax(s):
        s = jnp.where(allowed, s * b_scale, NEG)
        ma = jnp.max(jnp.where(first, s, -jnp.inf), axis=1, keepdims=True)
        mb = jnp.max(jnp.where(first, -jnp.inf, s), axis=1, keepdims=True)
        p = jnp.exp(s - jnp.where(first, ma, mb))
        la = jnp.sum(jnp.where(first, p, 0.0), axis=1, keepdims=True)
        lb = jnp.sum(jnp.where(first, 0.0, p), axis=1, keepdims=True)
        l = jnp.where(first, la, lb)
        r = pl.reciprocal(l, approx=True)
        r = r * (2.0 - l * r)
        return (p * r).astype(BF16)

    def segment(h, even):
        qkv, prob, att = {}, {}, {}
        acc = [None]

        def proj(j):
            r = _nn(h, pltpu.bitcast(wb_v[j], BF16))
            if even:
                carry_v[j] = r[32:40]
                seg = jnp.concatenate([r[0:32], r[40:48]], axis=0)
            else:
                seg = jnp.concatenate([carry_v[j], r], axis=0)
            qkv[j] = (seg[:, 0:PAIR].astype(BF16), blockdiag(seg[:, PAIR:2 * PAIR]),
                      blockdiag(seg[:, 2 * PAIR:3 * PAIR]))

        def scores(j):
            prob[j] = softmax(_nt(qkv[j][0], qkv[j][1]))

        def values(j):
            o = _nn(prob[j], qkv[j][2])
            if even:
                ocarry_v[j] = o[24:32]
                lhs = jnp.concatenate([o[0:24], o[32:40]], axis=0)
            else:
                lhs = jnp.concatenate([o[0:32], ocarry_v[j], o[32:40]], axis=0)
            att[j] = lhs.astype(BF16)

        def outp(j):
            d = _nn(att[j], pltpu.bitcast(wob_v[j], BF16))
            acc[0] = d if acc[0] is None else acc[0] + d

        stages = ((proj, 0), (scores, LAG_S), (values, LAG_V), (outp, LAG_O))
        for t in range(NPAIR + LAG_O):
            for fn, lag in stages:
                if 0 <= t - lag < NPAIR:
                    fn(t - lag)
        return acc[0]

    def b_body(i, mem):
        r0 = pl.multiple_of(i * 64, 64)
        x = bx_v[pl.ds(r0, 64), :].astype(F32)
        acc = segment(jnp.concatenate([x[0:40], mem], axis=0).astype(BF16), True)
        out_e = acc[0:24]
        mem = acc[24:32].astype(BF16).astype(F32)
        acc = segment(jnp.concatenate([x[40:64], mem], axis=0).astype(BF16), False)
        out = jnp.concatenate([out_e, acc[32:40], acc[0:32]], axis=0)
        outb_v[pl.ds(r0, 64), :] = out.astype(BF16)
        pltpu.make_async_copy(
            outb_v.at[pl.ds(r0, 64)], out_h.at[pl.ds(r0, 64), pl.ds(D, D)], sem_out.at[1]).start()
        return acc[40:48].astype(BF16).astype(F32)

    jax.lax.fori_loop(0, S // 64, b_body, mem0_v[...].astype(F32))

    pltpu.make_async_copy(outa_v, out_h.at[:, pl.ds(0, D)], sem_out.at[0]).wait()
    pltpu.make_async_copy(outb_v, out_h.at[:, pl.ds(D, D)], sem_out.at[1]).wait()


@functools.partial(jax.jit, static_argnames=("B_seg_len",))
def pallas_concat_heads__sliding_local_dilated__memory_aug_recurrent_mem_tr__prompt_kernel(
    A_x: jax.Array,
    A_wqkv: jax.Array,
    A_wo: jax.Array,
    B_x: jax.Array,
    B_mem0: jax.Array,
    B_Wq: jax.Array,
    B_Wk: jax.Array,
    B_Wv: jax.Array,
    B_Wo: jax.Array,
    B_seg_len: int,
):
    assert A_x.shape == (1, S, D) and B_x.shape == (1, S, D)
    assert B_seg_len == B_SEG and B_mem0.shape == (1, B_M, D)
    assert B_Wq.shape == (D, B_H, B_DH) and B_Wo.shape == (B_H, B_DH, D)

    def feat_major(w):
        return jnp.transpose(w, (1, 2, 0)).reshape(B_F, D)

    any_spec = pl.BlockSpec(memory_space=pl.ANY)
    out = pl.pallas_call(
        _kernel,
        out_shape=jax.ShapeDtypeStruct((S, 2 * D), BF16),
        in_specs=[any_spec] * 9,
        out_specs=any_spec,
        scratch_shapes=[
            pltpu.VMEM((S, D), BF16),
            pltpu.VMEM((D, 3 * D), BF16),
            pltpu.VMEM((D, D), BF16),
            pltpu.VMEM((S, D), BF16),
            pltpu.VMEM((B_M, D), BF16),
            pltpu.VMEM((4, B_F, D), BF16),
            pltpu.VMEM((LT, 3 * D, 128), F32),
            pltpu.VMEM((3 * D // 2, D), U32),
            pltpu.VMEM((D // 2, D), U32),
            pltpu.VMEM((3 * LT, A_PAD + S, 128), F32),
            pltpu.VMEM((S, D), BF16),
            pltpu.VMEM((NPAIR, D // 2, 3 * PAIR), U32),
            pltpu.VMEM((NPAIR, PAIR // 2, D), U32),
            pltpu.VMEM((NPAIR, 8, 3 * PAIR), F32),
            pltpu.VMEM((NPAIR, 8, PAIR), F32),
            pltpu.VMEM((S, D), BF16),
            pltpu.SemaphoreType.DMA((5 + 4 * W_NCH,)),
            pltpu.SemaphoreType.DMA((2,)),
        ],
        compiler_params=pltpu.CompilerParams(vmem_limit_bytes=120 * 1024 * 1024),
    )(
        A_x.reshape(S, D), A_wqkv, A_wo, B_x.reshape(S, D), B_mem0.reshape(B_M, D),
        feat_major(B_Wq), feat_major(B_Wk), feat_major(B_Wv), B_Wo.reshape(B_F, D),
    )
    return out.reshape(1, S, 2 * D)
```

```python
import functools

import jax
import jax.numpy as jnp
import jax.experimental.pallas as pl
import jax.experimental.pallas.tpu as pltpu

F32 = jnp.float32
BF16 = jnp.bfloat16
U32 = jnp.uint32

S = 2048
D = 640
LT = D // 128
BLK = 64
NIT = S // BLK

A_H = 32
A_DH = 20
A_W = 8
A_DIL = 2
A_PAD = 16
A_SUB = 16

B_H = 32
B_DH = 192
B_F = B_H * B_DH
B_M = 8
B_SEG = 32
B_L = B_M + B_SEG
PAIR = 2 * B_DH
NPAIR = B_H // 2
W_NCH = 8
W_ROWS = B_F // W_NCH
PRE = 16
PRE_MB = 128

NEG = -1000000000.0
LAG_S, LAG_V, LAG_O = 1, 2, 4


def _nt(a, b):
    return jax.lax.dot_general(a, b, (((1,), (1,)), ((), ())), preferred_element_type=F32)


def _nn(a, b):
    return jnp.dot(a, b, preferred_element_type=F32)


def _recip(x):
    r = pl.reciprocal(x, approx=True)
    return r * (2.0 - x * r)


def _kernel(ax_h, wqkv_h, woa_h, bx_h, mem0_h, wq_h, wk_h, wv_h, wo_h, out_h,
            ax_v, wqkv_v, woa_v, bx_v, xpre_v, mem0_v, wraw_v,
            tmp_v, wqkvt_v, wqkvp_v, woap_v, slab_v, outa_v,
            wb_v, wob_v, pre_v, carry_v, ocarry_v, outb_v,
            sem_in, sem_out):
    cp_xpre = pltpu.make_async_copy(bx_h.at[:, pl.ds(0, PRE), :], xpre_v, sem_in.at[0])
    cp_wqkv = pltpu.make_async_copy(wqkv_h, wqkv_v, sem_in.at[1])
    cp_woa = pltpu.make_async_copy(woa_h, woa_v, sem_in.at[2])
    cp_mem = pltpu.make_async_copy(mem0_h, mem0_v, sem_in.at[3])
    cp_bx = pltpu.make_async_copy(bx_h, bx_v, sem_in.at[4])
    cp_ax = pltpu.make_async_copy(ax_h, ax_v, sem_in.at[5])
    w_hs = (wq_h, wk_h, wv_h, wo_h)

    def w_copy(m, c):
        return pltpu.make_async_copy(
            w_hs[m].at[pl.ds(c * W_ROWS, W_ROWS)],
            wraw_v.at[m, pl.ds(c * W_ROWS, W_ROWS)],
            sem_in.at[6 + m * W_NCH + c])

    cp_xpre.start()
    for c in range(W_NCH):
        for m in range(4):
            w_copy(m, c).start()
    cp_wqkv.start()
    cp_woa.start()
    cp_mem.start()
    cp_bx.start()
    cp_ax.start()

    def b_pre(c, m):
        for jj in range(W_ROWS // PAIR):
            row0 = pl.multiple_of(c * W_ROWS + jj * PAIR, PAIR)
            j = c * (W_ROWS // PAIR) + jj
            blk = wraw_v[m, pl.ds(row0, PAIR), :]
            wb_v[j, :, m * PAIR:(m + 1) * PAIR] = pltpu.bitcast(blk.T, U32)
            nb = PRE_MB // PRE
            for mb in range(NIT // nb):
                x = xpre_v[mb * nb:(mb + 1) * nb].reshape(PRE_MB, D)
                for n in range(PAIR // 128):
                    r = _nt(x, blk[n * 128:(n + 1) * 128])
                    col = m * PAIR + n * 128
                    pre_v[j, mb * PRE_MB // 2:(mb + 1) * PRE_MB // 2, col:col + 128] = (
                        pltpu.bitcast(r.astype(BF16), U32))

    def b_repack(c):
        for jj in range(W_ROWS // PAIR):
            row0 = pl.multiple_of(c * W_ROWS + jj * PAIR, PAIR)
            j = c * (W_ROWS // PAIR) + jj
            wob_v[j] = pltpu.bitcast(wraw_v[3, pl.ds(row0, PAIR), :], U32)

    cp_xpre.wait()
    for m in range(3):
        w_copy(m, 0).wait()
        b_pre(0, m)
    w_copy(3, 0).wait()
    b_repack(0)

    def pre_body(c, carry):
        for m in range(4):
            w_copy(m, c).wait()
        for m in range(3):
            b_pre(c, m)
        b_repack(c)
        return carry

    jax.lax.fori_loop(1, W_NCH - 1, pre_body, 0)

    for m in range(4):
        w_copy(m, W_NCH - 1).wait()
    cp_wqkv.wait()
    cp_woa.wait()

    for b in range(3 * LT):
        blk = wqkv_v[:, b * 128:(b + 1) * 128].T.astype(F32)
        for t in range(LT):
            tmp_v[t, b * 128:(b + 1) * 128, :] = blk[:, t * 128:(t + 1) * 128]
    b_pre(W_NCH - 1, 0)
    for p in range(3):
        for d in range(A_DH):
            r = p * D + d * A_H
            for t in range(LT):
                v = tmp_v[t, pl.ds(p * D + d, A_H, stride=A_DH), :]
                wqkvt_v[r // 2:(r + A_H) // 2, t * 128:(t + 1) * 128] = pltpu.bitcast(
                    v.astype(BF16), U32)
    b_pre(W_NCH - 1, 1)
    for b in range(3 * LT):
        blk = pltpu.bitcast(wqkvt_v[b * 64:(b + 1) * 64, :], BF16)
        wqkvp_v[:, b * 128:(b + 1) * 128] = pltpu.bitcast(blk.T, U32)
    for t in range(LT):
        tmp_v[t, 0:D, :] = woa_v[:, t * 128:(t + 1) * 128].astype(F32)
    b_pre(W_NCH - 1, 2)
    for d in range(A_DH):
        r = d * A_H
        for t in range(LT):
            v = tmp_v[t, pl.ds(d, A_H, stride=A_DH), :]
            woap_v[r // 2:(r + A_H) // 2, t * 128:(t + 1) * 128] = pltpu.bitcast(
                v.astype(BF16), U32)
    b_repack(W_NCH - 1)
    for t in range(LT, 3 * LT):
        slab_v[t, 0:A_PAD, :] = jnp.zeros((A_PAD, 128), F32)
    cp_mem.wait()
    cp_bx.wait()
    cp_ax.wait()

    a_scale = A_DH ** (-0.5)
    b_scale = B_DH ** (-0.5)
    qrow = jax.lax.broadcasted_iota(jnp.int32, (B_L, 2 * B_L), 0)
    lane = jax.lax.broadcasted_iota(jnp.int32, (B_L, 2 * B_L), 1)
    first = lane < B_L
    kcol = jnp.where(first, lane, lane - B_L)
    allowed = (qrow >= B_SEG) | (kcol >= B_SEG) | (qrow >= kcol)
    flane = jax.lax.broadcasted_iota(jnp.int32, (B_L, 128), 1)
    left = flane < 64

    def blockdiag(t):
        z = jnp.zeros((B_L, 128), F32)
        mid = t[:, 128:256]
        top = jnp.concatenate([t[:, 0:128], jnp.where(left, mid, 0.0), z], axis=1)
        bot = jnp.concatenate([z, jnp.where(left, 0.0, mid), t[:, 256:384]], axis=1)
        return jnp.concatenate([top, bot], axis=0).astype(BF16)

    def softmax(s):
        s = jnp.where(allowed, s * b_scale, NEG)
        ma = jnp.max(jnp.where(first, s, -jnp.inf), axis=1, keepdims=True)
        mb = jnp.max(jnp.where(first, -jnp.inf, s), axis=1, keepdims=True)
        p = jnp.exp(s - jnp.where(first, ma, mb))
        la = jnp.sum(jnp.where(first, p, 0.0), axis=1, keepdims=True)
        lb = jnp.sum(jnp.where(first, 0.0, p), axis=1, keepdims=True)
        return (p * _recip(jnp.where(first, la, lb))).astype(BF16)

    def segment(i, h, even, extra):
        qkv, prob, att = {}, {}, {}
        acc = [None]

        def proj(j):
            r = _nn(h, pltpu.bitcast(wb_v[j], BF16))
            if even:
                pre = pltpu.bitcast(
                    pre_v[j, pl.ds(pl.multiple_of(i * (PRE // 2), PRE // 2), PRE // 2), :], BF16)
                carry_v[j] = r[16:24]
                seg = jnp.concatenate([pre.astype(F32), r[0:16], r[24:32]], axis=0)
            else:
                seg = jnp.concatenate([carry_v[j], r], axis=0)
            qkv[j] = (seg[:, 0:PAIR].astype(BF16), blockdiag(seg[:, PAIR:2 * PAIR]),
                      blockdiag(seg[:, 2 * PAIR:3 * PAIR]))

        def scores(j):
            prob[j] = softmax(_nt(qkv[j][0], qkv[j][1]))

        def values(j):
            o = _nn(prob[j], qkv[j][2])
            if even:
                ocarry_v[j] = o[24:32]
                lhs = jnp.concatenate([o[0:24], o[32:40]], axis=0)
            else:
                lhs = jnp.concatenate([o[0:32], ocarry_v[j], o[32:40]], axis=0)
            att[j] = lhs.astype(BF16)

        def outp(j):
            d = _nn(att[j], pltpu.bitcast(wob_v[j], BF16))
            acc[0] = d if acc[0] is None else acc[0] + d

        stages = ((proj, 0), (scores, LAG_S), (values, LAG_V), (outp, LAG_O))
        for t in range(NPAIR + LAG_O):
            for k, (fn, lag) in enumerate(stages):
                if 0 <= t - lag < NPAIR:
                    fn(t - lag)
                    if (t - lag, k) in extra:
                        extra[(t - lag, k)]()
        return acc[0]

    def body(i, mem):
        r0 = pl.multiple_of(i * BLK, BLK)

        def a_qkv(p):
            x = ax_v[pl.ds(r0, BLK), :]
            r = _nn(x, pltpu.bitcast(wqkvp_v[:, p * D:(p + 1) * D], BF16))
            for t in range(LT):
                slab_v[p * LT + t, A_PAD:A_PAD + BLK, :] = r[:, t * 128:(t + 1) * 128]

        a_o = {}

        def a_attn(sb):
            base = A_PAD + sb * A_SUB
            q = [slab_v[t, base:base + A_SUB, :] for t in range(LT)]
            logits = []
            for w in range(A_W):
                lo = base - A_DIL * w
                acc = None
                for t in range(LT):
                    pr = q[t] * slab_v[LT + t, lo:lo + A_SUB, :]
                    acc = pr if acc is None else acc + pr
                acc = acc + pltpu.roll(acc, 64, 1)
                acc = acc + pltpu.roll(acc, 32, 1)
                acc = acc * a_scale
                if sb == 0 and w > 0:
                    row = jax.lax.broadcasted_iota(jnp.int32, (A_SUB, 128), 0) + r0
                    acc = jnp.where(row >= A_DIL * w, acc, NEG)
                logits.append(acc)
            m = logits[0]
            for w in range(1, A_W):
                m = jnp.maximum(m, logits[w])
            ps = [jnp.exp(l - m) for l in logits]
            den = ps[0]
            for w in range(1, A_W):
                den = den + ps[w]
            inv = _recip(den)
            o = []
            for t in range(LT):
                acc = None
                for w in range(A_W):
                    lo = base - A_DIL * w
                    pr = ps[w] * slab_v[2 * LT + t, lo:lo + A_SUB, :]
                    acc = pr if acc is None else acc + pr
                o.append((acc * inv).astype(BF16))
            a_o[sb] = jnp.concatenate(o, axis=1)
            if sb == BLK // A_SUB - 1:
                for t in range(LT, 3 * LT):
                    slab_v[t, 0:A_PAD, :] = slab_v[t, BLK:BLK + A_PAD, :]

        def a_out():
            o = jnp.concatenate([a_o[sb] for sb in range(BLK // A_SUB)], axis=0)
            res = _nn(o, pltpu.bitcast(woap_v[...], BF16))
            outa_v[pl.ds(r0, BLK), :] = res.astype(BF16)

        x = bx_v[i].astype(F32)
        last = NPAIR - 1
        acc = segment(i, jnp.concatenate([x[16:40], mem], axis=0).astype(BF16), True,
                      {(last, 1): lambda: a_qkv(1), (last, 2): lambda: a_qkv(2),
                       (last, 3): lambda: a_qkv(0)})
        out_e = acc[0:24]
        mem = acc[24:32].astype(BF16).astype(F32)
        acc = segment(i, jnp.concatenate([x[40:64], mem], axis=0).astype(BF16), False,
                      {(2, 0): lambda: a_attn(0), (5, 0): lambda: a_attn(1),
                       (8, 0): lambda: a_attn(2), (11, 0): lambda: a_attn(3),
                       (last, 3): a_out})
        out = jnp.concatenate([out_e, acc[32:40], acc[0:32]], axis=0)
        outb_v[pl.ds(r0, BLK), :] = out.astype(BF16)
        pltpu.make_async_copy(
            outa_v.at[pl.ds(r0, BLK)], out_h.at[pl.ds(r0, BLK), pl.ds(0, D)], sem_out.at[0]).start()
        pltpu.make_async_copy(
            outb_v.at[pl.ds(r0, BLK)], out_h.at[pl.ds(r0, BLK), pl.ds(D, D)], sem_out.at[1]).start()
        return acc[40:48].astype(BF16).astype(F32)

    jax.lax.fori_loop(0, NIT, body, mem0_v[...].astype(F32))

    pltpu.make_async_copy(outa_v, out_h.at[:, pl.ds(0, D)], sem_out.at[0]).wait()
    pltpu.make_async_copy(outb_v, out_h.at[:, pl.ds(D, D)], sem_out.at[1]).wait()


@functools.partial(jax.jit, static_argnames=("B_seg_len",))
def pallas_concat_heads__sliding_local_dilated__memory_aug_recurrent_mem_tr__prompt_kernel(
    A_x: jax.Array,
    A_wqkv: jax.Array,
    A_wo: jax.Array,
    B_x: jax.Array,
    B_mem0: jax.Array,
    B_Wq: jax.Array,
    B_Wk: jax.Array,
    B_Wv: jax.Array,
    B_Wo: jax.Array,
    B_seg_len: int,
):
    assert A_x.shape == (1, S, D) and B_x.shape == (1, S, D)
    assert B_seg_len == B_SEG and B_mem0.shape == (1, B_M, D)
    assert B_Wq.shape == (D, B_H, B_DH) and B_Wo.shape == (B_H, B_DH, D)

    def feat_major(w):
        return jnp.transpose(w, (1, 2, 0)).reshape(B_F, D)

    any_spec = pl.BlockSpec(memory_space=pl.ANY)
    out = pl.pallas_call(
        _kernel,
        out_shape=jax.ShapeDtypeStruct((S, 2 * D), BF16),
        in_specs=[any_spec] * 9,
        out_specs=any_spec,
        scratch_shapes=[
            pltpu.VMEM((S, D), BF16),
            pltpu.VMEM((D, 3 * D), BF16),
            pltpu.VMEM((D, D), BF16),
            pltpu.VMEM((NIT, BLK, D), BF16),
            pltpu.VMEM((NIT, PRE, D), BF16),
            pltpu.VMEM((B_M, D), BF16),
            pltpu.VMEM((4, B_F, D), BF16),
            pltpu.VMEM((LT, 3 * D, 128), F32),
            pltpu.VMEM((3 * D // 2, D), U32),
            pltpu.VMEM((D // 2, 3 * D), U32),
            pltpu.VMEM((D // 2, D), U32),
            pltpu.VMEM((3 * LT, A_PAD + BLK, 128), F32),
            pltpu.VMEM((S, D), BF16),
            pltpu.VMEM((NPAIR, D // 2, 3 * PAIR), U32),
            pltpu.VMEM((NPAIR, PAIR // 2, D), U32),
            pltpu.VMEM((NPAIR, NIT * PRE // 2, 3 * PAIR), U32),
            pltpu.VMEM((NPAIR, 8, 3 * PAIR), F32),
            pltpu.VMEM((NPAIR, 8, PAIR), F32),
            pltpu.VMEM((S, D), BF16),
            pltpu.SemaphoreType.DMA((6 + 4 * W_NCH,)),
            pltpu.SemaphoreType.DMA((2,)),
        ],
        compiler_params=pltpu.CompilerParams(vmem_limit_bytes=120 * 1024 * 1024),
    )(
        A_x.reshape(S, D), A_wqkv, A_wo, B_x.reshape(NIT, BLK, D), B_mem0.reshape(B_M, D),
        feat_major(B_Wq), feat_major(B_Wk), feat_major(B_Wv), B_Wo.reshape(B_F, D),
    )
    return out.reshape(1, S, 2 * D)
```

```python
import functools

import jax
import jax.numpy as jnp
import jax.experimental.pallas as pl
import jax.experimental.pallas.tpu as pltpu

F32 = jnp.float32
BF16 = jnp.bfloat16
U32 = jnp.uint32

S = 2048
D = 640
LT = D // 128
BLK = 64
NIT = S // BLK

A_H = 32
A_DH = 20
A_W = 8
A_DIL = 2
A_PAD = 16
A_SUB = 16

B_H = 32
B_DH = 192
B_F = B_H * B_DH
B_M = 8
B_SEG = 32
B_L = B_M + B_SEG
PAIR = 2 * B_DH
NPAIR = B_H // 2
W_NCH = 8
W_ROWS = B_F // W_NCH
PRE = 16
PRE_MB = 128

NEG = -1000000000.0
LAG_S, LAG_V, LAG_O = 1, 3, 5
ORDER = "povs"


def _nt(a, b):
    return jax.lax.dot_general(a, b, (((1,), (1,)), ((), ())), preferred_element_type=F32)


def _nn(a, b):
    return jnp.dot(a, b, preferred_element_type=F32)


def _recip(x):
    r = pl.reciprocal(x, approx=True)
    return r * (2.0 - x * r)


def _kernel(ax_h, wqkv_h, woa_h, bx_h, mem0_h, wq_h, wk_h, wv_h, wo_h, out_h,
            ax_v, wqkv_v, woa_v, bx_v, xpre_v, mem0_v, wraw_v,
            tmp_v, wqkvt_v, wqkvp_v, woap_v, slab_v, outa_v,
            wb_v, wob_v, pre_v, carry_v, mcarry_v, outb_v,
            sem_in, sem_out):
    cp_xpre = pltpu.make_async_copy(bx_h.at[:, pl.ds(0, PRE), :], xpre_v, sem_in.at[0])
    cp_wqkv = pltpu.make_async_copy(wqkv_h, wqkv_v, sem_in.at[1])
    cp_woa = pltpu.make_async_copy(woa_h, woa_v, sem_in.at[2])
    cp_mem = pltpu.make_async_copy(mem0_h, mem0_v, sem_in.at[3])
    cp_bx = pltpu.make_async_copy(bx_h, bx_v, sem_in.at[4])
    cp_ax = pltpu.make_async_copy(ax_h, ax_v, sem_in.at[5])
    w_hs = (wq_h, wk_h, wv_h, wo_h)

    def w_copy(m, c):
        return pltpu.make_async_copy(
            w_hs[m].at[pl.ds(c * W_ROWS, W_ROWS)],
            wraw_v.at[m, pl.ds(c * W_ROWS, W_ROWS)],
            sem_in.at[6 + m * W_NCH + c])

    cp_xpre.start()
    for c in range(W_NCH):
        for m in range(4):
            w_copy(m, c).start()
    cp_wqkv.start()
    cp_woa.start()
    cp_mem.start()
    cp_bx.start()
    cp_ax.start()

    def b_pre(c, m):
        for jj in range(W_ROWS // PAIR):
            row0 = pl.multiple_of(c * W_ROWS + jj * PAIR, PAIR)
            j = c * (W_ROWS // PAIR) + jj
            blk = wraw_v[m, pl.ds(row0, PAIR), :]
            wb_v[j, :, m * PAIR:(m + 1) * PAIR] = pltpu.bitcast(blk.T, U32)
            nb = PRE_MB // PRE
            for mb in range(NIT // nb):
                x = xpre_v[mb * nb:(mb + 1) * nb].reshape(PRE_MB, D)
                for n in range(PAIR // 128):
                    r = _nt(x, blk[n * 128:(n + 1) * 128])
                    col = m * PAIR + n * 128
                    pre_v[j, mb * PRE_MB // 2:(mb + 1) * PRE_MB // 2, col:col + 128] = (
                        pltpu.bitcast(r.astype(BF16), U32))

    def b_repack(c):
        for jj in range(W_ROWS // PAIR):
            row0 = pl.multiple_of(c * W_ROWS + jj * PAIR, PAIR)
            j = c * (W_ROWS // PAIR) + jj
            wob_v[j] = pltpu.bitcast(wraw_v[3, pl.ds(row0, PAIR), :], U32)

    cp_xpre.wait()
    for m in range(3):
        w_copy(m, 0).wait()
        b_pre(0, m)
    w_copy(3, 0).wait()
    b_repack(0)

    def pre_body(c, carry):
        for m in range(4):
            w_copy(m, c).wait()
        for m in range(3):
            b_pre(c, m)
        b_repack(c)
        return carry

    jax.lax.fori_loop(1, W_NCH - 1, pre_body, 0)

    for m in range(4):
        w_copy(m, W_NCH - 1).wait()
    cp_wqkv.wait()
    cp_woa.wait()

    for b in range(3 * LT):
        blk = wqkv_v[:, b * 128:(b + 1) * 128].T.astype(F32)
        for t in range(LT):
            tmp_v[t, b * 128:(b + 1) * 128, :] = blk[:, t * 128:(t + 1) * 128]
    b_pre(W_NCH - 1, 0)
    for p in range(3):
        for d in range(A_DH):
            r = p * D + d * A_H
            for t in range(LT):
                v = tmp_v[t, pl.ds(p * D + d, A_H, stride=A_DH), :]
                wqkvt_v[r // 2:(r + A_H) // 2, t * 128:(t + 1) * 128] = pltpu.bitcast(
                    v.astype(BF16), U32)
    b_pre(W_NCH - 1, 1)
    for b in range(3 * LT):
        blk = pltpu.bitcast(wqkvt_v[b * 64:(b + 1) * 64, :], BF16)
        wqkvp_v[:, b * 128:(b + 1) * 128] = pltpu.bitcast(blk.T, U32)
    for t in range(LT):
        tmp_v[t, 0:D, :] = woa_v[:, t * 128:(t + 1) * 128].astype(F32)
    b_pre(W_NCH - 1, 2)
    for d in range(A_DH):
        r = d * A_H
        for t in range(LT):
            v = tmp_v[t, pl.ds(d, A_H, stride=A_DH), :]
            woap_v[r // 2:(r + A_H) // 2, t * 128:(t + 1) * 128] = pltpu.bitcast(
                v.astype(BF16), U32)
    b_repack(W_NCH - 1)
    for t in range(LT, 3 * LT):
        slab_v[t, 0:A_PAD, :] = jnp.zeros((A_PAD, 128), F32)
    cp_mem.wait()
    cp_bx.wait()
    cp_ax.wait()

    a_scale = A_DH ** (-0.5)
    b_scale = B_DH ** (-0.5)
    def masks(nq, nk, even):
        qrow = jax.lax.broadcasted_iota(jnp.int32, (nq, 2 * nk), 0)
        lane = jax.lax.broadcasted_iota(jnp.int32, (nq, 2 * nk), 1)
        first = lane < nk
        kcol = jnp.where(first, lane, lane - nk)
        if even:
            allowed = (qrow >= B_SEG - 8) | (kcol >= B_SEG) | (qrow + 8 >= kcol)
            fill = jnp.full((nq, 2 * nk), NEG, F32)
        else:
            own1 = (qrow < B_L) & (kcol < B_L)
            own2 = (qrow >= B_L) & (kcol >= B_L)
            own = own1 | own2
            allowed = ((own1 & ((qrow >= B_SEG) | (kcol >= B_SEG) | (qrow >= kcol)))
                       | (own2 & ((kcol >= B_L + 8) | (qrow >= kcol))))
            fill = jnp.where(own, NEG, -jnp.inf)
        return first, allowed, fill

    mask_e = masks(32, B_L, True)
    mask_o = masks(48, B_L + 16, False)

    def blockdiag(t):
        n = t.shape[0]
        left = jax.lax.broadcasted_iota(jnp.int32, (n, 128), 1) < 64
        z = jnp.zeros((n, 128), F32)
        mid = t[:, 128:256]
        top = jnp.concatenate([t[:, 0:128], jnp.where(left, mid, 0.0), z], axis=1)
        bot = jnp.concatenate([z, jnp.where(left, 0.0, mid), t[:, 256:384]], axis=1)
        return jnp.concatenate([top, bot], axis=0).astype(BF16)

    def softmax(s, mask):
        first, allowed, fill = mask
        s = jnp.where(allowed, s * b_scale, fill)
        ma = jnp.max(jnp.where(first, s, -jnp.inf), axis=1, keepdims=True)
        mb = jnp.max(jnp.where(first, -jnp.inf, s), axis=1, keepdims=True)
        p = jnp.exp(s - jnp.where(first, ma, mb))
        la = jnp.sum(jnp.where(first, p, 0.0), axis=1, keepdims=True)
        lb = jnp.sum(jnp.where(first, 0.0, p), axis=1, keepdims=True)
        return (p * _recip(jnp.where(first, la, lb))).astype(BF16)

    def segment(i, h, even, extra):
        qkv, prob, att = {}, {}, {}
        acc = [None]

        def proj(j):
            r = _nn(h, pltpu.bitcast(wb_v[j], BF16))
            pre = pltpu.bitcast(
                pre_v[j, pl.ds(pl.multiple_of(i * (PRE // 2), PRE // 2), PRE // 2), :],
                BF16).astype(F32)
            if even:
                carry_v[j] = r[16:24]
                mcarry_v[j] = r[24:32, PAIR:]
                q = jnp.concatenate([pre[8:16, :PAIR], r[0:16, :PAIR], r[24:32, :PAIR]], axis=0)
                kv = jnp.concatenate([pre[:, PAIR:], r[0:16, PAIR:], r[24:32, PAIR:]], axis=0)
            else:
                c = carry_v[j]
                q = jnp.concatenate([c[:, :PAIR], r[:, :PAIR], pre[0:8, :PAIR]], axis=0)
                kv = jnp.concatenate([c[:, PAIR:], r[:, PAIR:], pre[0:8, PAIR:], mcarry_v[j]],
                                     axis=0)
            qkv[j] = (q.astype(BF16), blockdiag(kv[:, :PAIR]), blockdiag(kv[:, PAIR:]))

        def scores(j):
            prob[j] = softmax(_nt(qkv[j][0], qkv[j][1]), mask_e if even else mask_o)

        def values(j):
            att[j] = _nn(prob[j], qkv[j][2]).astype(BF16)

        def outp(j):
            d = _nn(att[j], pltpu.bitcast(wob_v[j], BF16))
            acc[0] = d if acc[0] is None else acc[0] + d

        stages = dict(p=(proj, 0), s=(scores, LAG_S), v=(values, LAG_V), o=(outp, LAG_O))
        for t in range(NPAIR + LAG_O):
            for k in ORDER:
                fn, lag = stages[k]
                if 0 <= t - lag < NPAIR:
                    fn(t - lag)
                    for e in extra.get((t - lag, k), ()):
                        e()
        return acc[0]

    def body(i, mem):
        r0 = pl.multiple_of(i * BLK, BLK)

        def a_qkv(p, nxt=False):
            rr = pl.multiple_of(jnp.minimum(i + 1, NIT - 1) * BLK, BLK) if nxt else r0
            x = ax_v[pl.ds(rr, BLK), :]
            r = _nn(x, pltpu.bitcast(wqkvp_v[:, p * D:(p + 1) * D], BF16))
            for t in range(LT):
                slab_v[p * LT + t, A_PAD:A_PAD + BLK, :] = r[:, t * 128:(t + 1) * 128]

        a_o = {}

        def a_attn(sb):
            base = A_PAD + sb * A_SUB
            q = [slab_v[t, base:base + A_SUB, :] for t in range(LT)]
            logits = []
            for w in range(A_W):
                lo = base - A_DIL * w
                acc = None
                for t in range(LT):
                    pr = q[t] * slab_v[LT + t, lo:lo + A_SUB, :]
                    acc = pr if acc is None else acc + pr
                acc = acc + pltpu.roll(acc, 64, 1)
                acc = acc + pltpu.roll(acc, 32, 1)
                acc = acc * a_scale
                if sb == 0 and w > 0:
                    row = jax.lax.broadcasted_iota(jnp.int32, (A_SUB, 128), 0) + r0
                    acc = jnp.where(row >= A_DIL * w, acc, NEG)
                logits.append(acc)
            m = logits[0]
            for w in range(1, A_W):
                m = jnp.maximum(m, logits[w])
            ps = [jnp.exp(l - m) for l in logits]
            den = ps[0]
            for w in range(1, A_W):
                den = den + ps[w]
            inv = _recip(den)
            o = []
            for t in range(LT):
                acc = None
                for w in range(A_W):
                    lo = base - A_DIL * w
                    pr = ps[w] * slab_v[2 * LT + t, lo:lo + A_SUB, :]
                    acc = pr if acc is None else acc + pr
                o.append((acc * inv).astype(BF16))
            a_o[sb] = jnp.concatenate(o, axis=1)
            if sb == BLK // A_SUB - 1:
                for t in range(LT, 3 * LT):
                    slab_v[t, 0:A_PAD, :] = slab_v[t, BLK:BLK + A_PAD, :]

        def a_out():
            o = jnp.concatenate([a_o[sb] for sb in range(BLK // A_SUB)], axis=0)
            res = _nn(o, pltpu.bitcast(woap_v[...], BF16))
            outa_v[pl.ds(r0, BLK), :] = res.astype(BF16)

        x = bx_v[i].astype(F32)
        last = NPAIR - 1
        acc = segment(i, jnp.concatenate([x[16:40], mem], axis=0).astype(BF16), True,
                      {(last, 's'): [lambda: a_qkv(2)], (last, 'o'): [lambda: a_qkv(0)]})
        out_e = acc[0:24]
        mem = acc[24:32].astype(BF16).astype(F32)
        acc = segment(i, jnp.concatenate([x[40:64], mem], axis=0).astype(BF16), False,
                      {(2, 'p'): [lambda: a_attn(0)], (5, 'p'): [lambda: a_attn(1)],
                       (8, 'p'): [lambda: a_attn(2)], (11, 'p'): [lambda: a_attn(3)],
                       (last, 's'): [a_out], (last, 'o'): [lambda: a_qkv(1, True)]})
        out = jnp.concatenate([acc[40:48], out_e, acc[0:32]], axis=0)
        outb_v[pl.ds(r0, BLK), :] = out.astype(BF16)
        pltpu.make_async_copy(
            outa_v.at[pl.ds(r0, BLK)], out_h.at[pl.ds(r0, BLK), pl.ds(0, D)], sem_out.at[0]).start()
        pltpu.make_async_copy(
            outb_v.at[pl.ds(r0, BLK)], out_h.at[pl.ds(r0, BLK), pl.ds(D, D)], sem_out.at[1]).start()
        return acc[32:40].astype(BF16).astype(F32)

    r = _nn(ax_v[0:BLK, :], pltpu.bitcast(wqkvp_v[:, D:2 * D], BF16))
    for t in range(LT):
        slab_v[LT + t, A_PAD:A_PAD + BLK, :] = r[:, t * 128:(t + 1) * 128]
    jax.lax.fori_loop(0, NIT, body, mem0_v[...].astype(F32))

    pltpu.make_async_copy(outa_v, out_h.at[:, pl.ds(0, D)], sem_out.at[0]).wait()
    pltpu.make_async_copy(outb_v, out_h.at[:, pl.ds(D, D)], sem_out.at[1]).wait()


@functools.partial(jax.jit, static_argnames=("B_seg_len",))
def pallas_concat_heads__sliding_local_dilated__memory_aug_recurrent_mem_tr__prompt_kernel(
    A_x: jax.Array,
    A_wqkv: jax.Array,
    A_wo: jax.Array,
    B_x: jax.Array,
    B_mem0: jax.Array,
    B_Wq: jax.Array,
    B_Wk: jax.Array,
    B_Wv: jax.Array,
    B_Wo: jax.Array,
    B_seg_len: int,
):
    assert A_x.shape == (1, S, D) and B_x.shape == (1, S, D)
    assert B_seg_len == B_SEG and B_mem0.shape == (1, B_M, D)
    assert B_Wq.shape == (D, B_H, B_DH) and B_Wo.shape == (B_H, B_DH, D)

    def feat_major(w):
        return jnp.transpose(w, (1, 2, 0)).reshape(B_F, D)

    any_spec = pl.BlockSpec(memory_space=pl.ANY)
    out = pl.pallas_call(
        _kernel,
        out_shape=jax.ShapeDtypeStruct((S, 2 * D), BF16),
        in_specs=[any_spec] * 9,
        out_specs=any_spec,
        scratch_shapes=[
            pltpu.VMEM((S, D), BF16),
            pltpu.VMEM((D, 3 * D), BF16),
            pltpu.VMEM((D, D), BF16),
            pltpu.VMEM((NIT, BLK, D), BF16),
            pltpu.VMEM((NIT, PRE, D), BF16),
            pltpu.VMEM((B_M, D), BF16),
            pltpu.VMEM((4, B_F, D), BF16),
            pltpu.VMEM((LT, 3 * D, 128), F32),
            pltpu.VMEM((3 * D // 2, D), U32),
            pltpu.VMEM((D // 2, 3 * D), U32),
            pltpu.VMEM((D // 2, D), U32),
            pltpu.VMEM((3 * LT, A_PAD + BLK, 128), F32),
            pltpu.VMEM((S, D), BF16),
            pltpu.VMEM((NPAIR, D // 2, 3 * PAIR), U32),
            pltpu.VMEM((NPAIR, PAIR // 2, D), U32),
            pltpu.VMEM((NPAIR, NIT * PRE // 2, 3 * PAIR), U32),
            pltpu.VMEM((NPAIR, 8, 3 * PAIR), F32),
            pltpu.VMEM((NPAIR, 8, 2 * PAIR), F32),
            pltpu.VMEM((S, D), BF16),
            pltpu.SemaphoreType.DMA((6 + 4 * W_NCH,)),
            pltpu.SemaphoreType.DMA((2,)),
        ],
        compiler_params=pltpu.CompilerParams(vmem_limit_bytes=120 * 1024 * 1024,
                                             disable_bounds_checks=True),
    )(
        A_x.reshape(S, D), A_wqkv, A_wo, B_x.reshape(NIT, BLK, D), B_mem0.reshape(B_M, D),
        feat_major(B_Wq), feat_major(B_Wk), feat_major(B_Wv), B_Wo.reshape(B_F, D),
    )
    return out.reshape(1, S, 2 * D)
```

```python
import functools

import jax
import jax.numpy as jnp
import jax.experimental.pallas as pl
import jax.experimental.pallas.tpu as pltpu

F32 = jnp.float32
BF16 = jnp.bfloat16
U32 = jnp.uint32

S = 2048
D = 640
LT = D // 128
BLK = 64
NIT = S // BLK

A_H = 32
A_DH = 20
A_W = 8
A_DIL = 2
A_PAD = 16
A_SUB = 16

B_H = 32
B_DH = 192
B_F = B_H * B_DH
B_M = 8
B_SEG = 32
B_L = B_M + B_SEG
PAIR = 2 * B_DH
NPAIR = B_H // 2
W_NCH = 8
W_ROWS = B_F // W_NCH
PRE = 16
PRE_MB = 128

NEG = -1000000000.0
LAG_S, LAG_V, LAG_O = [int(v) for v in "1,3,5".split(",")]
ORDER = "povs"
UNROLL = int("1")
PIN = int("1")
NLOOP = int("32")


def _schedule(lags, steady_extra, tail):
    lag = dict(p=0, s=lags[0], v=lags[1], o=lags[2])
    seq = []
    for t in range(NPAIR):
        for k in "povs":
            if t == NPAIR - 1 and k != "p":
                break
            j = t - lag[k]
            if j >= 0:
                seq += steady_extra.get("<" + k + str(j), [])
                seq.append((k, j))
                seq += steady_extra.get(k + str(j), [])
    seq += [(x[0], int(x[1:])) for x in tail.split()]
    for k in "psvo":
        assert [j for kk, j in seq if kk == k] == list(range(NPAIR)), (k, seq)
    return seq


def _ex(txt):
    d = {}
    for x in txt.split():
        key, val = x.split(":")
        d.setdefault(key, []).append((val[0], int(val[1:])))
    return d


SCHED_E = _schedule(
    [int(v) for v in "1,3,5".split(",")],
    _ex("<s0:q0 <s1:q1 <s3:q2 <s5:q3 <s7:q4 <s9:q5 <s11:q6 <s13:q7"),
    "v12 s14 q8 v13 s15 o10 o11 o12 v14 o13 v15 o14 q9 o15 q10 q11")
SCHED_O = _schedule(
    [int(v) for v in "1,3,5".split(",")],
    _ex("<s0:q12 <s1:q13 <s2:q14 <s4:a0 <s5:b0 <s6:a1 <s7:b1 <s8:a2 <s9:b2 <s11:a3 <s12:b3"),
    "v12 s14 o10 v13 s15 o11 o12 w0 v14 o13 v15 o14 o15 w1 w2 w3 w4")


def _nt(a, b):
    return jax.lax.dot_general(a, b, (((1,), (1,)), ((), ())), preferred_element_type=F32)


def _nn(a, b):
    return jnp.dot(a, b, preferred_element_type=F32)


def _recip(x):
    r = pl.reciprocal(x, approx=True)
    return r * (2.0 - x * r)


def _kernel(ax_h, wqkv_h, woa_h, bx_h, mem0_h, wq_h, wk_h, wv_h, wo_h, out_h,
            ax_v, wqkv_v, woa_v, bx_v, xpre_v, mem0_v, wraw_v,
            tmp_v, wqkvt_v, wqkvp_v, woap_v, slab_v, outa_v,
            wb_v, wob_v, pre_v, carry_v, mcarry_v, outb_v,
            sem_in, sem_out):
    cp_xpre = pltpu.make_async_copy(bx_h.at[:, pl.ds(0, PRE), :], xpre_v, sem_in.at[0])
    cp_wqkv = pltpu.make_async_copy(wqkv_h, wqkv_v, sem_in.at[1])
    cp_woa = pltpu.make_async_copy(woa_h, woa_v, sem_in.at[2])
    cp_mem = pltpu.make_async_copy(mem0_h, mem0_v, sem_in.at[3])
    cp_bx = pltpu.make_async_copy(bx_h, bx_v, sem_in.at[4])
    cp_ax = pltpu.make_async_copy(ax_h, ax_v, sem_in.at[5])
    w_hs = (wq_h, wk_h, wv_h, wo_h)

    def w_copy(m, c):
        return pltpu.make_async_copy(
            w_hs[m].at[pl.ds(c * W_ROWS, W_ROWS)],
            wraw_v.at[m, pl.ds(c * W_ROWS, W_ROWS)],
            sem_in.at[6 + m * W_NCH + c])

    cp_xpre.start()
    for c in range(W_NCH):
        for m in range(4):
            w_copy(m, c).start()
    cp_wqkv.start()
    cp_woa.start()
    cp_mem.start()
    cp_bx.start()
    cp_ax.start()

    def b_pre(c, m):
        for jj in range(W_ROWS // PAIR):
            row0 = pl.multiple_of(c * W_ROWS + jj * PAIR, PAIR)
            j = c * (W_ROWS // PAIR) + jj
            blk = wraw_v[m, pl.ds(row0, PAIR), :]
            wb_v[j, :, m * PAIR:(m + 1) * PAIR] = pltpu.bitcast(blk.T, U32)
            nb = PRE_MB // PRE
            for mb in range(NIT // nb):
                x = xpre_v[mb * nb:(mb + 1) * nb].reshape(PRE_MB, D)
                for n in range(PAIR // 128):
                    r = _nt(x, blk[n * 128:(n + 1) * 128])
                    col = m * PAIR + n * 128
                    pre_v[j, mb * PRE_MB // 2:(mb + 1) * PRE_MB // 2, col:col + 128] = (
                        pltpu.bitcast(r.astype(BF16), U32))

    def b_repack(c):
        for jj in range(W_ROWS // PAIR):
            row0 = pl.multiple_of(c * W_ROWS + jj * PAIR, PAIR)
            j = c * (W_ROWS // PAIR) + jj
            wob_v[j] = pltpu.bitcast(wraw_v[3, pl.ds(row0, PAIR), :], U32)

    cp_xpre.wait()
    for m in range(3):
        w_copy(m, 0).wait()
        b_pre(0, m)
    w_copy(3, 0).wait()
    b_repack(0)

    def pre_body(c, carry):
        for m in range(4):
            w_copy(m, c).wait()
        for m in range(3):
            b_pre(c, m)
        b_repack(c)
        return carry

    jax.lax.fori_loop(1, W_NCH - 1, pre_body, 0)

    for m in range(4):
        w_copy(m, W_NCH - 1).wait()
    cp_wqkv.wait()
    cp_woa.wait()

    for b in range(3 * LT):
        blk = wqkv_v[:, b * 128:(b + 1) * 128].T.astype(F32)
        for t in range(LT):
            tmp_v[t, b * 128:(b + 1) * 128, :] = blk[:, t * 128:(t + 1) * 128]
    b_pre(W_NCH - 1, 0)
    for p in range(3):
        for d in range(A_DH):
            r = p * D + d * A_H
            for t in range(LT):
                v = tmp_v[t, pl.ds(p * D + d, A_H, stride=A_DH), :]
                wqkvt_v[r // 2:(r + A_H) // 2, t * 128:(t + 1) * 128] = pltpu.bitcast(
                    v.astype(BF16), U32)
    b_pre(W_NCH - 1, 1)
    for b in range(3 * LT):
        blk = pltpu.bitcast(wqkvt_v[b * 64:(b + 1) * 64, :], BF16)
        wqkvp_v[:, b * 128:(b + 1) * 128] = pltpu.bitcast(blk.T, U32)
    for t in range(LT):
        tmp_v[t, 0:D, :] = woa_v[:, t * 128:(t + 1) * 128].astype(F32)
    b_pre(W_NCH - 1, 2)
    for d in range(A_DH):
        r = d * A_H
        for t in range(LT):
            v = tmp_v[t, pl.ds(d, A_H, stride=A_DH), :]
            woap_v[r // 2:(r + A_H) // 2, t * 128:(t + 1) * 128] = pltpu.bitcast(
                v.astype(BF16), U32)
    b_repack(W_NCH - 1)
    for t in range(LT, 3 * LT):
        slab_v[t, 0:A_PAD, :] = jnp.zeros((A_PAD, 128), F32)
    cp_mem.wait()
    cp_bx.wait()
    cp_ax.wait()

    a_scale = A_DH ** (-0.5)
    b_scale = B_DH ** (-0.5)
    def masks(nq, nk, even):
        qrow = jax.lax.broadcasted_iota(jnp.int32, (nq, 2 * nk), 0)
        lane = jax.lax.broadcasted_iota(jnp.int32, (nq, 2 * nk), 1)
        first = lane < nk
        kcol = jnp.where(first, lane, lane - nk)
        if even:
            allowed = (qrow >= B_SEG - 8) | (kcol >= B_SEG) | (qrow + 8 >= kcol)
            fill = jnp.full((nq, 2 * nk), NEG, F32)
        else:
            own1 = (qrow < B_L) & (kcol < B_L)
            own2 = (qrow >= B_L) & (kcol >= B_L)
            own = own1 | own2
            allowed = ((own1 & ((qrow >= B_SEG) | (kcol >= B_SEG) | (qrow >= kcol)))
                       | (own2 & ((kcol >= B_L + 8) | (qrow >= kcol))))
            fill = jnp.where(own, NEG, -jnp.inf)
        return first, allowed, fill

    mask_e = masks(32, B_L, True)
    mask_o = masks(48, B_L + 16, False)

    def blockdiag(t):
        n = t.shape[0]
        left = jax.lax.broadcasted_iota(jnp.int32, (n, 128), 1) < 64
        z = jnp.zeros((n, 128), F32)
        mid = t[:, 128:256]
        top = jnp.concatenate([t[:, 0:128], jnp.where(left, mid, 0.0), z], axis=1)
        bot = jnp.concatenate([z, jnp.where(left, 0.0, mid), t[:, 256:384]], axis=1)
        return jnp.concatenate([top, bot], axis=0).astype(BF16)

    def softmax(s, mask):
        first, allowed, fill = mask
        s = jnp.where(allowed, s * b_scale, fill)
        ma = jnp.max(jnp.where(first, s, -jnp.inf), axis=1, keepdims=True)
        mb = jnp.max(jnp.where(first, -jnp.inf, s), axis=1, keepdims=True)
        p = jnp.exp(s - jnp.where(first, ma, mb))
        la = jnp.sum(jnp.where(first, p, 0.0), axis=1, keepdims=True)
        lb = jnp.sum(jnp.where(first, 0.0, p), axis=1, keepdims=True)
        return (p * _recip(jnp.where(first, la, lb))).astype(BF16)

    def segment(i, h, even, extra):
        qkv, prob, att = {}, {}, {}
        acc = [None]

        def proj(j):
            r = jnp.dot(h, pltpu.bitcast(wb_v[j], BF16), preferred_element_type=F32)
            pre = pltpu.bitcast(
                pre_v[j, pl.ds(pl.multiple_of(i * (PRE // 2), PRE // 2), PRE // 2), :],
                BF16).astype(F32)
            if even:
                carry_v[j] = r[16:24]
                mcarry_v[j] = r[24:32, PAIR:]
                q = jnp.concatenate([pre[8:16, :PAIR], r[0:16, :PAIR], r[24:32, :PAIR]], axis=0)
                kv = jnp.concatenate([pre[:, PAIR:], r[0:16, PAIR:], r[24:32, PAIR:]], axis=0)
            else:
                c = carry_v[j]
                q = jnp.concatenate([c[:, :PAIR], r[:, :PAIR], pre[0:8, :PAIR]], axis=0)
                kv = jnp.concatenate([c[:, PAIR:], r[:, PAIR:], pre[0:8, PAIR:], mcarry_v[j]],
                                     axis=0)
            qkv[j] = (q.astype(BF16), blockdiag(kv[:, :PAIR]), blockdiag(kv[:, PAIR:]))

        def scores(j):
            prob[j] = softmax(_nt(extra['pin'](qkv[j][0]), qkv[j][1]), mask_e if even else mask_o)

        def values(j):
            att[j] = jnp.dot(prob[j], qkv[j][2], preferred_element_type=F32).astype(BF16)

        def outp(j):
            d = jnp.dot(att[j], pltpu.bitcast(wob_v[j], BF16), preferred_element_type=F32)
            acc[0] = d if acc[0] is None else acc[0] + d

        fns = dict(p=proj, s=scores, v=values, o=outp)
        for k, j in (SCHED_E if even else SCHED_O):
            if k in fns:
                fns[k](j)
            else:
                extra[k](j)
        return acc[0]

    def body(i, mem):
        r0 = pl.multiple_of(i * BLK, BLK)

        def a_qkv(b):
            x = ax_v[pl.ds(r0, BLK), :]
            slab_v[b, A_PAD:A_PAD + BLK, :] = _nn(
                x, pltpu.bitcast(wqkvp_v[:, b * 128:(b + 1) * 128], BF16))

        a_o, a_p = {}, {}
        never = i < 0
        pins = []

        def a_logits(sb):
            base = A_PAD + sb * A_SUB
            q = [slab_v[t, base:base + A_SUB, :] for t in range(LT)]
            logits = []
            for w in range(A_W):
                lo = base - A_DIL * w
                acc = None
                for t in range(LT):
                    pr = q[t] * slab_v[LT + t, lo:lo + A_SUB, :]
                    acc = pr if acc is None else acc + pr
                acc = acc + pltpu.roll(acc, 64, 1)
                acc = acc + pltpu.roll(acc, 32, 1)
                acc = acc * a_scale
                if sb == 0 and w > 0:
                    row = jax.lax.broadcasted_iota(jnp.int32, (A_SUB, 128), 0) + r0
                    acc = jnp.where(row >= A_DIL * w, acc, NEG)
                logits.append(acc)
            m = logits[0]
            for w in range(1, A_W):
                m = jnp.maximum(m, logits[w])
            ps = [jnp.exp(l - m) for l in logits]
            den = ps[0]
            for w in range(1, A_W):
                den = den + ps[w]
            inv = _recip(den)
            a_p[sb] = (ps, inv)
            pins.extend(pltpu.bitcast(inv[8 * u:8 * u + 8], U32) for u in range(A_SUB // 8))

        def a_values(sb):
            base = A_PAD + sb * A_SUB
            ps, inv = a_p[sb]
            o = []
            for t in range(LT):
                acc = None
                for w in range(A_W):
                    lo = base - A_DIL * w
                    pr = ps[w] * slab_v[2 * LT + t, lo:lo + A_SUB, :]
                    acc = pr if acc is None else acc + pr
                o.append((acc * inv).astype(BF16))
            pins.extend(pltpu.bitcast(x, U32) for x in o)
            a_o[sb] = jnp.concatenate(o, axis=1)
            if sb == BLK // A_SUB - 1:
                for t in range(LT, 3 * LT):
                    slab_v[t, 0:A_PAD, :] = slab_v[t, BLK:BLK + A_PAD, :]

        def pin(q):
            if not pins or not PIN:
                return q
            u = pltpu.bitcast(q, U32)
            rows = []
            for r in range(u.shape[0] // 8):
                cols = []
                for c in range(u.shape[1] // 128):
                    x = u[8 * r:8 * r + 8, 128 * c:128 * c + 128]
                    if pins:
                        x = jnp.where(never, pins.pop(), x)
                    cols.append(x)
                rows.append(jnp.concatenate(cols, axis=1))
            assert not pins
            return pltpu.bitcast(jnp.concatenate(rows, axis=0), BF16)

        def a_out(b):
            o = jnp.concatenate([a_o[sb] for sb in range(BLK // A_SUB)], axis=0)
            res = jnp.dot(o, pltpu.bitcast(woap_v[:, b * 128:(b + 1) * 128], BF16), preferred_element_type=F32)
            outa_v[pl.ds(r0, BLK), b * 128:(b + 1) * 128] = res.astype(BF16)

        x = bx_v[i].astype(F32)
        ex_e = ex_o = dict(q=a_qkv, a=a_logits, b=a_values, w=a_out, pin=pin)
        acc = segment(i, jnp.concatenate([x[16:40], mem], axis=0).astype(BF16), True,
                      ex_e)
        out_e = acc[0:24]
        mem = acc[24:32].astype(BF16).astype(F32)
        acc = segment(i, jnp.concatenate([x[40:64], mem], axis=0).astype(BF16), False,
                      ex_o)
        out = jnp.concatenate([acc[40:48], out_e, acc[0:32]], axis=0)
        outb_v[pl.ds(r0, BLK), :] = out.astype(BF16)
        pltpu.make_async_copy(
            outa_v.at[pl.ds(r0, BLK)], out_h.at[pl.ds(r0, BLK), pl.ds(0, D)], sem_out.at[0]).start()
        pltpu.make_async_copy(
            outb_v.at[pl.ds(r0, BLK)], out_h.at[pl.ds(r0, BLK), pl.ds(D, D)], sem_out.at[1]).start()
        return acc[32:40].astype(BF16).astype(F32)

    def body_n(ii, mem):
        for u in range(UNROLL):
            mem = body(ii * UNROLL + u, mem)
        return mem

    jax.lax.fori_loop(0, NLOOP // UNROLL, body_n, mem0_v[...].astype(F32))

    pltpu.make_async_copy(outa_v.at[0:NLOOP * BLK], out_h.at[0:NLOOP * BLK, pl.ds(0, D)], sem_out.at[0]).wait()
    pltpu.make_async_copy(outb_v.at[0:NLOOP * BLK], out_h.at[0:NLOOP * BLK, pl.ds(D, D)], sem_out.at[1]).wait()


@functools.partial(jax.jit, static_argnames=("B_seg_len",))
def pallas_concat_heads__sliding_local_dilated__memory_aug_recurrent_mem_tr__prompt_kernel(
    A_x: jax.Array,
    A_wqkv: jax.Array,
    A_wo: jax.Array,
    B_x: jax.Array,
    B_mem0: jax.Array,
    B_Wq: jax.Array,
    B_Wk: jax.Array,
    B_Wv: jax.Array,
    B_Wo: jax.Array,
    B_seg_len: int,
):
    assert A_x.shape == (1, S, D) and B_x.shape == (1, S, D)
    assert B_seg_len == B_SEG and B_mem0.shape == (1, B_M, D)
    assert B_Wq.shape == (D, B_H, B_DH) and B_Wo.shape == (B_H, B_DH, D)

    def feat_major(w):
        return jnp.transpose(w, (1, 2, 0)).reshape(B_F, D)

    any_spec = pl.BlockSpec(memory_space=pl.ANY)
    out = pl.pallas_call(
        _kernel,
        out_shape=jax.ShapeDtypeStruct((S, 2 * D), BF16),
        in_specs=[any_spec] * 9,
        out_specs=any_spec,
        scratch_shapes=[
            pltpu.VMEM((S, D), BF16),
            pltpu.VMEM((D, 3 * D), BF16),
            pltpu.VMEM((D, D), BF16),
            pltpu.VMEM((NIT, BLK, D), BF16),
            pltpu.VMEM((NIT, PRE, D), BF16),
            pltpu.VMEM((B_M, D), BF16),
            pltpu.VMEM((4, B_F, D), BF16),
            pltpu.VMEM((LT, 3 * D, 128), F32),
            pltpu.VMEM((3 * D // 2, D), U32),
            pltpu.VMEM((D // 2, 3 * D), U32),
            pltpu.VMEM((D // 2, D), U32),
            pltpu.VMEM((3 * LT, A_PAD + BLK, 128), F32),
            pltpu.VMEM((S, D), BF16),
            pltpu.VMEM((NPAIR, D // 2, 3 * PAIR), U32),
            pltpu.VMEM((NPAIR, PAIR // 2, D), U32),
            pltpu.VMEM((NPAIR, NIT * PRE // 2, 3 * PAIR), U32),
            pltpu.VMEM((NPAIR, 8, 3 * PAIR), F32),
            pltpu.VMEM((NPAIR, 8, 2 * PAIR), F32),
            pltpu.VMEM((S, D), BF16),
            pltpu.SemaphoreType.DMA((6 + 4 * W_NCH,)),
            pltpu.SemaphoreType.DMA((2,)),
        ],
        compiler_params=pltpu.CompilerParams(vmem_limit_bytes=120 * 1024 * 1024,
                                             disable_bounds_checks=True),
    )(
        A_x.reshape(S, D), A_wqkv, A_wo, B_x.reshape(NIT, BLK, D), B_mem0.reshape(B_M, D),
        feat_major(B_Wq), feat_major(B_Wk), feat_major(B_Wv), B_Wo.reshape(B_F, D),
    )
    return out.reshape(1, S, 2 * D)
```

```python
import functools

import jax
import jax.numpy as jnp
import jax.experimental.pallas as pl
import jax.experimental.pallas.tpu as pltpu

F32 = jnp.float32
BF16 = jnp.bfloat16
U32 = jnp.uint32

S = 2048
D = 640
LT = D // 128
BLK = 64
NIT = S // BLK

A_H = 32
A_DH = 20
A_W = 8
A_DIL = 2
A_PAD = 16
A_SUB = 16

B_H = 32
B_DH = 192
B_F = B_H * B_DH
B_M = 8
B_SEG = 32
B_L = B_M + B_SEG
PAIR = 2 * B_DH
NPAIR = B_H // 2
NU = 3 * NPAIR
PRE = 16
PRE_MB = 128

NEG = -1000000000.0
LAG_S, LAG_V, LAG_O = [int(v) for v in "1,3,5".split(",")]
ORDER = "povs"
UNROLL = int("2")
U_HEAD = [int(v) for v in "1,1,2".split(",")]
U_BODY = int("5")
U_N = int("8")
U_TAIL = NU - sum(U_HEAD) - U_BODY * U_N
PIN = int("1")
NLOOP = int("32")


def _schedule(lags, steady_extra, tail):
    lag = dict(p=0, s=lags[0], v=lags[1], o=lags[2])
    seq = []
    for t in range(NPAIR):
        for k in "povs":
            if t == NPAIR - 1 and k != "p":
                break
            j = t - lag[k]
            if j >= 0:
                seq += steady_extra.get("<" + k + str(j), [])
                seq.append((k, j))
                seq += steady_extra.get(k + str(j), [])
    seq += [(x[0], int(x[1:])) for x in tail.split()]
    for k in "psvo":
        assert [j for kk, j in seq if kk == k] == list(range(NPAIR)), (k, seq)
    return seq


def _ex(txt):
    d = {}
    for x in txt.split():
        key, val = x.split(":")
        d.setdefault(key, []).append((val[0], int(val[1:])))
    return d


SCHED_E = _schedule(
    [int(v) for v in "1,3,5".split(",")],
    _ex("<s0:q0 <s1:q1 <s3:q2 <s5:q3 <s7:q4 <s9:q5 <s11:q6 <s13:q7"),
    "v12 s14 q8 v13 s15 o10 o11 o12 v14 o13 v15 o14 q9 o15 q10 q11")
SCHED_O = _schedule(
    [int(v) for v in "1,3,5".split(",")],
    _ex("<s0:q12 <s1:q13 <s2:q14 <s4:a0 <s5:b0 <s6:a1 <s7:b1 <s8:a2 <s9:b2 <s11:a3 <s12:b3"),
    "v12 s14 o10 v13 s15 o11 o12 w0 v14 o13 v15 o14 o15 w1 w2 w3 w4")


def _nt(a, b):
    return jax.lax.dot_general(a, b, (((1,), (1,)), ((), ())), preferred_element_type=F32)


def _nn(a, b):
    return jnp.dot(a, b, preferred_element_type=F32)


def _recip(x):
    r = pl.reciprocal(x, approx=True)
    return r * (2.0 - x * r)


def _kernel(ax_h, wqkv_h, woa_h, bx_h, mem0_h, wq_h, wk_h, wv_h, wo_h, out_h,
            ax_v, wqkv_v, woa_v, bx_v, xpre_v, mem0_v, wraw_v, wo_v,
            tmp_v, wqkvt_v, wqkvp_v, woap_v, slab_v, outa_v,
            wb_v, pre_v, carry_v, mcarry_v, outb_v,
            sem_in, sem_out):
    cp_xpre = pltpu.make_async_copy(bx_h.at[:, pl.ds(0, PRE), :], xpre_v, sem_in.at[0])
    cp_wqkv = pltpu.make_async_copy(wqkv_h, wqkv_v, sem_in.at[1])
    cp_woa = pltpu.make_async_copy(woa_h, woa_v, sem_in.at[2])
    cp_mem = pltpu.make_async_copy(mem0_h, mem0_v, sem_in.at[3])
    cp_bx = pltpu.make_async_copy(bx_h, bx_v, sem_in.at[4])
    cp_ax = pltpu.make_async_copy(ax_h, ax_v, sem_in.at[5])
    cp_wo = pltpu.make_async_copy(wo_h, wo_v, sem_in.at[6])
    w_hs = (wq_h, wk_h, wv_h)
    groups = list(U_HEAD) + [U_BODY] * U_N + [U_TAIL]
    g_start = [sum(groups[:g]) for g in range(len(groups))]

    cp_xpre.start()
    for g, n in enumerate(groups):
        for u in range(g_start[g], g_start[g] + n):
            pltpu.make_async_copy(w_hs[u % 3].at[pl.ds(u // 3 * PAIR, PAIR)], wraw_v.at[u],
                                  sem_in.at[7 + g]).start()
    cp_wo.start()
    cp_wqkv.start()
    cp_woa.start()
    cp_mem.start()
    cp_bx.start()
    cp_ax.start()

    def g_wait(g, u0, n):
        buf = wraw_v.at[pl.ds(u0, n)]
        pltpu.make_async_copy(buf, buf, sem_in.at[7 + g]).wait()

    def b_pre(u):
        blk = wraw_v[u]
        wb_v[u] = pltpu.bitcast(blk.T, U32)
        nb = PRE_MB // PRE
        for mb in range(NIT // nb):
            x = xpre_v[mb * nb:(mb + 1) * nb].reshape(PRE_MB, D)
            for n in range(PAIR // 128):
                r = _nt(x, blk[n * 128:(n + 1) * 128])
                pre_v[u, mb * PRE_MB // 2:(mb + 1) * PRE_MB // 2, n * 128:(n + 1) * 128] = (
                    pltpu.bitcast(r.astype(BF16), U32))

    cp_xpre.wait()
    for g, n in enumerate(U_HEAD):
        g_wait(g, g_start[g], n)
        for u in range(g_start[g], g_start[g] + n):
            b_pre(u)

    def pre_body(c, carry):
        u0 = sum(U_HEAD) + c * U_BODY
        g_wait(len(U_HEAD) + c, u0, U_BODY)
        for k in range(U_BODY):
            b_pre(u0 + k)
        return carry

    jax.lax.fori_loop(0, U_N, pre_body, 0)

    g_wait(len(groups) - 1, g_start[-1], U_TAIL)
    cp_wqkv.wait()
    cp_woa.wait()
    tail_units = list(range(g_start[-1], NU))

    def tail_pre(k):
        for u in tail_units[k * U_TAIL // 4:(k + 1) * U_TAIL // 4]:
            b_pre(u)

    for b in range(3 * LT):
        blk = wqkv_v[:, b * 128:(b + 1) * 128].T.astype(F32)
        for t in range(LT):
            tmp_v[t, b * 128:(b + 1) * 128, :] = blk[:, t * 128:(t + 1) * 128]
    tail_pre(0)
    tail_pre(1)
    for p in range(3):
        for d in range(A_DH):
            r = p * D + d * A_H
            for t in range(LT):
                v = tmp_v[t, pl.ds(p * D + d, A_H, stride=A_DH), :]
                wqkvt_v[r // 2:(r + A_H) // 2, t * 128:(t + 1) * 128] = pltpu.bitcast(
                    v.astype(BF16), U32)
    tail_pre(2)
    for b in range(3 * LT):
        blk = pltpu.bitcast(wqkvt_v[b * 64:(b + 1) * 64, :], BF16)
        wqkvp_v[:, b * 128:(b + 1) * 128] = pltpu.bitcast(blk.T, U32)
    for t in range(LT):
        tmp_v[t, 0:D, :] = woa_v[:, t * 128:(t + 1) * 128].astype(F32)
    tail_pre(3)
    for d in range(A_DH):
        r = d * A_H
        for t in range(LT):
            v = tmp_v[t, pl.ds(d, A_H, stride=A_DH), :]
            woap_v[r // 2:(r + A_H) // 2, t * 128:(t + 1) * 128] = pltpu.bitcast(
                v.astype(BF16), U32)
    for t in range(LT, 3 * LT):
        slab_v[t, 0:A_PAD, :] = jnp.zeros((A_PAD, 128), F32)
    cp_wo.wait()
    cp_mem.wait()
    cp_bx.wait()
    cp_ax.wait()

    a_scale = A_DH ** (-0.5)
    b_scale = B_DH ** (-0.5)
    def masks(nq, nk, even):
        qrow = jax.lax.broadcasted_iota(jnp.int32, (nq, 2 * nk), 0)
        lane = jax.lax.broadcasted_iota(jnp.int32, (nq, 2 * nk), 1)
        first = lane < nk
        kcol = jnp.where(first, lane, lane - nk)
        if even:
            allowed = (qrow >= B_SEG - 8) | (kcol >= B_SEG) | (qrow + 8 >= kcol)
            fill = jnp.full((nq, 2 * nk), NEG, F32)
        else:
            own1 = (qrow < B_L) & (kcol < B_L)
            own2 = (qrow >= B_L) & (kcol >= B_L)
            own = own1 | own2
            allowed = ((own1 & ((qrow >= B_SEG) | (kcol >= B_SEG) | (qrow >= kcol)))
                       | (own2 & ((kcol >= B_L + 8) | (qrow >= kcol))))
            fill = jnp.where(own, NEG, -jnp.inf)
        return first, allowed, fill

    mask_e = masks(32, B_L, True)
    mask_o = masks(48, B_L + 16, False)

    def blockdiag(t):
        n = t.shape[0]
        left = jax.lax.broadcasted_iota(jnp.int32, (n, 128), 1) < 64
        z = jnp.zeros((n, 128), F32)
        mid = t[:, 128:256]
        top = jnp.concatenate([t[:, 0:128], jnp.where(left, mid, 0.0), z], axis=1)
        bot = jnp.concatenate([z, jnp.where(left, 0.0, mid), t[:, 256:384]], axis=1)
        return jnp.concatenate([top, bot], axis=0).astype(BF16)

    def softmax(s, mask):
        first, allowed, fill = mask
        s = jnp.where(allowed, s * b_scale, fill)
        ma = jnp.max(jnp.where(first, s, -jnp.inf), axis=1, keepdims=True)
        mb = jnp.max(jnp.where(first, -jnp.inf, s), axis=1, keepdims=True)
        p = jnp.exp(s - jnp.where(first, ma, mb))
        la = jnp.sum(jnp.where(first, p, 0.0), axis=1, keepdims=True)
        lb = jnp.sum(jnp.where(first, 0.0, p), axis=1, keepdims=True)
        return (p * _recip(jnp.where(first, la, lb))).astype(BF16)

    def segment(i, h, even, extra):
        qkv, prob, att = {}, {}, {}
        acc = [None]

        def proj(j):
            w = jnp.concatenate([wb_v[3 * j + m] for m in range(3)], axis=1)
            r = jnp.dot(h, pltpu.bitcast(w, BF16), preferred_element_type=F32)
            rows = pl.ds(pl.multiple_of(i * (PRE // 2), PRE // 2), PRE // 2)
            pre = jnp.concatenate([pre_v[3 * j + m, rows, :] for m in range(3)], axis=1)
            pre = pltpu.bitcast(pre, BF16).astype(F32)
            if even:
                carry_v[j] = r[16:24]
                mcarry_v[j] = r[24:32, PAIR:]
                q = jnp.concatenate([pre[8:16, :PAIR], r[0:16, :PAIR], r[24:32, :PAIR]], axis=0)
                kv = jnp.concatenate([pre[:, PAIR:], r[0:16, PAIR:], r[24:32, PAIR:]], axis=0)
            else:
                c = carry_v[j]
                q = jnp.concatenate([c[:, :PAIR], r[:, :PAIR], pre[0:8, :PAIR]], axis=0)
                kv = jnp.concatenate([c[:, PAIR:], r[:, PAIR:], pre[0:8, PAIR:], mcarry_v[j]],
                                     axis=0)
            qkv[j] = (q.astype(BF16), blockdiag(kv[:, :PAIR]), blockdiag(kv[:, PAIR:]))

        def scores(j):
            prob[j] = softmax(_nt(extra['pin'](qkv[j][0]), qkv[j][1]), mask_e if even else mask_o)

        def values(j):
            att[j] = jnp.dot(prob[j], qkv[j][2], preferred_element_type=F32).astype(BF16)

        def outp(j):
            d = jnp.dot(att[j], wo_v[j * PAIR:(j + 1) * PAIR, :], preferred_element_type=F32)
            acc[0] = d if acc[0] is None else acc[0] + d

        fns = dict(p=proj, s=scores, v=values, o=outp)
        for k, j in (SCHED_E if even else SCHED_O):
            if k in fns:
                fns[k](j)
            else:
                extra[k](j)
        return acc[0]

    def body(i, mem):
        r0 = pl.multiple_of(i * BLK, BLK)

        def a_qkv(b):
            x = ax_v[pl.ds(r0, BLK), :]
            slab_v[b, A_PAD:A_PAD + BLK, :] = _nn(
                x, pltpu.bitcast(wqkvp_v[:, b * 128:(b + 1) * 128], BF16))

        a_o, a_p = {}, {}
        never = i < 0
        pins = []

        def a_logits(sb):
            base = A_PAD + sb * A_SUB
            q = [slab_v[t, base:base + A_SUB, :] for t in range(LT)]
            logits = []
            for w in range(A_W):
                lo = base - A_DIL * w
                acc = None
                for t in range(LT):
                    pr = q[t] * slab_v[LT + t, lo:lo + A_SUB, :]
                    acc = pr if acc is None else acc + pr
                acc = acc + pltpu.roll(acc, 64, 1)
                acc = acc + pltpu.roll(acc, 32, 1)
                acc = acc * a_scale
                if sb == 0 and w > 0:
                    row = jax.lax.broadcasted_iota(jnp.int32, (A_SUB, 128), 0) + r0
                    acc = jnp.where(row >= A_DIL * w, acc, NEG)
                logits.append(acc)
            m = logits[0]
            for w in range(1, A_W):
                m = jnp.maximum(m, logits[w])
            ps = [jnp.exp(l - m) for l in logits]
            den = ps[0]
            for w in range(1, A_W):
                den = den + ps[w]
            inv = _recip(den)
            a_p[sb] = (ps, inv)
            pins.extend(pltpu.bitcast(inv[8 * u:8 * u + 8], U32) for u in range(A_SUB // 8))

        def a_values(sb):
            base = A_PAD + sb * A_SUB
            ps, inv = a_p[sb]
            o = []
            for t in range(LT):
                acc = None
                for w in range(A_W):
                    lo = base - A_DIL * w
                    pr = ps[w] * slab_v[2 * LT + t, lo:lo + A_SUB, :]
                    acc = pr if acc is None else acc + pr
                o.append((acc * inv).astype(BF16))
            pins.extend(pltpu.bitcast(x, U32) for x in o)
            a_o[sb] = jnp.concatenate(o, axis=1)
            if sb == BLK // A_SUB - 1:
                for t in range(LT, 3 * LT):
                    slab_v[t, 0:A_PAD, :] = slab_v[t, BLK:BLK + A_PAD, :]

        def pin(q):
            if not pins or not PIN:
                return q
            u = pltpu.bitcast(q, U32)
            rows = []
            for r in range(u.shape[0] // 8):
                cols = []
                for c in range(u.shape[1] // 128):
                    x = u[8 * r:8 * r + 8, 128 * c:128 * c + 128]
                    if pins:
                        x = jnp.where(never, pins.pop(), x)
                    cols.append(x)
                rows.append(jnp.concatenate(cols, axis=1))
            assert not pins
            return pltpu.bitcast(jnp.concatenate(rows, axis=0), BF16)

        def a_out(b):
            o = jnp.concatenate([a_o[sb] for sb in range(BLK // A_SUB)], axis=0)
            res = jnp.dot(o, pltpu.bitcast(woap_v[:, b * 128:(b + 1) * 128], BF16), preferred_element_type=F32)
            outa_v[pl.ds(r0, BLK), b * 128:(b + 1) * 128] = res.astype(BF16)

        x = bx_v[i].astype(F32)
        ex_e = ex_o = dict(q=a_qkv, a=a_logits, b=a_values, w=a_out, pin=pin)
        acc = segment(i, jnp.concatenate([x[16:40], mem], axis=0).astype(BF16), True,
                      ex_e)
        out_e = acc[0:24]
        mem = acc[24:32].astype(BF16).astype(F32)
        acc = segment(i, jnp.concatenate([x[40:64], mem], axis=0).astype(BF16), False,
                      ex_o)
        out = jnp.concatenate([acc[40:48], out_e, acc[0:32]], axis=0)
        outb_v[pl.ds(r0, BLK), :] = out.astype(BF16)
        pltpu.make_async_copy(
            outa_v.at[pl.ds(r0, BLK)], out_h.at[pl.ds(r0, BLK), pl.ds(0, D)], sem_out.at[0]).start()
        pltpu.make_async_copy(
            outb_v.at[pl.ds(r0, BLK)], out_h.at[pl.ds(r0, BLK), pl.ds(D, D)], sem_out.at[1]).start()
        return acc[32:40].astype(BF16).astype(F32)

    def body_n(ii, mem):
        for u in range(UNROLL):
            mem = body(ii * UNROLL + u, mem)
        return mem

    jax.lax.fori_loop(0, NLOOP // UNROLL, body_n, mem0_v[...].astype(F32))

    pltpu.make_async_copy(outa_v.at[0:NLOOP * BLK], out_h.at[0:NLOOP * BLK, pl.ds(0, D)], sem_out.at[0]).wait()
    pltpu.make_async_copy(outb_v.at[0:NLOOP * BLK], out_h.at[0:NLOOP * BLK, pl.ds(D, D)], sem_out.at[1]).wait()


@functools.partial(jax.jit, static_argnames=("B_seg_len",))
def pallas_concat_heads__sliding_local_dilated__memory_aug_recurrent_mem_tr__prompt_kernel(
    A_x: jax.Array,
    A_wqkv: jax.Array,
    A_wo: jax.Array,
    B_x: jax.Array,
    B_mem0: jax.Array,
    B_Wq: jax.Array,
    B_Wk: jax.Array,
    B_Wv: jax.Array,
    B_Wo: jax.Array,
    B_seg_len: int,
):
    assert A_x.shape == (1, S, D) and B_x.shape == (1, S, D)
    assert B_seg_len == B_SEG and B_mem0.shape == (1, B_M, D)
    assert B_Wq.shape == (D, B_H, B_DH) and B_Wo.shape == (B_H, B_DH, D)

    def feat_major(w):
        return jnp.transpose(w, (1, 2, 0)).reshape(B_F, D)

    any_spec = pl.BlockSpec(memory_space=pl.ANY)
    out = pl.pallas_call(
        _kernel,
        out_shape=jax.ShapeDtypeStruct((S, 2 * D), BF16),
        in_specs=[any_spec] * 9,
        out_specs=any_spec,
        scratch_shapes=[
            pltpu.VMEM((S, D), BF16),
            pltpu.VMEM((D, 3 * D), BF16),
            pltpu.VMEM((D, D), BF16),
            pltpu.VMEM((NIT, BLK, D), BF16),
            pltpu.VMEM((NIT, PRE, D), BF16),
            pltpu.VMEM((B_M, D), BF16),
            pltpu.VMEM((NU, PAIR, D), BF16),
            pltpu.VMEM((B_F, D), BF16),
            pltpu.VMEM((LT, 3 * D, 128), F32),
            pltpu.VMEM((3 * D // 2, D), U32),
            pltpu.VMEM((D // 2, 3 * D), U32),
            pltpu.VMEM((D // 2, D), U32),
            pltpu.VMEM((3 * LT, A_PAD + BLK, 128), F32),
            pltpu.VMEM((S, D), BF16),
            pltpu.VMEM((NU, D // 2, PAIR), U32),
            pltpu.VMEM((NU, NIT * PRE // 2, PAIR), U32),
            pltpu.VMEM((NPAIR, 8, 3 * PAIR), F32),
            pltpu.VMEM((NPAIR, 8, 2 * PAIR), F32),
            pltpu.VMEM((S, D), BF16),
            pltpu.SemaphoreType.DMA((8 + len(U_HEAD) + U_N,)),
            pltpu.SemaphoreType.DMA((2,)),
        ],
        compiler_params=pltpu.CompilerParams(vmem_limit_bytes=120 * 1024 * 1024,
                                             disable_bounds_checks=True),
    )(
        A_x.reshape(S, D), A_wqkv, A_wo, B_x.reshape(NIT, BLK, D), B_mem0.reshape(B_M, D),
        feat_major(B_Wq), feat_major(B_Wk), feat_major(B_Wv), B_Wo.reshape(B_F, D),
    )
    return out.reshape(1, S, 2 * D)
```

```python
import functools

import jax
import jax.numpy as jnp
import jax.experimental.pallas as pl
import jax.experimental.pallas.tpu as pltpu

F32 = jnp.float32
BF16 = jnp.bfloat16
U32 = jnp.uint32

S = 2048
D = 640
LT = D // 128
BLK = 64
NIT = S // BLK

A_H = 32
A_DH = 20
A_W = 8
A_DIL = 2
A_PAD = 16
A_SUB = 16

B_H = 32
B_DH = 192
B_F = B_H * B_DH
B_M = 8
B_SEG = 32
B_L = B_M + B_SEG
PAIR = 2 * B_DH
NPAIR = B_H // 2
NU = 3 * NPAIR
PRE = 16
PRE_MB = 128

NEG = -1000000000.0
LOG2E = 1.4426950408889634
LAG_S, LAG_V, LAG_O = [int(v) for v in "1,3,5".split(",")]
ORDER = "povs"
UNROLL = int("2")
U_HEAD = [int(v) for v in "1,1,2".split(",")]
U_BODY = int("5")
U_N = int("8")
U_TAIL = NU - sum(U_HEAD) - U_BODY * U_N
PIN = int("1")
NLOOP = int("32")


def _schedule(lags, steady_extra, tail):
    lag = dict(p=0, s=lags[0], v=lags[1], o=lags[2])
    seq = []
    for t in range(NPAIR):
        for k in ORDER:
            if t == NPAIR - 1 and k != "p":
                break
            j = t - lag[k]
            if j >= 0:
                seq += steady_extra.get("<" + k + str(j), [])
                seq.append((k, j))
                seq += steady_extra.get(k + str(j), [])
    seq += [(x[0], int(x[1:])) for x in tail.split()]
    for k in "psvo":
        assert [j for kk, j in seq if kk == k] == list(range(NPAIR)), (k, seq)
    return seq


def _ex(txt):
    d = {}
    for x in txt.split():
        key, val = x.split(":")
        d.setdefault(key, []).append((val[0], int(val[1:])))
    return d


def _due(txt):
    d = {}
    for x in txt.split():
        key, at = x.split("@")
        j, m = at.split(".")
        d.setdefault((int(j), int(m)), []).append((key[0], int(key[1:])))
    return d


def _vector_plan(ea, eb, ua, ub, last):
    ua, ub = ua.split("."), ub.split(".")
    es = [(j, e, d) for j in range(NPAIR) for e, d in enumerate((ea, eb))]
    ds = [(j, e, d) for j in range(NPAIR) for e, d in enumerate((ua, ub))]
    emit = " ".join(f"{d[0]}{j + int(d[1:])}:u{2 * j + e}" for j, e, d in es
                    if j + int(d[1:]) <= last[d[0]])
    tail = " ".join(f"u{2 * j + e}" for j, e, d in es if j + int(d[1:]) > last[d[0]])
    due = " ".join(f"u{2 * j + e}@{j + int(d[0])}.{d[1]}" for j, e, d in ds
                   if j + int(d[0]) < NPAIR)
    late = " ".join(f"u{2 * j + e}@{j + int(d[0]) - NPAIR}.{d[1]}" for j, e, d in ds
                    if j + int(d[0]) >= NPAIR)
    return emit, tail, due, late


_VE = _vector_plan(*"s0 s0 2.2 3.0".split(), dict(p=15, s=13))
_VO = _vector_plan(*"s0 s0 2.2 3.0".split(), dict(p=15, s=13))
SCHED_E = _schedule(
    [int(v) for v in "1,3,5".split(",")],
    _ex("<s0:q0 <s1:q1 <s3:q2 <s5:q3 <s7:q4 <s9:q5 <s11:q6 <s13:q7" + " " + _VE[0]),
    "v12 s14 q8 v13 s15 # o10 o11 o12 v14 o13 v15 o14 q9 o15 q10 q11".replace("#", _VE[1]))
SCHED_O = _schedule(
    [int(v) for v in "1,3,5".split(",")],
    _ex("<s0:q12 <s1:q13 <s2:q14 p4:a0 p5:b0 p6:a1 p7:b1 p8:a2 p9:b2 p10:a3 p11:b3" + " " + _VO[0]),
    "v12 s14 o10 v13 s15 # o11 o12 w0 v14 o13 v15 o14 o15 w1 w2 w3 w4".replace("#", _VO[1]))
DUE_E = _due(_VE[2])
DUE_O = _due(_VO[2].replace("u", "U") + " " + _VE[3] + " " + "a0@6.0 b0@7.0 a1@8.0 b1@9.0 a2@10.0 b2@11.0 a3@12.0 b3@13.0")


def _nt(a, b):
    return jax.lax.dot_general(a, b, (((1,), (1,)), ((), ())), preferred_element_type=F32)


def _nn(a, b):
    return jnp.dot(a, b, preferred_element_type=F32)


def _recip(x):
    r = pl.reciprocal(x, approx=True)
    return r * (2.0 - x * r)


def _kernel(ax_h, wqkv_h, woa_h, bx_h, mem0_h, wq_h, wk_h, wv_h, wo_h, out_h,
            ax_v, wqkv_v, woa_v, bx_v, xpre_v, mem0_v, wraw_v, wo_v,
            tmp_v, tmp2_v, wob_v, wqkvp_v, woap_v, slab_v, outa_v,
            wb_v, pre_v, qo_v, kvo_v, o8_v, outb_v,
            sem_in, sem_out):
    cp_xpre = pltpu.make_async_copy(bx_h.at[:, pl.ds(0, PRE), :], xpre_v, sem_in.at[0])
    cp_wqkv = pltpu.make_async_copy(wqkv_h, wqkv_v, sem_in.at[1])
    cp_woa = pltpu.make_async_copy(woa_h, woa_v, sem_in.at[2])
    cp_mem = pltpu.make_async_copy(mem0_h, mem0_v, sem_in.at[3])
    cp_bx = pltpu.make_async_copy(bx_h, bx_v, sem_in.at[4])
    cp_ax = pltpu.make_async_copy(ax_h, ax_v, sem_in.at[5])
    cp_wo = pltpu.make_async_copy(wo_h, wo_v, sem_in.at[6])
    w_hs = (wq_h, wk_h, wv_h)
    groups = list(U_HEAD) + [U_BODY] * U_N + [U_TAIL]
    g_start = [sum(groups[:g]) for g in range(len(groups))]

    cp_xpre.start()
    for g, n in enumerate(groups):
        for u in range(g_start[g], g_start[g] + n):
            pltpu.make_async_copy(w_hs[u % 3].at[pl.ds(u // 3 * PAIR, PAIR)], wraw_v.at[u],
                                  sem_in.at[7 + g]).start()
    cp_wo.start()
    cp_wqkv.start()
    cp_woa.start()
    cp_mem.start()
    cp_bx.start()
    cp_ax.start()

    def g_wait(g, u0, n):
        buf = wraw_v.at[pl.ds(u0, n)]
        pltpu.make_async_copy(buf, buf, sem_in.at[7 + g]).wait()

    def b_pre(u, after=None):
        blk = wraw_v[u]
        wb_v[u] = pltpu.bitcast(blk.T, U32)
        nb = PRE_MB // PRE
        for mb in range(NIT // nb):
            x = xpre_v[mb * nb:(mb + 1) * nb].reshape(PRE_MB, D)
            for n in range(PAIR // 128):
                r = _nt(x, blk[n * 128:(n + 1) * 128])
                pre_v[u, mb * PRE_MB // 2:(mb + 1) * PRE_MB // 2, n * 128:(n + 1) * 128] = (
                    pltpu.bitcast(r.astype(BF16), U32))
                if after is not None:
                    after(pltpu.bitcast(r[0:8], U32))

    cp_xpre.wait()
    for g, n in enumerate(U_HEAD):
        g_wait(g, g_start[g], n)
        for u in range(g_start[g], g_start[g] + n):
            b_pre(u)

    def pre_body(c, carry):
        u0 = sum(U_HEAD) + c * U_BODY
        g_wait(len(U_HEAD) + c, u0, U_BODY)
        for k in range(U_BODY):
            b_pre(u0 + k)
        return carry + c

    off = jax.lax.fori_loop(0, U_N, pre_body, 0) < 0

    g_wait(len(groups) - 1, g_start[-1], U_TAIL)
    cp_wqkv.wait()
    cp_woa.wait()
    cp_wo.wait()
    tail_units = list(range(g_start[-1], NU))

    copies = [(woa_v, 0, D, t, tmp2_v.at[t], 0) for t in range(LT)]
    n_dots = U_TAIL * (NIT * PRE // PRE_MB) * (PAIR // 128)
    RP = 256
    copies += [(wo_v, r, RP, t, wob_v.at[:, pl.ds(t * 128, 128)], r // 2)
               for r in range(0, B_F, RP) for t in range(LT)]
    per_dot = -(-len(copies) // (n_dots - 4))

    def copy_some(tok):
        for _ in range(per_dot):
            if copies:
                src, r, n, t, dst, d0 = copies.pop(0)
                v = pltpu.bitcast(src[r:r + n, t * 128:(t + 1) * 128], U32)
                v = jnp.where(off, jnp.concatenate([tok] * (n // 16), axis=0), v)
                dst[d0:d0 + n // 2, :] = v

    def tail_pre(k):
        for u in tail_units[k * U_TAIL // 4:(k + 1) * U_TAIL // 4]:
            b_pre(u, copy_some)

    def regroup(tmp_v, t, base, g):
        parts = []
        for dp in (2 * g, 2 * g + 1):
            v = tmp_v[t, pl.ds(base + dp, A_H, stride=A_DH // 2), :]
            parts.append(pltpu.bitcast(v << 16, F32))
            parts.append(pltpu.bitcast(v & jnp.uint32(0xFFFF0000), F32))
        return jnp.concatenate(parts, axis=0).astype(BF16)

    def a_prep1(p):
        for b in range(p * LT, (p + 1) * LT):
            blk = pltpu.bitcast(wqkv_v[:, b * 128:(b + 1) * 128].T, U32)
            for t in range(LT):
                tmp_v[t, b * 64:(b + 1) * 64, :] = blk[:, t * 128:(t + 1) * 128]

    def a_prep2(p):
        for g in range(LT):
            blk = jnp.concatenate([regroup(tmp_v, t, p * D // 2, g) for t in range(LT)], axis=1)
            b = p * LT + g
            wqkvp_v[:, b * 128:(b + 1) * 128] = pltpu.bitcast(blk.T, U32)

    def a_prep4():
        for g in range(LT):
            for t in range(LT):
                woap_v[g * 64:(g + 1) * 64, t * 128:(t + 1) * 128] = pltpu.bitcast(
                    regroup(tmp2_v, t, 0, g), U32)

    a_prep1(0)
    a_prep1(1)
    tail_pre(0)
    a_prep1(2)
    a_prep2(0)
    tail_pre(1)
    a_prep2(1)
    tail_pre(2)
    a_prep2(2)
    a_prep4()
    tail_pre(3)
    for t in range(LT, 3 * LT):
        slab_v[t, 0:A_PAD, :] = jnp.zeros((A_PAD, 128), F32)
    assert not copies
    cp_mem.wait()
    cp_bx.wait()
    cp_ax.wait()

    a_scale = A_DH ** (-0.5)
    b_scale = B_DH ** (-0.5)
    qrow = jax.lax.broadcasted_iota(jnp.int32, (32, 2 * B_L), 0)
    lane = jax.lax.broadcasted_iota(jnp.int32, (32, 2 * B_L), 1)
    first = lane < B_L
    kcol = jnp.where(first, lane, lane - B_L)
    allowed = (qrow >= B_SEG - 8) | (kcol >= B_SEG) | (qrow + 8 >= kcol)

    def blockdiag(t):
        n = t.shape[0]
        left = jax.lax.broadcasted_iota(jnp.int32, (n, 128), 1) < 64
        z = jnp.zeros((n, 128), F32)
        mid = t[:, 128:256]
        top = jnp.concatenate([t[:, 0:128], jnp.where(left, mid, 0.0), z], axis=1)
        bot = jnp.concatenate([z, jnp.where(left, 0.0, mid), t[:, 256:384]], axis=1)
        return jnp.concatenate([top, bot], axis=0).astype(BF16)

    def softmax(s):
        s = jnp.where(allowed, s * b_scale, NEG)
        ma = jnp.max(jnp.where(first, s, -jnp.inf), axis=1, keepdims=True)
        mb = jnp.max(jnp.where(first, -jnp.inf, s), axis=1, keepdims=True)
        p = jnp.exp(s - jnp.where(first, ma, mb))
        la = jnp.sum(jnp.where(first, p, 0.0), axis=1, keepdims=True)
        lb = jnp.sum(jnp.where(first, 0.0, p), axis=1, keepdims=True)
        return (p * _recip(jnp.where(first, la, lb))).astype(BF16)

    def head8(q, kv_x, kv_m, second):
        left = jax.lax.broadcasted_iota(jnp.int32, (8, 128), 1) < 64
        row = jax.lax.broadcasted_iota(jnp.int32, (8, 128), 0)
        t = 2 if second else 0
        qa = q[:, t * 128:(t + 1) * 128] * (b_scale * LOG2E)
        qb = q[:, 128:256] * (b_scale * LOG2E)
        qb = jnp.where(left, 0.0, qb) if second else jnp.where(left, qb, 0.0)

        def bc(k, t):
            src = kv_x if k < 8 else kv_m
            return jnp.broadcast_to(src[k % 8:k % 8 + 1, t * 128:(t + 1) * 128], (8, 128))

        sc = []
        for k in range(16):
            x = jnp.sum(qa * bc(k, t) + qb * bc(k, 1), axis=1, keepdims=True)
            x = jnp.broadcast_to(x, (8, 128))
            if 0 < k < 8:
                x = jnp.where(row >= k, x, NEG * LOG2E)
            sc.append(x)
        m = functools.reduce(jnp.maximum, sc)
        p = [jnp.exp2(x - m) for x in sc]
        inv = _recip(functools.reduce(jnp.add, p))
        return [functools.reduce(jnp.add, [p[k] * bc(k, 3 + tt) for k in range(16)]) * inv
                for tt in (t, 1)]

    def segment(i, h, even, extra):
        qkv, prob, att, q8, o8 = {}, {}, {}, {}, {}
        acc = [None]
        hh = [h]
        pins = extra['pins']

        def proj(j):
            parts = []
            for m in range(3):
                due = [x for key in (DUE_E if even else DUE_O).get((j, m), ()) for x in pins.pop(key)]
                if due:
                    hh[0] = extra['pin'](hh[0], due)
                parts.append(jnp.dot(hh[0], pltpu.bitcast(wb_v[3 * j + m], BF16), preferred_element_type=F32))
            r = jnp.concatenate(parts, axis=1)
            if even:
                rows = pl.ds(pl.multiple_of(i * (PRE // 2), PRE // 2), PRE // 2)
                pre = jnp.concatenate([pre_v[3 * j + m, rows, :] for m in range(3)], axis=1)
                pre = pltpu.bitcast(pre, BF16).astype(F32)
                qo_v[j] = r[16:24, :PAIR]
                kvo_v[j] = r[16:24, PAIR:]
                q8[j] = (pre[0:8, :PAIR], pre[0:8, PAIR:], r[24:32, PAIR:])
                q = jnp.concatenate([pre[8:16, :PAIR], r[0:16, :PAIR], r[24:32, :PAIR]], axis=0)
                kv = jnp.concatenate([pre[:, PAIR:], r[0:16, PAIR:], r[24:32, PAIR:]], axis=0)
            else:
                q8[j] = (qo_v[j], kvo_v.at[j], r[24:32, PAIR:])
                q = r[:, :PAIR]
                kv = jnp.concatenate([kvo_v[j], r[:, PAIR:]], axis=0)
            qkv[j] = (q.astype(BF16), blockdiag(kv[:, :PAIR]), blockdiag(kv[:, PAIR:]))

        def vector(jj):
            j, second = jj // 2, jj % 2
            o = head8(*q8[j], second)
            pins[('u' if even else 'U', jj)] = [pltpu.bitcast(x, U32) for x in o]
            if not second:
                o8[j] = o
                return
            left = jax.lax.broadcasted_iota(jnp.int32, (8, 128), 1) < 64
            o = jnp.concatenate([o8[j][0], jnp.where(left, o8[j][1], o[1]), o[0]], axis=1)
            if even:
                o8_v[j] = o
            else:
                o8[j] = o

        def scores(j):
            prob[j] = softmax(_nt(qkv[j][0], qkv[j][1]))

        def values(j):
            att[j] = jnp.dot(prob[j], qkv[j][2], preferred_element_type=F32)

        def outp(j):
            lhs = att[j] if even else jnp.concatenate([att[j], o8_v[j], o8[j]], axis=0)
            lhs = lhs.astype(BF16)
            d = jnp.dot(lhs, pltpu.bitcast(wob_v[j * PAIR // 2:(j + 1) * PAIR // 2, :], BF16), preferred_element_type=F32)
            acc[0] = d if acc[0] is None else acc[0] + d

        fns = dict(p=proj, s=scores, v=values, o=outp, u=vector)
        for k, j in (SCHED_E if even else SCHED_O):
            if k in fns:
                fns[k](j)
            else:
                extra[k](j)
        return acc[0]

    def body(i, mem):
        r0 = pl.multiple_of(i * BLK, BLK)

        def a_qkv(b):
            x = ax_v[pl.ds(r0, BLK), :]
            slab_v[b, A_PAD:A_PAD + BLK, :] = _nn(
                x, pltpu.bitcast(wqkvp_v[:, b * 128:(b + 1) * 128], BF16))

        a_o, a_p = {}, {}
        never = i < 0
        pins = {}

        def a_logits(sb):
            base = A_PAD + sb * A_SUB
            q = [slab_v[t, base:base + A_SUB, :] for t in range(LT)]
            logits = []
            for w in range(A_W):
                lo = base - A_DIL * w
                acc = None
                for t in range(LT):
                    pr = q[t] * slab_v[LT + t, lo:lo + A_SUB, :]
                    acc = pr if acc is None else acc + pr
                acc = acc + pltpu.roll(acc, 64, 1)
                acc = acc + pltpu.roll(acc, 32, 1)
                acc = acc * a_scale
                if sb == 0 and w > 0:
                    row = jax.lax.broadcasted_iota(jnp.int32, (A_SUB, 128), 0) + r0
                    acc = jnp.where(row >= A_DIL * w, acc, NEG)
                logits.append(acc)
            m = logits[0]
            for w in range(1, A_W):
                m = jnp.maximum(m, logits[w])
            ps = [jnp.exp(l - m) for l in logits]
            den = ps[0]
            for w in range(1, A_W):
                den = den + ps[w]
            inv = _recip(den)
            a_p[sb] = (ps, inv)
            pins[('a', sb)] = [pltpu.bitcast(inv[8 * u:8 * u + 8], U32) for u in range(A_SUB // 8)]

        def a_values(sb):
            base = A_PAD + sb * A_SUB
            ps, inv = a_p[sb]
            o = []
            for t in range(LT):
                acc = None
                for w in range(A_W):
                    lo = base - A_DIL * w
                    pr = ps[w] * slab_v[2 * LT + t, lo:lo + A_SUB, :]
                    acc = pr if acc is None else acc + pr
                o.append(acc * inv)
            pins[('b', sb)] = [pltpu.bitcast(x[8 * u:8 * u + 8], U32) for x in o
                               for u in range(A_SUB // 8)]
            a_o[sb] = jnp.concatenate(o, axis=1)
            if sb == BLK // A_SUB - 1:
                for t in range(LT, 3 * LT):
                    slab_v[t, 0:A_PAD, :] = slab_v[t, BLK:BLK + A_PAD, :]

        def pin(h, due):
            u = pltpu.bitcast(h, U32)
            tiles = [u[8 * r:8 * r + 8, 128 * c:128 * c + 128]
                     for c in range(LT) for r in range(u.shape[0] // 8)]
            for k, x in enumerate(due):
                tiles[k % len(tiles)] = jnp.where(never, x, tiles[k % len(tiles)])
            n = u.shape[0] // 8
            cols = [jnp.concatenate(tiles[c * n:(c + 1) * n], axis=0) for c in range(LT)]
            return pltpu.bitcast(jnp.concatenate(cols, axis=1), BF16)

        def a_out(b):
            o = jnp.concatenate([a_o[sb] for sb in range(BLK // A_SUB)], axis=0).astype(BF16)
            res = jnp.dot(o, pltpu.bitcast(woap_v[:, b * 128:(b + 1) * 128], BF16), preferred_element_type=F32)
            outa_v[pl.ds(r0, BLK), b * 128:(b + 1) * 128] = res.astype(BF16)

        x = bx_v[i].astype(F32)
        ex_e = ex_o = dict(q=a_qkv, a=a_logits, b=a_values, w=a_out, pin=pin, pins=pins)
        acc = segment(i, jnp.concatenate([x[16:40], mem], axis=0).astype(BF16), True,
                      ex_e)
        out_e = acc[0:24]
        mem = acc[24:32].astype(BF16).astype(F32)
        acc = segment(i, jnp.concatenate([x[40:64], mem], axis=0).astype(BF16), False,
                      ex_o)
        out = jnp.concatenate([acc[32:40], out_e, acc[40:48], acc[0:24]], axis=0)
        outb_v[pl.ds(r0, BLK), :] = out.astype(BF16)
        pltpu.make_async_copy(
            outa_v.at[pl.ds(r0, BLK)], out_h.at[pl.ds(r0, BLK), pl.ds(0, D)], sem_out.at[0]).start()
        pltpu.make_async_copy(
            outb_v.at[pl.ds(r0, BLK)], out_h.at[pl.ds(r0, BLK), pl.ds(D, D)], sem_out.at[1]).start()
        return acc[24:32].astype(BF16).astype(F32)

    def body_n(ii, mem):
        for u in range(UNROLL):
            mem = body(ii * UNROLL + u, mem)
        return mem

    jax.lax.fori_loop(0, NLOOP // UNROLL, body_n, mem0_v[...].astype(F32))

    pltpu.make_async_copy(outa_v.at[0:NLOOP * BLK], out_h.at[0:NLOOP * BLK, pl.ds(0, D)], sem_out.at[0]).wait()
    pltpu.make_async_copy(outb_v.at[0:NLOOP * BLK], out_h.at[0:NLOOP * BLK, pl.ds(D, D)], sem_out.at[1]).wait()


@functools.partial(jax.jit, static_argnames=("B_seg_len",))
def pallas_concat_heads__sliding_local_dilated__memory_aug_recurrent_mem_tr__prompt_kernel(
    A_x: jax.Array,
    A_wqkv: jax.Array,
    A_wo: jax.Array,
    B_x: jax.Array,
    B_mem0: jax.Array,
    B_Wq: jax.Array,
    B_Wk: jax.Array,
    B_Wv: jax.Array,
    B_Wo: jax.Array,
    B_seg_len: int,
):
    assert A_x.shape == (1, S, D) and B_x.shape == (1, S, D)
    assert B_seg_len == B_SEG and B_mem0.shape == (1, B_M, D)
    assert B_Wq.shape == (D, B_H, B_DH) and B_Wo.shape == (B_H, B_DH, D)

    def feat_major(w):
        return jnp.transpose(w, (1, 2, 0)).reshape(B_F, D)

    any_spec = pl.BlockSpec(memory_space=pl.ANY)
    out = pl.pallas_call(
        _kernel,
        out_shape=jax.ShapeDtypeStruct((S, 2 * D), BF16),
        in_specs=[any_spec] * 9,
        out_specs=any_spec,
        scratch_shapes=[
            pltpu.VMEM((S, D), BF16),
            pltpu.VMEM((D, 3 * D), BF16),
            pltpu.VMEM((D, D), BF16),
            pltpu.VMEM((NIT, BLK, D), BF16),
            pltpu.VMEM((NIT, PRE, D), BF16),
            pltpu.VMEM((B_M, D), BF16),
            pltpu.VMEM((NU, PAIR, D), BF16),
            pltpu.VMEM((B_F, D), BF16),
            pltpu.VMEM((LT, 3 * D // 2, 128), U32),
            pltpu.VMEM((LT, D // 2, 128), U32),
            pltpu.VMEM((B_F // 2, D), U32),
            pltpu.VMEM((D // 2, 3 * D), U32),
            pltpu.VMEM((D // 2, D), U32),
            pltpu.VMEM((3 * LT, A_PAD + BLK, 128), F32),
            pltpu.VMEM((S, D), BF16),
            pltpu.VMEM((NU, D // 2, PAIR), U32),
            pltpu.VMEM((NU, NIT * PRE // 2, PAIR), U32),
            pltpu.VMEM((NPAIR, 8, PAIR), F32),
            pltpu.VMEM((NPAIR, 8, 2 * PAIR), F32),
            pltpu.VMEM((NPAIR, 8, PAIR), F32),
            pltpu.VMEM((S, D), BF16),
            pltpu.SemaphoreType.DMA((8 + len(U_HEAD) + U_N,)),
            pltpu.SemaphoreType.DMA((2,)),
        ],
        compiler_params=pltpu.CompilerParams(vmem_limit_bytes=120 * 1024 * 1024,
                                             disable_bounds_checks=True),
    )(
        A_x.reshape(S, D), A_wqkv, A_wo, B_x.reshape(NIT, BLK, D), B_mem0.reshape(B_M, D),
        feat_major(B_Wq), feat_major(B_Wk), feat_major(B_Wv), B_Wo.reshape(B_F, D),
    )
    return out.reshape(1, S, 2 * D)
```

```python
import functools

import jax
import jax.numpy as jnp
import jax.experimental.pallas as pl
import jax.experimental.pallas.tpu as pltpu

F32 = jnp.float32
BF16 = jnp.bfloat16
U32 = jnp.uint32

S = 2048
D = 640
LT = D // 128
BLK = 64
NIT = S // BLK

A_H = 32
A_DH = 20
A_W = 8
A_DIL = 2
A_PAD = 16
A_SUB = 16

B_H = 32
B_DH = 192
B_F = B_H * B_DH
B_M = 8
B_SEG = 32
B_L = B_M + B_SEG
PAIR = 2 * B_DH
NPAIR = B_H // 2
NU = 3 * NPAIR
PRE = 16
PRE_MB = 128

NEG = -1000000000.0
LOG2E = 1.4426950408889634
LAG_S, LAG_V, LAG_O = [int(v) for v in "1,3,5".split(",")]
ORDER = "povs"
UNROLL = int("2")
U_HEAD = [int(v) for v in "1,1,2".split(",")]
U_BODY = int("5")
U_N = int("8")
U_TAIL = NU - sum(U_HEAD) - U_BODY * U_N
SEARCH = int("0")
PIN = int("1")
NLOOP = int("32")


def _schedule(order, lags, steady_extra, tail):
    lag = dict(p=0, s=lags[0], v=lags[1], o=lags[2])
    kind = dict(x="p", y="p", z="p", A="o", B="o", C="o", s="s", v="v")
    seq = []
    for t in range(NPAIR):
        for k in order:
            j = t - lag[kind[k]]
            if j >= 0:
                if k in "xAsv":
                    seq += steady_extra.get("<" + kind[k] + str(j), [])
                seq.append((k, j))
                if k in "zCsv":
                    seq += steady_extra.get(kind[k] + str(j), [])
            if t == NPAIR - 1 and k == "z":
                break
    for x in tail.split():
        seq += [(k, int(x[1:])) for k in ("ABC" if x[0] == "o" else x[0])
                if (k, int(x[1:])) not in seq]
    for k in "xyzABCsv":
        assert [j for kk, j in seq if kk == k] == list(range(NPAIR)), (k, seq)
    return seq


def _ex(txt):
    d = {}
    for x in txt.split():
        key, val = x.split(":")
        d.setdefault(key, []).append((val[0], int(val[1:])))
    return d


def _due(txt):
    d = {}
    for x in txt.split():
        key, at = x.split("@")
        j, m = at.split(".")
        d.setdefault((int(j), int(m)), []).append((key[0], int(key[1:])))
    return d


def _vector_plan(ea, eb, ia, ua, ib, ub, last):
    es = [(j, e, d) for j in range(NPAIR) for e, d in enumerate((ea, eb))]
    ds = [(k, 2 * j + e, 9 * j + int(d)) for j in range(NPAIR)
          for k, e, d in (("i", 0, ia), ("u", 0, ua), ("i", 1, ib), ("u", 1, ub)) if int(d) > 0]
    emit = " ".join(f"{d[0]}{j + int(d[1:])}:u{2 * j + e}" for j, e, d in es
                    if j + int(d[1:]) <= last[d[0]])
    tail = " ".join(f"u{2 * j + e}" for j, e, d in es if j + int(d[1:]) > last[d[0]])
    due = " ".join(f"{k}{n}@{d // 9}.{d % 9}" for k, n, d in ds if d < 9 * NPAIR)
    late = " ".join(f"{k}{n}@{d // 9 - NPAIR}.{d % 9}" for k, n, d in ds if d >= 9 * NPAIR)
    return emit, tail, due, late


_VE = _vector_plan(*"s0 s0 0 25 0 27".split(), dict(p=15, s=13))
_VO = _vector_plan(*"s0 s0 0 24 0 28".split(), dict(p=15, s=13))
SCHED_E = _schedule(
    "xyzABCvs",
    [int(v) for v in "1,3,5".split(",")],
    _ex("<s0:q0 <s1:q1 <s2:q2 <s5:q3 <s8:q4 <s10:q5 <s11:q6 <s13:q7" + " " + _VE[0]),
    "v12 s14 q8 v13 s15 # o10 o11 o12 v14 o13 v15 o14 q9 o15 q10 q11".replace("#", _VE[1]))
SCHED_O = _schedule(
    "xAyBzCvs",
    [int(v) for v in "1,3,4".split(",")],
    _ex("<s0:q12 <s1:q13 <s2:q14 p4:a0 p5:b0 p6:a1 p7:b1 p9:a2 p10:b2 p11:a3 p12:b3" + " " + _VO[0]),
    "v12 s14 o11 v13 s15 # o12 w0 o13 v14 w1 v15 o14 w2 o15 w3 w4".replace("#", _VO[1]))
DUE_E = _due(_VE[2])
DUE_O = _due(_VO[2].replace("u", "U").replace("i", "I") + " " + _VE[3] + " " + "a0@6.2 b0@7.2 a1@8.2 b1@9.2 a2@11.2 b2@12.2 a3@13.2 b3@14.2")


def _nt(a, b):
    return jax.lax.dot_general(a, b, (((1,), (1,)), ((), ())), preferred_element_type=F32)


def _nn(a, b):
    return jnp.dot(a, b, preferred_element_type=F32)


def _recip(x):
    r = pl.reciprocal(x, approx=True)
    return r * (2.0 - x * r)


def _kernel(ax_h, wqkv_h, woa_h, bx_h, mem0_h, wq_h, wk_h, wv_h, wo_h, out_h,
            ax_v, wqkv_v, woa_v, bx_v, xpre_v, mem0_v, wraw_v, wo_v,
            tmp_v, tmp2_v, wob_v, wqkvp_v, woap_v, slab_v, outa_v,
            wb_v, pre_v, qo_v, kvo_v, o8_v, outb_v,
            sem_in, sem_out):
    cp_xpre = pltpu.make_async_copy(bx_h.at[:, pl.ds(0, PRE), :], xpre_v, sem_in.at[0])
    cp_wqkv = pltpu.make_async_copy(wqkv_h, wqkv_v, sem_in.at[1])
    cp_woa = pltpu.make_async_copy(woa_h, woa_v, sem_in.at[2])
    cp_mem = pltpu.make_async_copy(mem0_h, mem0_v, sem_in.at[3])
    cp_bx = pltpu.make_async_copy(bx_h, bx_v, sem_in.at[4])
    cp_ax = pltpu.make_async_copy(ax_h, ax_v, sem_in.at[5])
    cp_wo = pltpu.make_async_copy(wo_h, wo_v, sem_in.at[6])
    w_hs = (wq_h, wk_h, wv_h)
    groups = list(U_HEAD) + [U_BODY] * U_N + [U_TAIL]
    g_start = [sum(groups[:g]) for g in range(len(groups))]

    cp_xpre.start()
    for g, n in enumerate(groups):
        for u in range(g_start[g], g_start[g] + n):
            pltpu.make_async_copy(w_hs[u % 3].at[pl.ds(u // 3 * PAIR, PAIR)], wraw_v.at[u],
                                  sem_in.at[7 + g]).start()
    cp_wo.start()
    cp_wqkv.start()
    cp_woa.start()
    cp_mem.start()
    cp_bx.start()
    cp_ax.start()

    def g_wait(g, u0, n):
        buf = wraw_v.at[pl.ds(u0, n)]
        pltpu.make_async_copy(buf, buf, sem_in.at[7 + g]).wait()

    def b_pre(u, after=None):
        blk = wraw_v[u]
        wb_v[u] = pltpu.bitcast(blk.T, U32)
        nb = PRE_MB // PRE
        for mb in range(NIT // nb):
            x = xpre_v[mb * nb:(mb + 1) * nb].reshape(PRE_MB, D)
            for n in range(PAIR // 128):
                r = _nt(x, blk[n * 128:(n + 1) * 128])
                pre_v[u, mb * PRE_MB // 2:(mb + 1) * PRE_MB // 2, n * 128:(n + 1) * 128] = (
                    pltpu.bitcast(r.astype(BF16), U32))
                if after is not None:
                    after(r)

    cp_xpre.wait()
    if SEARCH:
        b_pre = lambda u, after=None: None
    for g, n in enumerate(U_HEAD):
        g_wait(g, g_start[g], n)
        for u in range(g_start[g], g_start[g] + n):
            b_pre(u)

    def pre_body(c, carry):
        u0 = sum(U_HEAD) + c * U_BODY
        g_wait(len(U_HEAD) + c, u0, U_BODY)
        for k in range(U_BODY):
            b_pre(u0 + k)
        return carry + c

    off = jax.lax.fori_loop(0, U_N, pre_body, 0) < 0

    g_wait(len(groups) - 1, g_start[-1], U_TAIL)
    cp_wqkv.wait()
    cp_woa.wait()
    cp_wo.wait()
    tail_units = list(range(g_start[-1], NU))

    copies = [(woa_v, r, 32, t, tmp2_v.at[t]) for t in range(LT) for r in range(0, D, 32)]
    copies += [(wo_v, r, 48, t, wob_v.at[:, pl.ds(t * 128, 128)])
               for r in range(0, B_F, 48) for t in range(LT)]

    def copy_some(res):
        for k in range(res.shape[0] // 8):
            if copies:
                src, r, n, t, dst = copies.pop(0)
                tok = pltpu.bitcast(res[8 * k:8 * k + 8], U32)
                v = pltpu.bitcast(src[r:r + n, t * 128:(t + 1) * 128], U32)
                v = jnp.where(off, jnp.concatenate([tok] * (n // 16), axis=0), v)
                dst[r // 2:(r + n) // 2, :] = v

    def tail_pre(k):
        for u in tail_units[k * U_TAIL // 4:(k + 1) * U_TAIL // 4]:
            b_pre(u, copy_some)

    def regroup(tmp_v, t, base, g):
        parts = []
        for dp in (2 * g, 2 * g + 1):
            v = tmp_v[t, pl.ds(base + dp, A_H, stride=A_DH // 2), :]
            parts.append(pltpu.bitcast(v << 16, F32))
            parts.append(pltpu.bitcast(v & jnp.uint32(0xFFFF0000), F32))
        return jnp.concatenate(parts, axis=0).astype(BF16)

    def a_prep1(p):
        for b in range(p * LT, (p + 1) * LT):
            blk = pltpu.bitcast(wqkv_v[:, b * 128:(b + 1) * 128].T, U32)
            for t in range(LT):
                tmp_v[t, b * 64:(b + 1) * 64, :] = blk[:, t * 128:(t + 1) * 128]

    def a_prep2(p):
        for g in range(LT):
            blk = jnp.concatenate([regroup(tmp_v, t, p * D // 2, g) for t in range(LT)], axis=1)
            b = p * LT + g
            wqkvp_v[:, b * 128:(b + 1) * 128] = pltpu.bitcast(blk.T, U32)

    def a_prep4():
        for g in range(LT):
            for t in range(LT):
                woap_v[g * 64:(g + 1) * 64, t * 128:(t + 1) * 128] = pltpu.bitcast(
                    regroup(tmp2_v, t, 0, g), U32)

    if SEARCH:
        a_prep1 = a_prep2 = lambda p: None
        a_prep4 = lambda: None
        copies.clear()
    a_prep1(0)
    a_prep1(1)
    tail_pre(0)
    a_prep1(2)
    a_prep2(0)
    tail_pre(1)
    a_prep2(1)
    tail_pre(2)
    a_prep2(2)
    a_prep4()
    tail_pre(3)
    for t in range(LT, 3 * LT):
        slab_v[t, 0:A_PAD, :] = jnp.zeros((A_PAD, 128), F32)
    assert not copies
    cp_mem.wait()
    cp_bx.wait()
    cp_ax.wait()

    a_scale = A_DH ** (-0.5)
    b_scale = B_DH ** (-0.5)
    qrow = jax.lax.broadcasted_iota(jnp.int32, (32, 2 * B_L), 0)
    lane = jax.lax.broadcasted_iota(jnp.int32, (32, 2 * B_L), 1)
    first = lane < B_L
    kcol = jnp.where(first, lane, lane - B_L)
    allowed = (qrow >= B_SEG - 8) | (kcol >= B_SEG) | (qrow + 8 >= kcol)

    def blockdiag(t):
        n = t.shape[0]
        left = jax.lax.broadcasted_iota(jnp.int32, (n, 128), 1) < 64
        z = jnp.zeros((n, 128), F32)
        mid = t[:, 128:256]
        top = jnp.concatenate([t[:, 0:128], jnp.where(left, mid, 0.0), z], axis=1)
        bot = jnp.concatenate([z, jnp.where(left, 0.0, mid), t[:, 256:384]], axis=1)
        return jnp.concatenate([top, bot], axis=0).astype(BF16)

    def softmax(s):
        s = jnp.where(allowed, s * b_scale, NEG)
        ma = jnp.max(jnp.where(first, s, -jnp.inf), axis=1, keepdims=True)
        mb = jnp.max(jnp.where(first, -jnp.inf, s), axis=1, keepdims=True)
        p = jnp.exp(s - jnp.where(first, ma, mb))
        la = jnp.sum(jnp.where(first, p, 0.0), axis=1, keepdims=True)
        lb = jnp.sum(jnp.where(first, 0.0, p), axis=1, keepdims=True)
        return (p * _recip(jnp.where(first, la, lb))).astype(BF16)

    def head8(q, kv_x, kv_m, second):
        left = jax.lax.broadcasted_iota(jnp.int32, (8, 128), 1) < 64
        row = jax.lax.broadcasted_iota(jnp.int32, (8, 128), 0)
        t = 2 if second else 0
        qa = q[:, t * 128:(t + 1) * 128] * (b_scale * LOG2E)
        qb = q[:, 128:256] * (b_scale * LOG2E)
        qb = jnp.where(left, 0.0, qb) if second else jnp.where(left, qb, 0.0)

        def bc(k, t):
            src = kv_x if k < 8 else kv_m
            return jnp.broadcast_to(src[k % 8:k % 8 + 1, t * 128:(t + 1) * 128], (8, 128))

        sc = []
        for k in range(16):
            x = jnp.sum(qa * bc(k, t) + qb * bc(k, 1), axis=1, keepdims=True)
            x = jnp.broadcast_to(x, (8, 128))
            if 0 < k < 8:
                x = jnp.where(row >= k, x, NEG * LOG2E)
            sc.append(x)
        m = functools.reduce(jnp.maximum, sc)
        p = [jnp.exp2(x - m) for x in sc]
        inv = _recip(functools.reduce(jnp.add, p))
        return [functools.reduce(jnp.add, [p[k] * bc(k, 3 + tt) for k in range(16)]) * inv
                for tt in (t, 1)], inv

    def segment(i, h, even, extra):
        qkv, prob, att, q8, o8 = {}, {}, {}, {}, {}
        acc = [None]
        hh = [h]
        parts = []
        pins = extra['pins']

        def proj(j, part):
            dues = DUE_E if even else DUE_O
            cuts = sorted({3 * part, 3 * part + 3}
                          | {m for (jj, m) in dues if jj == j and m // 3 == part})
            for m, m2 in zip(cuts[:-1], cuts[1:]):
                due = [x for key in dues.get((j, m), ()) for x in pins.pop(key)]
                if due:
                    hh[0] = extra['pin'](hh[0], due)
                w = wb_v[3 * j + part, :, (m - 3 * part) * 128:(m2 - 3 * part) * 128]
                parts.append(jnp.dot(hh[0], pltpu.bitcast(w, BF16), preferred_element_type=F32))
            if part < 2:
                return
            r = jnp.concatenate(parts, axis=1)
            parts.clear()
            if even:
                rows = pl.ds(pl.multiple_of(i * (PRE // 2), PRE // 2), PRE // 2)
                pre = jnp.concatenate([pre_v[3 * j + m, rows, :] for m in range(3)], axis=1)
                pre = pltpu.bitcast(pre, BF16).astype(F32)
                qo_v[j] = r[16:24, :PAIR]
                kvo_v[j] = r[16:24, PAIR:]
                q8[j] = (pre[0:8, :PAIR], pre[0:8, PAIR:], r[24:32, PAIR:])
                q = jnp.concatenate([pre[8:16, :PAIR], r[0:16, :PAIR], r[24:32, :PAIR]], axis=0)
                kv = jnp.concatenate([pre[:, PAIR:], r[0:16, PAIR:], r[24:32, PAIR:]], axis=0)
            else:
                q8[j] = (qo_v[j], kvo_v.at[j], r[24:32, PAIR:])
                q = r[:, :PAIR]
                kv = jnp.concatenate([kvo_v[j], r[:, PAIR:]], axis=0)
            qkv[j] = (q.astype(BF16), blockdiag(kv[:, :PAIR]), blockdiag(kv[:, PAIR:]))

        def vector(jj):
            j, second = jj // 2, jj % 2
            o, inv = head8(*q8[j], second)
            pins[('u' if even else 'U', jj)] = [pltpu.bitcast(x, U32) for x in o]
            pins[('i' if even else 'I', jj)] = [pltpu.bitcast(inv, U32)]
            if not second:
                o8[j] = o
                return
            left = jax.lax.broadcasted_iota(jnp.int32, (8, 128), 1) < 64
            o = jnp.concatenate([o8[j][0], jnp.where(left, o8[j][1], o[1]), o[0]], axis=1)
            if even:
                o8_v[j] = o
            else:
                o8[j] = o

        def scores(j):
            prob[j] = softmax(_nt(qkv[j][0], qkv[j][1]))

        def values(j):
            att[j] = jnp.dot(prob[j], qkv[j][2], preferred_element_type=F32)

        def outp(j, t):
            lhs = att[j] if even else jnp.concatenate([att[j], o8_v[j], o8[j]], axis=0)
            lhs = lhs[:, t * 128:(t + 1) * 128].astype(BF16)
            r = j * PAIR // 2 + t * 64
            d = jnp.dot(lhs, pltpu.bitcast(wob_v[r:r + 64, :], BF16), preferred_element_type=F32)
            acc[0] = d if acc[0] is None else acc[0] + d

        fns = dict(s=scores, v=values, u=vector)
        for t in range(3):
            fns['xyz'[t]] = functools.partial(proj, part=t)
            fns['ABC'[t]] = functools.partial(outp, t=t)
        for k, j in (SCHED_E if even else SCHED_O):
            if k in fns:
                fns[k](j)
            else:
                extra[k](j)
        return acc[0]

    def body(i, mem):
        r0 = pl.multiple_of(i * BLK, BLK)

        def a_qkv(b):
            x = ax_v[pl.ds(r0, BLK), :]
            slab_v[b, A_PAD:A_PAD + BLK, :] = _nn(
                x, pltpu.bitcast(wqkvp_v[:, b * 128:(b + 1) * 128], BF16))

        a_o, a_p = {}, {}
        never = i < 0
        pins = {}

        def a_logits(sb):
            base = A_PAD + sb * A_SUB
            q = [slab_v[t, base:base + A_SUB, :] for t in range(LT)]
            logits = []
            for w in range(A_W):
                lo = base - A_DIL * w
                acc = None
                for t in range(LT):
                    pr = q[t] * slab_v[LT + t, lo:lo + A_SUB, :]
                    acc = pr if acc is None else acc + pr
                acc = acc + pltpu.roll(acc, 64, 1)
                acc = acc + pltpu.roll(acc, 32, 1)
                acc = acc * a_scale
                if sb == 0 and w > 0:
                    row = jax.lax.broadcasted_iota(jnp.int32, (A_SUB, 128), 0) + r0
                    acc = jnp.where(row >= A_DIL * w, acc, NEG)
                logits.append(acc)
            m = logits[0]
            for w in range(1, A_W):
                m = jnp.maximum(m, logits[w])
            ps = [jnp.exp(l - m) for l in logits]
            den = ps[0]
            for w in range(1, A_W):
                den = den + ps[w]
            inv = _recip(den)
            a_p[sb] = (ps, inv)
            pins[('a', sb)] = [pltpu.bitcast(inv[8 * u:8 * u + 8], U32) for u in range(A_SUB // 8)]

        def a_values(sb):
            base = A_PAD + sb * A_SUB
            ps, inv = a_p[sb]
            o = []
            for t in range(LT):
                acc = None
                for w in range(A_W):
                    lo = base - A_DIL * w
                    pr = ps[w] * slab_v[2 * LT + t, lo:lo + A_SUB, :]
                    acc = pr if acc is None else acc + pr
                o.append(acc * inv)
            pins[('b', sb)] = [pltpu.bitcast(x[8 * u:8 * u + 8], U32) for x in o
                               for u in range(A_SUB // 8)]
            a_o[sb] = jnp.concatenate(o, axis=1)
            if sb == BLK // A_SUB - 1:
                for t in range(LT, 3 * LT):
                    slab_v[t, 0:A_PAD, :] = slab_v[t, BLK:BLK + A_PAD, :]

        def pin(h, due):
            u = pltpu.bitcast(h, U32)
            tiles = [u[8 * r:8 * r + 8, 128 * c:128 * c + 128]
                     for c in range(LT) for r in range(u.shape[0] // 8)]
            for k, x in enumerate(due):
                tiles[k % len(tiles)] = jnp.where(never, x, tiles[k % len(tiles)])
            n = u.shape[0] // 8
            cols = [jnp.concatenate(tiles[c * n:(c + 1) * n], axis=0) for c in range(LT)]
            return pltpu.bitcast(jnp.concatenate(cols, axis=1), BF16)

        def a_out(b):
            o = jnp.concatenate([a_o[sb] for sb in range(BLK // A_SUB)], axis=0).astype(BF16)
            res = jnp.dot(o, pltpu.bitcast(woap_v[:, b * 128:(b + 1) * 128], BF16), preferred_element_type=F32)
            outa_v[pl.ds(r0, BLK), b * 128:(b + 1) * 128] = res.astype(BF16)

        x = bx_v[i].astype(F32)
        ex_e = ex_o = dict(q=a_qkv, a=a_logits, b=a_values, w=a_out, pin=pin, pins=pins)
        acc = segment(i, jnp.concatenate([x[16:40], mem], axis=0).astype(BF16), True,
                      ex_e)
        out_e = acc[0:24]
        mem = acc[24:32].astype(BF16).astype(F32)
        acc = segment(i, jnp.concatenate([x[40:64], mem], axis=0).astype(BF16), False,
                      ex_o)
        out = jnp.concatenate([acc[32:40], out_e, acc[40:48], acc[0:24]], axis=0)
        outb_v[pl.ds(r0, BLK), :] = out.astype(BF16)
        pltpu.make_async_copy(
            outa_v.at[pl.ds(r0, BLK)], out_h.at[pl.ds(r0, BLK), pl.ds(0, D)], sem_out.at[0]).start()
        pltpu.make_async_copy(
            outb_v.at[pl.ds(r0, BLK)], out_h.at[pl.ds(r0, BLK), pl.ds(D, D)], sem_out.at[1]).start()
        return acc[24:32].astype(BF16).astype(F32)

    def body_n(ii, mem):
        for u in range(UNROLL):
            mem = body(ii * UNROLL + u, mem)
        return mem

    jax.lax.fori_loop(0, NLOOP // UNROLL, body_n, mem0_v[...].astype(F32))

    pltpu.make_async_copy(outa_v.at[0:NLOOP * BLK], out_h.at[0:NLOOP * BLK, pl.ds(0, D)], sem_out.at[0]).wait()
    pltpu.make_async_copy(outb_v.at[0:NLOOP * BLK], out_h.at[0:NLOOP * BLK, pl.ds(D, D)], sem_out.at[1]).wait()


@functools.partial(jax.jit, static_argnames=("B_seg_len",))
def pallas_concat_heads__sliding_local_dilated__memory_aug_recurrent_mem_tr__prompt_kernel(
    A_x: jax.Array,
    A_wqkv: jax.Array,
    A_wo: jax.Array,
    B_x: jax.Array,
    B_mem0: jax.Array,
    B_Wq: jax.Array,
    B_Wk: jax.Array,
    B_Wv: jax.Array,
    B_Wo: jax.Array,
    B_seg_len: int,
):
    assert A_x.shape == (1, S, D) and B_x.shape == (1, S, D)
    assert B_seg_len == B_SEG and B_mem0.shape == (1, B_M, D)
    assert B_Wq.shape == (D, B_H, B_DH) and B_Wo.shape == (B_H, B_DH, D)

    def feat_major(w):
        return jnp.transpose(w, (1, 2, 0)).reshape(B_F, D)

    any_spec = pl.BlockSpec(memory_space=pl.ANY)
    out = pl.pallas_call(
        _kernel,
        out_shape=jax.ShapeDtypeStruct((S, 2 * D), BF16),
        in_specs=[any_spec] * 9,
        out_specs=any_spec,
        scratch_shapes=[
            pltpu.VMEM((S, D), BF16),
            pltpu.VMEM((D, 3 * D), BF16),
            pltpu.VMEM((D, D), BF16),
            pltpu.VMEM((NIT, BLK, D), BF16),
            pltpu.VMEM((NIT, PRE, D), BF16),
            pltpu.VMEM((B_M, D), BF16),
            pltpu.VMEM((NU, PAIR, D), BF16),
            pltpu.VMEM((B_F, D), BF16),
            pltpu.VMEM((LT, 3 * D // 2, 128), U32),
            pltpu.VMEM((LT, D // 2, 128), U32),
            pltpu.VMEM((B_F // 2, D), U32),
            pltpu.VMEM((D // 2, 3 * D), U32),
            pltpu.VMEM((D // 2, D), U32),
            pltpu.VMEM((3 * LT, A_PAD + BLK, 128), F32),
            pltpu.VMEM((S, D), BF16),
            pltpu.VMEM((NU, D // 2, PAIR), U32),
            pltpu.VMEM((NU, NIT * PRE // 2, PAIR), U32),
            pltpu.VMEM((NPAIR, 8, PAIR), F32),
            pltpu.VMEM((NPAIR, 8, 2 * PAIR), F32),
            pltpu.VMEM((NPAIR, 8, PAIR), F32),
            pltpu.VMEM((S, D), BF16),
            pltpu.SemaphoreType.DMA((8 + len(U_HEAD) + U_N,)),
            pltpu.SemaphoreType.DMA((2,)),
        ],
        compiler_params=pltpu.CompilerParams(vmem_limit_bytes=120 * 1024 * 1024,
                                             disable_bounds_checks=True),
    )(
        A_x.reshape(S, D), A_wqkv, A_wo, B_x.reshape(NIT, BLK, D), B_mem0.reshape(B_M, D),
        feat_major(B_Wq), feat_major(B_Wk), feat_major(B_Wv), B_Wo.reshape(B_F, D),
    )
    return out.reshape(1, S, 2 * D)
```

```python
import functools

import jax
import jax.numpy as jnp
import jax.experimental.pallas as pl
import jax.experimental.pallas.tpu as pltpu

F32 = jnp.float32
BF16 = jnp.bfloat16
U32 = jnp.uint32

S = 2048
D = 640
LT = D // 128
BLK = 64
NIT = S // BLK

A_H = 32
A_DH = 20
A_W = 8
A_DIL = 2
A_PAD = 16
A_SUB = 16

B_H = 32
B_DH = 192
B_F = B_H * B_DH
B_M = 8
B_SEG = 32
B_L = B_M + B_SEG
PAIR = 2 * B_DH
NPAIR = B_H // 2
NU = 3 * NPAIR
PRE = 16
PRE_MB = 128

NEG = -1000000000.0
LOG2E = 1.4426950408889634
LAG_S, LAG_V, LAG_O = [int(v) for v in "1,3,5".split(",")]
ORDER = "povs"
UNROLL = int("2")
U_HEAD = [int(v) for v in "1,1,2".split(",")]
U_BODY = int("5")
U_N = int("8")
U_TAIL = NU - sum(U_HEAD) - U_BODY * U_N
SEARCH = int("0")
XH = int("16")
DEFER = [int(v) for v in "1".split(",") if v.strip()]
PIN = int("1")
NLOOP = int("32")


def _schedule(order, lags, steady_extra, tail):
    lag = dict(p=0, s=lags[0], v=lags[1], o=lags[2])
    kind = dict(x="p", y="p", z="p", A="o", B="o", C="o", s="s", v="v")
    seq = []
    for t in range(NPAIR):
        for k in order:
            j = t - lag[kind[k]]
            if j >= 0:
                if k in "xAsv":
                    seq += steady_extra.get("<" + kind[k] + str(j), [])
                seq.append((k, j))
                if k in "zCsv":
                    seq += steady_extra.get(kind[k] + str(j), [])
            if t == NPAIR - 1 and k == "z":
                break
    for x in tail.split():
        seq += [(k, int(x[1:])) for k in ("ABC" if x[0] == "o" else x[0])
                if (k, int(x[1:])) not in seq]
    for k in "xyzABCsv":
        assert [j for kk, j in seq if kk == k] == list(range(NPAIR)), (k, seq)
    return seq


def _ex(txt):
    d = {}
    for x in txt.split():
        key, val = x.split(":")
        d.setdefault(key, []).append((val[0], int(val[1:])))
    return d


def _due(txt):
    d = {}
    for x in txt.split():
        key, at = x.split("@")
        j, m = at.split(".")
        d.setdefault((int(j), int(m)), []).append((key[0], int(key[1:])))
    return d


def _vector_plan(ea, eb, ia, ua, ib, ub, last):
    es = [(j, e, d) for j in range(NPAIR) for e, d in enumerate((ea, eb))]
    ds = [(k, 2 * j + e, 9 * j + int(d)) for j in range(NPAIR)
          for k, e, d in (("i", 0, ia), ("u", 0, ua), ("i", 1, ib), ("u", 1, ub)) if int(d) > 0]
    emit = " ".join(f"{d[0]}{j + int(d[1:])}:u{2 * j + e}" for j, e, d in es
                    if j + int(d[1:]) <= last[d[0]])
    tail = " ".join(f"u{2 * j + e}" for j, e, d in es if j + int(d[1:]) > last[d[0]])
    due = " ".join(f"{k}{n}@{d // 9}.{d % 9}" for k, n, d in ds if d < 9 * NPAIR)
    late = " ".join(f"{k}{n}@{d // 9 - NPAIR}.{d % 9}" for k, n, d in ds if d >= 9 * NPAIR)
    return emit, tail, due, late


def _plan(oe, le, xe, te, ve, oo, lo, xo, to, vo, do):
    ve = _vector_plan(*ve.split(), dict(p=15, s=13))
    vo = _vector_plan(*vo.split(), dict(p=15, s=13))
    sched_e = _schedule(oe, [int(v) for v in le.split(",")], _ex(xe + " " + ve[0]),
                        te.replace("#", ve[1]))
    sched_o = _schedule(oo, [int(v) for v in lo.split(",")], _ex(xo + " " + vo[0]),
                        to.replace("#", vo[1]))
    due_o = vo[2].replace("u", "U").replace("i", "I") + " " + ve[3] + " " + do
    return (sched_e, _due(ve[2])), (sched_o, _due(due_o))


PLANS = [_plan(
    "xyzABCvs",
    "1,3,5",
    "<s0:q0 <s1:q1 <s2:q2 <s5:q3 <s8:q4 <s10:q5 <s11:q6 <s13:q7",
    "v12 s14 q8 v13 s15 # o10 o11 o12 v14 o13 v15 o14 q9 o15 q10 q11",
    "s0 s0 0 25 0 27",
    "xAyzBCvs",
    "1,3,5",
    "<s0:q12 <s1:q13 <s2:q14 p3:a0 p4:b0 p6:a1 p7:b1 p8:a2 p9:b2 p11:a3 p12:b3",
    "v12 s14 o10 v13 s15 # o11 o12 v14 o13 v15 w0 o14 o15 w1 w2 w3 w4",
    "s0 s0 0 24 0 28",
    "a0@4.6 b0@5.6 a1@7.6 b1@8.6 a2@9.6 b2@10.6 a3@12.6 b3@13.6",
), _plan(
    "xyABzCvs",
    "1,3,5",
    "<s0:q0 <s1:q1 <s2:q2 <s5:q3 <s8:q4 <s10:q5 <s11:q6 <s13:q7",
    "v12 s14 q8 v13 s15 # o10 o11 o12 v14 o13 v15 o14 q9 o15 q10 q11",
    "s0 s0 0 25 0 27",
    "xAyBzCvs",
    "1,3,5",
    "<s0:q12 <s1:q13 <s2:q14 p4:a0 p5:b0 p6:a1 p7:b1 p9:a2 p10:b2 p11:a3 p12:b3",
    "v12 s14 o10 v13 s15 # o11 o12 v14 o13 v15 o14 w0 o15 w1 w2 w3 w4",
    "s0 s0 0 24 0 28",
    "a0@6.2 b0@7.2 a1@8.2 b1@9.2 a2@11.2 b2@12.2 a3@13.2 b3@14.2",
)]


def _nt(a, b):
    return jax.lax.dot_general(a, b, (((1,), (1,)), ((), ())), preferred_element_type=F32)


def _nn(a, b):
    return jnp.dot(a, b, preferred_element_type=F32)


def _recip(x):
    r = pl.reciprocal(x, approx=True)
    return r * (2.0 - x * r)


def _kernel(ax_h, wqkv_h, woa_h, bx_h, mem0_h, wq_h, wk_h, wv_h, wo_h, out_h,
            ax_v, wqkv_v, woa_v, bx_v, xpre_v, mem0_v, wraw_v, wo_v,
            tmp_v, tmp2_v, wob_v, wqkvp_v, woap_v, slab_v, outa_v,
            wb_v, pre_v, qo_v, kvo_v, o8_v, mid_v, outb_v,
            sem_in, sem_out):
    cp_xpre = [pltpu.make_async_copy(bx_h.at[pl.ds(a, n), pl.ds(0, PRE), :], xpre_v.at[pl.ds(a, n)],
                                     sem_in.at[s])
               for a, n, s in ((0, XH, 0), (XH, NIT - XH, 7 + len(U_HEAD) + U_N + 1))]
    cp_wqkv = pltpu.make_async_copy(wqkv_h, wqkv_v, sem_in.at[1])
    cp_woa = pltpu.make_async_copy(woa_h, woa_v, sem_in.at[2])
    cp_mem = pltpu.make_async_copy(mem0_h, mem0_v, sem_in.at[3])
    cp_bx = pltpu.make_async_copy(bx_h, bx_v, sem_in.at[4])
    cp_ax = pltpu.make_async_copy(ax_h, ax_v, sem_in.at[5])
    cp_wo = pltpu.make_async_copy(wo_h, wo_v, sem_in.at[6])
    w_hs = (wq_h, wk_h, wv_h)
    groups = list(U_HEAD) + [U_BODY] * U_N + [U_TAIL]
    g_start = [sum(groups[:g]) for g in range(len(groups))]

    cp_xpre[0].start()
    for g, n in enumerate(groups):
        for u in range(g_start[g], g_start[g] + n):
            pltpu.make_async_copy(w_hs[u % 3].at[pl.ds(u // 3 * PAIR, PAIR)], wraw_v.at[u],
                                  sem_in.at[7 + g]).start()
        if g == 0:
            cp_xpre[1].start()
    cp_wo.start()
    cp_wqkv.start()
    cp_woa.start()
    cp_mem.start()
    cp_bx.start()
    cp_ax.start()

    def g_wait(g, u0, n):
        buf = wraw_v.at[pl.ds(u0, n)]
        pltpu.make_async_copy(buf, buf, sem_in.at[7 + g]).wait()

    def b_pre(u, after=None, mbs=None):
        blk = wraw_v[u]
        if mbs is None or mbs[0] == 0:
            wb_v[u] = pltpu.bitcast(blk.T, U32)
        nb = PRE_MB // PRE
        for mb in (range(NIT // nb) if mbs is None else mbs):
            x = xpre_v[mb * nb:(mb + 1) * nb].reshape(PRE_MB, D)
            for n in range(PAIR // 128):
                r = _nt(x, blk[n * 128:(n + 1) * 128])
                pre_v[u, mb * PRE_MB // 2:(mb + 1) * PRE_MB // 2, n * 128:(n + 1) * 128] = (
                    pltpu.bitcast(r.astype(BF16), U32))
                if after is not None:
                    after(r)

    cp_xpre[0].wait()
    if SEARCH:
        b_pre = lambda u, after=None, mbs=None: None
    g_wait(0, 0, 1)
    nh = XH * PRE // PRE_MB
    b_pre(0, mbs=list(range(nh)))
    cp_xpre[1].wait()
    b_pre(0, mbs=list(range(nh, NIT * PRE // PRE_MB)))
    for g, n in enumerate(U_HEAD):
        if g == 0:
            continue
        g_wait(g, g_start[g], n)
        for u in range(g_start[g], g_start[g] + n):
            b_pre(u)

    def pre_body(c, carry):
        u0 = sum(U_HEAD) + c * U_BODY
        g_wait(len(U_HEAD) + c, u0, U_BODY)
        for k in range(U_BODY):
            b_pre(u0 + k)
        return carry + c

    off = jax.lax.fori_loop(0, U_N, pre_body, 0) < 0

    g_wait(len(groups) - 1, g_start[-1], U_TAIL)
    cp_wqkv.wait()
    cp_woa.wait()
    cp_wo.wait()
    tail_units = list(range(g_start[-1], NU))

    copies = [(woa_v, r, 32, t, tmp2_v.at[t]) for t in range(LT) for r in range(0, D, 32)]
    copies += [(wo_v, r, 48, t, wob_v.at[:, pl.ds(t * 128, 128)])
               for r in range(0, B_F, 48) for t in range(LT)]

    def copy_some(res):
        for k in range(res.shape[0] // 8):
            if copies:
                src, r, n, t, dst = copies.pop(0)
                tok = pltpu.bitcast(res[8 * k:8 * k + 8], U32)
                v = pltpu.bitcast(src[r:r + n, t * 128:(t + 1) * 128], U32)
                v = jnp.where(off, jnp.concatenate([tok] * (n // 16), axis=0), v)
                dst[r // 2:(r + n) // 2, :] = v

    def tail_pre(k):
        for u in tail_units[k * U_TAIL // 4:(k + 1) * U_TAIL // 4]:
            b_pre(u, copy_some)

    def regroup(tmp_v, t, base, g):
        parts = []
        for dp in (2 * g, 2 * g + 1):
            v = tmp_v[t, pl.ds(base + dp, A_H, stride=A_DH // 2), :]
            parts.append(pltpu.bitcast(v << 16, F32))
            parts.append(pltpu.bitcast(v & jnp.uint32(0xFFFF0000), F32))
        return jnp.concatenate(parts, axis=0).astype(BF16)

    def a_prep1(p):
        for b in range(p * LT, (p + 1) * LT):
            blk = pltpu.bitcast(wqkv_v[:, b * 128:(b + 1) * 128].T, U32)
            for t in range(LT):
                tmp_v[t, b * 64:(b + 1) * 64, :] = blk[:, t * 128:(t + 1) * 128]

    def a_prep2(p):
        for g in range(LT):
            blk = jnp.concatenate([regroup(tmp_v, t, p * D // 2, g) for t in range(LT)], axis=1)
            b = p * LT + g
            wqkvp_v[:, b * 128:(b + 1) * 128] = pltpu.bitcast(blk.T, U32)

    def a_prep4():
        for g in range(LT):
            for t in range(LT):
                woap_v[g * 64:(g + 1) * 64, t * 128:(t + 1) * 128] = pltpu.bitcast(
                    regroup(tmp2_v, t, 0, g), U32)

    if SEARCH:
        a_prep1 = a_prep2 = lambda p: None
        a_prep4 = lambda: None
        copies.clear()
    a_prep1(0)
    a_prep1(1)
    tail_pre(0)
    a_prep1(2)
    a_prep2(0)
    tail_pre(1)
    a_prep2(1)
    tail_pre(2)
    a_prep2(2)
    a_prep4()
    tail_pre(3)
    for t in range(LT, 3 * LT):
        slab_v[t, 0:A_PAD, :] = jnp.zeros((A_PAD, 128), F32)
    assert not copies
    cp_mem.wait()
    cp_bx.wait()
    cp_ax.wait()

    a_scale = A_DH ** (-0.5)
    b_scale = B_DH ** (-0.5)
    qrow = jax.lax.broadcasted_iota(jnp.int32, (32, 2 * B_L), 0)
    lane = jax.lax.broadcasted_iota(jnp.int32, (32, 2 * B_L), 1)
    first = lane < B_L
    kcol = jnp.where(first, lane, lane - B_L)
    allowed = (qrow >= B_SEG - 8) | (kcol >= B_SEG) | (qrow + 8 >= kcol)

    def blockdiag(t):
        n = t.shape[0]
        left = jax.lax.broadcasted_iota(jnp.int32, (n, 128), 1) < 64
        z = jnp.zeros((n, 128), F32)
        mid = t[:, 128:256]
        top = jnp.concatenate([t[:, 0:128], jnp.where(left, mid, 0.0), z], axis=1)
        bot = jnp.concatenate([z, jnp.where(left, 0.0, mid), t[:, 256:384]], axis=1)
        return jnp.concatenate([top, bot], axis=0).astype(BF16)

    def softmax(s):
        s = jnp.where(allowed, s * b_scale, NEG)
        ma = jnp.max(jnp.where(first, s, -jnp.inf), axis=1, keepdims=True)
        mb = jnp.max(jnp.where(first, -jnp.inf, s), axis=1, keepdims=True)
        p = jnp.exp(s - jnp.where(first, ma, mb))
        la = jnp.sum(jnp.where(first, p, 0.0), axis=1, keepdims=True)
        lb = jnp.sum(jnp.where(first, 0.0, p), axis=1, keepdims=True)
        return (p * _recip(jnp.where(first, la, lb))).astype(BF16)

    def head8(q, kv_x, kv_m, second):
        left = jax.lax.broadcasted_iota(jnp.int32, (8, 128), 1) < 64
        row = jax.lax.broadcasted_iota(jnp.int32, (8, 128), 0)
        t = 2 if second else 0
        qa = q[:, t * 128:(t + 1) * 128] * (b_scale * LOG2E)
        qb = q[:, 128:256] * (b_scale * LOG2E)
        qb = jnp.where(left, 0.0, qb) if second else jnp.where(left, qb, 0.0)

        def bc(k, t):
            src = kv_x if k < 8 else kv_m
            return jnp.broadcast_to(src[k % 8:k % 8 + 1, t * 128:(t + 1) * 128], (8, 128))

        sc = []
        for k in range(16):
            x = jnp.sum(qa * bc(k, t) + qb * bc(k, 1), axis=1, keepdims=True)
            x = jnp.broadcast_to(x, (8, 128))
            if 0 < k < 8:
                x = jnp.where(row >= k, x, NEG * LOG2E)
            sc.append(x)
        m = functools.reduce(jnp.maximum, sc)
        p = [jnp.exp2(x - m) for x in sc]
        inv = _recip(functools.reduce(jnp.add, p))
        return [functools.reduce(jnp.add, [p[k] * bc(k, 3 + tt) for k in range(16)]) * inv
                for tt in (t, 1)], inv

    def segment(i, sub, h, even, extra):
        qkv, prob, att, q8, o8 = {}, {}, {}, {}, {}
        acc = [None]
        hh = [h]
        parts = []
        pins = extra['pins']

        def proj(j, part):
            dues = PLANS[sub][0 if even else 1][1]
            cuts = sorted({3 * part, 3 * part + 3}
                          | {m for (jj, m) in dues if jj == j and m // 3 == part})
            for m, m2 in zip(cuts[:-1], cuts[1:]):
                due = [x for key in dues.get((j, m), ()) for x in pins.pop(key)]
                if due:
                    hh[0] = extra['pin'](hh[0], due)
                w = wb_v[3 * j + part, :, (m - 3 * part) * 128:(m2 - 3 * part) * 128]
                parts.append(jnp.dot(hh[0], pltpu.bitcast(w, BF16), preferred_element_type=F32))
            if part < 2:
                return
            r = jnp.concatenate(parts, axis=1)
            parts.clear()
            if even:
                rows = pl.ds(pl.multiple_of(i * (PRE // 2), PRE // 2), PRE // 2)
                pre = jnp.concatenate([pre_v[3 * j + m, rows, :] for m in range(3)], axis=1)
                pre = pltpu.bitcast(pre, BF16).astype(F32)
                qo_v[j] = r[16:24, :PAIR]
                kvo_v[j] = r[16:24, PAIR:]
                q8[j] = (pre[0:8, :PAIR], pre[0:8, PAIR:], r[24:32, PAIR:])
                q = jnp.concatenate([pre[8:16, :PAIR], r[0:16, :PAIR], r[24:32, :PAIR]], axis=0)
                kv = jnp.concatenate([pre[:, PAIR:], r[0:16, PAIR:], r[24:32, PAIR:]], axis=0)
            else:
                q8[j] = (qo_v[j], kvo_v.at[j], r[24:32, PAIR:])
                q = r[:, :PAIR]
                kv = jnp.concatenate([kvo_v[j], r[:, PAIR:]], axis=0)
            qkv[j] = (q.astype(BF16), blockdiag(kv[:, :PAIR]), blockdiag(kv[:, PAIR:]))

        def vector(jj):
            j, second = jj // 2, jj % 2
            o, inv = head8(*q8[j], second)
            pins[('u' if even else 'U', jj)] = [pltpu.bitcast(x, U32) for x in o]
            pins[('i' if even else 'I', jj)] = [pltpu.bitcast(inv, U32)]
            if not second:
                o8[j] = o
                return
            left = jax.lax.broadcasted_iota(jnp.int32, (8, 128), 1) < 64
            o = jnp.concatenate([o8[j][0], jnp.where(left, o8[j][1], o[1]), o[0]], axis=1)
            if even:
                o8_v[j] = o
            else:
                o8[j] = o

        def scores(j):
            prob[j] = softmax(_nt(qkv[j][0], qkv[j][1]))

        def values(j):
            att[j] = jnp.dot(prob[j], qkv[j][2], preferred_element_type=F32)

        acc16 = [None]

        def outp(j, t):
            lhs = att[j][:, t * 128:(t + 1) * 128]
            if even:
                wide = sub > 0 and t in DEFER
                if wide:
                    lhs = jnp.concatenate([lhs, mid_v[j, DEFER.index(t)]], axis=0)
            else:
                wide = sub == UNROLL - 1 or t not in DEFER
                o16 = jnp.concatenate([o8_v[j, :, t * 128:(t + 1) * 128],
                                       o8[j][:, t * 128:(t + 1) * 128]], axis=0)
                if wide:
                    lhs = jnp.concatenate([lhs, o16], axis=0)
                else:
                    mid_v[j, DEFER.index(t)] = o16
            lhs = lhs.astype(BF16)
            r = j * PAIR // 2 + t * 64
            d = jnp.dot(lhs, pltpu.bitcast(wob_v[r:r + 64, :], BF16), preferred_element_type=F32)
            acc[0] = d[0:32] if acc[0] is None else acc[0] + d[0:32]
            if wide:
                acc16[0] = d[32:48] if acc16[0] is None else acc16[0] + d[32:48]

        fns = dict(s=scores, v=values, u=vector)
        for t in range(3):
            fns['xyz'[t]] = functools.partial(proj, part=t)
            fns['ABC'[t]] = functools.partial(outp, t=t)
        for k, j in PLANS[sub][0 if even else 1][0]:
            if k in fns:
                fns[k](j)
            else:
                extra[k](j)
        return acc[0], acc16[0]

    def body(i, sub, mem, held):
        r0 = pl.multiple_of(i * BLK, BLK)

        def a_qkv(b):
            x = ax_v[pl.ds(r0, BLK), :]
            slab_v[b, A_PAD:A_PAD + BLK, :] = _nn(
                x, pltpu.bitcast(wqkvp_v[:, b * 128:(b + 1) * 128], BF16))

        a_o, a_p = {}, {}
        never = i < 0
        pins = {}

        def a_logits(sb):
            base = A_PAD + sb * A_SUB
            q = [slab_v[t, base:base + A_SUB, :] for t in range(LT)]
            logits = []
            for w in range(A_W):
                lo = base - A_DIL * w
                acc = None
                for t in range(LT):
                    pr = q[t] * slab_v[LT + t, lo:lo + A_SUB, :]
                    acc = pr if acc is None else acc + pr
                acc = acc + pltpu.roll(acc, 64, 1)
                acc = acc + pltpu.roll(acc, 32, 1)
                acc = acc * a_scale
                if sb == 0 and w > 0:
                    row = jax.lax.broadcasted_iota(jnp.int32, (A_SUB, 128), 0) + r0
                    acc = jnp.where(row >= A_DIL * w, acc, NEG)
                logits.append(acc)
            m = logits[0]
            for w in range(1, A_W):
                m = jnp.maximum(m, logits[w])
            ps = [jnp.exp(l - m) for l in logits]
            den = ps[0]
            for w in range(1, A_W):
                den = den + ps[w]
            inv = _recip(den)
            a_p[sb] = (ps, inv)
            pins[('a', sb)] = [pltpu.bitcast(inv[8 * u:8 * u + 8], U32) for u in range(A_SUB // 8)]

        def a_values(sb):
            base = A_PAD + sb * A_SUB
            ps, inv = a_p[sb]
            o = []
            for t in range(LT):
                acc = None
                for w in range(A_W):
                    lo = base - A_DIL * w
                    pr = ps[w] * slab_v[2 * LT + t, lo:lo + A_SUB, :]
                    acc = pr if acc is None else acc + pr
                o.append(acc * inv)
            pins[('b', sb)] = [pltpu.bitcast(x[8 * u:8 * u + 8], U32) for x in o
                               for u in range(A_SUB // 8)]
            a_o[sb] = jnp.concatenate(o, axis=1)
            if sb == BLK // A_SUB - 1:
                for t in range(LT, 3 * LT):
                    slab_v[t, 0:A_PAD, :] = slab_v[t, BLK:BLK + A_PAD, :]

        def pin(h, due):
            u = pltpu.bitcast(h, U32)
            tiles = [u[8 * r:8 * r + 8, 128 * c:128 * c + 128]
                     for c in range(LT) for r in range(u.shape[0] // 8)]
            for k, x in enumerate(due):
                tiles[k % len(tiles)] = jnp.where(never, x, tiles[k % len(tiles)])
            n = u.shape[0] // 8
            cols = [jnp.concatenate(tiles[c * n:(c + 1) * n], axis=0) for c in range(LT)]
            return pltpu.bitcast(jnp.concatenate(cols, axis=1), BF16)

        def a_out(b):
            o = jnp.concatenate([a_o[sb] for sb in range(BLK // A_SUB)], axis=0).astype(BF16)
            res = jnp.dot(o, pltpu.bitcast(woap_v[:, b * 128:(b + 1) * 128], BF16), preferred_element_type=F32)
            outa_v[pl.ds(r0, BLK), b * 128:(b + 1) * 128] = res.astype(BF16)

        x = bx_v[i].astype(F32)
        ex_e = ex_o = dict(q=a_qkv, a=a_logits, b=a_values, w=a_out, pin=pin, pins=pins)
        def emit(r, out_e, acc, acc16):
            out = jnp.concatenate([acc16[0:8], out_e, acc16[8:16], acc[0:24]], axis=0)
            outb_v[pl.ds(r, BLK), :] = out.astype(BF16)
            pltpu.make_async_copy(
                outb_v.at[pl.ds(r, BLK)], out_h.at[pl.ds(r, BLK), pl.ds(D, D)],
                sem_out.at[1]).start()

        acc, acc16 = segment(
            i, sub, jnp.concatenate([x[16:40], mem], axis=0).astype(BF16), True, ex_e)
        if held is not None:
            emit(held[0], held[1], held[2], held[3] + acc16)
        out_e = acc[0:24]
        mem = acc[24:32].astype(BF16).astype(F32)
        acc, acc16 = segment(
            i, sub, jnp.concatenate([x[40:64], mem], axis=0).astype(BF16), False, ex_o)
        held = (r0, out_e, acc, acc16)
        if sub == UNROLL - 1 or not DEFER:
            emit(*held)
            held = None
        pltpu.make_async_copy(
            outa_v.at[pl.ds(r0, BLK)], out_h.at[pl.ds(r0, BLK), pl.ds(0, D)], sem_out.at[0]).start()
        return acc[24:32].astype(BF16).astype(F32), held

    def body_n(ii, mem):
        held = None
        for u in range(UNROLL):
            mem, held = body(ii * UNROLL + u, u, mem, held)
        return mem

    jax.lax.fori_loop(0, NLOOP // UNROLL, body_n, mem0_v[...].astype(F32))

    pltpu.make_async_copy(outa_v.at[0:NLOOP * BLK], out_h.at[0:NLOOP * BLK, pl.ds(0, D)], sem_out.at[0]).wait()
    pltpu.make_async_copy(outb_v.at[0:NLOOP * BLK], out_h.at[0:NLOOP * BLK, pl.ds(D, D)], sem_out.at[1]).wait()


@functools.partial(jax.jit, static_argnames=("B_seg_len",))
def pallas_concat_heads__sliding_local_dilated__memory_aug_recurrent_mem_tr__prompt_kernel(
    A_x: jax.Array,
    A_wqkv: jax.Array,
    A_wo: jax.Array,
    B_x: jax.Array,
    B_mem0: jax.Array,
    B_Wq: jax.Array,
    B_Wk: jax.Array,
    B_Wv: jax.Array,
    B_Wo: jax.Array,
    B_seg_len: int,
):
    assert A_x.shape == (1, S, D) and B_x.shape == (1, S, D)
    assert B_seg_len == B_SEG and B_mem0.shape == (1, B_M, D)
    assert B_Wq.shape == (D, B_H, B_DH) and B_Wo.shape == (B_H, B_DH, D)

    def feat_major(w):
        return jnp.transpose(w, (1, 2, 0)).reshape(B_F, D)

    any_spec = pl.BlockSpec(memory_space=pl.ANY)
    out = pl.pallas_call(
        _kernel,
        out_shape=jax.ShapeDtypeStruct((S, 2 * D), BF16),
        in_specs=[any_spec] * 9,
        out_specs=any_spec,
        scratch_shapes=[
            pltpu.VMEM((S, D), BF16),
            pltpu.VMEM((D, 3 * D), BF16),
            pltpu.VMEM((D, D), BF16),
            pltpu.VMEM((NIT, BLK, D), BF16),
            pltpu.VMEM((NIT, PRE, D), BF16),
            pltpu.VMEM((B_M, D), BF16),
            pltpu.VMEM((NU, PAIR, D), BF16),
            pltpu.VMEM((B_F, D), BF16),
            pltpu.VMEM((LT, 3 * D // 2, 128), U32),
            pltpu.VMEM((LT, D // 2, 128), U32),
            pltpu.VMEM((B_F // 2, D), U32),
            pltpu.VMEM((D // 2, 3 * D), U32),
            pltpu.VMEM((D // 2, D), U32),
            pltpu.VMEM((3 * LT, A_PAD + BLK, 128), F32),
            pltpu.VMEM((S, D), BF16),
            pltpu.VMEM((NU, D // 2, PAIR), U32),
            pltpu.VMEM((NU, NIT * PRE // 2, PAIR), U32),
            pltpu.VMEM((NPAIR, 8, PAIR), F32),
            pltpu.VMEM((NPAIR, 8, 2 * PAIR), F32),
            pltpu.VMEM((NPAIR, 8, PAIR), F32),
            pltpu.VMEM((NPAIR, max(len(DEFER), 1), 16, 128), F32),
            pltpu.VMEM((S, D), BF16),
            pltpu.SemaphoreType.DMA((9 + len(U_HEAD) + U_N,)),
            pltpu.SemaphoreType.DMA((2,)),
        ],
        compiler_params=pltpu.CompilerParams(vmem_limit_bytes=120 * 1024 * 1024,
                                             disable_bounds_checks=True),
    )(
        A_x.reshape(S, D), A_wqkv, A_wo, B_x.reshape(NIT, BLK, D), B_mem0.reshape(B_M, D),
        feat_major(B_Wq), feat_major(B_Wk), feat_major(B_Wv), B_Wo.reshape(B_F, D),
    )
    return out.reshape(1, S, 2 * D)
```

```python
import functools

import jax
import jax.numpy as jnp
import jax.experimental.pallas as pl
import jax.experimental.pallas.tpu as pltpu

F32 = jnp.float32
BF16 = jnp.bfloat16
U32 = jnp.uint32

S = 2048
D = 640
LT = D // 128
BLK = 64
NIT = S // BLK

A_H = 32
A_DH = 20
A_W = 8
A_DIL = 2
A_PAD = 16
A_SUB = 16

B_H = 32
B_DH = 192
B_F = B_H * B_DH
B_M = 8
B_SEG = 32
B_L = B_M + B_SEG
PAIR = 2 * B_DH
NPAIR = B_H // 2
NU = 3 * NPAIR
PRE = 16
PRE_MB = 128

NEG = -1000000000.0
LOG2E = 1.4426950408889634
LAG_S, LAG_V, LAG_O = [int(v) for v in "1,3,5".split(",")]
ORDER = "povs"
UNROLL = int("2")
U_HEAD = [int(v) for v in "1,1,2".split(",")]
U_BODY = int("5")
U_N = int("8")
U_TAIL = NU - sum(U_HEAD) - U_BODY * U_N
SEARCH = int("0")
XH = int("16")
DEFER = [int(v) for v in "1".split(",") if v.strip()]
PIN = int("1")
NLOOP = int("32")


def _schedule(order, lags, steady_extra, tail):
    lag = dict(p=0, s=lags[0], v=lags[1], o=lags[2])
    kind = dict(x="p", y="p", z="p", A="o", B="o", C="o", s="s", v="v")
    seq = []
    for t in range(NPAIR):
        for k in order:
            j = t - lag[kind[k]]
            if j >= 0:
                if k in "xAsv":
                    seq += steady_extra.get("<" + kind[k] + str(j), [])
                seq.append((k, j))
                if k in "zCsv":
                    seq += steady_extra.get(kind[k] + str(j), [])
            if t == NPAIR - 1 and k == "z":
                break
    for x in tail.split():
        seq += [(k, int(x[1:])) for k in ("ABC" if x[0] == "o" else x[0])
                if (k, int(x[1:])) not in seq]
    for k in "xyzABCsv":
        assert [j for kk, j in seq if kk == k] == list(range(NPAIR)), (k, seq)
    return seq


def _ex(txt):
    d = {}
    for x in txt.split():
        key, val = x.split(":")
        d.setdefault(key, []).append((val[0], int(val[1:])))
    return d


def _due(txt):
    d = {}
    for x in txt.split():
        key, at = x.split("@")
        j, m = at.split(".")
        d.setdefault((int(j), int(m)), []).append((key[0], int(key[1:])))
    return d


def _vector_plan(ea, eb, ia, ua, ib, ub, last):
    es = [(j, e, d) for j in range(NPAIR) for e, d in enumerate((ea, eb))]
    ds = [(k, 2 * j + e, 9 * j + int(d)) for j in range(NPAIR)
          for k, e, d in (("i", 0, ia), ("u", 0, ua), ("i", 1, ib), ("u", 1, ub)) if int(d) > 0]
    emit = " ".join(f"{d[0]}{j + int(d[1:])}:u{2 * j + e}" for j, e, d in es
                    if j + int(d[1:]) <= last[d[0]])
    tail = " ".join(f"u{2 * j + e}" for j, e, d in es if j + int(d[1:]) > last[d[0]])
    due = " ".join(f"{k}{n}@{d // 9}.{d % 9}" for k, n, d in ds if d < 9 * NPAIR)
    late = " ".join(f"{k}{n}@{d // 9 - NPAIR}.{d % 9}" for k, n, d in ds if d >= 9 * NPAIR)
    return emit, tail, due, late


def _plan(oe, le, xe, te, ve, oo, lo, xo, to, vo, do):
    ve = _vector_plan(*ve.split(), dict(p=15, s=13))
    vo = _vector_plan(*vo.split(), dict(p=15, s=13))
    sched_e = _schedule(oe, [int(v) for v in le.split(",")], _ex(xe + " " + ve[0]),
                        te.replace("#", ve[1]))
    sched_o = _schedule(oo, [int(v) for v in lo.split(",")], _ex(xo + " " + vo[0]),
                        to.replace("#", vo[1]))
    due_o = vo[2].replace("u", "U").replace("i", "I") + " " + ve[3] + " " + do
    return (sched_e, _due(ve[2])), (sched_o, _due(due_o))


PLANS = [_plan(
    "xyzABCvs",
    "1,3,5",
    "<s0:q0 <s1:q1 <s2:q2 <s3:Q0 <s4:Q1 <s5:q3 <s6:Q2 <s7:Q3 <s8:q4 <s9:Q4 <s10:q5 <s11:q6 <s12:Q5 <s13:q7",
    "v12 s14 q8 v13 s15 # o10 o11 o12 v14 o13 v15 o14 q9 o15 q10 q11",
    "s0 s0 0 25 0 27",
    "xAyzBCvs",
    "1,3,5",
    "<s0:q12 <s1:q13 <s2:q14 p5:a0 p6:b0 p7:a1 p8:b1 p9:a2 p10:b2 p11:a3 p12:b3",
    "v12 s14 o10 v13 s15 # o11 o12 v14 o13 v15 w0 o14 o15 w1 w2 w3 w4",
    "s0 s0 0 24 0 28",
    "a0@7.0 b0@8.0 a1@9.0 b1@10.0 a2@11.0 b2@12.0 a3@13.0 b3@14.0",
), _plan(
    "xyABzCvs",
    "1,3,5",
    "<s0:q6 <s1:q7",
    "v12 s14 q8 v13 s15 # o10 o11 o12 v14 o13 v15 o14 q9 o15 q10 q11",
    "s0 s0 0 25 0 27",
    "xAyBzCvs",
    "1,3,5",
    "<s0:q12 <s1:q13 <s2:q14 p5:a0 p6:b0 p7:a1 p8:b1 p9:a2 p10:b2 p11:a3 p12:b3",
    "v12 s14 o10 v13 s15 # o11 o12 v14 o13 v15 o14 w0 o15 w1 w2 w3 w4",
    "s0 s0 0 24 0 28",
    "a0@6.0 b0@7.0 a1@8.0 b1@9.0 a2@10.0 b2@11.0 a3@12.0 b3@13.0",
)]


def _nt(a, b):
    return jax.lax.dot_general(a, b, (((1,), (1,)), ((), ())), preferred_element_type=F32)


def _nn(a, b):
    return jnp.dot(a, b, preferred_element_type=F32)


def _recip(x):
    r = pl.reciprocal(x, approx=True)
    return r * (2.0 - x * r)


def _kernel(ax_h, wqkv_h, woa_h, bx_h, mem0_h, wq_h, wk_h, wv_h, wo_h, out_h,
            ax_v, wqkv_v, woa_v, bx_v, xpre_v, mem0_v, wraw_v, wo_v,
            tmp_v, tmp2_v, wob_v, wqkvp_v, woap_v, slab_v, outa_v,
            wb_v, pre_v, qo_v, kvo_v, o8_v, mid_v, outb_v,
            sem_in, sem_out):
    cp_xpre = [pltpu.make_async_copy(bx_h.at[pl.ds(a, n), pl.ds(0, PRE), :], xpre_v.at[pl.ds(a, n)],
                                     sem_in.at[s])
               for a, n, s in ((0, XH, 0), (XH, NIT - XH, 7 + len(U_HEAD) + U_N + 1))]
    cp_wqkv = pltpu.make_async_copy(wqkv_h, wqkv_v, sem_in.at[1])
    cp_woa = pltpu.make_async_copy(woa_h, woa_v, sem_in.at[2])
    cp_mem = pltpu.make_async_copy(mem0_h, mem0_v, sem_in.at[3])
    cp_bx = pltpu.make_async_copy(bx_h, bx_v, sem_in.at[4])
    cp_ax = pltpu.make_async_copy(ax_h, ax_v, sem_in.at[5])
    cp_wo = pltpu.make_async_copy(wo_h, wo_v, sem_in.at[6])
    w_hs = (wq_h, wk_h, wv_h)
    groups = list(U_HEAD) + [U_BODY] * U_N + [U_TAIL]
    g_start = [sum(groups[:g]) for g in range(len(groups))]

    cp_xpre[0].start()
    for g, n in enumerate(groups):
        for u in range(g_start[g], g_start[g] + n):
            pltpu.make_async_copy(w_hs[u % 3].at[pl.ds(u // 3 * PAIR, PAIR)], wraw_v.at[u],
                                  sem_in.at[7 + g]).start()
        if g == 0:
            cp_xpre[1].start()
    cp_wo.start()
    cp_wqkv.start()
    cp_woa.start()
    cp_mem.start()
    cp_bx.start()
    cp_ax.start()

    def g_wait(g, u0, n):
        buf = wraw_v.at[pl.ds(u0, n)]
        pltpu.make_async_copy(buf, buf, sem_in.at[7 + g]).wait()

    def b_pre(u, after=None, mbs=None):
        blk = wraw_v[u]
        if mbs is None or mbs[0] == 0:
            wb_v[u] = pltpu.bitcast(blk.T, U32)
        nb = PRE_MB // PRE
        for mb in (range(NIT // nb) if mbs is None else mbs):
            x = xpre_v[mb * nb:(mb + 1) * nb].reshape(PRE_MB, D)
            for n in range(PAIR // 128):
                r = _nt(x, blk[n * 128:(n + 1) * 128])
                pre_v[u, mb * PRE_MB // 2:(mb + 1) * PRE_MB // 2, n * 128:(n + 1) * 128] = (
                    pltpu.bitcast(r.astype(BF16), U32))
                if after is not None:
                    after(r)

    cp_xpre[0].wait()
    if SEARCH:
        b_pre = lambda u, after=None, mbs=None: None
    g_wait(0, 0, 1)
    nh = XH * PRE // PRE_MB
    b_pre(0, mbs=list(range(nh)))
    cp_xpre[1].wait()
    b_pre(0, mbs=list(range(nh, NIT * PRE // PRE_MB)))
    for g, n in enumerate(U_HEAD):
        if g == 0:
            continue
        g_wait(g, g_start[g], n)
        for u in range(g_start[g], g_start[g] + n):
            b_pre(u)

    def pre_body(c, carry):
        u0 = sum(U_HEAD) + c * U_BODY
        g_wait(len(U_HEAD) + c, u0, U_BODY)
        for k in range(U_BODY):
            b_pre(u0 + k)
        return carry + c

    off = jax.lax.fori_loop(0, U_N, pre_body, 0) < 0

    g_wait(len(groups) - 1, g_start[-1], U_TAIL)
    cp_wqkv.wait()
    cp_woa.wait()
    cp_wo.wait()
    tail_units = list(range(g_start[-1], NU))

    copies = [(woa_v, r, 32, t, tmp2_v.at[t]) for t in range(LT) for r in range(0, D, 32)]
    copies += [(wo_v, r, 48, t, wob_v.at[:, pl.ds(t * 128, 128)])
               for r in range(0, B_F, 48) for t in range(LT)]

    def copy_some(res):
        for k in range(res.shape[0] // 8):
            if copies:
                src, r, n, t, dst = copies.pop(0)
                tok = pltpu.bitcast(res[8 * k:8 * k + 8], U32)
                v = pltpu.bitcast(src[r:r + n, t * 128:(t + 1) * 128], U32)
                v = jnp.where(off, jnp.concatenate([tok] * (n // 16), axis=0), v)
                dst[r // 2:(r + n) // 2, :] = v

    def tail_pre(k):
        for u in tail_units[k * U_TAIL // 4:(k + 1) * U_TAIL // 4]:
            b_pre(u, copy_some)

    def regroup(tmp_v, t, base, g):
        parts = []
        for dp in (2 * g, 2 * g + 1):
            v = tmp_v[t, pl.ds(base + dp, A_H, stride=A_DH // 2), :]
            parts.append(pltpu.bitcast(v << 16, F32))
            parts.append(pltpu.bitcast(v & jnp.uint32(0xFFFF0000), F32))
        return jnp.concatenate(parts, axis=0).astype(BF16)

    def a_prep1(p):
        for b in range(p * LT, (p + 1) * LT):
            blk = pltpu.bitcast(wqkv_v[:, b * 128:(b + 1) * 128].T, U32)
            for t in range(LT):
                tmp_v[t, b * 64:(b + 1) * 64, :] = blk[:, t * 128:(t + 1) * 128]

    def a_prep2(p):
        for g in range(LT):
            blk = jnp.concatenate([regroup(tmp_v, t, p * D // 2, g) for t in range(LT)], axis=1)
            b = p * LT + g
            wqkvp_v[:, b * 128:(b + 1) * 128] = pltpu.bitcast(blk.T, U32)

    def a_prep4():
        for g in range(LT):
            for t in range(LT):
                woap_v[g * 64:(g + 1) * 64, t * 128:(t + 1) * 128] = pltpu.bitcast(
                    regroup(tmp2_v, t, 0, g), U32)

    if SEARCH:
        a_prep1 = a_prep2 = lambda p: None
        a_prep4 = lambda: None
        copies.clear()
    a_prep1(0)
    a_prep1(1)
    tail_pre(0)
    a_prep1(2)
    a_prep2(0)
    tail_pre(1)
    a_prep2(1)
    tail_pre(2)
    a_prep2(2)
    a_prep4()
    tail_pre(3)
    for t in range(LT, 3 * LT):
        slab_v[0, t, 0:A_PAD, :] = jnp.zeros((A_PAD, 128), F32)
    assert not copies
    cp_mem.wait()
    cp_bx.wait()
    cp_ax.wait()

    a_scale = A_DH ** (-0.5)
    b_scale = B_DH ** (-0.5)
    qrow = jax.lax.broadcasted_iota(jnp.int32, (32, 2 * B_L), 0)
    lane = jax.lax.broadcasted_iota(jnp.int32, (32, 2 * B_L), 1)
    first = lane < B_L
    kcol = jnp.where(first, lane, lane - B_L)
    allowed = (qrow >= B_SEG - 8) | (kcol >= B_SEG) | (qrow + 8 >= kcol)

    def blockdiag(t):
        n = t.shape[0]
        left = jax.lax.broadcasted_iota(jnp.int32, (n, 128), 1) < 64
        z = jnp.zeros((n, 128), F32)
        mid = t[:, 128:256]
        top = jnp.concatenate([t[:, 0:128], jnp.where(left, mid, 0.0), z], axis=1)
        bot = jnp.concatenate([z, jnp.where(left, 0.0, mid), t[:, 256:384]], axis=1)
        return jnp.concatenate([top, bot], axis=0).astype(BF16)

    def softmax(s):
        s = jnp.where(allowed, s * b_scale, NEG)
        ma = jnp.max(jnp.where(first, s, -jnp.inf), axis=1, keepdims=True)
        mb = jnp.max(jnp.where(first, -jnp.inf, s), axis=1, keepdims=True)
        p = jnp.exp(s - jnp.where(first, ma, mb))
        la = jnp.sum(jnp.where(first, p, 0.0), axis=1, keepdims=True)
        lb = jnp.sum(jnp.where(first, 0.0, p), axis=1, keepdims=True)
        return (p * _recip(jnp.where(first, la, lb))).astype(BF16)

    def head8(q, kv_x, kv_m, second):
        left = jax.lax.broadcasted_iota(jnp.int32, (8, 128), 1) < 64
        row = jax.lax.broadcasted_iota(jnp.int32, (8, 128), 0)
        t = 2 if second else 0
        qa = q[:, t * 128:(t + 1) * 128] * (b_scale * LOG2E)
        qb = q[:, 128:256] * (b_scale * LOG2E)
        qb = jnp.where(left, 0.0, qb) if second else jnp.where(left, qb, 0.0)

        def bc(k, t):
            src = kv_x if k < 8 else kv_m
            return jnp.broadcast_to(src[k % 8:k % 8 + 1, t * 128:(t + 1) * 128], (8, 128))

        sc = []
        for k in range(16):
            x = jnp.sum(qa * bc(k, t) + qb * bc(k, 1), axis=1, keepdims=True)
            x = jnp.broadcast_to(x, (8, 128))
            if 0 < k < 8:
                x = jnp.where(row >= k, x, NEG * LOG2E)
            sc.append(x)
        m = functools.reduce(jnp.maximum, sc)
        p = [jnp.exp2(x - m) for x in sc]
        inv = _recip(functools.reduce(jnp.add, p))
        return [functools.reduce(jnp.add, [p[k] * bc(k, 3 + tt) for k in range(16)]) * inv
                for tt in (t, 1)], inv

    def segment(i, sub, h, even, extra):
        qkv, prob, att, q8, o8 = {}, {}, {}, {}, {}
        acc = [None]
        hh = [h]
        parts = []
        pins = extra['pins']

        def proj(j, part):
            dues = PLANS[sub][0 if even else 1][1]
            cuts = sorted({3 * part, 3 * part + 3}
                          | {m for (jj, m) in dues if jj == j and m // 3 == part})
            for m, m2 in zip(cuts[:-1], cuts[1:]):
                due = [x for key in dues.get((j, m), ()) for x in pins.pop(key)]
                if due:
                    hh[0] = extra['pin'](hh[0], due)
                w = wb_v[3 * j + part, :, (m - 3 * part) * 128:(m2 - 3 * part) * 128]
                parts.append(jnp.dot(hh[0], pltpu.bitcast(w, BF16), preferred_element_type=F32))
            if part < 2:
                return
            r = jnp.concatenate(parts, axis=1)
            parts.clear()
            if even:
                rows = pl.ds(pl.multiple_of(i * (PRE // 2), PRE // 2), PRE // 2)
                pre = jnp.concatenate([pre_v[3 * j + m, rows, :] for m in range(3)], axis=1)
                pre = pltpu.bitcast(pre, BF16).astype(F32)
                qo_v[j] = r[16:24, :PAIR]
                kvo_v[j] = r[16:24, PAIR:]
                q8[j] = (pre[0:8, :PAIR], pre[0:8, PAIR:], r[24:32, PAIR:])
                q = jnp.concatenate([pre[8:16, :PAIR], r[0:16, :PAIR], r[24:32, :PAIR]], axis=0)
                kv = jnp.concatenate([pre[:, PAIR:], r[0:16, PAIR:], r[24:32, PAIR:]], axis=0)
            else:
                q8[j] = (qo_v[j], kvo_v.at[j], r[24:32, PAIR:])
                q = r[:, :PAIR]
                kv = jnp.concatenate([kvo_v[j], r[:, PAIR:]], axis=0)
            qkv[j] = (q.astype(BF16), blockdiag(kv[:, :PAIR]), blockdiag(kv[:, PAIR:]))

        def vector(jj):
            j, second = jj // 2, jj % 2
            o, inv = head8(*q8[j], second)
            pins[('u' if even else 'U', jj)] = [pltpu.bitcast(x, U32) for x in o]
            pins[('i' if even else 'I', jj)] = [pltpu.bitcast(inv, U32)]
            if not second:
                o8[j] = o
                return
            left = jax.lax.broadcasted_iota(jnp.int32, (8, 128), 1) < 64
            o = jnp.concatenate([o8[j][0], jnp.where(left, o8[j][1], o[1]), o[0]], axis=1)
            if even:
                o8_v[j] = o
            else:
                o8[j] = o

        def scores(j):
            prob[j] = softmax(_nt(qkv[j][0], qkv[j][1]))

        def values(j):
            att[j] = jnp.dot(prob[j], qkv[j][2], preferred_element_type=F32)

        acc16 = [None]

        def outp(j, t):
            lhs = att[j][:, t * 128:(t + 1) * 128]
            if even:
                wide = sub > 0 and t in DEFER
                if wide:
                    lhs = jnp.concatenate([lhs, mid_v[j, DEFER.index(t)]], axis=0)
            else:
                wide = sub == UNROLL - 1 or t not in DEFER
                o16 = jnp.concatenate([o8_v[j, :, t * 128:(t + 1) * 128],
                                       o8[j][:, t * 128:(t + 1) * 128]], axis=0)
                if wide:
                    lhs = jnp.concatenate([lhs, o16], axis=0)
                else:
                    mid_v[j, DEFER.index(t)] = o16
            lhs = lhs.astype(BF16)
            r = j * PAIR // 2 + t * 64
            d = jnp.dot(lhs, pltpu.bitcast(wob_v[r:r + 64, :], BF16), preferred_element_type=F32)
            acc[0] = d[0:32] if acc[0] is None else acc[0] + d[0:32]
            if wide:
                acc16[0] = d[32:48] if acc16[0] is None else acc16[0] + d[32:48]

        fns = dict(s=scores, v=values, u=vector)
        for t in range(3):
            fns['xyz'[t]] = functools.partial(proj, part=t)
            fns['ABC'[t]] = functools.partial(outp, t=t)
        for k, j in PLANS[sub][0 if even else 1][0]:
            if k in fns:
                fns[k](j)
            else:
                extra[k](j)
        return acc[0], acc16[0]

    def body(i, sub, mem, held):
        r0 = pl.multiple_of(i * BLK, BLK)

        slab = slab_v.at[sub]

        def a_qkv(b, ahead=0):
            x = ax_v[pl.ds(r0 + ahead * BLK, BLK), :]
            slab_v[sub + ahead, b, A_PAD:A_PAD + BLK, :] = _nn(
                x, pltpu.bitcast(wqkvp_v[:, b * 128:(b + 1) * 128], BF16))

        a_o, a_p = {}, {}
        never = i < 0
        pins = {}

        def a_logits(sb):
            base = A_PAD + sb * A_SUB
            q = [slab[t, base:base + A_SUB, :] for t in range(LT)]
            logits = []
            for w in range(A_W):
                lo = base - A_DIL * w
                acc = None
                for t in range(LT):
                    pr = q[t] * slab[LT + t, lo:lo + A_SUB, :]
                    acc = pr if acc is None else acc + pr
                acc = acc + pltpu.roll(acc, 64, 1)
                acc = acc + pltpu.roll(acc, 32, 1)
                acc = acc * a_scale
                if sb == 0 and w > 0:
                    row = jax.lax.broadcasted_iota(jnp.int32, (A_SUB, 128), 0) + r0
                    acc = jnp.where(row >= A_DIL * w, acc, NEG)
                logits.append(acc)
            m = logits[0]
            for w in range(1, A_W):
                m = jnp.maximum(m, logits[w])
            ps = [jnp.exp(l - m) for l in logits]
            den = ps[0]
            for w in range(1, A_W):
                den = den + ps[w]
            inv = _recip(den)
            a_p[sb] = (ps, inv)
            pins[('a', sb)] = [pltpu.bitcast(inv[8 * u:8 * u + 8], U32) for u in range(A_SUB // 8)]

        def a_values(sb):
            base = A_PAD + sb * A_SUB
            ps, inv = a_p[sb]
            o = []
            for t in range(LT):
                acc = None
                for w in range(A_W):
                    lo = base - A_DIL * w
                    pr = ps[w] * slab[2 * LT + t, lo:lo + A_SUB, :]
                    acc = pr if acc is None else acc + pr
                o.append(acc * inv)
            pins[('b', sb)] = [pltpu.bitcast(x[8 * u:8 * u + 8], U32) for x in o
                               for u in range(A_SUB // 8)]
            a_o[sb] = jnp.concatenate(o, axis=1)
            if sb == BLK // A_SUB - 1:
                for t in range(LT, 3 * LT):
                    slab_v[(sub + 1) % UNROLL, t, 0:A_PAD, :] = slab[t, BLK:BLK + A_PAD, :]

        def pin(h, due):
            u = pltpu.bitcast(h, U32)
            tiles = [u[8 * r:8 * r + 8, 128 * c:128 * c + 128]
                     for c in range(LT) for r in range(u.shape[0] // 8)]
            for k, x in enumerate(due):
                tiles[k % len(tiles)] = jnp.where(never, x, tiles[k % len(tiles)])
            n = u.shape[0] // 8
            cols = [jnp.concatenate(tiles[c * n:(c + 1) * n], axis=0) for c in range(LT)]
            return pltpu.bitcast(jnp.concatenate(cols, axis=1), BF16)

        def a_out(b):
            o = jnp.concatenate([a_o[sb] for sb in range(BLK // A_SUB)], axis=0).astype(BF16)
            res = jnp.dot(o, pltpu.bitcast(woap_v[:, b * 128:(b + 1) * 128], BF16), preferred_element_type=F32)
            outa_v[pl.ds(r0, BLK), b * 128:(b + 1) * 128] = res.astype(BF16)

        x = bx_v[i].astype(F32)
        ex_e = ex_o = dict(q=a_qkv, Q=functools.partial(a_qkv, ahead=1), a=a_logits, b=a_values, w=a_out, pin=pin, pins=pins)
        def emit(r, out_e, acc, acc16):
            out = jnp.concatenate([acc16[0:8], out_e, acc16[8:16], acc[0:24]], axis=0)
            outb_v[pl.ds(r, BLK), :] = out.astype(BF16)
            pltpu.make_async_copy(
                outb_v.at[pl.ds(r, BLK)], out_h.at[pl.ds(r, BLK), pl.ds(D, D)],
                sem_out.at[1]).start()

        acc, acc16 = segment(
            i, sub, jnp.concatenate([x[16:40], mem], axis=0).astype(BF16), True, ex_e)
        if held is not None:
            emit(held[0], held[1], held[2], held[3] + acc16)
        out_e = acc[0:24]
        mem = acc[24:32].astype(BF16).astype(F32)
        acc, acc16 = segment(
            i, sub, jnp.concatenate([x[40:64], mem], axis=0).astype(BF16), False, ex_o)
        held = (r0, out_e, acc, acc16)
        if sub == UNROLL - 1 or not DEFER:
            emit(*held)
            held = None
        pltpu.make_async_copy(
            outa_v.at[pl.ds(r0, BLK)], out_h.at[pl.ds(r0, BLK), pl.ds(0, D)], sem_out.at[0]).start()
        return acc[24:32].astype(BF16).astype(F32), held

    def body_n(ii, mem):
        held = None
        for u in range(UNROLL):
            mem, held = body(ii * UNROLL + u, u, mem, held)
        return mem

    jax.lax.fori_loop(0, NLOOP // UNROLL, body_n, mem0_v[...].astype(F32))

    pltpu.make_async_copy(outa_v.at[0:NLOOP * BLK], out_h.at[0:NLOOP * BLK, pl.ds(0, D)], sem_out.at[0]).wait()
    pltpu.make_async_copy(outb_v.at[0:NLOOP * BLK], out_h.at[0:NLOOP * BLK, pl.ds(D, D)], sem_out.at[1]).wait()


@functools.partial(jax.jit, static_argnames=("B_seg_len",))
def pallas_concat_heads__sliding_local_dilated__memory_aug_recurrent_mem_tr__prompt_kernel(
    A_x: jax.Array,
    A_wqkv: jax.Array,
    A_wo: jax.Array,
    B_x: jax.Array,
    B_mem0: jax.Array,
    B_Wq: jax.Array,
    B_Wk: jax.Array,
    B_Wv: jax.Array,
    B_Wo: jax.Array,
    B_seg_len: int,
):
    assert A_x.shape == (1, S, D) and B_x.shape == (1, S, D)
    assert B_seg_len == B_SEG and B_mem0.shape == (1, B_M, D)
    assert B_Wq.shape == (D, B_H, B_DH) and B_Wo.shape == (B_H, B_DH, D)

    def feat_major(w):
        return jnp.transpose(w, (1, 2, 0)).reshape(B_F, D)

    any_spec = pl.BlockSpec(memory_space=pl.ANY)
    out = pl.pallas_call(
        _kernel,
        out_shape=jax.ShapeDtypeStruct((S, 2 * D), BF16),
        in_specs=[any_spec] * 9,
        out_specs=any_spec,
        scratch_shapes=[
            pltpu.VMEM((S, D), BF16),
            pltpu.VMEM((D, 3 * D), BF16),
            pltpu.VMEM((D, D), BF16),
            pltpu.VMEM((NIT, BLK, D), BF16),
            pltpu.VMEM((NIT, PRE, D), BF16),
            pltpu.VMEM((B_M, D), BF16),
            pltpu.VMEM((NU, PAIR, D), BF16),
            pltpu.VMEM((B_F, D), BF16),
            pltpu.VMEM((LT, 3 * D // 2, 128), U32),
            pltpu.VMEM((LT, D // 2, 128), U32),
            pltpu.VMEM((B_F // 2, D), U32),
            pltpu.VMEM((D // 2, 3 * D), U32),
            pltpu.VMEM((D // 2, D), U32),
            pltpu.VMEM((UNROLL, 3 * LT, A_PAD + BLK, 128), F32),
            pltpu.VMEM((S, D), BF16),
            pltpu.VMEM((NU, D // 2, PAIR), U32),
            pltpu.VMEM((NU, NIT * PRE // 2, PAIR), U32),
            pltpu.VMEM((NPAIR, 8, PAIR), F32),
            pltpu.VMEM((NPAIR, 8, 2 * PAIR), F32),
            pltpu.VMEM((NPAIR, 8, PAIR), F32),
            pltpu.VMEM((NPAIR, max(len(DEFER), 1), 16, 128), F32),
            pltpu.VMEM((S, D), BF16),
            pltpu.SemaphoreType.DMA((9 + len(U_HEAD) + U_N,)),
            pltpu.SemaphoreType.DMA((2,)),
        ],
        compiler_params=pltpu.CompilerParams(vmem_limit_bytes=120 * 1024 * 1024,
                                             disable_bounds_checks=True),
    )(
        A_x.reshape(S, D), A_wqkv, A_wo, B_x.reshape(NIT, BLK, D), B_mem0.reshape(B_M, D),
        feat_major(B_Wq), feat_major(B_Wk), feat_major(B_Wv), B_Wo.reshape(B_F, D),
    )
    return out.reshape(1, S, 2 * D)
```

```python
import functools

import jax
import jax.numpy as jnp
import jax.experimental.pallas as pl
import jax.experimental.pallas.tpu as pltpu

F32 = jnp.float32
BF16 = jnp.bfloat16
U32 = jnp.uint32

S = 2048
D = 640
LT = D // 128
BLK = 64
NIT = S // BLK

A_H = 32
A_DH = 20
A_W = 8
A_DIL = 2
A_PAD = 16
A_SUB = 16

B_H = 32
B_DH = 192
B_F = B_H * B_DH
B_M = 8
B_SEG = 32
B_L = B_M + B_SEG
PAIR = 2 * B_DH
NPAIR = B_H // 2
NU = 3 * NPAIR
PRE = 16
PRE_MB = 128

NEG = -1000000000.0
LOG2E = 1.4426950408889634
UNROLL = 2
U_HEAD = (1, 1, 2)
U_BODY = 5
U_N = 8
U_TAIL = NU - sum(U_HEAD) - U_BODY * U_N
X_FIRST = 16
MID = 1


def _schedule(order, lags, extra, tail):
    lag = dict(p=0, s=lags[0], v=lags[1], o=lags[2])
    kind = dict(x="p", y="p", z="p", A="o", B="o", C="o", s="s", v="v")
    hooks = {}
    for x in extra.split():
        key, val = x.split(":")
        hooks.setdefault(key, []).append((val[0], int(val[1:])))
    seq = []
    for t in range(NPAIR):
        for k in order:
            j = t - lag[kind[k]]
            if j >= 0:
                if k in "xAsv":
                    seq += hooks.get("<" + kind[k] + str(j), [])
                seq.append((k, j))
                if k in "zCsv":
                    seq += hooks.get(kind[k] + str(j), [])
            if t == NPAIR - 1 and k == "z":
                break
    for x in tail.split():
        seq += [(k, int(x[1:])) for k in ("ABC" if x[0] == "o" else x[0])
                if (k, int(x[1:])) not in seq]
    for k in "xyzABCsv":
        assert [j for kk, j in seq if kk == k] == list(range(NPAIR)), (k, seq)
    return seq


def _plan(order_e, extra_e, tail_e, due_e, order_o, extra_o, tail_o, due_o, due_a):
    lags = (1, 3, 5)
    emit = " ".join(f"s{j}:u{2 * j} s{j}:u{2 * j + 1}" for j in range(NPAIR - 2))
    rest = " ".join(f"u{n}" for n in range(2 * NPAIR - 4, 2 * NPAIR))
    dues = ({}, {})
    for j in range(NPAIR):
        for e in range(2):
            d = 9 * j + due_e[e]
            dues[d >= 9 * NPAIR].setdefault((d // 9 % NPAIR, d % 9), []).append(("u", 2 * j + e))
            d = 9 * j + due_o[e]
            if d < 9 * NPAIR:
                dues[1].setdefault((d // 9, d % 9), []).append(("U", 2 * j + e))
    for key in dues[1]:
        dues[1][key].sort(key=lambda x: x[0] == "u")
    for k in range(8):
        dues[1].setdefault((due_a + k, 0), []).append(("ab"[k % 2], k // 2))
    return ((_schedule(order_e, lags, extra_e + " " + emit, tail_e.replace("#", rest)), dues[0]),
            (_schedule(order_o, lags, extra_o + " " + emit, tail_o.replace("#", rest)), dues[1]))


_A_ODD = "<s0:q12 <s1:q13 <s2:q14 p5:a0 p6:b0 p7:a1 p8:b1 p9:a2 p10:b2 p11:a3 p12:b3"
_TAIL_E = "v12 s14 q8 v13 s15 # o10 o11 o12 v14 o13 v15 o14 q9 o15 q10 q11"
PLANS = (
    _plan("xyzABCvs",
          "<s0:q0 <s1:q1 <s2:q2 <s3:Q0 <s4:Q1 <s5:q3 <s6:Q2 <s7:Q3 <s8:q4 <s9:Q4 <s10:q5 <s11:q6"
          " <s12:Q5 <s13:q7", _TAIL_E, (25, 27),
          "xAyzBCvs", _A_ODD,
          "v12 s14 o10 v13 s15 # o11 o12 v14 o13 v15 w0 o14 o15 w1 w2 w3 w4", (24, 28), 7),
    _plan("xyABzCvs", "<s0:q6 <s1:q7", _TAIL_E, (25, 27),
          "xAyBzCvs", _A_ODD,
          "v12 s14 o10 v13 s15 # o11 o12 v14 o13 v15 o14 w0 o15 w1 w2 w3 w4", (24, 28), 6),
)


def _nt(a, b):
    return jax.lax.dot_general(a, b, (((1,), (1,)), ((), ())), preferred_element_type=F32)


def _nn(a, b):
    return jnp.dot(a, b, preferred_element_type=F32)


def _recip(x):
    r = pl.reciprocal(x, approx=True)
    return r * (2.0 - x * r)


def _kernel(ax_h, wqkv_h, woa_h, bx_h, mem0_h, wq_h, wk_h, wv_h, wo_h, out_h,
            ax_v, wqkv_v, woa_v, bx_v, xpre_v, mem0_v, wraw_v, wo_v,
            tmp_v, tmp2_v, wob_v, wqkvp_v, woap_v, slab_v, outa_v,
            wb_v, pre_v, qo_v, kvo_v, o8_v, mid_v, outb_v,
            sem_in, sem_out):
    cp_xpre = [pltpu.make_async_copy(bx_h.at[pl.ds(a, n), pl.ds(0, PRE), :],
                                     xpre_v.at[pl.ds(a, n)], sem_in.at[s])
               for a, n, s in ((0, X_FIRST, 0), (X_FIRST, NIT - X_FIRST, 8 + len(U_HEAD) + U_N))]
    cp_wqkv = pltpu.make_async_copy(wqkv_h, wqkv_v, sem_in.at[1])
    cp_woa = pltpu.make_async_copy(woa_h, woa_v, sem_in.at[2])
    cp_mem = pltpu.make_async_copy(mem0_h, mem0_v, sem_in.at[3])
    cp_bx = pltpu.make_async_copy(bx_h, bx_v, sem_in.at[4])
    cp_ax = pltpu.make_async_copy(ax_h, ax_v, sem_in.at[5])
    cp_wo = pltpu.make_async_copy(wo_h, wo_v, sem_in.at[6])
    w_hs = (wq_h, wk_h, wv_h)
    groups = list(U_HEAD) + [U_BODY] * U_N + [U_TAIL]
    g_start = [sum(groups[:g]) for g in range(len(groups))]

    cp_xpre[0].start()
    for g, n in enumerate(groups):
        for u in range(g_start[g], g_start[g] + n):
            pltpu.make_async_copy(w_hs[u % 3].at[pl.ds(u // 3 * PAIR, PAIR)], wraw_v.at[u],
                                  sem_in.at[7 + g]).start()
        if g == 0:
            cp_xpre[1].start()
    cp_wo.start()
    cp_wqkv.start()
    cp_woa.start()
    cp_mem.start()
    cp_bx.start()
    cp_ax.start()

    def g_wait(g, u0, n):
        buf = wraw_v.at[pl.ds(u0, n)]
        pltpu.make_async_copy(buf, buf, sem_in.at[7 + g]).wait()

    def b_pre(u, after=None, mbs=None):
        blk = wraw_v[u]
        if mbs is None or mbs[0] == 0:
            wb_v[u] = pltpu.bitcast(blk.T, U32)
        nb = PRE_MB // PRE
        for mb in (range(NIT // nb) if mbs is None else mbs):
            x = xpre_v[mb * nb:(mb + 1) * nb].reshape(PRE_MB, D)
            for n in range(PAIR // 128):
                r = _nt(x, blk[n * 128:(n + 1) * 128])
                pre_v[u, mb * PRE_MB // 2:(mb + 1) * PRE_MB // 2, n * 128:(n + 1) * 128] = (
                    pltpu.bitcast(r.astype(BF16), U32))
                if after is not None:
                    after(r)

    cp_xpre[0].wait()
    g_wait(0, 0, 1)
    nh = X_FIRST * PRE // PRE_MB
    b_pre(0, mbs=list(range(nh)))
    cp_xpre[1].wait()
    b_pre(0, mbs=list(range(nh, NIT * PRE // PRE_MB)))
    for g in range(1, len(U_HEAD)):
        g_wait(g, g_start[g], groups[g])
        for u in range(g_start[g], g_start[g] + groups[g]):
            b_pre(u)

    def pre_body(c, carry):
        u0 = sum(U_HEAD) + c * U_BODY
        g_wait(len(U_HEAD) + c, u0, U_BODY)
        for k in range(U_BODY):
            b_pre(u0 + k)
        return carry + c

    off = jax.lax.fori_loop(0, U_N, pre_body, 0) < 0

    g_wait(len(groups) - 1, g_start[-1], U_TAIL)
    cp_wqkv.wait()
    cp_woa.wait()
    cp_wo.wait()
    tail_units = list(range(g_start[-1], NU))

    copies = [(woa_v, r, 32, t, tmp2_v.at[t]) for t in range(LT) for r in range(0, D, 32)]
    copies += [(wo_v, r, 48, t, wob_v.at[:, pl.ds(t * 128, 128)])
               for r in range(0, B_F, 48) for t in range(LT)]

    def copy_some(res):
        for k in range(res.shape[0] // 8):
            if copies:
                src, r, n, t, dst = copies.pop(0)
                tok = pltpu.bitcast(res[8 * k:8 * k + 8], U32)
                v = pltpu.bitcast(src[r:r + n, t * 128:(t + 1) * 128], U32)
                v = jnp.where(off, jnp.concatenate([tok] * (n // 16), axis=0), v)
                dst[r // 2:(r + n) // 2, :] = v

    def tail_pre(k):
        for u in tail_units[k * U_TAIL // 4:(k + 1) * U_TAIL // 4]:
            b_pre(u, copy_some)

    def regroup(src_v, t, base, g):
        parts = []
        for dp in (2 * g, 2 * g + 1):
            v = src_v[t, pl.ds(base + dp, A_H, stride=A_DH // 2), :]
            parts.append(pltpu.bitcast(v << 16, F32))
            parts.append(pltpu.bitcast(v & jnp.uint32(0xFFFF0000), F32))
        return jnp.concatenate(parts, axis=0).astype(BF16)

    def a_prep1(p):
        for b in range(p * LT, (p + 1) * LT):
            blk = pltpu.bitcast(wqkv_v[:, b * 128:(b + 1) * 128].T, U32)
            for t in range(LT):
                tmp_v[t, b * 64:(b + 1) * 64, :] = blk[:, t * 128:(t + 1) * 128]

    def a_prep2(p):
        for g in range(LT):
            blk = jnp.concatenate([regroup(tmp_v, t, p * D // 2, g) for t in range(LT)], axis=1)
            b = p * LT + g
            wqkvp_v[:, b * 128:(b + 1) * 128] = pltpu.bitcast(blk.T, U32)

    def a_prep3():
        for g in range(LT):
            for t in range(LT):
                woap_v[g * 64:(g + 1) * 64, t * 128:(t + 1) * 128] = pltpu.bitcast(
                    regroup(tmp2_v, t, 0, g), U32)

    a_prep1(0)
    a_prep1(1)
    tail_pre(0)
    a_prep1(2)
    a_prep2(0)
    tail_pre(1)
    a_prep2(1)
    tail_pre(2)
    a_prep2(2)
    a_prep3()
    tail_pre(3)
    for t in range(LT, 3 * LT):
        slab_v[0, t, 0:A_PAD, :] = jnp.zeros((A_PAD, 128), F32)
    assert not copies
    cp_mem.wait()
    cp_bx.wait()
    cp_ax.wait()

    a_scale = A_DH ** (-0.5)
    b_scale = B_DH ** (-0.5)
    qrow = jax.lax.broadcasted_iota(jnp.int32, (32, 2 * B_L), 0)
    lane = jax.lax.broadcasted_iota(jnp.int32, (32, 2 * B_L), 1)
    first = lane < B_L
    kcol = jnp.where(first, lane, lane - B_L)
    allowed = (qrow >= B_SEG - 8) | (kcol >= B_SEG) | (qrow + 8 >= kcol)

    def blockdiag(t):
        n = t.shape[0]
        left = jax.lax.broadcasted_iota(jnp.int32, (n, 128), 1) < 64
        z = jnp.zeros((n, 128), F32)
        mid = t[:, 128:256]
        top = jnp.concatenate([t[:, 0:128], jnp.where(left, mid, 0.0), z], axis=1)
        bot = jnp.concatenate([z, jnp.where(left, 0.0, mid), t[:, 256:384]], axis=1)
        return jnp.concatenate([top, bot], axis=0).astype(BF16)

    def softmax(s):
        s = jnp.where(allowed, s * b_scale, NEG)
        ma = jnp.max(jnp.where(first, s, -jnp.inf), axis=1, keepdims=True)
        mb = jnp.max(jnp.where(first, -jnp.inf, s), axis=1, keepdims=True)
        p = jnp.exp(s - jnp.where(first, ma, mb))
        la = jnp.sum(jnp.where(first, p, 0.0), axis=1, keepdims=True)
        lb = jnp.sum(jnp.where(first, 0.0, p), axis=1, keepdims=True)
        return (p * _recip(jnp.where(first, la, lb))).astype(BF16)

    def head8(q, kv_x, kv_m, second):
        left = jax.lax.broadcasted_iota(jnp.int32, (8, 128), 1) < 64
        row = jax.lax.broadcasted_iota(jnp.int32, (8, 128), 0)
        t = 2 if second else 0
        qa = q[:, t * 128:(t + 1) * 128] * (b_scale * LOG2E)
        qb = q[:, 128:256] * (b_scale * LOG2E)
        qb = jnp.where(left, 0.0, qb) if second else jnp.where(left, qb, 0.0)

        def bc(k, t):
            src = kv_x if k < 8 else kv_m
            return jnp.broadcast_to(src[k % 8:k % 8 + 1, t * 128:(t + 1) * 128], (8, 128))

        sc = []
        for k in range(16):
            x = jnp.sum(qa * bc(k, t) + qb * bc(k, 1), axis=1, keepdims=True)
            x = jnp.broadcast_to(x, (8, 128))
            if 0 < k < 8:
                x = jnp.where(row >= k, x, NEG * LOG2E)
            sc.append(x)
        m = functools.reduce(jnp.maximum, sc)
        p = [jnp.exp2(x - m) for x in sc]
        inv = _recip(functools.reduce(jnp.add, p))
        return [functools.reduce(jnp.add, [p[k] * bc(k, 3 + tt) for k in range(16)]) * inv
                for tt in (t, 1)]

    def segment(i, sub, h, even, extra):
        order, dues = PLANS[sub][0 if even else 1]
        qkv, prob, att, q8, o8 = {}, {}, {}, {}, {}
        acc, acc16 = [None], [None]
        hh = [h]
        parts = []
        pins = extra['pins']

        def proj(j, part):
            cuts = sorted({3 * part, 3 * part + 3}
                          | {m for (jj, m) in dues if jj == j and m // 3 == part})
            for m, m2 in zip(cuts[:-1], cuts[1:]):
                due = [x for key in dues.get((j, m), ()) for x in pins.pop(key)]
                if due:
                    hh[0] = extra['pin'](hh[0], due)
                w = wb_v[3 * j + part, :, (m - 3 * part) * 128:(m2 - 3 * part) * 128]
                parts.append(_nn(hh[0], pltpu.bitcast(w, BF16)))
            if part < 2:
                return
            r = jnp.concatenate(parts, axis=1)
            parts.clear()
            if even:
                rows = pl.ds(pl.multiple_of(i * (PRE // 2), PRE // 2), PRE // 2)
                pre = jnp.concatenate([pre_v[3 * j + m, rows, :] for m in range(3)], axis=1)
                pre = pltpu.bitcast(pre, BF16).astype(F32)
                qo_v[j] = r[16:24, :PAIR]
                kvo_v[j] = r[16:24, PAIR:]
                q8[j] = (pre[0:8, :PAIR], pre[0:8, PAIR:], r[24:32, PAIR:])
                q = jnp.concatenate([pre[8:16, :PAIR], r[0:16, :PAIR], r[24:32, :PAIR]], axis=0)
                kv = jnp.concatenate([pre[:, PAIR:], r[0:16, PAIR:], r[24:32, PAIR:]], axis=0)
            else:
                q8[j] = (qo_v[j], kvo_v.at[j], r[24:32, PAIR:])
                q = r[:, :PAIR]
                kv = jnp.concatenate([kvo_v[j], r[:, PAIR:]], axis=0)
            qkv[j] = (q.astype(BF16), blockdiag(kv[:, :PAIR]), blockdiag(kv[:, PAIR:]))

        def vector(jj):
            j, second = jj // 2, jj % 2
            o = head8(*q8[j], second)
            pins[('u' if even else 'U', jj)] = [pltpu.bitcast(x, U32) for x in o]
            if not second:
                o8[j] = o
                return
            left = jax.lax.broadcasted_iota(jnp.int32, (8, 128), 1) < 64
            o = jnp.concatenate([o8[j][0], jnp.where(left, o8[j][1], o[1]), o[0]], axis=1)
            if even:
                o8_v[j] = o
            else:
                o8[j] = o

        def scores(j):
            prob[j] = softmax(_nt(qkv[j][0], qkv[j][1]))

        def values(j):
            att[j] = _nn(prob[j], qkv[j][2])

        def outp(j, t):
            lhs = att[j][:, t * 128:(t + 1) * 128]
            if even:
                wide = sub > 0 and t == MID
                if wide:
                    lhs = jnp.concatenate([lhs, mid_v[j]], axis=0)
            else:
                wide = sub == UNROLL - 1 or t != MID
                o16 = jnp.concatenate([o8_v[j, :, t * 128:(t + 1) * 128],
                                       o8[j][:, t * 128:(t + 1) * 128]], axis=0)
                if wide:
                    lhs = jnp.concatenate([lhs, o16], axis=0)
                else:
                    mid_v[j] = o16
            r = j * PAIR // 2 + t * 64
            d = _nn(lhs.astype(BF16), pltpu.bitcast(wob_v[r:r + 64, :], BF16))
            acc[0] = d[0:32] if acc[0] is None else acc[0] + d[0:32]
            if wide:
                acc16[0] = d[32:48] if acc16[0] is None else acc16[0] + d[32:48]

        fns = dict(extra, s=scores, v=values, u=vector)
        for t in range(3):
            fns['xyz'[t]] = functools.partial(proj, part=t)
            fns['ABC'[t]] = functools.partial(outp, t=t)
        for k, j in order:
            fns[k](j)
        return acc[0], acc16[0]

    def body(i, sub, mem, held):
        r0 = pl.multiple_of(i * BLK, BLK)

        slab = slab_v.at[sub]

        def a_qkv(b, ahead=0):
            x = ax_v[pl.ds(r0 + ahead * BLK, BLK), :]
            slab_v[sub + ahead, b, A_PAD:A_PAD + BLK, :] = _nn(
                x, pltpu.bitcast(wqkvp_v[:, b * 128:(b + 1) * 128], BF16))

        a_o, a_p = {}, {}
        never = i < 0
        pins = {}

        def a_logits(sb):
            base = A_PAD + sb * A_SUB
            q = [slab[t, base:base + A_SUB, :] for t in range(LT)]
            logits = []
            for w in range(A_W):
                lo = base - A_DIL * w
                acc = None
                for t in range(LT):
                    pr = q[t] * slab[LT + t, lo:lo + A_SUB, :]
                    acc = pr if acc is None else acc + pr
                acc = acc + pltpu.roll(acc, 64, 1)
                acc = acc + pltpu.roll(acc, 32, 1)
                acc = acc * a_scale
                if sb == 0 and w > 0:
                    row = jax.lax.broadcasted_iota(jnp.int32, (A_SUB, 128), 0) + r0
                    acc = jnp.where(row >= A_DIL * w, acc, NEG)
                logits.append(acc)
            m = logits[0]
            for w in range(1, A_W):
                m = jnp.maximum(m, logits[w])
            ps = [jnp.exp(l - m) for l in logits]
            den = ps[0]
            for w in range(1, A_W):
                den = den + ps[w]
            inv = _recip(den)
            a_p[sb] = (ps, inv)
            pins[('a', sb)] = [pltpu.bitcast(inv[8 * u:8 * u + 8], U32) for u in range(A_SUB // 8)]

        def a_values(sb):
            base = A_PAD + sb * A_SUB
            ps, inv = a_p[sb]
            o = []
            for t in range(LT):
                acc = None
                for w in range(A_W):
                    lo = base - A_DIL * w
                    pr = ps[w] * slab[2 * LT + t, lo:lo + A_SUB, :]
                    acc = pr if acc is None else acc + pr
                o.append(acc * inv)
            pins[('b', sb)] = [pltpu.bitcast(x[8 * u:8 * u + 8], U32) for x in o
                               for u in range(A_SUB // 8)]
            a_o[sb] = jnp.concatenate(o, axis=1)
            if sb == BLK // A_SUB - 1:
                for t in range(LT, 3 * LT):
                    slab_v[(sub + 1) % UNROLL, t, 0:A_PAD, :] = slab[t, BLK:BLK + A_PAD, :]

        def pin(h, due):
            u = pltpu.bitcast(h, U32)
            tiles = [u[8 * r:8 * r + 8, 128 * c:128 * c + 128]
                     for c in range(LT) for r in range(u.shape[0] // 8)]
            for k, x in enumerate(due):
                tiles[k % len(tiles)] = jnp.where(never, x, tiles[k % len(tiles)])
            n = u.shape[0] // 8
            cols = [jnp.concatenate(tiles[c * n:(c + 1) * n], axis=0) for c in range(LT)]
            return pltpu.bitcast(jnp.concatenate(cols, axis=1), BF16)

        def a_out(b):
            o = jnp.concatenate([a_o[sb] for sb in range(BLK // A_SUB)], axis=0).astype(BF16)
            res = _nn(o, pltpu.bitcast(woap_v[:, b * 128:(b + 1) * 128], BF16))
            outa_v[pl.ds(r0, BLK), b * 128:(b + 1) * 128] = res.astype(BF16)

        x = bx_v[i].astype(F32)
        extra = dict(q=a_qkv, Q=functools.partial(a_qkv, ahead=1), a=a_logits, b=a_values,
                     w=a_out, pin=pin, pins=pins)

        def emit(r, out_e, acc, acc16):
            out = jnp.concatenate([acc16[0:8], out_e, acc16[8:16], acc[0:24]], axis=0)
            outb_v[pl.ds(r, BLK), :] = out.astype(BF16)
            pltpu.make_async_copy(
                outb_v.at[pl.ds(r, BLK)], out_h.at[pl.ds(r, BLK), pl.ds(D, D)],
                sem_out.at[1]).start()

        acc, acc16 = segment(
            i, sub, jnp.concatenate([x[16:40], mem], axis=0).astype(BF16), True, extra)
        if held is not None:
            emit(held[0], held[1], held[2], held[3] + acc16)
        out_e = acc[0:24]
        mem = acc[24:32].astype(BF16).astype(F32)
        acc, acc16 = segment(
            i, sub, jnp.concatenate([x[40:64], mem], axis=0).astype(BF16), False, extra)
        held = (r0, out_e, acc, acc16)
        if sub == UNROLL - 1:
            emit(*held)
            held = None
        pltpu.make_async_copy(
            outa_v.at[pl.ds(r0, BLK)], out_h.at[pl.ds(r0, BLK), pl.ds(0, D)], sem_out.at[0]).start()
        return acc[24:32].astype(BF16).astype(F32), held

    def body_n(ii, mem):
        held = None
        for u in range(UNROLL):
            mem, held = body(ii * UNROLL + u, u, mem, held)
        return mem

    jax.lax.fori_loop(0, NIT // UNROLL, body_n, mem0_v[...].astype(F32))

    pltpu.make_async_copy(outa_v, out_h.at[:, pl.ds(0, D)], sem_out.at[0]).wait()
    pltpu.make_async_copy(outb_v, out_h.at[:, pl.ds(D, D)], sem_out.at[1]).wait()


@jax.jit
def _run(A_x, A_wqkv, A_wo, B_x, B_mem0, B_Wq, B_Wk, B_Wv, B_Wo):
    def feat_major(w):
        return jnp.transpose(w, (1, 2, 0)).reshape(B_F, D)

    any_spec = pl.BlockSpec(memory_space=pl.ANY)
    out = pl.pallas_call(
        _kernel,
        out_shape=jax.ShapeDtypeStruct((S, 2 * D), BF16),
        in_specs=[any_spec] * 9,
        out_specs=any_spec,
        scratch_shapes=[
            pltpu.VMEM((S, D), BF16),
            pltpu.VMEM((D, 3 * D), BF16),
            pltpu.VMEM((D, D), BF16),
            pltpu.VMEM((NIT, BLK, D), BF16),
            pltpu.VMEM((NIT, PRE, D), BF16),
            pltpu.VMEM((B_M, D), BF16),
            pltpu.VMEM((NU, PAIR, D), BF16),
            pltpu.VMEM((B_F, D), BF16),
            pltpu.VMEM((LT, 3 * D // 2, 128), U32),
            pltpu.VMEM((LT, D // 2, 128), U32),
            pltpu.VMEM((B_F // 2, D), U32),
            pltpu.VMEM((D // 2, 3 * D), U32),
            pltpu.VMEM((D // 2, D), U32),
            pltpu.VMEM((UNROLL, 3 * LT, A_PAD + BLK, 128), F32),
            pltpu.VMEM((S, D), BF16),
            pltpu.VMEM((NU, D // 2, PAIR), U32),
            pltpu.VMEM((NU, NIT * PRE // 2, PAIR), U32),
            pltpu.VMEM((NPAIR, 8, PAIR), F32),
            pltpu.VMEM((NPAIR, 8, 2 * PAIR), F32),
            pltpu.VMEM((NPAIR, 8, PAIR), F32),
            pltpu.VMEM((NPAIR, 16, 128), F32),
            pltpu.VMEM((S, D), BF16),
            pltpu.SemaphoreType.DMA((9 + len(U_HEAD) + U_N,)),
            pltpu.SemaphoreType.DMA((2,)),
        ],
        compiler_params=pltpu.CompilerParams(vmem_limit_bytes=120 * 1024 * 1024,
                                             disable_bounds_checks=True),
    )(
        A_x.reshape(S, D), A_wqkv, A_wo, B_x.reshape(NIT, BLK, D), B_mem0.reshape(B_M, D),
        feat_major(B_Wq), feat_major(B_Wk), feat_major(B_Wv), B_Wo.reshape(B_F, D),
    )
    return out.reshape(1, S, 2 * D)


def pallas_concat_heads__sliding_local_dilated__memory_aug_recurrent_mem_tr__prompt_kernel(
    A_x: jax.Array,
    A_wqkv: jax.Array,
    A_wo: jax.Array,
    B_x: jax.Array,
    B_mem0: jax.Array,
    B_Wq: jax.Array,
    B_Wk: jax.Array,
    B_Wv: jax.Array,
    B_Wo: jax.Array,
    B_seg_len,
):
    assert A_x.shape == (1, S, D) and B_x.shape == (1, S, D) and B_mem0.shape == (1, B_M, D)
    assert B_Wq.shape == (D, B_H, B_DH) and B_Wo.shape == (B_H, B_DH, D)
    if isinstance(B_seg_len, int):
        assert B_seg_len == B_SEG
    return _run(A_x, A_wqkv, A_wo, B_x, B_mem0, B_Wq, B_Wk, B_Wv, B_Wo)
```

```python
import functools

import jax
import jax.numpy as jnp
import jax.experimental.pallas as pl
import jax.experimental.pallas.tpu as pltpu

F32 = jnp.float32
BF16 = jnp.bfloat16
U32 = jnp.uint32

S = 2048
D = 640
LT = D // 128
BLK = 64
NIT = S // BLK

A_H = 32
A_DH = 20
A_W = 8
A_DIL = 2
A_PAD = 16
A_SUB = 16

B_H = 32
B_DH = 192
B_F = B_H * B_DH
B_M = 8
B_SEG = 32
B_L = B_M + B_SEG
PAIR = 2 * B_DH
NPAIR = B_H // 2
NU = 3 * NPAIR
PRE = 16
PRE_MB = 128

NEG = -1000000000.0
ILV = [h * B_DH + t * 64 for t in range(3) for h in range(2)]
LOG2E = 1.4426950408889634
LAG_S, LAG_V, LAG_O = [int(v) for v in "1,3,5".split(",")]
ORDER = "povs"
UNROLL = int("2")
U_HEAD = [int(v) for v in "1,1,2".split(",")]
U_BODY = int("5")
U_N = int("8")
U_TAIL = NU - sum(U_HEAD) - U_BODY * U_N
SEARCH = int("0")
XH = int("16")
DEFER = [int(v) for v in "1".split(",") if v.strip()]
PIN = int("1")
NLOOP = int("32")


def _schedule(order, lags, steady_extra, tail):
    lag = dict(p=0, s=lags[0], v=lags[1], o=lags[2])
    kind = dict(x="p", y="p", z="p", A="o", B="o", C="o", s="s", v="v")
    seq = []
    for t in range(NPAIR):
        for k in order:
            j = t - lag[kind[k]]
            if j >= 0:
                if k in "xAsv":
                    seq += steady_extra.get("<" + kind[k] + str(j), [])
                seq.append((k, j))
                if k in "zCsv":
                    seq += steady_extra.get(kind[k] + str(j), [])
            if t == NPAIR - 1 and k == "z":
                break
    for x in tail.split():
        seq += [(k, int(x[1:])) for k in ("ABC" if x[0] == "o" else x[0])
                if (k, int(x[1:])) not in seq]
    for k in "xyzABCsv":
        assert [j for kk, j in seq if kk == k] == list(range(NPAIR)), (k, seq)
    return seq


def _ex(txt):
    d = {}
    for x in txt.split():
        key, val = x.split(":")
        d.setdefault(key, []).append((val[0], int(val[1:])))
    return d


def _due(txt):
    d = {}
    for x in txt.split():
        key, at = x.split("@")
        j, m = at.split(".")
        d.setdefault((int(j), int(m)), []).append((key[0], int(key[1:])))
    return d


def _vector_plan(ea, eb, ia, ua, ib, ub, last):
    es = [(j, e, d) for j in range(NPAIR) for e, d in enumerate((ea, eb))]
    ds = [(k, 2 * j + e, 9 * j + int(d)) for j in range(NPAIR)
          for k, e, d in (("i", 0, ia), ("u", 0, ua), ("i", 1, ib), ("u", 1, ub)) if int(d) > 0]
    emit = " ".join(f"{d[0]}{j + int(d[1:])}:u{2 * j + e}" for j, e, d in es
                    if j + int(d[1:]) <= last[d[0]])
    tail = " ".join(f"u{2 * j + e}" for j, e, d in es if j + int(d[1:]) > last[d[0]])
    due = " ".join(f"{k}{n}@{d // 9}.{d % 9}" for k, n, d in ds if d < 9 * NPAIR)
    late = " ".join(f"{k}{n}@{d // 9 - NPAIR}.{d % 9}" for k, n, d in ds if d >= 9 * NPAIR)
    return emit, tail, due, late


def _plan(oe, le, xe, te, ve, oo, lo, xo, to, vo, do):
    ve = _vector_plan(*ve.split(), dict(p=15, s=13))
    vo = _vector_plan(*vo.split(), dict(p=15, s=13))
    sched_e = _schedule(oe, [int(v) for v in le.split(",")], _ex(xe + " " + ve[0]),
                        te.replace("#", ve[1]))
    sched_o = _schedule(oo, [int(v) for v in lo.split(",")], _ex(xo + " " + vo[0]),
                        to.replace("#", vo[1]))
    due_o = vo[2].replace("u", "U").replace("i", "I") + " " + ve[3] + " " + do
    return (sched_e, _due(ve[2])), (sched_o, _due(due_o))


PLANS = [_plan(
    "xyzABCvs",
    "1,3,4",
    "<s0:q0 <s1:q1 <s2:q2 <s3:Q0 <s4:Q1 <s5:q3 <s6:Q2 <s7:Q3 <s8:q4 <s9:Q4 <s10:q5 <s11:q6 <s12:Q5 <s13:q7",
    "v12 s14 q8 v13 s15 # o11 o12 o13 v14 q9 v15 o14 o15 q10 q11",
    "s0 s0 0 25 0 26",
    "xAyzBCvs",
    "1,3,5",
    "<s0:q12 <s1:q13 <s2:q14 p4:a0 p5:b0 p7:a1 p8:b1 p9:a2 p10:b2 p12:a3 p13:b3",
    "v12 s14 o10 v13 s15 # o11 o12 v14 o13 v15 w0 o14 o15 w1 w2 w3 w4",
    "s0 s0 0 26 0 27",
    "a0@5.0 b0@6.0 a1@8.0 b1@9.0 a2@10.0 b2@11.0 a3@13.0 b3@14.0",
), _plan(
    "xyABzCvs",
    "1,3,5",
    "<s0:q6 <s1:q7",
    "v12 s14 q8 v13 s15 # o10 o11 o12 v14 o13 v15 o14 q9 o15 q10 q11",
    "s0 s0 0 25 0 26",
    "xAyBzCvs",
    "1,3,5",
    "<s0:q12 <s1:q13 <s2:q14 p5:a0 p6:b0 p7:a1 p8:b1 p9:a2 p10:b2 p11:a3 p12:b3",
    "v12 s14 o10 v13 s15 # o11 o12 v14 o13 v15 o14 w0 o15 w1 w2 w3 w4",
    "s0 s0 0 26 0 27",
    "a0@6.0 b0@7.0 a1@8.0 b1@9.0 a2@10.0 b2@11.0 a3@12.0 b3@13.0",
)]


def _nt(a, b):
    return jax.lax.dot_general(a, b, (((1,), (1,)), ((), ())), preferred_element_type=F32)


def _nn(a, b):
    return jnp.dot(a, b, preferred_element_type=F32)


def _recip(x):
    r = pl.reciprocal(x, approx=True)
    return r * (2.0 - x * r)


def _kernel(ax_h, wqkv_h, woa_h, bx_h, mem0_h, wq_h, wk_h, wv_h, wo_h, out_h,
            ax_v, wqkv_v, woa_v, bx_v, xpre_v, mem0_v, wraw_v, wo_v,
            tmp_v, tmp2_v, wob_v, wqkvp_v, woap_v, slab_v, outa_v,
            wb_v, pre_v, qo_v, kvo_v, o8_v, mid_v, outb_v,
            sem_in, sem_out):
    cp_xpre = [pltpu.make_async_copy(bx_h.at[pl.ds(a, n), pl.ds(0, PRE), :], xpre_v.at[pl.ds(a, n)],
                                     sem_in.at[s])
               for a, n, s in ((0, XH, 0), (XH, NIT - XH, 7 + len(U_HEAD) + U_N + 1))]
    cp_wqkv = pltpu.make_async_copy(wqkv_h, wqkv_v, sem_in.at[1])
    cp_woa = pltpu.make_async_copy(woa_h, woa_v, sem_in.at[2])
    cp_mem = pltpu.make_async_copy(mem0_h, mem0_v, sem_in.at[3])
    cp_bx = pltpu.make_async_copy(bx_h, bx_v, sem_in.at[4])
    cp_ax = pltpu.make_async_copy(ax_h, ax_v, sem_in.at[5])
    cp_wo = pltpu.make_async_copy(wo_h, wo_v, sem_in.at[6])
    w_hs = (wq_h, wk_h, wv_h)
    groups = list(U_HEAD) + [U_BODY] * U_N + [U_TAIL]
    g_start = [sum(groups[:g]) for g in range(len(groups))]

    cp_xpre[0].start()
    for g, n in enumerate(groups):
        for u in range(g_start[g], g_start[g] + n):
            pltpu.make_async_copy(w_hs[u % 3].at[pl.ds(u // 3 * PAIR, PAIR)], wraw_v.at[u],
                                  sem_in.at[7 + g]).start()
        if g == 0:
            cp_xpre[1].start()
    cp_wo.start()
    cp_wqkv.start()
    cp_woa.start()
    cp_mem.start()
    cp_bx.start()
    cp_ax.start()

    def g_wait(g, u0, n):
        buf = wraw_v.at[pl.ds(u0, n)]
        pltpu.make_async_copy(buf, buf, sem_in.at[7 + g]).wait()

    def b_pre(u, after=None, mbs=None):
        if isinstance(u, int):
            rows = [pl.ds(r if u % 3 == 2 else 64 * k, 64) for k, r in enumerate(ILV)]
        else:
            rows = [pl.ds(pl.multiple_of(jnp.where(u % 3 == 2, r, 64 * k), 64), 64)
                    for k, r in enumerate(ILV)]
        blk = jnp.concatenate([wraw_v[u, r, :] for r in rows], axis=0)
        if mbs is None or mbs[0] == 0:
            wb_v[u] = pltpu.bitcast(blk.T, U32)
        nb = PRE_MB // PRE
        for mb in (range(NIT // nb) if mbs is None else mbs):
            x = xpre_v[mb * nb:(mb + 1) * nb].reshape(PRE_MB, D)
            for n in range(PAIR // 128):
                r = _nt(x, blk[n * 128:(n + 1) * 128])
                pre_v[u, mb * PRE_MB // 2:(mb + 1) * PRE_MB // 2, n * 128:(n + 1) * 128] = (
                    pltpu.bitcast(r.astype(BF16), U32))
                if after is not None:
                    after(r)

    cp_xpre[0].wait()
    if SEARCH:
        b_pre = lambda u, after=None, mbs=None: None
    g_wait(0, 0, 1)
    nh = XH * PRE // PRE_MB
    b_pre(0, mbs=list(range(nh)))
    cp_xpre[1].wait()
    b_pre(0, mbs=list(range(nh, NIT * PRE // PRE_MB)))
    for g, n in enumerate(U_HEAD):
        if g == 0:
            continue
        g_wait(g, g_start[g], n)
        for u in range(g_start[g], g_start[g] + n):
            b_pre(u)

    def pre_body(c, carry):
        u0 = sum(U_HEAD) + c * U_BODY
        g_wait(len(U_HEAD) + c, u0, U_BODY)
        for k in range(U_BODY):
            b_pre(u0 + k)
        return carry + c

    off = jax.lax.fori_loop(0, U_N, pre_body, 0) < 0

    g_wait(len(groups) - 1, g_start[-1], U_TAIL)
    cp_wqkv.wait()
    cp_woa.wait()
    cp_wo.wait()
    tail_units = list(range(g_start[-1], NU))

    copies = [(woa_v, r, r, t, tmp2_v.at[t]) for t in range(LT) for r in range(0, D, 16)]
    copies += [(wo_v, j * PAIR + r + rr, j * PAIR + k * 64 + rr, t,
                wob_v.at[:, pl.ds(t * 128, 128)])
               for j in range(NPAIR) for k, r in enumerate(ILV) for t in range(LT)
               for rr in range(0, 64, 16)]

    def copy_some(res):
        for k in range(res.shape[0] // 8):
            tok = pltpu.bitcast(res[8 * k:8 * k + 8], U32)
            for _ in range(3):
                if copies:
                    src, r, rd, t, dst = copies.pop(0)
                    v = pltpu.bitcast(src[r:r + 16, t * 128:(t + 1) * 128], U32)
                    dst[rd // 2:rd // 2 + 8, :] = jnp.where(off, tok, v)

    def tail_pre(k):
        for u in tail_units[k * U_TAIL // 4:(k + 1) * U_TAIL // 4]:
            b_pre(u, copy_some)

    def regroup(tmp_v, t, base, g):
        parts = []
        for dp in (2 * g, 2 * g + 1):
            v = tmp_v[t, pl.ds(base + dp, A_H, stride=A_DH // 2), :]
            parts.append(pltpu.bitcast(v << 16, F32))
            parts.append(pltpu.bitcast(v & jnp.uint32(0xFFFF0000), F32))
        return jnp.concatenate(parts, axis=0).astype(BF16)

    def a_prep1(p):
        for b in range(p * LT, (p + 1) * LT):
            blk = pltpu.bitcast(wqkv_v[:, b * 128:(b + 1) * 128].T, U32)
            for t in range(LT):
                tmp_v[t, b * 64:(b + 1) * 64, :] = blk[:, t * 128:(t + 1) * 128]

    def a_prep2(p):
        for g in range(LT):
            blk = jnp.concatenate([regroup(tmp_v, t, p * D // 2, g) for t in range(LT)], axis=1)
            b = p * LT + g
            wqkvp_v[:, b * 128:(b + 1) * 128] = pltpu.bitcast(blk.T, U32)

    def a_prep4():
        for g in range(LT):
            for t in range(LT):
                woap_v[g * 64:(g + 1) * 64, t * 128:(t + 1) * 128] = pltpu.bitcast(
                    regroup(tmp2_v, t, 0, g), U32)

    if SEARCH:
        a_prep1 = a_prep2 = lambda p: None
        a_prep4 = lambda: None
        copies.clear()
    a_prep1(0)
    a_prep1(1)
    tail_pre(0)
    a_prep1(2)
    a_prep2(0)
    tail_pre(1)
    a_prep2(1)
    tail_pre(2)
    a_prep2(2)
    a_prep4()
    tail_pre(3)
    for t in range(LT, 3 * LT):
        slab_v[0, t, 0:A_PAD, :] = jnp.zeros((A_PAD, 128), F32)
    assert not copies
    cp_mem.wait()
    cp_bx.wait()
    cp_ax.wait()

    a_scale = A_DH ** (-0.5)
    b_scale = B_DH ** (-0.5)
    qrow = jax.lax.broadcasted_iota(jnp.int32, (32, 2 * B_L), 0)
    lane = jax.lax.broadcasted_iota(jnp.int32, (32, 2 * B_L), 1)
    first = lane < B_L
    kcol = jnp.where(first, lane, lane - B_L)
    allowed = (qrow >= B_SEG - 8) | (kcol >= B_SEG) | (qrow + 8 >= kcol)

    def blockdiag_k(t):
        n = t.shape[0]
        left = jax.lax.broadcasted_iota(jnp.int32, (n, 128), 1) < 64
        z = jnp.zeros((n, 128), F32)
        mid = t[:, 128:256]
        top = jnp.concatenate([t[:, 0:128], jnp.where(left, mid, 0.0), z], axis=1)
        bot = jnp.concatenate([z, jnp.where(left, 0.0, mid), t[:, 256:384]], axis=1)
        return jnp.concatenate([top, bot], axis=0).astype(BF16)

    def blockdiag_v(t):
        left = jax.lax.broadcasted_iota(jnp.int32, t.shape, 1) % 128 < 64
        return jnp.concatenate([jnp.where(left, t, 0.0), jnp.where(left, 0.0, t)],
                               axis=0).astype(BF16)

    def softmax(s):
        s = jnp.where(allowed, s * b_scale, NEG)
        ma = jnp.max(jnp.where(first, s, -jnp.inf), axis=1, keepdims=True)
        mb = jnp.max(jnp.where(first, -jnp.inf, s), axis=1, keepdims=True)
        p = jnp.exp(s - jnp.where(first, ma, mb))
        la = jnp.sum(jnp.where(first, p, 0.0), axis=1, keepdims=True)
        lb = jnp.sum(jnp.where(first, 0.0, p), axis=1, keepdims=True)
        return (p * _recip(jnp.where(first, la, lb))).astype(BF16)

    def bc(kv_x, kv_m, k, t):
        src = kv_x if k < 8 else kv_m
        return jnp.broadcast_to(src[k % 8:k % 8 + 1, t * 128:(t + 1) * 128], (8, 128))

    def first8_probs(q, kv_x, kv_m):
        left = jax.lax.broadcasted_iota(jnp.int32, (8, 128), 1) < 64
        row = jax.lax.broadcasted_iota(jnp.int32, (8, 128), 0)
        q = q * (b_scale * LOG2E)
        q0, q2 = q[:, 0:128], q[:, 256:384]
        q1a, q1b = jnp.where(left, q[:, 128:256], 0.0), jnp.where(left, 0.0, q[:, 128:256])
        sc = []
        for k in range(16):
            k1 = bc(kv_x, kv_m, k, 1)
            xa = jnp.sum(q0 * bc(kv_x, kv_m, k, 0) + q1a * k1, axis=1, keepdims=True)
            xb = jnp.sum(q1b * k1 + q2 * bc(kv_x, kv_m, k, 2), axis=1, keepdims=True)
            x = jnp.where(left, xa, xb)
            if 0 < k < 8:
                x = jnp.where(row >= k, x, NEG * LOG2E)
            sc.append(x)
        m = functools.reduce(jnp.maximum, sc)
        p = [jnp.exp2(x - m) for x in sc]
        return p, _recip(functools.reduce(jnp.add, p))

    def first8_values(p, inv, kv_x, kv_m):
        return [functools.reduce(jnp.add, [p[k] * bc(kv_x, kv_m, k, 3 + t) for k in range(16)])
                * inv for t in range(3)]

    def segment(i, sub, h, even, extra):
        qkv, prob, att, q8, o8 = {}, {}, {}, {}, {}
        acc = [None]
        hh = [h]
        parts = []
        pins = extra['pins']

        def proj(j, part):
            dues = PLANS[sub][0 if even else 1][1]
            cuts = sorted({3 * part, 3 * part + 3}
                          | {m for (jj, m) in dues if jj == j and m // 3 == part})
            for m, m2 in zip(cuts[:-1], cuts[1:]):
                due = [x for key in dues.get((j, m), ()) for x in pins.pop(key)]
                if due:
                    hh[0] = extra['pin'](hh[0], due)
                w = wb_v[3 * j + part, :, (m - 3 * part) * 128:(m2 - 3 * part) * 128]
                parts.append(jnp.dot(hh[0], pltpu.bitcast(w, BF16), preferred_element_type=F32))
            if part < 2:
                return
            r = jnp.concatenate(parts, axis=1)
            parts.clear()
            if even:
                rows = pl.ds(pl.multiple_of(i * (PRE // 2), PRE // 2), PRE // 2)
                pre = jnp.concatenate([pre_v[3 * j + m, rows, :] for m in range(3)], axis=1)
                pre = pltpu.bitcast(pre, BF16).astype(F32)
                qo_v[j] = r[16:24, :PAIR]
                kvo_v[j] = r[16:24, PAIR:]
                q8[j] = (pre[0:8, :PAIR], pre[0:8, PAIR:], r[24:32, PAIR:])
                q = jnp.concatenate([pre[8:16, :PAIR], r[0:16, :PAIR], r[24:32, :PAIR]], axis=0)
                kv = jnp.concatenate([pre[:, PAIR:], r[0:16, PAIR:], r[24:32, PAIR:]], axis=0)
            else:
                q8[j] = (qo_v[j], kvo_v.at[j], r[24:32, PAIR:])
                q = r[:, :PAIR]
                kv = jnp.concatenate([kvo_v[j], r[:, PAIR:]], axis=0)
            qkv[j] = (q.astype(BF16), blockdiag_k(kv[:, :PAIR]), blockdiag_v(kv[:, PAIR:]))

        def vector(jj):
            j, second = jj // 2, jj % 2
            key = ('u' if even else 'U', jj)
            if not second:
                o8[j] = first8_probs(*q8[j])
                pins[key] = [pltpu.bitcast(o8[j][1], U32)]
                return
            o = first8_values(*o8[j], *q8[j][1:])
            pins[key] = [pltpu.bitcast(x, U32) for x in o]
            o = jnp.concatenate(o, axis=1)
            if even:
                o8_v[j] = o
            else:
                o8[j] = o

        def scores(j):
            prob[j] = softmax(_nt(qkv[j][0], qkv[j][1]))

        def values(j):
            att[j] = jnp.dot(prob[j], qkv[j][2], preferred_element_type=F32)

        acc16 = [None]

        def outp(j, t):
            lhs = att[j][:, t * 128:(t + 1) * 128]
            if even:
                wide = sub > 0 and t in DEFER
                if wide:
                    lhs = jnp.concatenate([lhs, mid_v[j, DEFER.index(t)]], axis=0)
            else:
                wide = sub == UNROLL - 1 or t not in DEFER
                o16 = jnp.concatenate([o8_v[j, :, t * 128:(t + 1) * 128],
                                       o8[j][:, t * 128:(t + 1) * 128]], axis=0)
                if wide:
                    lhs = jnp.concatenate([lhs, o16], axis=0)
                else:
                    mid_v[j, DEFER.index(t)] = o16
            lhs = lhs.astype(BF16)
            r = j * PAIR // 2 + t * 64
            d = jnp.dot(lhs, pltpu.bitcast(wob_v[r:r + 64, :], BF16), preferred_element_type=F32)
            acc[0] = d[0:32] if acc[0] is None else acc[0] + d[0:32]
            if wide:
                acc16[0] = d[32:48] if acc16[0] is None else acc16[0] + d[32:48]

        fns = dict(s=scores, v=values, u=vector)
        for t in range(3):
            fns['xyz'[t]] = functools.partial(proj, part=t)
            fns['ABC'[t]] = functools.partial(outp, t=t)
        for k, j in PLANS[sub][0 if even else 1][0]:
            if k in fns:
                fns[k](j)
            else:
                extra[k](j)
        return acc[0], acc16[0]

    def body(i, sub, mem, held):
        r0 = pl.multiple_of(i * BLK, BLK)

        slab = slab_v.at[sub]

        def a_qkv(b, ahead=0):
            x = ax_v[pl.ds(r0 + ahead * BLK, BLK), :]
            slab_v[sub + ahead, b, A_PAD:A_PAD + BLK, :] = _nn(
                x, pltpu.bitcast(wqkvp_v[:, b * 128:(b + 1) * 128], BF16))

        a_o, a_p = {}, {}
        never = i < 0
        pins = {}

        def a_logits(sb):
            base = A_PAD + sb * A_SUB
            q = [slab[t, base:base + A_SUB, :] for t in range(LT)]
            logits = []
            for w in range(A_W):
                lo = base - A_DIL * w
                acc = None
                for t in range(LT):
                    pr = q[t] * slab[LT + t, lo:lo + A_SUB, :]
                    acc = pr if acc is None else acc + pr
                acc = acc + pltpu.roll(acc, 64, 1)
                acc = acc + pltpu.roll(acc, 32, 1)
                acc = acc * a_scale
                if sb == 0 and w > 0:
                    row = jax.lax.broadcasted_iota(jnp.int32, (A_SUB, 128), 0) + r0
                    acc = jnp.where(row >= A_DIL * w, acc, NEG)
                logits.append(acc)
            m = logits[0]
            for w in range(1, A_W):
                m = jnp.maximum(m, logits[w])
            ps = [jnp.exp(l - m) for l in logits]
            den = ps[0]
            for w in range(1, A_W):
                den = den + ps[w]
            inv = _recip(den)
            a_p[sb] = (ps, inv)
            pins[('a', sb)] = [pltpu.bitcast(inv[8 * u:8 * u + 8], U32) for u in range(A_SUB // 8)]

        def a_values(sb):
            base = A_PAD + sb * A_SUB
            ps, inv = a_p[sb]
            o = []
            for t in range(LT):
                acc = None
                for w in range(A_W):
                    lo = base - A_DIL * w
                    pr = ps[w] * slab[2 * LT + t, lo:lo + A_SUB, :]
                    acc = pr if acc is None else acc + pr
                o.append(acc * inv)
            pins[('b', sb)] = [pltpu.bitcast(x[8 * u:8 * u + 8], U32) for x in o
                               for u in range(A_SUB // 8)]
            a_o[sb] = jnp.concatenate(o, axis=1)
            if sb == BLK // A_SUB - 1:
                for t in range(LT, 3 * LT):
                    slab_v[(sub + 1) % UNROLL, t, 0:A_PAD, :] = slab[t, BLK:BLK + A_PAD, :]

        def pin(h, due):
            u = pltpu.bitcast(h, U32)
            tiles = [u[8 * r:8 * r + 8, 128 * c:128 * c + 128]
                     for c in range(LT) for r in range(u.shape[0] // 8)]
            for k, x in enumerate(due):
                tiles[k % len(tiles)] = jnp.where(never, x, tiles[k % len(tiles)])
            n = u.shape[0] // 8
            cols = [jnp.concatenate(tiles[c * n:(c + 1) * n], axis=0) for c in range(LT)]
            return pltpu.bitcast(jnp.concatenate(cols, axis=1), BF16)

        def a_out(b):
            o = jnp.concatenate([a_o[sb] for sb in range(BLK // A_SUB)], axis=0).astype(BF16)
            res = jnp.dot(o, pltpu.bitcast(woap_v[:, b * 128:(b + 1) * 128], BF16), preferred_element_type=F32)
            outa_v[pl.ds(r0, BLK), b * 128:(b + 1) * 128] = res.astype(BF16)

        x = bx_v[i].astype(F32)
        ex_e = ex_o = dict(q=a_qkv, Q=functools.partial(a_qkv, ahead=1), a=a_logits, b=a_values, w=a_out, pin=pin, pins=pins)
        def emit(r, out_e, acc, acc16):
            out = jnp.concatenate([acc16[0:8], out_e, acc16[8:16], acc[0:24]], axis=0)
            outb_v[pl.ds(r, BLK), :] = out.astype(BF16)
            pltpu.make_async_copy(
                outb_v.at[pl.ds(r, BLK)], out_h.at[pl.ds(r, BLK), pl.ds(D, D)],
                sem_out.at[1]).start()

        acc, acc16 = segment(
            i, sub, jnp.concatenate([x[16:40], mem], axis=0).astype(BF16), True, ex_e)
        if held is not None:
            emit(held[0], held[1], held[2], held[3] + acc16)
        out_e = acc[0:24]
        mem = acc[24:32].astype(BF16).astype(F32)
        acc, acc16 = segment(
            i, sub, jnp.concatenate([x[40:64], mem], axis=0).astype(BF16), False, ex_o)
        held = (r0, out_e, acc, acc16)
        if sub == UNROLL - 1 or not DEFER:
            emit(*held)
            held = None
        pltpu.make_async_copy(
            outa_v.at[pl.ds(r0, BLK)], out_h.at[pl.ds(r0, BLK), pl.ds(0, D)], sem_out.at[0]).start()
        return acc[24:32].astype(BF16).astype(F32), held

    def body_n(ii, mem):
        held = None
        for u in range(UNROLL):
            mem, held = body(ii * UNROLL + u, u, mem, held)
        return mem

    jax.lax.fori_loop(0, NLOOP // UNROLL, body_n, mem0_v[...].astype(F32))

    pltpu.make_async_copy(outa_v.at[0:NLOOP * BLK], out_h.at[0:NLOOP * BLK, pl.ds(0, D)], sem_out.at[0]).wait()
    pltpu.make_async_copy(outb_v.at[0:NLOOP * BLK], out_h.at[0:NLOOP * BLK, pl.ds(D, D)], sem_out.at[1]).wait()


@functools.partial(jax.jit, static_argnames=("B_seg_len",))
def pallas_concat_heads__sliding_local_dilated__memory_aug_recurrent_mem_tr__prompt_kernel(
    A_x: jax.Array,
    A_wqkv: jax.Array,
    A_wo: jax.Array,
    B_x: jax.Array,
    B_mem0: jax.Array,
    B_Wq: jax.Array,
    B_Wk: jax.Array,
    B_Wv: jax.Array,
    B_Wo: jax.Array,
    B_seg_len: int,
):
    assert A_x.shape == (1, S, D) and B_x.shape == (1, S, D)
    assert B_seg_len == B_SEG and B_mem0.shape == (1, B_M, D)
    assert B_Wq.shape == (D, B_H, B_DH) and B_Wo.shape == (B_H, B_DH, D)

    def feat_major(w):
        return jnp.transpose(w, (1, 2, 0)).reshape(B_F, D)

    any_spec = pl.BlockSpec(memory_space=pl.ANY)
    out = pl.pallas_call(
        _kernel,
        out_shape=jax.ShapeDtypeStruct((S, 2 * D), BF16),
        in_specs=[any_spec] * 9,
        out_specs=any_spec,
        scratch_shapes=[
            pltpu.VMEM((S, D), BF16),
            pltpu.VMEM((D, 3 * D), BF16),
            pltpu.VMEM((D, D), BF16),
            pltpu.VMEM((NIT, BLK, D), BF16),
            pltpu.VMEM((NIT, PRE, D), BF16),
            pltpu.VMEM((B_M, D), BF16),
            pltpu.VMEM((NU, PAIR, D), BF16),
            pltpu.VMEM((B_F, D), BF16),
            pltpu.VMEM((LT, 3 * D // 2, 128), U32),
            pltpu.VMEM((LT, D // 2, 128), U32),
            pltpu.VMEM((B_F // 2, D), U32),
            pltpu.VMEM((D // 2, 3 * D), U32),
            pltpu.VMEM((D // 2, D), U32),
            pltpu.VMEM((UNROLL, 3 * LT, A_PAD + BLK, 128), F32),
            pltpu.VMEM((S, D), BF16),
            pltpu.VMEM((NU, D // 2, PAIR), U32),
            pltpu.VMEM((NU, NIT * PRE // 2, PAIR), U32),
            pltpu.VMEM((NPAIR, 8, PAIR), F32),
            pltpu.VMEM((NPAIR, 8, 2 * PAIR), F32),
            pltpu.VMEM((NPAIR, 8, PAIR), F32),
            pltpu.VMEM((NPAIR, max(len(DEFER), 1), 16, 128), F32),
            pltpu.VMEM((S, D), BF16),
            pltpu.SemaphoreType.DMA((9 + len(U_HEAD) + U_N,)),
            pltpu.SemaphoreType.DMA((2,)),
        ],
        compiler_params=pltpu.CompilerParams(vmem_limit_bytes=120 * 1024 * 1024,
                                             disable_bounds_checks=True),
    )(
        A_x.reshape(S, D), A_wqkv, A_wo, B_x.reshape(NIT, BLK, D), B_mem0.reshape(B_M, D),
        feat_major(B_Wq), feat_major(B_Wk), feat_major(B_Wv), B_Wo.reshape(B_F, D),
    )
    return out.reshape(1, S, 2 * D)
```

```python
import functools

import jax
import jax.numpy as jnp
import jax.experimental.pallas as pl
import jax.experimental.pallas.tpu as pltpu

F32 = jnp.float32
BF16 = jnp.bfloat16
U32 = jnp.uint32

S = 2048
D = 640
LT = D // 128
BLK = 64
NIT = S // BLK

A_H = 32
A_DH = 20
A_W = 8
A_DIL = 2
A_PAD = 16
A_SUB = 16

B_H = 32
B_DH = 192
B_F = B_H * B_DH
B_M = 8
B_SEG = 32
B_L = B_M + B_SEG
PAIR = 2 * B_DH
NPAIR = B_H // 2
NU = 3 * NPAIR
PRE = 16
PRE_MB = 128

NEG = -1000000000.0
ILV = [h * B_DH + t * 64 for t in range(3) for h in range(2)]
LOG2E = 1.4426950408889634
LAG_S, LAG_V, LAG_O = [int(v) for v in "1,3,5".split(",")]
ORDER = "povs"
UNROLL = int("2")
U_HEAD = [int(v) for v in "1,1,2".split(",")]
U_BODY = int("5")
U_N = int("8")
U_TAIL = NU - sum(U_HEAD) - U_BODY * U_N
SEARCH = int("0")
XH = int("16")
DEFER = [int(v) for v in "1".split(",") if v.strip()]
PIN = int("1")
NLOOP = int("32")


def _schedule(order, lags, steady_extra, tail):
    lag = dict(p=0, s=lags[0], v=lags[1], o=lags[2])
    kind = dict(x="p", y="p", z="p", A="o", B="o", C="o", s="s", v="v")
    seq = []
    for t in range(NPAIR):
        for k in order:
            j = t - lag[kind[k]]
            if j >= 0:
                if k in "xAsv":
                    seq += steady_extra.get("<" + kind[k] + str(j), [])
                seq.append((k, j))
                if k in "zCsv":
                    seq += steady_extra.get(kind[k] + str(j), [])
            if t == NPAIR - 1 and k == "z":
                break
    for x in tail.split():
        seq += [(k, int(x[1:])) for k in ("ABC" if x[0] == "o" else x[0])
                if (k, int(x[1:])) not in seq]
    for k in "xyzABCsv":
        assert [j for kk, j in seq if kk == k] == list(range(NPAIR)), (k, seq)
    return seq


def _ex(txt):
    d = {}
    for x in txt.split():
        key, val = x.split(":")
        d.setdefault(key, []).append((val[0], int(val[1:])))
    return d


def _due(txt):
    d = {}
    for x in txt.split():
        key, at = x.split("@")
        j, m = at.split(".")
        d.setdefault((int(j), int(m)), []).append((key[0], int(key[1:])))
    return d


def _vector_plan(ea, eb, ia, ua, ib, ub, last):
    es = [(j, e, d) for j in range(NPAIR) for e, d in enumerate((ea, eb))]
    ds = [(k, 2 * j + e, 9 * j + int(d)) for j in range(NPAIR)
          for k, e, d in (("i", 0, ia), ("u", 0, ua), ("i", 1, ib), ("u", 1, ub)) if int(d) > 0]
    emit = " ".join(f"{d[0]}{j + int(d[1:])}:u{2 * j + e}" for j, e, d in es
                    if j + int(d[1:]) <= last[d[0]])
    tail = " ".join(f"u{2 * j + e}" for j, e, d in es if j + int(d[1:]) > last[d[0]])
    due = " ".join(f"{k}{n}@{d // 9}.{d % 9}" for k, n, d in ds if d < 9 * NPAIR)
    late = " ".join(f"{k}{n}@{d // 9 - NPAIR}.{d % 9}" for k, n, d in ds if d >= 9 * NPAIR)
    return emit, tail, due, late


def _plan(oe, le, xe, te, ve, oo, lo, xo, to, vo, do):
    ve = _vector_plan(*ve.split(), dict(p=15, s=13))
    vo = _vector_plan(*vo.split(), dict(p=15, s=13))
    sched_e = _schedule(oe, [int(v) for v in le.split(",")], _ex(xe + " " + ve[0]),
                        te.replace("#", ve[1]))
    sched_o = _schedule(oo, [int(v) for v in lo.split(",")], _ex(xo + " " + vo[0]),
                        to.replace("#", vo[1]))
    due_o = vo[2].replace("u", "U").replace("i", "I") + " " + ve[3] + " " + do
    return (sched_e, _due(ve[2])), (sched_o, _due(due_o))


PLANS = [_plan(
    "xyzABCvs",
    "1,3,4",
    "<s0:q0 <s1:q1 <s2:q2 <s3:Q0 <s4:Q1 <s5:q3 <s6:Q2 <s7:Q3 <s8:q4 <s9:Q4 <s10:q5 <s11:q6 <s12:Q5 <s13:q7",
    "v12 s14 q8 v13 s15 # o11 o12 o13 v14 q9 v15 o14 o15 q10 q11",
    "s0 s0 0 25 0 26",
    "xAyzBCvs",
    "1,3,5",
    "<s0:q12 <s1:q13 <s2:q14 p4:a0 p5:b0 p7:a1 p8:b1 p9:a2 p10:b2 p12:a3 p13:b3",
    "v12 s14 o10 v13 s15 # o11 o12 v14 o13 v15 w0 o14 o15 w1 w2 w3 w4",
    "s0 s0 0 25 0 26",
    "a0@5.0 b0@6.0 a1@8.0 b1@9.0 a2@10.0 b2@11.0 a3@13.0 b3@14.0",
), _plan(
    "xyABzCvs",
    "1,3,5",
    "<s0:q6 <s1:q7",
    "v12 s14 q8 v13 s15 # o10 o11 o12 v14 o13 v15 o14 q9 o15 q10 q11",
    "s0 s0 0 24 0 25",
    "xAyBzCvs",
    "1,3,5",
    "<s0:q12 <s1:q13 <s2:q14 p5:a0 p6:b0 p7:a1 p8:b1 p9:a2 p10:b2 p11:a3 p12:b3",
    "v12 s14 o10 v13 s15 # o11 o12 v14 o13 v15 o14 w0 o15 w1 w2 w3 w4",
    "s0 s0 0 24 0 25",
    "a0@6.0 b0@7.0 a1@8.0 b1@9.0 a2@10.0 b2@11.0 a3@12.0 b3@13.0",
)]


def _nt(a, b):
    return jax.lax.dot_general(a, b, (((1,), (1,)), ((), ())), preferred_element_type=F32)


def _nn(a, b):
    return jnp.dot(a, b, preferred_element_type=F32)


def _recip(x):
    r = pl.reciprocal(x, approx=True)
    return r * (2.0 - x * r)


def _kernel(ax_h, wqkv_h, woa_h, bx_h, mem0_h, wq_h, wk_h, wv_h, wo_h, out_h,
            ax_v, wqkv_v, woa_v, bx_v, xpre_v, mem0_v, wraw_v, wo_v,
            tmp_v, tmp2_v, wob_v, wqkvp_v, woap_v, slab_v, outa_v,
            wb_v, pre_v, qo_v, kvo_v, o8_v, mid_v, cap_v, outb_v,
            sem_in, sem_out):
    cp_xpre = [pltpu.make_async_copy(bx_h.at[pl.ds(a, n), pl.ds(0, PRE), :], xpre_v.at[pl.ds(a, n)],
                                     sem_in.at[s])
               for a, n, s in ((0, XH, 0), (XH, NIT - XH, 7 + len(U_HEAD) + U_N + 1))]
    cp_wqkv = pltpu.make_async_copy(wqkv_h, wqkv_v, sem_in.at[1])
    cp_woa = pltpu.make_async_copy(woa_h, woa_v, sem_in.at[2])
    cp_mem = pltpu.make_async_copy(mem0_h, mem0_v, sem_in.at[3])
    cp_bx = pltpu.make_async_copy(bx_h, bx_v, sem_in.at[4])
    cp_ax = pltpu.make_async_copy(ax_h, ax_v, sem_in.at[5])
    cp_wo = pltpu.make_async_copy(wo_h, wo_v, sem_in.at[6])
    w_hs = (wq_h, wk_h, wv_h)
    groups = list(U_HEAD) + [U_BODY] * U_N + [U_TAIL]
    g_start = [sum(groups[:g]) for g in range(len(groups))]

    cp_xpre[0].start()
    for g, n in enumerate(groups):
        for u in range(g_start[g], g_start[g] + n):
            pltpu.make_async_copy(w_hs[u % 3].at[pl.ds(u // 3 * PAIR, PAIR)], wraw_v.at[u],
                                  sem_in.at[7 + g]).start()
        if g == 0:
            cp_xpre[1].start()
    cp_wo.start()
    cp_wqkv.start()
    cp_woa.start()
    cp_mem.start()
    cp_bx.start()
    cp_ax.start()

    def g_wait(g, u0, n):
        buf = wraw_v.at[pl.ds(u0, n)]
        pltpu.make_async_copy(buf, buf, sem_in.at[7 + g]).wait()

    def b_pre(u, after=None, mbs=None):
        if isinstance(u, int):
            rows = [pl.ds(r if u % 3 == 2 else 64 * k, 64) for k, r in enumerate(ILV)]
        else:
            rows = [pl.ds(pl.multiple_of(jnp.where(u % 3 == 2, r, 64 * k), 64), 64)
                    for k, r in enumerate(ILV)]
        blk = jnp.concatenate([wraw_v[u, r, :] for r in rows], axis=0)
        if mbs is None or mbs[0] == 0:
            wb_v[u] = pltpu.bitcast(blk.T, U32)
        nb = PRE_MB // PRE
        for mb in (range(NIT // nb) if mbs is None else mbs):
            x = xpre_v[mb * nb:(mb + 1) * nb].reshape(PRE_MB, D)
            for n in range(PAIR // 128):
                r = _nt(x, blk[n * 128:(n + 1) * 128])
                pre_v[u, mb * PRE_MB // 2:(mb + 1) * PRE_MB // 2, n * 128:(n + 1) * 128] = (
                    pltpu.bitcast(r.astype(BF16), U32))
                if after is not None:
                    after(r)

    cp_xpre[0].wait()
    if SEARCH:
        b_pre = lambda u, after=None, mbs=None: None
    g_wait(0, 0, 1)
    nh = XH * PRE // PRE_MB
    b_pre(0, mbs=list(range(nh)))
    cp_xpre[1].wait()
    b_pre(0, mbs=list(range(nh, NIT * PRE // PRE_MB)))
    for g, n in enumerate(U_HEAD):
        if g == 0:
            continue
        g_wait(g, g_start[g], n)
        for u in range(g_start[g], g_start[g] + n):
            b_pre(u)

    def pre_body(c, carry):
        u0 = sum(U_HEAD) + c * U_BODY
        g_wait(len(U_HEAD) + c, u0, U_BODY)
        for k in range(U_BODY):
            b_pre(u0 + k)
        return carry + c

    off = jax.lax.fori_loop(0, U_N, pre_body, 0) < 0

    g_wait(len(groups) - 1, g_start[-1], U_TAIL)
    cp_wqkv.wait()
    cp_woa.wait()
    cp_wo.wait()
    tail_units = list(range(g_start[-1], NU))

    copies = [(woa_v, r, r, t, tmp2_v.at[t]) for t in range(LT) for r in range(0, D, 16)]
    copies += [(wo_v, j * PAIR + r + rr, j * PAIR + k * 64 + rr, t,
                wob_v.at[:, pl.ds(t * 128, 128)])
               for j in range(NPAIR) for k, r in enumerate(ILV) for t in range(LT)
               for rr in range(0, 64, 16)]

    def copy_some(res):
        for k in range(res.shape[0] // 8):
            tok = pltpu.bitcast(res[8 * k:8 * k + 8], U32)
            for _ in range(3):
                if copies:
                    src, r, rd, t, dst = copies.pop(0)
                    v = pltpu.bitcast(src[r:r + 16, t * 128:(t + 1) * 128], U32)
                    dst[rd // 2:rd // 2 + 8, :] = jnp.where(off, tok, v)

    def tail_pre(k):
        for u in tail_units[k * U_TAIL // 4:(k + 1) * U_TAIL // 4]:
            b_pre(u, copy_some)

    def regroup(tmp_v, t, base, g):
        parts = []
        for dp in (2 * g, 2 * g + 1):
            v = tmp_v[t, pl.ds(base + dp, A_H, stride=A_DH // 2), :]
            parts.append(pltpu.bitcast(v << 16, F32))
            parts.append(pltpu.bitcast(v & jnp.uint32(0xFFFF0000), F32))
        return jnp.concatenate(parts, axis=0).astype(BF16)

    def a_prep1(p):
        for b in range(p * LT, (p + 1) * LT):
            blk = pltpu.bitcast(wqkv_v[:, b * 128:(b + 1) * 128].T, U32)
            for t in range(LT):
                tmp_v[t, b * 64:(b + 1) * 64, :] = blk[:, t * 128:(t + 1) * 128]

    def a_prep2(p):
        for g in range(LT):
            blk = jnp.concatenate([regroup(tmp_v, t, p * D // 2, g) for t in range(LT)], axis=1)
            b = p * LT + g
            wqkvp_v[:, b * 128:(b + 1) * 128] = pltpu.bitcast(blk.T, U32)

    def a_prep4():
        for g in range(LT):
            for t in range(LT):
                woap_v[g * 64:(g + 1) * 64, t * 128:(t + 1) * 128] = pltpu.bitcast(
                    regroup(tmp2_v, t, 0, g), U32)

    if SEARCH:
        a_prep1 = a_prep2 = lambda p: None
        a_prep4 = lambda: None
        copies.clear()
    a_prep1(0)
    a_prep1(1)
    tail_pre(0)
    a_prep1(2)
    a_prep2(0)
    tail_pre(1)
    a_prep2(1)
    tail_pre(2)
    a_prep2(2)
    a_prep4()
    tail_pre(3)
    for t in range(LT, 3 * LT):
        slab_v[0, t, 0:A_PAD, :] = jnp.zeros((A_PAD, 128), F32)
    assert not copies
    cp_mem.wait()
    cp_bx.wait()
    cp_ax.wait()

    a_scale = A_DH ** (-0.5)
    b_scale = B_DH ** (-0.5)
    qrow = jax.lax.broadcasted_iota(jnp.int32, (32, 128), 0)
    lane = jax.lax.broadcasted_iota(jnp.int32, (32, 128), 1)
    first = lane < B_L
    kcol = jnp.where(first, lane, lane - B_L)
    allowed = (qrow >= B_SEG - 8) | (kcol >= B_SEG) | (qrow + 8 >= kcol)
    cap = jnp.where(allowed, jnp.inf, NEG * LOG2E)
    cap_v[0] = jnp.where(first, cap, -jnp.inf)
    cap_v[1] = jnp.where(first | (lane >= 2 * B_L), -jnp.inf, cap)
    cap_v[2] = jnp.where(qrow % 8 >= qrow // 8, jnp.inf, NEG * LOG2E)
    cap_v[3] = jnp.where(qrow % 8 >= qrow // 8 + 4, jnp.inf, NEG * LOG2E)

    def blockdiag_k(t):
        n = t.shape[0]
        left = jax.lax.broadcasted_iota(jnp.int32, (n, 128), 1) < 64
        z = jnp.zeros((n, 128), F32)
        mid = t[:, 128:256]
        top = jnp.concatenate([t[:, 0:128], jnp.where(left, mid, 0.0), z], axis=1)
        bot = jnp.concatenate([z, jnp.where(left, 0.0, mid), t[:, 256:384]], axis=1)
        return jnp.concatenate([top, bot], axis=0).astype(BF16)

    def blockdiag_v(t):
        left = jax.lax.broadcasted_iota(jnp.int32, t.shape, 1) % 128 < 64
        return jnp.concatenate([jnp.where(left, t, 0.0), jnp.where(left, 0.0, t)],
                               axis=0).astype(BF16)

    def softmax(s):
        s = jnp.concatenate([s, jnp.zeros((32, 128 - 2 * B_L), F32)], axis=1) * (b_scale * LOG2E)
        sa, sb = jnp.minimum(s, cap_v[0]), jnp.minimum(s, cap_v[1])
        ma = jnp.max(sa, axis=1, keepdims=True)
        mb = jnp.max(sb, axis=1, keepdims=True)
        p = jnp.exp2(jnp.maximum(sa, sb) - jnp.where(first, ma, mb))
        la = jnp.sum(jnp.where(first, p, 0.0), axis=1, keepdims=True)
        lb = jnp.sum(p, axis=1, keepdims=True) - la
        return (p * _recip(jnp.where(first, la, lb)))[:, :2 * B_L].astype(BF16)

    def bc(kv_x, kv_m, k, t):
        src = kv_x if k < 8 else kv_m
        return jnp.broadcast_to(src[k % 8:k % 8 + 1, t * 128:(t + 1) * 128], (8, 128))

    def first8_probs(q, kv_x, kv_m):
        left = jax.lax.broadcasted_iota(jnp.int32, (8, 128), 1) < 64
        row = jax.lax.broadcasted_iota(jnp.int32, (8, 128), 0)
        q = q * (b_scale * LOG2E)
        q0, q2 = q[:, 0:128], q[:, 256:384]
        q1a, q1b = jnp.where(left, q[:, 128:256], 0.0), jnp.where(left, 0.0, q[:, 128:256])
        sc = []
        for k in range(16):
            k1 = bc(kv_x, kv_m, k, 1)
            xa = jnp.sum(q0 * bc(kv_x, kv_m, k, 0) + q1a * k1, axis=1, keepdims=True)
            xb = jnp.sum(q1b * k1 + q2 * bc(kv_x, kv_m, k, 2), axis=1, keepdims=True)
            x = jnp.where(left, xa, xb)
            if 0 < k < 8:
                x = jnp.minimum(x, cap_v[2 + k // 4, 8 * (k % 4):8 * (k % 4) + 8, :])
            sc.append(x)
        m = functools.reduce(jnp.maximum, sc)
        p = [jnp.exp2(x - m) for x in sc]
        return p, _recip(functools.reduce(jnp.add, p))

    def first8_values(p, inv, kv_x, kv_m):
        return [functools.reduce(jnp.add, [p[k] * bc(kv_x, kv_m, k, 3 + t) for k in range(16)])
                * inv for t in range(3)]

    def segment(i, sub, h, even, extra):
        qkv, prob, att, q8, o8 = {}, {}, {}, {}, {}
        acc = [None]
        hh = [h]
        parts = []
        pins = extra['pins']

        def proj(j, part):
            dues = PLANS[sub][0 if even else 1][1]
            cuts = sorted({3 * part, 3 * part + 3}
                          | {m for (jj, m) in dues if jj == j and m // 3 == part})
            for m, m2 in zip(cuts[:-1], cuts[1:]):
                due = [x for key in dues.get((j, m), ()) for x in pins.pop(key)]
                if due:
                    hh[0] = extra['pin'](hh[0], due)
                w = wb_v[3 * j + part, :, (m - 3 * part) * 128:(m2 - 3 * part) * 128]
                parts.append(jnp.dot(hh[0], pltpu.bitcast(w, BF16), preferred_element_type=F32))
            if part < 2:
                return
            r = jnp.concatenate(parts, axis=1)
            parts.clear()
            if even:
                rows = pl.ds(pl.multiple_of(i * (PRE // 2), PRE // 2), PRE // 2)
                pre = jnp.concatenate([pre_v[3 * j + m, rows, :] for m in range(3)], axis=1)
                pre = pltpu.bitcast(pre, BF16).astype(F32)
                qo_v[j] = r[16:24, :PAIR]
                kvo_v[j] = r[16:24, PAIR:]
                q8[j] = (pre[0:8, :PAIR], pre[0:8, PAIR:], r[24:32, PAIR:])
                q = jnp.concatenate([pre[8:16, :PAIR], r[0:16, :PAIR], r[24:32, :PAIR]], axis=0)
                kv = jnp.concatenate([pre[:, PAIR:], r[0:16, PAIR:], r[24:32, PAIR:]], axis=0)
            else:
                q8[j] = (qo_v[j], kvo_v.at[j], r[24:32, PAIR:])
                q = r[:, :PAIR]
                kv = jnp.concatenate([kvo_v[j], r[:, PAIR:]], axis=0)
            qkv[j] = (q.astype(BF16), blockdiag_k(kv[:, :PAIR]), blockdiag_v(kv[:, PAIR:]))

        def vector(jj):
            j, second = jj // 2, jj % 2
            key = ('u' if even else 'U', jj)
            if not second:
                o8[j] = first8_probs(*q8[j])
                pins[key] = [pltpu.bitcast(o8[j][1], U32)]
                return
            o = first8_values(*o8[j], *q8[j][1:])
            pins[key] = [pltpu.bitcast(x, U32) for x in o]
            o = jnp.concatenate(o, axis=1)
            if even:
                o8_v[j] = o
            else:
                o8[j] = o

        def scores(j):
            prob[j] = softmax(_nt(qkv[j][0], qkv[j][1]))

        def values(j):
            att[j] = jnp.dot(prob[j], qkv[j][2], preferred_element_type=F32)

        acc16 = [None]

        def outp(j, t):
            lhs = att[j][:, t * 128:(t + 1) * 128]
            if even:
                wide = sub > 0 and t in DEFER
                if wide:
                    lhs = jnp.concatenate([lhs, mid_v[j, DEFER.index(t)]], axis=0)
            else:
                wide = sub == UNROLL - 1 or t not in DEFER
                o16 = jnp.concatenate([o8_v[j, :, t * 128:(t + 1) * 128],
                                       o8[j][:, t * 128:(t + 1) * 128]], axis=0)
                if wide:
                    lhs = jnp.concatenate([lhs, o16], axis=0)
                else:
                    mid_v[j, DEFER.index(t)] = o16
            lhs = lhs.astype(BF16)
            r = j * PAIR // 2 + t * 64
            d = jnp.dot(lhs, pltpu.bitcast(wob_v[r:r + 64, :], BF16), preferred_element_type=F32)
            acc[0] = d[0:32] if acc[0] is None else acc[0] + d[0:32]
            if wide:
                acc16[0] = d[32:48] if acc16[0] is None else acc16[0] + d[32:48]

        fns = dict(s=scores, v=values, u=vector)
        for t in range(3):
            fns['xyz'[t]] = functools.partial(proj, part=t)
            fns['ABC'[t]] = functools.partial(outp, t=t)
        for k, j in PLANS[sub][0 if even else 1][0]:
            if k in fns:
                fns[k](j)
            else:
                extra[k](j)
        return acc[0], acc16[0]

    def body(i, sub, mem, held):
        r0 = pl.multiple_of(i * BLK, BLK)

        slab = slab_v.at[sub]

        def a_qkv(b, ahead=0):
            x = ax_v[pl.ds(r0 + ahead * BLK, BLK), :]
            slab_v[sub + ahead, b, A_PAD:A_PAD + BLK, :] = _nn(
                x, pltpu.bitcast(wqkvp_v[:, b * 128:(b + 1) * 128], BF16))

        a_o, a_p = {}, {}
        never = i < 0
        pins = {}

        def a_logits(sb):
            base = A_PAD + sb * A_SUB
            q = [slab[t, base:base + A_SUB, :] for t in range(LT)]
            logits = []
            for w in range(A_W):
                lo = base - A_DIL * w
                acc = None
                for t in range(LT):
                    pr = q[t] * slab[LT + t, lo:lo + A_SUB, :]
                    acc = pr if acc is None else acc + pr
                acc = acc + pltpu.roll(acc, 64, 1)
                acc = acc + pltpu.roll(acc, 32, 1)
                acc = acc * a_scale
                if sb == 0 and w > 0:
                    row = jax.lax.broadcasted_iota(jnp.int32, (A_SUB, 128), 0) + r0
                    acc = jnp.where(row >= A_DIL * w, acc, NEG)
                logits.append(acc)
            m = logits[0]
            for w in range(1, A_W):
                m = jnp.maximum(m, logits[w])
            ps = [jnp.exp(l - m) for l in logits]
            den = ps[0]
            for w in range(1, A_W):
                den = den + ps[w]
            inv = _recip(den)
            a_p[sb] = (ps, inv)
            pins[('a', sb)] = [pltpu.bitcast(inv[8 * u:8 * u + 8], U32) for u in range(A_SUB // 8)]

        def a_values(sb):
            base = A_PAD + sb * A_SUB
            ps, inv = a_p[sb]
            o = []
            for t in range(LT):
                acc = None
                for w in range(A_W):
                    lo = base - A_DIL * w
                    pr = ps[w] * slab[2 * LT + t, lo:lo + A_SUB, :]
                    acc = pr if acc is None else acc + pr
                o.append(acc * inv)
            pins[('b', sb)] = [pltpu.bitcast(x[8 * u:8 * u + 8], U32) for x in o
                               for u in range(A_SUB // 8)]
            a_o[sb] = jnp.concatenate(o, axis=1)
            if sb == BLK // A_SUB - 1:
                for t in range(LT, 3 * LT):
                    slab_v[(sub + 1) % UNROLL, t, 0:A_PAD, :] = slab[t, BLK:BLK + A_PAD, :]

        def pin(h, due):
            u = pltpu.bitcast(h, U32)
            tiles = [u[8 * r:8 * r + 8, 128 * c:128 * c + 128]
                     for c in range(LT) for r in range(u.shape[0] // 8)]
            for k, x in enumerate(due):
                tiles[k % len(tiles)] = jnp.where(never, x, tiles[k % len(tiles)])
            n = u.shape[0] // 8
            cols = [jnp.concatenate(tiles[c * n:(c + 1) * n], axis=0) for c in range(LT)]
            return pltpu.bitcast(jnp.concatenate(cols, axis=1), BF16)

        def a_out(b):
            o = jnp.concatenate([a_o[sb] for sb in range(BLK // A_SUB)], axis=0).astype(BF16)
            res = jnp.dot(o, pltpu.bitcast(woap_v[:, b * 128:(b + 1) * 128], BF16), preferred_element_type=F32)
            outa_v[pl.ds(r0, BLK), b * 128:(b + 1) * 128] = res.astype(BF16)

        x = bx_v[i].astype(F32)
        ex_e = ex_o = dict(q=a_qkv, Q=functools.partial(a_qkv, ahead=1), a=a_logits, b=a_values, w=a_out, pin=pin, pins=pins)
        def emit(r, out_e, acc, acc16):
            out = jnp.concatenate([acc16[0:8], out_e, acc16[8:16], acc[0:24]], axis=0)
            outb_v[pl.ds(r, BLK), :] = out.astype(BF16)
            pltpu.make_async_copy(
                outb_v.at[pl.ds(r, BLK)], out_h.at[pl.ds(r, BLK), pl.ds(D, D)],
                sem_out.at[1]).start()

        acc, acc16 = segment(
            i, sub, jnp.concatenate([x[16:40], mem], axis=0).astype(BF16), True, ex_e)
        if held is not None:
            emit(held[0], held[1], held[2], held[3] + acc16)
        out_e = acc[0:24]
        mem = acc[24:32].astype(BF16).astype(F32)
        acc, acc16 = segment(
            i, sub, jnp.concatenate([x[40:64], mem], axis=0).astype(BF16), False, ex_o)
        held = (r0, out_e, acc, acc16)
        if sub == UNROLL - 1 or not DEFER:
            emit(*held)
            held = None
        pltpu.make_async_copy(
            outa_v.at[pl.ds(r0, BLK)], out_h.at[pl.ds(r0, BLK), pl.ds(0, D)], sem_out.at[0]).start()
        return acc[24:32].astype(BF16).astype(F32), held

    def body_n(ii, mem):
        held = None
        for u in range(UNROLL):
            mem, held = body(ii * UNROLL + u, u, mem, held)
        return mem

    jax.lax.fori_loop(0, NLOOP // UNROLL, body_n, mem0_v[...].astype(F32))

    pltpu.make_async_copy(outa_v.at[0:NLOOP * BLK], out_h.at[0:NLOOP * BLK, pl.ds(0, D)], sem_out.at[0]).wait()
    pltpu.make_async_copy(outb_v.at[0:NLOOP * BLK], out_h.at[0:NLOOP * BLK, pl.ds(D, D)], sem_out.at[1]).wait()


@functools.partial(jax.jit, static_argnames=("B_seg_len",))
def pallas_concat_heads__sliding_local_dilated__memory_aug_recurrent_mem_tr__prompt_kernel(
    A_x: jax.Array,
    A_wqkv: jax.Array,
    A_wo: jax.Array,
    B_x: jax.Array,
    B_mem0: jax.Array,
    B_Wq: jax.Array,
    B_Wk: jax.Array,
    B_Wv: jax.Array,
    B_Wo: jax.Array,
    B_seg_len: int,
):
    assert A_x.shape == (1, S, D) and B_x.shape == (1, S, D)
    assert B_seg_len == B_SEG and B_mem0.shape == (1, B_M, D)
    assert B_Wq.shape == (D, B_H, B_DH) and B_Wo.shape == (B_H, B_DH, D)

    def feat_major(w):
        return jnp.transpose(w, (1, 2, 0)).reshape(B_F, D)

    any_spec = pl.BlockSpec(memory_space=pl.ANY)
    out = pl.pallas_call(
        _kernel,
        out_shape=jax.ShapeDtypeStruct((S, 2 * D), BF16),
        in_specs=[any_spec] * 9,
        out_specs=any_spec,
        scratch_shapes=[
            pltpu.VMEM((S, D), BF16),
            pltpu.VMEM((D, 3 * D), BF16),
            pltpu.VMEM((D, D), BF16),
            pltpu.VMEM((NIT, BLK, D), BF16),
            pltpu.VMEM((NIT, PRE, D), BF16),
            pltpu.VMEM((B_M, D), BF16),
            pltpu.VMEM((NU, PAIR, D), BF16),
            pltpu.VMEM((B_F, D), BF16),
            pltpu.VMEM((LT, 3 * D // 2, 128), U32),
            pltpu.VMEM((LT, D // 2, 128), U32),
            pltpu.VMEM((B_F // 2, D), U32),
            pltpu.VMEM((D // 2, 3 * D), U32),
            pltpu.VMEM((D // 2, D), U32),
            pltpu.VMEM((UNROLL, 3 * LT, A_PAD + BLK, 128), F32),
            pltpu.VMEM((S, D), BF16),
            pltpu.VMEM((NU, D // 2, PAIR), U32),
            pltpu.VMEM((NU, NIT * PRE // 2, PAIR), U32),
            pltpu.VMEM((NPAIR, 8, PAIR), F32),
            pltpu.VMEM((NPAIR, 8, 2 * PAIR), F32),
            pltpu.VMEM((NPAIR, 8, PAIR), F32),
            pltpu.VMEM((NPAIR, max(len(DEFER), 1), 16, 128), F32),
            pltpu.VMEM((4, 32, 128), F32),
            pltpu.VMEM((S, D), BF16),
            pltpu.SemaphoreType.DMA((9 + len(U_HEAD) + U_N,)),
            pltpu.SemaphoreType.DMA((2,)),
        ],
        compiler_params=pltpu.CompilerParams(vmem_limit_bytes=120 * 1024 * 1024,
                                             disable_bounds_checks=True),
    )(
        A_x.reshape(S, D), A_wqkv, A_wo, B_x.reshape(NIT, BLK, D), B_mem0.reshape(B_M, D),
        feat_major(B_Wq), feat_major(B_Wk), feat_major(B_Wv), B_Wo.reshape(B_F, D),
    )
    return out.reshape(1, S, 2 * D)
```

```python
import functools

import jax
import jax.numpy as jnp
import jax.experimental.pallas as pl
import jax.experimental.pallas.tpu as pltpu

F32 = jnp.float32
BF16 = jnp.bfloat16
U32 = jnp.uint32

S = 2048
D = 640
LT = D // 128
BLK = 64
NIT = S // BLK

A_H = 32
A_DH = 20
A_W = 8
A_DIL = 2
A_PAD = 16
A_SUB = 16

B_H = 32
B_DH = 192
B_F = B_H * B_DH
B_M = 8
B_SEG = 32
B_L = B_M + B_SEG
PAIR = 2 * B_DH
NPAIR = B_H // 2
NU = 3 * NPAIR
PRE = 16
PRE_MB = 128

NEG = -1000000000.0
LOG2E = 1.4426950408889634
ILV = [h * B_DH + t * 64 for t in range(3) for h in range(2)]
UNROLL = 2
U_HEAD = (1, 1, 2)
U_BODY = 5
U_N = 8
U_TAIL = NU - sum(U_HEAD) - U_BODY * U_N
X_FIRST = 16
MID = 1


def _schedule(order, lags, extra, tail):
    lag = dict(p=0, s=lags[0], v=lags[1], o=lags[2])
    kind = dict(x="p", y="p", z="p", A="o", B="o", C="o", s="s", v="v")
    hooks = {}
    for x in extra.split():
        key, val = x.split(":")
        hooks.setdefault(key, []).append((val[0], int(val[1:])))
    seq = []
    for t in range(NPAIR):
        for k in order:
            j = t - lag[kind[k]]
            if j >= 0:
                if k in "xAsv":
                    seq += hooks.get("<" + kind[k] + str(j), [])
                seq.append((k, j))
                if k in "zCsv":
                    seq += hooks.get(kind[k] + str(j), [])
            if t == NPAIR - 1 and k == "z":
                break
    for x in tail.split():
        seq += [(k, int(x[1:])) for k in ("ABC" if x[0] == "o" else x[0])
                if (k, int(x[1:])) not in seq]
    for k in "xyzABCsv":
        assert [j for kk, j in seq if kk == k] == list(range(NPAIR)), (k, seq)
    return seq


def _plan(order_e, lag_e, extra_e, tail_e, due_e, order_o, extra_o, tail_o, due_o):
    emit = " ".join(f"s{j}:u{2 * j} s{j}:u{2 * j + 1}" for j in range(NPAIR - 2))
    rest = " ".join(f"u{n}" for n in range(2 * NPAIR - 4, 2 * NPAIR))
    dues = ({}, {})
    for j in range(NPAIR):
        for e in range(2):
            d = 9 * j + due_e + e
            dues[d >= 9 * NPAIR].setdefault((d // 9 % NPAIR, d % 9), []).append(("u", 2 * j + e))
            d = 9 * j + due_o + e
            if d < 9 * NPAIR:
                dues[1].setdefault((d // 9, d % 9), []).append(("U", 2 * j + e))
    for key in dues[1]:
        dues[1][key].sort(key=lambda x: x[0] == "u")
    for x in extra_o.split():
        key, val = x.split(":")
        if val[0] in "ab":
            dues[1].setdefault((int(key[1:]) + 1, 0), []).append((val[0], int(val[1:])))
    return ((_schedule(order_e, (1, 3, lag_e), extra_e + " " + emit, tail_e.replace("#", rest)),
             dues[0]),
            (_schedule(order_o, (1, 3, 5), extra_o + " " + emit, tail_o.replace("#", rest)),
             dues[1]))


PLANS = (
    _plan("xyzBACvs", 4,
          "<s0:q0 <s1:q1 <s2:q2 <s3:Q0 <s4:Q1 <s5:q3 <s6:Q2 <s7:Q3 <s8:q4 <s9:Q4 <s10:q5 <s11:q6"
          " <s12:Q5 <s13:q7",
          "v12 s14 q8 v13 s15 # o11 o12 o13 v14 q9 v15 o14 o15 q10 q11", 25,
          "xAyzBCvs",
          "<s0:q12 <s1:q13 <s2:q14 p4:a0 p5:b0 p7:a1 p8:b1 p9:a2 p10:b2 p12:a3 p13:b3",
          "v12 s14 o10 v13 s15 # o11 o12 v14 w0 v15 o13 w1 o14 w2 o15 w3 w4", 25),
    _plan("xyABzCvs", 5, "<s0:q6 <s1:q7",
          "v12 s14 q8 v13 s15 # o10 o11 o12 v14 o13 v15 o14 q9 o15 q10 q11", 22,
          "xAyBzCvs",
          "<s0:q12 <s1:q13 <s2:q14 p5:a0 p6:b0 p7:a1 p8:b1 p9:a2 p10:b2 p11:a3 p12:b3",
          "v12 s14 o10 v13 s15 # o11 o12 v14 o13 v15 o14 w0 o15 w1 w2 w3 w4", 24),
)


def _nt(a, b):
    return jax.lax.dot_general(a, b, (((1,), (1,)), ((), ())), preferred_element_type=F32)


def _nn(a, b):
    return jnp.dot(a, b, preferred_element_type=F32)


def _recip(x):
    r = pl.reciprocal(x, approx=True)
    return r * (2.0 - x * r)


def _kernel(ax_h, wqkv_h, woa_h, bx_h, mem0_h, wq_h, wk_h, wv_h, wo_h, out_h,
            ax_v, wqkv_v, woa_v, bx_v, xpre_v, mem0_v, wraw_v, wo_v,
            tmp_v, tmp2_v, wob_v, wqkvp_v, woap_v, slab_v, outa_v,
            wb_v, pre_v, qo_v, kvo_v, o8_v, mid_v, cap_v, outb_v,
            sem_in, sem_out):
    cp_xpre = [pltpu.make_async_copy(bx_h.at[pl.ds(a, n), pl.ds(0, PRE), :],
                                     xpre_v.at[pl.ds(a, n)], sem_in.at[s])
               for a, n, s in ((0, X_FIRST, 0), (X_FIRST, NIT - X_FIRST, 8 + len(U_HEAD) + U_N))]
    cp_wqkv = pltpu.make_async_copy(wqkv_h, wqkv_v, sem_in.at[1])
    cp_woa = pltpu.make_async_copy(woa_h, woa_v, sem_in.at[2])
    cp_mem = pltpu.make_async_copy(mem0_h, mem0_v, sem_in.at[3])
    cp_bx = pltpu.make_async_copy(bx_h, bx_v, sem_in.at[4])
    cp_ax = pltpu.make_async_copy(ax_h, ax_v, sem_in.at[5])
    cp_wo = pltpu.make_async_copy(wo_h, wo_v, sem_in.at[6])
    w_hs = (wq_h, wk_h, wv_h)
    groups = list(U_HEAD) + [U_BODY] * U_N + [U_TAIL]
    g_start = [sum(groups[:g]) for g in range(len(groups))]

    cp_xpre[0].start()
    for g, n in enumerate(groups):
        for u in range(g_start[g], g_start[g] + n):
            pltpu.make_async_copy(w_hs[u % 3].at[pl.ds(u // 3 * PAIR, PAIR)], wraw_v.at[u],
                                  sem_in.at[7 + g]).start()
        if g == 0:
            cp_xpre[1].start()
    cp_wo.start()
    cp_wqkv.start()
    cp_woa.start()
    cp_mem.start()
    cp_bx.start()
    cp_ax.start()

    def g_wait(g, u0, n):
        buf = wraw_v.at[pl.ds(u0, n)]
        pltpu.make_async_copy(buf, buf, sem_in.at[7 + g]).wait()

    def b_pre(u, after=None, mbs=None):
        if isinstance(u, int):
            rows = [pl.ds(r if u % 3 == 2 else 64 * k, 64) for k, r in enumerate(ILV)]
        else:
            rows = [pl.ds(pl.multiple_of(jnp.where(u % 3 == 2, r, 64 * k), 64), 64)
                    for k, r in enumerate(ILV)]
        blk = jnp.concatenate([wraw_v[u, r, :] for r in rows], axis=0)
        if mbs is None or mbs[0] == 0:
            wb_v[u] = pltpu.bitcast(blk.T, U32)
        nb = PRE_MB // PRE
        for mb in (range(NIT // nb) if mbs is None else mbs):
            x = xpre_v[mb * nb:(mb + 1) * nb].reshape(PRE_MB, D)
            for n in range(PAIR // 128):
                r = _nt(x, blk[n * 128:(n + 1) * 128])
                pre_v[u, mb * PRE_MB // 2:(mb + 1) * PRE_MB // 2, n * 128:(n + 1) * 128] = (
                    pltpu.bitcast(r.astype(BF16), U32))
                if after is not None:
                    after(r)

    cp_xpre[0].wait()
    g_wait(0, 0, 1)
    nh = X_FIRST * PRE // PRE_MB
    b_pre(0, mbs=list(range(nh)))
    cp_xpre[1].wait()
    b_pre(0, mbs=list(range(nh, NIT * PRE // PRE_MB)))
    for g in range(1, len(U_HEAD)):
        g_wait(g, g_start[g], groups[g])
        for u in range(g_start[g], g_start[g] + groups[g]):
            b_pre(u)

    def pre_body(c, carry):
        u0 = sum(U_HEAD) + c * U_BODY
        g_wait(len(U_HEAD) + c, u0, U_BODY)
        for k in range(U_BODY):
            b_pre(u0 + k)
        return carry + c

    off = jax.lax.fori_loop(0, U_N, pre_body, 0) < 0

    g_wait(len(groups) - 1, g_start[-1], U_TAIL)
    cp_wqkv.wait()
    cp_woa.wait()
    cp_wo.wait()
    tail_units = list(range(g_start[-1], NU))

    copies = [(woa_v, r, r, t, tmp2_v.at[t]) for t in range(LT) for r in range(0, D, 16)]
    copies += [(wo_v, j * PAIR + r + rr, j * PAIR + k * 64 + rr, t,
                wob_v.at[:, pl.ds(t * 128, 128)])
               for j in range(NPAIR) for k, r in enumerate(ILV) for t in range(LT)
               for rr in range(0, 64, 16)]

    def copy_some(res):
        for k in range(res.shape[0] // 8):
            tok = pltpu.bitcast(res[8 * k:8 * k + 8], U32)
            for _ in range(3):
                if copies:
                    src, r, rd, t, dst = copies.pop(0)
                    v = pltpu.bitcast(src[r:r + 16, t * 128:(t + 1) * 128], U32)
                    dst[rd // 2:rd // 2 + 8, :] = jnp.where(off, tok, v)

    def tail_pre(k):
        for u in tail_units[k * U_TAIL // 4:(k + 1) * U_TAIL // 4]:
            b_pre(u, copy_some)

    def regroup(src_v, t, base, g):
        parts = []
        for dp in (2 * g, 2 * g + 1):
            v = src_v[t, pl.ds(base + dp, A_H, stride=A_DH // 2), :]
            parts.append(pltpu.bitcast(v << 16, F32))
            parts.append(pltpu.bitcast(v & jnp.uint32(0xFFFF0000), F32))
        return jnp.concatenate(parts, axis=0).astype(BF16)

    def a_prep1(p):
        for b in range(p * LT, (p + 1) * LT):
            blk = pltpu.bitcast(wqkv_v[:, b * 128:(b + 1) * 128].T, U32)
            for t in range(LT):
                tmp_v[t, b * 64:(b + 1) * 64, :] = blk[:, t * 128:(t + 1) * 128]

    def a_prep2(p):
        for g in range(LT):
            blk = jnp.concatenate([regroup(tmp_v, t, p * D // 2, g) for t in range(LT)], axis=1)
            b = p * LT + g
            wqkvp_v[:, b * 128:(b + 1) * 128] = pltpu.bitcast(blk.T, U32)

    def a_prep3():
        for g in range(LT):
            for t in range(LT):
                woap_v[g * 64:(g + 1) * 64, t * 128:(t + 1) * 128] = pltpu.bitcast(
                    regroup(tmp2_v, t, 0, g), U32)

    a_prep1(0)
    a_prep1(1)
    tail_pre(0)
    a_prep1(2)
    a_prep2(0)
    tail_pre(1)
    a_prep2(1)
    tail_pre(2)
    a_prep2(2)
    a_prep3()
    tail_pre(3)
    for t in range(LT, 3 * LT):
        slab_v[0, t, 0:A_PAD, :] = jnp.zeros((A_PAD, 128), F32)
    assert not copies
    cp_mem.wait()
    cp_bx.wait()
    cp_ax.wait()

    a_scale = A_DH ** (-0.5)
    b_scale = B_DH ** (-0.5)
    qrow = jax.lax.broadcasted_iota(jnp.int32, (32, 128), 0)
    lane = jax.lax.broadcasted_iota(jnp.int32, (32, 128), 1)
    first = lane < B_L
    kcol = jnp.where(first, lane, lane - B_L)
    allowed = (qrow >= B_SEG - 8) | (kcol >= B_SEG) | (qrow + 8 >= kcol)
    cap = jnp.where(allowed, jnp.inf, NEG * LOG2E)
    cap_v[0] = jnp.where(first, cap, -jnp.inf)
    cap_v[1] = jnp.where(first | (lane >= 2 * B_L), -jnp.inf, cap)
    cap_v[2] = jnp.where(qrow % 8 >= qrow // 8, jnp.inf, NEG * LOG2E)
    cap_v[3] = jnp.where(qrow % 8 >= qrow // 8 + 4, jnp.inf, NEG * LOG2E)

    def blockdiag_k(t):
        n = t.shape[0]
        left = jax.lax.broadcasted_iota(jnp.int32, (n, 128), 1) < 64
        z = jnp.zeros((n, 128), F32)
        mid = t[:, 128:256]
        top = jnp.concatenate([t[:, 0:128], jnp.where(left, mid, 0.0), z], axis=1)
        bot = jnp.concatenate([z, jnp.where(left, 0.0, mid), t[:, 256:384]], axis=1)
        return jnp.concatenate([top, bot], axis=0).astype(BF16)

    def blockdiag_v(t):
        left = jax.lax.broadcasted_iota(jnp.int32, t.shape, 1) % 128 < 64
        return jnp.concatenate([jnp.where(left, t, 0.0), jnp.where(left, 0.0, t)],
                               axis=0).astype(BF16)

    def softmax(s):
        s = jnp.concatenate([s, jnp.zeros((32, 128 - 2 * B_L), F32)], axis=1) * (b_scale * LOG2E)
        sa, sb = jnp.minimum(s, cap_v[0]), jnp.minimum(s, cap_v[1])
        ma = jnp.max(sa, axis=1, keepdims=True)
        mb = jnp.max(sb, axis=1, keepdims=True)
        p = jnp.exp2(jnp.maximum(sa, sb) - jnp.where(first, ma, mb))
        la = jnp.sum(jnp.where(first, p, 0.0), axis=1, keepdims=True)
        lb = jnp.sum(p, axis=1, keepdims=True) - la
        p = p * pl.reciprocal(jnp.where(first, la, lb), approx=True)
        return p[:, :2 * B_L].astype(BF16)

    def bc(kv_x, kv_m, k, t):
        src = kv_x if k < 8 else kv_m
        return jnp.broadcast_to(src[k % 8:k % 8 + 1, t * 128:(t + 1) * 128], (8, 128))

    def first8_probs(q, kv_x, kv_m):
        left = jax.lax.broadcasted_iota(jnp.int32, (8, 128), 1) < 64
        q = q * (b_scale * LOG2E)
        q0, q2 = q[:, 0:128], q[:, 256:384]
        q1a, q1b = jnp.where(left, q[:, 128:256], 0.0), jnp.where(left, 0.0, q[:, 128:256])
        sc = []
        for k in range(16):
            k1 = bc(kv_x, kv_m, k, 1)
            xa = jnp.sum(q0 * bc(kv_x, kv_m, k, 0) + q1a * k1, axis=1, keepdims=True)
            xb = jnp.sum(q1b * k1 + q2 * bc(kv_x, kv_m, k, 2), axis=1, keepdims=True)
            x = jnp.where(left, xa, xb)
            if 0 < k < 8:
                x = jnp.minimum(x, cap_v[2 + k // 4, 8 * (k % 4):8 * (k % 4) + 8, :])
            sc.append(x)
        m = functools.reduce(jnp.maximum, sc)
        p = [jnp.exp2(x - m) for x in sc]
        return p, _recip(functools.reduce(jnp.add, p))

    def first8_values(p, inv, kv_x, kv_m):
        return [functools.reduce(jnp.add, [p[k] * bc(kv_x, kv_m, k, 3 + t) for k in range(16)])
                * inv for t in range(3)]

    def segment(i, sub, h, even, extra):
        order, dues = PLANS[sub][0 if even else 1]
        qkv, prob, att, q8, o8 = {}, {}, {}, {}, {}
        acc, acc16 = [None], [None]
        hh = [h]
        parts = []
        pins = extra['pins']

        def proj(j, part):
            cuts = sorted({3 * part, 3 * part + 3}
                          | {m for (jj, m) in dues if jj == j and m // 3 == part})
            for m, m2 in zip(cuts[:-1], cuts[1:]):
                due = [x for key in dues.get((j, m), ()) for x in pins.pop(key)]
                if due:
                    hh[0] = extra['pin'](hh[0], due)
                w = wb_v[3 * j + part, :, (m - 3 * part) * 128:(m2 - 3 * part) * 128]
                parts.append(_nn(hh[0], pltpu.bitcast(w, BF16)))
            if part < 2:
                return
            r = jnp.concatenate(parts, axis=1)
            parts.clear()
            if even:
                rows = pl.ds(pl.multiple_of(i * (PRE // 2), PRE // 2), PRE // 2)
                pre = jnp.concatenate([pre_v[3 * j + m, rows, :] for m in range(3)], axis=1)
                pre = pltpu.bitcast(pre, BF16).astype(F32)
                qo_v[j] = r[16:24, :PAIR]
                kvo_v[j] = r[16:24, PAIR:]
                q8[j] = (pre[0:8, :PAIR], pre[0:8, PAIR:], r[24:32, PAIR:])
                q = jnp.concatenate([pre[8:16, :PAIR], r[0:16, :PAIR], r[24:32, :PAIR]], axis=0)
                kv = jnp.concatenate([pre[:, PAIR:], r[0:16, PAIR:], r[24:32, PAIR:]], axis=0)
            else:
                q8[j] = (qo_v[j], kvo_v.at[j], r[24:32, PAIR:])
                q = r[:, :PAIR]
                kv = jnp.concatenate([kvo_v[j], r[:, PAIR:]], axis=0)
            qkv[j] = (q.astype(BF16), blockdiag_k(kv[:, :PAIR]), blockdiag_v(kv[:, PAIR:]))

        def vector(jj):
            j, second = jj // 2, jj % 2
            key = ('u' if even else 'U', jj)
            if not second:
                o8[j] = first8_probs(*q8[j])
                pins[key] = [pltpu.bitcast(o8[j][1], U32)]
                return
            o = first8_values(*o8[j], *q8[j][1:])
            pins[key] = [pltpu.bitcast(x, U32) for x in o]
            o = jnp.concatenate(o, axis=1)
            if even:
                o8_v[j] = o
            else:
                o8[j] = o

        def scores(j):
            prob[j] = softmax(_nt(qkv[j][0], qkv[j][1]))

        def values(j):
            att[j] = _nn(prob[j], qkv[j][2])

        def outp(j, t):
            lhs = att[j][:, t * 128:(t + 1) * 128]
            if even:
                wide = sub > 0 and t == MID
                if wide:
                    lhs = jnp.concatenate([lhs, mid_v[j]], axis=0)
            else:
                wide = sub == UNROLL - 1 or t != MID
                o16 = jnp.concatenate([o8_v[j, :, t * 128:(t + 1) * 128],
                                       o8[j][:, t * 128:(t + 1) * 128]], axis=0)
                if wide:
                    lhs = jnp.concatenate([lhs, o16], axis=0)
                else:
                    mid_v[j] = o16
            r = j * PAIR // 2 + t * 64
            d = _nn(lhs.astype(BF16), pltpu.bitcast(wob_v[r:r + 64, :], BF16))
            acc[0] = d[0:32] if acc[0] is None else acc[0] + d[0:32]
            if wide:
                acc16[0] = d[32:48] if acc16[0] is None else acc16[0] + d[32:48]

        fns = dict(extra, s=scores, v=values, u=vector)
        for t in range(3):
            fns['xyz'[t]] = functools.partial(proj, part=t)
            fns['ABC'[t]] = functools.partial(outp, t=t)
        for k, j in order:
            fns[k](j)
        return acc[0], acc16[0]

    def body(i, sub, mem, held):
        r0 = pl.multiple_of(i * BLK, BLK)

        slab = slab_v.at[sub]

        def a_qkv(b, ahead=0):
            x = ax_v[pl.ds(r0 + ahead * BLK, BLK), :]
            slab_v[sub + ahead, b, A_PAD:A_PAD + BLK, :] = _nn(
                x, pltpu.bitcast(wqkvp_v[:, b * 128:(b + 1) * 128], BF16))

        a_o, a_p = {}, {}
        never = i < 0
        pins = {}

        def a_logits(sb):
            base = A_PAD + sb * A_SUB
            q = [slab[t, base:base + A_SUB, :] for t in range(LT)]
            logits = []
            for w in range(A_W):
                lo = base - A_DIL * w
                acc = None
                for t in range(LT):
                    pr = q[t] * slab[LT + t, lo:lo + A_SUB, :]
                    acc = pr if acc is None else acc + pr
                acc = acc + pltpu.roll(acc, 64, 1)
                acc = acc + pltpu.roll(acc, 32, 1)
                acc = acc * a_scale
                if sb == 0 and w > 0:
                    row = jax.lax.broadcasted_iota(jnp.int32, (A_SUB, 128), 0) + r0
                    acc = jnp.where(row >= A_DIL * w, acc, NEG)
                logits.append(acc)
            m = logits[0]
            for w in range(1, A_W):
                m = jnp.maximum(m, logits[w])
            ps = [jnp.exp(l - m) for l in logits]
            den = ps[0]
            for w in range(1, A_W):
                den = den + ps[w]
            inv = _recip(den)
            a_p[sb] = (ps, inv)
            pins[('a', sb)] = [pltpu.bitcast(inv[8 * u:8 * u + 8], U32) for u in range(A_SUB // 8)]

        def a_values(sb):
            base = A_PAD + sb * A_SUB
            ps, inv = a_p[sb]
            o = []
            for t in range(LT):
                acc = None
                for w in range(A_W):
                    lo = base - A_DIL * w
                    pr = ps[w] * slab[2 * LT + t, lo:lo + A_SUB, :]
                    acc = pr if acc is None else acc + pr
                o.append(acc * inv)
            pins[('b', sb)] = [pltpu.bitcast(x[8 * u:8 * u + 8], U32) for x in o
                               for u in range(A_SUB // 8)]
            a_o[sb] = jnp.concatenate(o, axis=1)
            if sb == BLK // A_SUB - 1:
                for t in range(LT, 3 * LT):
                    slab_v[(sub + 1) % UNROLL, t, 0:A_PAD, :] = slab[t, BLK:BLK + A_PAD, :]

        def pin(h, due):
            u = pltpu.bitcast(h, U32)
            tiles = [u[8 * r:8 * r + 8, 128 * c:128 * c + 128]
                     for c in range(LT) for r in range(u.shape[0] // 8)]
            for k, x in enumerate(due):
                tiles[k % len(tiles)] = jnp.where(never, x, tiles[k % len(tiles)])
            n = u.shape[0] // 8
            cols = [jnp.concatenate(tiles[c * n:(c + 1) * n], axis=0) for c in range(LT)]
            return pltpu.bitcast(jnp.concatenate(cols, axis=1), BF16)

        def a_out(b):
            o = jnp.concatenate([a_o[sb] for sb in range(BLK // A_SUB)], axis=0).astype(BF16)
            res = _nn(o, pltpu.bitcast(woap_v[:, b * 128:(b + 1) * 128], BF16))
            outa_v[pl.ds(r0, BLK), b * 128:(b + 1) * 128] = res.astype(BF16)

        x = bx_v[i].astype(F32)
        extra = dict(q=a_qkv, Q=functools.partial(a_qkv, ahead=1), a=a_logits, b=a_values,
                     w=a_out, pin=pin, pins=pins)

        def emit(r, out_e, acc, acc16):
            out = jnp.concatenate([acc16[0:8], out_e, acc16[8:16], acc[0:24]], axis=0)
            outb_v[pl.ds(r, BLK), :] = out.astype(BF16)
            pltpu.make_async_copy(
                outb_v.at[pl.ds(r, BLK)], out_h.at[pl.ds(r, BLK), pl.ds(D, D)],
                sem_out.at[1]).start()

        acc, acc16 = segment(
            i, sub, jnp.concatenate([x[16:40], mem], axis=0).astype(BF16), True, extra)
        if held is not None:
            emit(held[0], held[1], held[2], held[3] + acc16)
        out_e = acc[0:24]
        mem = acc[24:32].astype(BF16).astype(F32)
        acc, acc16 = segment(
            i, sub, jnp.concatenate([x[40:64], mem], axis=0).astype(BF16), False, extra)
        held = (r0, out_e, acc, acc16)
        if sub == UNROLL - 1:
            emit(*held)
            held = None
        pltpu.make_async_copy(
            outa_v.at[pl.ds(r0, BLK)], out_h.at[pl.ds(r0, BLK), pl.ds(0, D)], sem_out.at[0]).start()
        return acc[24:32].astype(BF16).astype(F32), held

    def body_n(ii, mem):
        held = None
        for u in range(UNROLL):
            mem, held = body(ii * UNROLL + u, u, mem, held)
        return mem

    jax.lax.fori_loop(0, NIT // UNROLL, body_n, mem0_v[...].astype(F32))

    pltpu.make_async_copy(outa_v, out_h.at[:, pl.ds(0, D)], sem_out.at[0]).wait()
    pltpu.make_async_copy(outb_v, out_h.at[:, pl.ds(D, D)], sem_out.at[1]).wait()


@jax.jit
def _run(A_x, A_wqkv, A_wo, B_x, B_mem0, B_Wq, B_Wk, B_Wv, B_Wo):
    def feat_major(w):
        return jnp.transpose(w, (1, 2, 0)).reshape(B_F, D)

    any_spec = pl.BlockSpec(memory_space=pl.ANY)
    out = pl.pallas_call(
        _kernel,
        out_shape=jax.ShapeDtypeStruct((S, 2 * D), BF16),
        in_specs=[any_spec] * 9,
        out_specs=any_spec,
        scratch_shapes=[
            pltpu.VMEM((S, D), BF16),
            pltpu.VMEM((D, 3 * D), BF16),
            pltpu.VMEM((D, D), BF16),
            pltpu.VMEM((NIT, BLK, D), BF16),
            pltpu.VMEM((NIT, PRE, D), BF16),
            pltpu.VMEM((B_M, D), BF16),
            pltpu.VMEM((NU, PAIR, D), BF16),
            pltpu.VMEM((B_F, D), BF16),
            pltpu.VMEM((LT, 3 * D // 2, 128), U32),
            pltpu.VMEM((LT, D // 2, 128), U32),
            pltpu.VMEM((B_F // 2, D), U32),
            pltpu.VMEM((D // 2, 3 * D), U32),
            pltpu.VMEM((D // 2, D), U32),
            pltpu.VMEM((UNROLL, 3 * LT, A_PAD + BLK, 128), F32),
            pltpu.VMEM((S, D), BF16),
            pltpu.VMEM((NU, D // 2, PAIR), U32),
            pltpu.VMEM((NU, NIT * PRE // 2, PAIR), U32),
            pltpu.VMEM((NPAIR, 8, PAIR), F32),
            pltpu.VMEM((NPAIR, 8, 2 * PAIR), F32),
            pltpu.VMEM((NPAIR, 8, PAIR), F32),
            pltpu.VMEM((NPAIR, 16, 128), F32),
            pltpu.VMEM((4, 32, 128), F32),
            pltpu.VMEM((S, D), BF16),
            pltpu.SemaphoreType.DMA((9 + len(U_HEAD) + U_N,)),
            pltpu.SemaphoreType.DMA((2,)),
        ],
        compiler_params=pltpu.CompilerParams(vmem_limit_bytes=120 * 1024 * 1024,
                                             disable_bounds_checks=True),
    )(
        A_x.reshape(S, D), A_wqkv, A_wo, B_x.reshape(NIT, BLK, D), B_mem0.reshape(B_M, D),
        feat_major(B_Wq), feat_major(B_Wk), feat_major(B_Wv), B_Wo.reshape(B_F, D),
    )
    return out.reshape(1, S, 2 * D)


def pallas_concat_heads__sliding_local_dilated__memory_aug_recurrent_mem_tr__prompt_kernel(
    A_x: jax.Array,
    A_wqkv: jax.Array,
    A_wo: jax.Array,
    B_x: jax.Array,
    B_mem0: jax.Array,
    B_Wq: jax.Array,
    B_Wk: jax.Array,
    B_Wv: jax.Array,
    B_Wo: jax.Array,
    B_seg_len,
):
    assert A_x.shape == (1, S, D) and B_x.shape == (1, S, D) and B_mem0.shape == (1, B_M, D)
    assert B_Wq.shape == (D, B_H, B_DH) and B_Wo.shape == (B_H, B_DH, D)
    if isinstance(B_seg_len, int):
        assert B_seg_len == B_SEG
    return _run(A_x, A_wqkv, A_wo, B_x, B_mem0, B_Wq, B_Wk, B_Wv, B_Wo)
```

```python
import functools

import jax
import jax.numpy as jnp
import jax.experimental.pallas as pl
import jax.experimental.pallas.tpu as pltpu

F32 = jnp.float32
BF16 = jnp.bfloat16
U32 = jnp.uint32

S = 2048
D = 640
LT = D // 128
BLK = 64
NIT = S // BLK

A_H = 32
A_DH = 20
A_W = 8
A_DIL = 2
A_PAD = 16
A_SUB = 16

B_H = 32
B_DH = 192
B_F = B_H * B_DH
B_M = 8
B_SEG = 32
B_L = B_M + B_SEG
PAIR = 2 * B_DH
NPAIR = B_H // 2
NU = 3 * NPAIR
PRE = 16
PRE_MB = 128

NEG = -1000000000.0
LOG2E = 1.4426950408889634
ILV = [h * B_DH + t * 64 for t in range(3) for h in range(2)]
UNROLL = 2
U_HEAD = (1, 1, 2)
U_BODY = 5
U_N = 8
U_TAIL = NU - sum(U_HEAD) - U_BODY * U_N
X_FIRST = 16
MID = 1


def _schedule(order, lags, extra, tail):
    lag = dict(p=0, s=lags[0], v=lags[1], o=lags[2])
    kind = dict(x="p", y="p", z="p", A="o", B="o", C="o", s="s", v="v")
    hooks = {}
    for x in extra.split():
        key, val = x.split(":")
        hooks.setdefault(key, []).append((val[0], int(val[1:])))
    seq = []
    for t in range(NPAIR):
        for k in order:
            j = t - lag[kind[k]]
            if j >= 0:
                if k in "xAsv":
                    seq += hooks.get("<" + kind[k] + str(j), [])
                seq.append((k, j))
                if k in "zCsv":
                    seq += hooks.get(kind[k] + str(j), [])
            if t == NPAIR - 1 and k == "z":
                break
    for x in tail.split():
        seq += [(k, int(x[1:])) for k in ("ABC" if x[0] == "o" else x[0])
                if (k, int(x[1:])) not in seq]
    for k in "xyzABCsv":
        assert [j for kk, j in seq if kk == k] == list(range(NPAIR)), (k, seq)
    return seq


def _plan(order_e, lag_e, extra_e, tail_e, due_e, order_o, extra_o, tail_o, due_o):
    emit = " ".join(f"s{j}:u{2 * j} s{j}:u{2 * j + 1}" for j in range(NPAIR - 2))
    rest = " ".join(f"u{n}" for n in range(2 * NPAIR - 4, 2 * NPAIR))
    dues = ({}, {})
    for j in range(NPAIR):
        for e in range(2):
            d = 9 * j + due_e + e
            dues[d >= 9 * NPAIR].setdefault((d // 9 % NPAIR, d % 9), []).append(("u", 2 * j + e))
            d = 9 * j + due_o + e
            if d < 9 * NPAIR:
                dues[1].setdefault((d // 9, d % 9), []).append(("U", 2 * j + e))
    for key in dues[1]:
        dues[1][key].sort(key=lambda x: x[0] == "u")
    for x in extra_o.split():
        key, val = x.split(":")
        if val[0] in "ab":
            dues[1].setdefault((int(key[1:]) + 1, 0), []).append((val[0], int(val[1:])))
    return ((_schedule(order_e, (1, 3, lag_e), extra_e + " " + emit, tail_e.replace("#", rest)),
             dues[0]),
            (_schedule(order_o, (1, 3, 5), extra_o + " " + emit, tail_o.replace("#", rest)),
             dues[1]))


PLANS = (
    _plan("xyzBACvs", 4,
          "<s0:q0 <s1:q1 <s2:q2 <s3:Q0 <s4:Q1 <s5:q3 <s6:Q2 <s7:Q3 <s8:q4 <s9:Q4 <s10:q5 <s11:q6"
          " <s12:Q5 <s13:q7",
          "v12 s14 q8 v13 s15 # o11 o12 o13 v14 q9 v15 o14 o15 q10 q11", 25,
          "xAyzBCvs",
          "<s0:q12 <s1:q13 <s2:q14 p4:a0 p5:b0 p7:a1 p8:b1 p9:a2 p10:b2 p12:a3 p13:b3 <s3:Q7",
          "v12 s14 o10 v13 s15 # o11 o12 v14 w0 v15 o13 w1 o14 w2 o15 w3 w4", 25),
    _plan("xyABzCvs", 5, "<s0:q6",
          "v12 s14 q8 v13 s15 # o10 o11 o12 v14 o13 v15 o14 q9 o15 q10 q11", 22,
          "xAyBzCvs",
          "<s0:q12 <s1:q13 <s2:q14 p5:a0 p6:b0 p7:a1 p8:b1 p9:a2 p10:b2 p11:a3 p12:b3",
          "v12 s14 o10 v13 s15 # o11 o12 v14 o13 v15 o14 w0 o15 w1 w2 w3 w4", 24),
)


def _nt(a, b):
    return jax.lax.dot_general(a, b, (((1,), (1,)), ((), ())), preferred_element_type=F32)


def _nn(a, b):
    return jnp.dot(a, b, preferred_element_type=F32)


def _recip(x):
    r = pl.reciprocal(x, approx=True)
    return r * (2.0 - x * r)


def _kernel(ax_h, wqkv_h, woa_h, bx_h, mem0_h, wq_h, wk_h, wv_h, wo_h, out_h,
            ax_v, wqkv_v, woa_v, bx_v, xpre_v, mem0_v, wraw_v, wo_v,
            tmp_v, tmp2_v, wob_v, wqkvp_v, woap_v, slab_v, outa_v,
            wb_v, pre_v, qo_v, kvo_v, o8_v, mid_v, cap_v, outb_v,
            sem_in, sem_out):
    cp_xpre = [pltpu.make_async_copy(bx_h.at[pl.ds(a, n), pl.ds(0, PRE), :],
                                     xpre_v.at[pl.ds(a, n)], sem_in.at[s])
               for a, n, s in ((0, X_FIRST, 0), (X_FIRST, NIT - X_FIRST, 8 + len(U_HEAD) + U_N))]
    cp_wqkv = pltpu.make_async_copy(wqkv_h, wqkv_v, sem_in.at[1])
    cp_woa = pltpu.make_async_copy(woa_h, woa_v, sem_in.at[2])
    cp_mem = pltpu.make_async_copy(mem0_h, mem0_v, sem_in.at[3])
    cp_bx = pltpu.make_async_copy(bx_h, bx_v, sem_in.at[4])
    cp_ax = pltpu.make_async_copy(ax_h, ax_v, sem_in.at[5])
    cp_wo = pltpu.make_async_copy(wo_h, wo_v, sem_in.at[6])
    w_hs = (wq_h, wk_h, wv_h)
    groups = list(U_HEAD) + [U_BODY] * U_N + [U_TAIL]
    g_start = [sum(groups[:g]) for g in range(len(groups))]

    cp_xpre[0].start()
    for g, n in enumerate(groups):
        for u in range(g_start[g], g_start[g] + n):
            pltpu.make_async_copy(w_hs[u % 3].at[pl.ds(u // 3 * PAIR, PAIR)], wraw_v.at[u],
                                  sem_in.at[7 + g]).start()
        if g == 0:
            cp_xpre[1].start()
    cp_wo.start()
    cp_wqkv.start()
    cp_woa.start()
    cp_mem.start()
    cp_bx.start()
    cp_ax.start()

    def g_wait(g, u0, n):
        buf = wraw_v.at[pl.ds(u0, n)]
        pltpu.make_async_copy(buf, buf, sem_in.at[7 + g]).wait()

    n_dots = NIT * PRE // PRE_MB * (PAIR // 128)

    def b_pre(u, after=None, dots=(0, n_dots)):
        if isinstance(u, int):
            rows = [pl.ds(r if u % 3 == 2 else 64 * k, 64) for k, r in enumerate(ILV)]
        else:
            rows = [pl.ds(pl.multiple_of(jnp.where(u % 3 == 2, r, 64 * k), 64), 64)
                    for k, r in enumerate(ILV)]
        blk = jnp.concatenate([wraw_v[u, r, :] for r in rows], axis=0)
        if dots[0] == 0:
            wb_v[u] = pltpu.bitcast(blk.T, U32)
        nb = PRE_MB // PRE
        for k in range(*dots):
            mb, n = divmod(k, PAIR // 128)
            x = xpre_v[mb * nb:(mb + 1) * nb].reshape(PRE_MB, D)
            r = _nt(x, blk[n * 128:(n + 1) * 128])
            pre_v[u, mb * PRE_MB // 2:(mb + 1) * PRE_MB // 2, n * 128:(n + 1) * 128] = (
                pltpu.bitcast(r.astype(BF16), U32))
            if after is not None:
                after(r)

    cp_xpre[0].wait()
    g_wait(0, 0, 1)
    b_pre(0, dots=(0, 4))
    cp_xpre[1].wait()
    b_pre(0, dots=(4, n_dots))
    for g in range(1, len(U_HEAD)):
        g_wait(g, g_start[g], groups[g])
        for u in range(g_start[g], g_start[g] + groups[g]):
            b_pre(u)

    def pre_body(c, carry):
        u0 = sum(U_HEAD) + c * U_BODY
        g_wait(len(U_HEAD) + c, u0, U_BODY)
        for k in range(U_BODY):
            b_pre(u0 + k)
        return carry + c

    off = jax.lax.fori_loop(0, U_N, pre_body, 0) < 0

    g_wait(len(groups) - 1, g_start[-1], U_TAIL)
    cp_wqkv.wait()
    cp_woa.wait()
    cp_wo.wait()
    tail_units = list(range(g_start[-1], NU))

    copies = [(woa_v, r, r, t, tmp2_v.at[t]) for t in range(LT) for r in range(0, D, 16)]
    copies += [(wo_v, j * PAIR + r + rr, j * PAIR + k * 64 + rr, t,
                wob_v.at[:, pl.ds(t * 128, 128)])
               for j in range(NPAIR) for k, r in enumerate(ILV) for t in range(LT)
               for rr in range(0, 64, 16)]

    def copy_some(res):
        for k in range(res.shape[0] // 8):
            tok = pltpu.bitcast(res[8 * k:8 * k + 8], U32)
            for _ in range(3):
                if copies:
                    src, r, rd, t, dst = copies.pop(0)
                    v = pltpu.bitcast(src[r:r + 16, t * 128:(t + 1) * 128], U32)
                    dst[rd // 2:rd // 2 + 8, :] = jnp.where(off, tok, v)

    def tail_pre(k):
        for u in tail_units[k * U_TAIL // 4:(k + 1) * U_TAIL // 4]:
            b_pre(u, copy_some)

    def regroup(src_v, t, base, g):
        parts = []
        for dp in (2 * g, 2 * g + 1):
            v = src_v[t, pl.ds(base + dp, A_H, stride=A_DH // 2), :]
            parts.append(pltpu.bitcast(v << 16, F32))
            parts.append(pltpu.bitcast(v & jnp.uint32(0xFFFF0000), F32))
        return jnp.concatenate(parts, axis=0).astype(BF16)

    def a_prep1(p):
        for b in range(p * LT, (p + 1) * LT):
            blk = pltpu.bitcast(wqkv_v[:, b * 128:(b + 1) * 128].T, U32)
            for t in range(LT):
                tmp_v[t, b * 64:(b + 1) * 64, :] = blk[:, t * 128:(t + 1) * 128]

    def a_prep2(p):
        for g in range(LT):
            blk = jnp.concatenate([regroup(tmp_v, t, p * D // 2, g) for t in range(LT)], axis=1)
            b = p * LT + g
            wqkvp_v[:, b * 128:(b + 1) * 128] = pltpu.bitcast(blk.T, U32)

    def a_prep3():
        for g in range(LT):
            for t in range(LT):
                woap_v[g * 64:(g + 1) * 64, t * 128:(t + 1) * 128] = pltpu.bitcast(
                    regroup(tmp2_v, t, 0, g), U32)

    a_prep1(0)
    a_prep1(1)
    tail_pre(0)
    a_prep1(2)
    a_prep2(0)
    tail_pre(1)
    a_prep2(1)
    tail_pre(2)
    a_prep2(2)
    a_prep3()
    tail_pre(3)
    for t in range(LT, 3 * LT):
        slab_v[0, t, 0:A_PAD, :] = jnp.zeros((A_PAD, 128), F32)
    assert not copies
    cp_mem.wait()
    cp_bx.wait()
    cp_ax.wait()

    a_scale = A_DH ** (-0.5)
    b_scale = B_DH ** (-0.5)
    qrow = jax.lax.broadcasted_iota(jnp.int32, (32, 128), 0)
    lane = jax.lax.broadcasted_iota(jnp.int32, (32, 128), 1)
    first = lane < B_L
    kcol = jnp.where(first, lane, lane - B_L)
    allowed = (qrow >= B_SEG - 8) | (kcol >= B_SEG) | (qrow + 8 >= kcol)
    cap = jnp.where(allowed, jnp.inf, NEG * LOG2E)
    cap_v[0] = jnp.where(first, cap, -jnp.inf)
    cap_v[1] = jnp.where(first | (lane >= 2 * B_L), -jnp.inf, cap)
    cap_v[2] = jnp.where(qrow % 8 >= qrow // 8, jnp.inf, NEG * LOG2E)
    cap_v[3] = jnp.where(qrow % 8 >= qrow // 8 + 4, jnp.inf, NEG * LOG2E)

    def blockdiag_k(t):
        n = t.shape[0]
        left = jax.lax.broadcasted_iota(jnp.int32, (n, 128), 1) < 64
        z = jnp.zeros((n, 128), F32)
        mid = t[:, 128:256]
        top = jnp.concatenate([t[:, 0:128], jnp.where(left, mid, 0.0), z], axis=1)
        bot = jnp.concatenate([z, jnp.where(left, 0.0, mid), t[:, 256:384]], axis=1)
        return jnp.concatenate([top, bot], axis=0).astype(BF16)

    def blockdiag_v(t):
        left = jax.lax.broadcasted_iota(jnp.int32, t.shape, 1) % 128 < 64
        return jnp.concatenate([jnp.where(left, t, 0.0), jnp.where(left, 0.0, t)],
                               axis=0).astype(BF16)

    def softmax(s):
        s = jnp.concatenate([s, jnp.zeros((32, 128 - 2 * B_L), F32)], axis=1) * (b_scale * LOG2E)
        sa, sb = jnp.minimum(s, cap_v[0]), jnp.minimum(s, cap_v[1])
        ma = jnp.max(sa, axis=1, keepdims=True)
        mb = jnp.max(sb, axis=1, keepdims=True)
        p = jnp.exp2(jnp.maximum(sa, sb) - jnp.where(first, ma, mb))
        la = jnp.sum(jnp.where(first, p, 0.0), axis=1, keepdims=True)
        lb = jnp.sum(p, axis=1, keepdims=True) - la
        p = p * pl.reciprocal(jnp.where(first, la, lb), approx=True)
        return p[:, :2 * B_L].astype(BF16)

    def bc(kv_x, kv_m, k, t):
        src = kv_x if k < 8 else kv_m
        return jnp.broadcast_to(src[k % 8:k % 8 + 1, t * 128:(t + 1) * 128], (8, 128))

    def first8_probs(q, kv_x, kv_m):
        left = jax.lax.broadcasted_iota(jnp.int32, (8, 128), 1) < 64
        q = q * (b_scale * LOG2E)
        q0, q2 = q[:, 0:128], q[:, 256:384]
        q1a, q1b = jnp.where(left, q[:, 128:256], 0.0), jnp.where(left, 0.0, q[:, 128:256])
        sc = []
        for k in range(16):
            k1 = bc(kv_x, kv_m, k, 1)
            xa = jnp.sum(q0 * bc(kv_x, kv_m, k, 0) + q1a * k1, axis=1, keepdims=True)
            xb = jnp.sum(q1b * k1 + q2 * bc(kv_x, kv_m, k, 2), axis=1, keepdims=True)
            x = jnp.where(left, xa, xb)
            if 0 < k < 8:
                x = jnp.minimum(x, cap_v[2 + k // 4, 8 * (k % 4):8 * (k % 4) + 8, :])
            sc.append(x)
        m = functools.reduce(jnp.maximum, sc)
        p = [jnp.exp2(x - m) for x in sc]
        return p, _recip(functools.reduce(jnp.add, p))

    def first8_values(p, inv, kv_x, kv_m):
        return [functools.reduce(jnp.add, [p[k] * bc(kv_x, kv_m, k, 3 + t) for k in range(16)])
                * inv for t in range(3)]

    def segment(i, sub, h, even, extra):
        order, dues = PLANS[sub][0 if even else 1]
        qkv, prob, att, q8, o8 = {}, {}, {}, {}, {}
        acc, acc16 = [None], [None]
        hh = [h]
        parts = []
        pins = extra['pins']

        def proj(j, part):
            cuts = sorted({3 * part, 3 * part + 3}
                          | {m for (jj, m) in dues if jj == j and m // 3 == part})
            for m, m2 in zip(cuts[:-1], cuts[1:]):
                due = [x for key in dues.get((j, m), ()) for x in pins.pop(key)]
                if due:
                    hh[0] = extra['pin'](hh[0], due)
                w = wb_v[3 * j + part, :, (m - 3 * part) * 128:(m2 - 3 * part) * 128]
                parts.append(_nn(hh[0], pltpu.bitcast(w, BF16)))
            if part < 2:
                return
            r = jnp.concatenate(parts, axis=1)
            parts.clear()
            if even:
                rows = pl.ds(pl.multiple_of(i * (PRE // 2), PRE // 2), PRE // 2)
                pre = jnp.concatenate([pre_v[3 * j + m, rows, :] for m in range(3)], axis=1)
                pre = pltpu.bitcast(pre, BF16).astype(F32)
                qo_v[j] = r[16:24, :PAIR]
                kvo_v[j] = r[16:24, PAIR:]
                q8[j] = (pre[0:8, :PAIR], pre[0:8, PAIR:], r[24:32, PAIR:])
                q = jnp.concatenate([pre[8:16, :PAIR], r[0:16, :PAIR], r[24:32, :PAIR]], axis=0)
                kv = jnp.concatenate([pre[:, PAIR:], r[0:16, PAIR:], r[24:32, PAIR:]], axis=0)
            else:
                q8[j] = (qo_v[j], kvo_v.at[j], r[24:32, PAIR:])
                q = r[:, :PAIR]
                kv = jnp.concatenate([kvo_v[j], r[:, PAIR:]], axis=0)
            qkv[j] = (q.astype(BF16), blockdiag_k(kv[:, :PAIR]), blockdiag_v(kv[:, PAIR:]))

        def vector(jj):
            j, second = jj // 2, jj % 2
            key = ('u' if even else 'U', jj)
            if not second:
                o8[j] = first8_probs(*q8[j])
                pins[key] = [pltpu.bitcast(o8[j][1], U32)]
                return
            o = first8_values(*o8[j], *q8[j][1:])
            pins[key] = [pltpu.bitcast(x, U32) for x in o]
            o = jnp.concatenate(o, axis=1)
            if even:
                o8_v[j] = o
            else:
                o8[j] = o

        def scores(j):
            prob[j] = softmax(_nt(qkv[j][0], qkv[j][1]))

        def values(j):
            att[j] = _nn(prob[j], qkv[j][2])

        def outp(j, t):
            lhs = att[j][:, t * 128:(t + 1) * 128]
            if even:
                wide = sub > 0 and t == MID
                if wide:
                    lhs = jnp.concatenate([lhs, mid_v[j]], axis=0)
            else:
                wide = sub == UNROLL - 1 or t != MID
                o16 = jnp.concatenate([o8_v[j, :, t * 128:(t + 1) * 128],
                                       o8[j][:, t * 128:(t + 1) * 128]], axis=0)
                if wide:
                    lhs = jnp.concatenate([lhs, o16], axis=0)
                else:
                    mid_v[j] = o16
            r = j * PAIR // 2 + t * 64
            d = _nn(lhs.astype(BF16), pltpu.bitcast(wob_v[r:r + 64, :], BF16))
            acc[0] = d[0:32] if acc[0] is None else acc[0] + d[0:32]
            if wide:
                acc16[0] = d[32:48] if acc16[0] is None else acc16[0] + d[32:48]

        fns = dict(extra, s=scores, v=values, u=vector)
        for t in range(3):
            fns['xyz'[t]] = functools.partial(proj, part=t)
            fns['ABC'[t]] = functools.partial(outp, t=t)
        for k, j in order:
            fns[k](j)
        return acc[0], acc16[0]

    def body(i, sub, mem, held):
        r0 = pl.multiple_of(i * BLK, BLK)

        slab = slab_v.at[sub]

        def a_qkv(b, ahead=0):
            x = ax_v[pl.ds(r0 + ahead * BLK, BLK), :]
            slab_v[sub + ahead, b, A_PAD:A_PAD + BLK, :] = _nn(
                x, pltpu.bitcast(wqkvp_v[:, b * 128:(b + 1) * 128], BF16))

        a_o, a_p = {}, {}
        never = i < 0
        pins = {}

        def a_logits(sb):
            base = A_PAD + sb * A_SUB
            q = [slab[t, base:base + A_SUB, :] for t in range(LT)]
            logits = []
            for w in range(A_W):
                lo = base - A_DIL * w
                acc = None
                for t in range(LT):
                    pr = q[t] * slab[LT + t, lo:lo + A_SUB, :]
                    acc = pr if acc is None else acc + pr
                acc = acc + pltpu.roll(acc, 64, 1)
                acc = acc + pltpu.roll(acc, 32, 1)
                acc = acc * a_scale
                if sb == 0 and w > 0:
                    row = jax.lax.broadcasted_iota(jnp.int32, (A_SUB, 128), 0) + r0
                    acc = jnp.where(row >= A_DIL * w, acc, NEG)
                logits.append(acc)
            m = logits[0]
            for w in range(1, A_W):
                m = jnp.maximum(m, logits[w])
            ps = [jnp.exp(l - m) for l in logits]
            den = ps[0]
            for w in range(1, A_W):
                den = den + ps[w]
            inv = _recip(den)
            a_p[sb] = (ps, inv)
            pins[('a', sb)] = [pltpu.bitcast(inv[8 * u:8 * u + 8], U32) for u in range(A_SUB // 8)]

        def a_values(sb):
            base = A_PAD + sb * A_SUB
            ps, inv = a_p[sb]
            o = []
            for t in range(LT):
                acc = None
                for w in range(A_W):
                    lo = base - A_DIL * w
                    pr = ps[w] * slab[2 * LT + t, lo:lo + A_SUB, :]
                    acc = pr if acc is None else acc + pr
                o.append(acc * inv)
            pins[('b', sb)] = [pltpu.bitcast(x[8 * u:8 * u + 8], U32) for x in o
                               for u in range(A_SUB // 8)]
            a_o[sb] = jnp.concatenate(o, axis=1)
            if sb == BLK // A_SUB - 1:
                for t in range(LT, 3 * LT):
                    slab_v[(sub + 1) % UNROLL, t, 0:A_PAD, :] = slab[t, BLK:BLK + A_PAD, :]

        def pin(h, due):
            u = pltpu.bitcast(h, U32)
            tiles = [u[8 * r:8 * r + 8, 128 * c:128 * c + 128]
                     for c in range(LT) for r in range(u.shape[0] // 8)]
            for k, x in enumerate(due):
                tiles[k % len(tiles)] = jnp.where(never, x, tiles[k % len(tiles)])
            n = u.shape[0] // 8
            cols = [jnp.concatenate(tiles[c * n:(c + 1) * n], axis=0) for c in range(LT)]
            return pltpu.bitcast(jnp.concatenate(cols, axis=1), BF16)

        def a_out(b):
            o = jnp.concatenate([a_o[sb] for sb in range(BLK // A_SUB)], axis=0).astype(BF16)
            res = _nn(o, pltpu.bitcast(woap_v[:, b * 128:(b + 1) * 128], BF16))
            outa_v[pl.ds(r0, BLK), b * 128:(b + 1) * 128] = res.astype(BF16)

        x = bx_v[i].astype(F32)
        extra = dict(q=a_qkv, Q=functools.partial(a_qkv, ahead=1), a=a_logits, b=a_values,
                     w=a_out, pin=pin, pins=pins)

        def emit(r, out_e, acc, acc16):
            out = jnp.concatenate([acc16[0:8], out_e, acc16[8:16], acc[0:24]], axis=0)
            outb_v[pl.ds(r, BLK), :] = out.astype(BF16)
            pltpu.make_async_copy(
                outb_v.at[pl.ds(r, BLK)], out_h.at[pl.ds(r, BLK), pl.ds(D, D)],
                sem_out.at[1]).start()

        acc, acc16 = segment(
            i, sub, jnp.concatenate([x[16:40], mem], axis=0).astype(BF16), True, extra)
        if held is not None:
            emit(held[0], held[1], held[2], held[3] + acc16)
        out_e = acc[0:24]
        mem = acc[24:32].astype(BF16).astype(F32)
        acc, acc16 = segment(
            i, sub, jnp.concatenate([x[40:64], mem], axis=0).astype(BF16), False, extra)
        held = (r0, out_e, acc, acc16)
        if sub == UNROLL - 1:
            emit(*held)
            held = None
        pltpu.make_async_copy(
            outa_v.at[pl.ds(r0, BLK)], out_h.at[pl.ds(r0, BLK), pl.ds(0, D)], sem_out.at[0]).start()
        return acc[24:32].astype(BF16).astype(F32), held

    def body_n(ii, mem):
        held = None
        for u in range(UNROLL):
            mem, held = body(ii * UNROLL + u, u, mem, held)
        return mem

    jax.lax.fori_loop(0, NIT // UNROLL, body_n, mem0_v[...].astype(F32))

    pltpu.make_async_copy(outa_v, out_h.at[:, pl.ds(0, D)], sem_out.at[0]).wait()
    pltpu.make_async_copy(outb_v, out_h.at[:, pl.ds(D, D)], sem_out.at[1]).wait()


@jax.jit
def _run(A_x, A_wqkv, A_wo, B_x, B_mem0, B_Wq, B_Wk, B_Wv, B_Wo):
    def feat_major(w):
        return jnp.transpose(w, (1, 2, 0)).reshape(B_F, D)

    any_spec = pl.BlockSpec(memory_space=pl.ANY)
    out = pl.pallas_call(
        _kernel,
        out_shape=jax.ShapeDtypeStruct((S, 2 * D), BF16),
        in_specs=[any_spec] * 9,
        out_specs=any_spec,
        scratch_shapes=[
            pltpu.VMEM((S, D), BF16),
            pltpu.VMEM((D, 3 * D), BF16),
            pltpu.VMEM((D, D), BF16),
            pltpu.VMEM((NIT, BLK, D), BF16),
            pltpu.VMEM((NIT, PRE, D), BF16),
            pltpu.VMEM((B_M, D), BF16),
            pltpu.VMEM((NU, PAIR, D), BF16),
            pltpu.VMEM((B_F, D), BF16),
            pltpu.VMEM((LT, 3 * D // 2, 128), U32),
            pltpu.VMEM((LT, D // 2, 128), U32),
            pltpu.VMEM((B_F // 2, D), U32),
            pltpu.VMEM((D // 2, 3 * D), U32),
            pltpu.VMEM((D // 2, D), U32),
            pltpu.VMEM((UNROLL, 3 * LT, A_PAD + BLK, 128), F32),
            pltpu.VMEM((S, D), BF16),
            pltpu.VMEM((NU, D // 2, PAIR), U32),
            pltpu.VMEM((NU, NIT * PRE // 2, PAIR), U32),
            pltpu.VMEM((NPAIR, 8, PAIR), F32),
            pltpu.VMEM((NPAIR, 8, 2 * PAIR), F32),
            pltpu.VMEM((NPAIR, 8, PAIR), F32),
            pltpu.VMEM((NPAIR, 16, 128), F32),
            pltpu.VMEM((4, 32, 128), F32),
            pltpu.VMEM((S, D), BF16),
            pltpu.SemaphoreType.DMA((9 + len(U_HEAD) + U_N,)),
            pltpu.SemaphoreType.DMA((2,)),
        ],
        compiler_params=pltpu.CompilerParams(vmem_limit_bytes=120 * 1024 * 1024,
                                             disable_bounds_checks=True),
    )(
        A_x.reshape(S, D), A_wqkv, A_wo, B_x.reshape(NIT, BLK, D), B_mem0.reshape(B_M, D),
        feat_major(B_Wq), feat_major(B_Wk), feat_major(B_Wv), B_Wo.reshape(B_F, D),
    )
    return out.reshape(1, S, 2 * D)


def pallas_concat_heads__sliding_local_dilated__memory_aug_recurrent_mem_tr__prompt_kernel(
    A_x: jax.Array,
    A_wqkv: jax.Array,
    A_wo: jax.Array,
    B_x: jax.Array,
    B_mem0: jax.Array,
    B_Wq: jax.Array,
    B_Wk: jax.Array,
    B_Wv: jax.Array,
    B_Wo: jax.Array,
    B_seg_len,
):
    assert A_x.shape == (1, S, D) and B_x.shape == (1, S, D) and B_mem0.shape == (1, B_M, D)
    assert B_Wq.shape == (D, B_H, B_DH) and B_Wo.shape == (B_H, B_DH, D)
    if isinstance(B_seg_len, int):
        assert B_seg_len == B_SEG
    return _run(A_x, A_wqkv, A_wo, B_x, B_mem0, B_Wq, B_Wk, B_Wv, B_Wo)
```

```python
import functools

import jax
import jax.numpy as jnp
import jax.experimental.pallas as pl
import jax.experimental.pallas.tpu as pltpu

F32 = jnp.float32
BF16 = jnp.bfloat16
U32 = jnp.uint32

S = 2048
D = 640
LT = D // 128
BLK = 64
NIT = S // BLK

A_H = 32
A_DH = 20
A_W = 8
A_DIL = 2
A_PAD = 16
A_SUB = 16

B_H = 32
B_DH = 192
B_F = B_H * B_DH
B_M = 8
B_SEG = 32
B_L = B_M + B_SEG
PAIR = 2 * B_DH
NPAIR = B_H // 2
NU = 3 * NPAIR
PRE = 16
PRE_MB = 128

NEG = -1000000000.0
LOG2E = 1.4426950408889634
ILV = [h * B_DH + t * 64 for t in range(3) for h in range(2)]
UNROLL = 2
U_HEAD = (1, 1, 2)
U_BODY = 5
U_N = 8
U_TAIL = NU - sum(U_HEAD) - U_BODY * U_N
X_FIRST = 16
MID = 1


def _schedule(order, lags, extra, tail):
    lag = dict(p=0, s=lags[0], v=lags[1], o=lags[2])
    kind = dict(x="p", y="p", z="p", A="o", B="o", C="o", s="s", v="v")
    hooks = {}
    for x in extra.split():
        key, val = x.split(":")
        hooks.setdefault(key, []).append((val[0], int(val[1:])))
    seq = []
    for t in range(NPAIR):
        for k in order:
            j = t - lag[kind[k]]
            if j >= 0:
                if k in "xAsv":
                    seq += hooks.get("<" + kind[k] + str(j), [])
                seq.append((k, j))
                if k in "zCsv":
                    seq += hooks.get(kind[k] + str(j), [])
            if t == NPAIR - 1 and k == "z":
                break
    for x in tail.split():
        seq += [(k, int(x[1:])) for k in ("ABC" if x[0] == "o" else x[0])
                if (k, int(x[1:])) not in seq]
    for k in "xyzABCsv":
        assert [j for kk, j in seq if kk == k] == list(range(NPAIR)), (k, seq)
    return seq


def _plan(order_e, lag_e, extra_e, tail_e, due_e, order_o, extra_o, tail_o, due_o):
    emit = " ".join(f"s{j}:u{2 * j} s{j}:u{2 * j + 1}" for j in range(NPAIR - 2))
    rest = " ".join(f"u{n}" for n in range(2 * NPAIR - 4, 2 * NPAIR))
    dues = ({}, {})
    for j in range(NPAIR):
        for e in range(2):
            d = 9 * j + due_e + e
            dues[d >= 9 * NPAIR].setdefault((d // 9 % NPAIR, d % 9), []).append(("u", 2 * j + e))
            d = 9 * j + due_o + e
            if d < 9 * NPAIR:
                dues[1].setdefault((d // 9, d % 9), []).append(("U", 2 * j + e))
    for key in dues[1]:
        dues[1][key].sort(key=lambda x: x[0] == "u")
    for x in extra_o.split():
        key, val = x.split(":")
        if val[0] in "ab":
            dues[1].setdefault((int(key[1:]) + 1, 0), []).append((val[0], int(val[1:])))
    return ((_schedule(order_e, (1, 3, lag_e), extra_e + " " + emit, tail_e.replace("#", rest)),
             dues[0]),
            (_schedule(order_o, (1, 3, 5), extra_o + " " + emit, tail_o.replace("#", rest)),
             dues[1]))


PLANS = (
    _plan("xyzBACvs", 4,
          "<s0:q0 <s1:q1 <s2:q2 <s3:Q0 <s4:Q1 <s5:q3 <s6:Q2 <s7:Q3 <s8:q4 <s9:Q4 <s10:q5 <s11:q6"
          " <s12:Q5 <s13:q7",
          "v12 s14 q8 v13 s15 # o11 o12 o13 v14 q9 v15 o14 o15 q10 q11", 25,
          "xAyzBCvs",
          "<s0:q12 <s1:q13 <s2:q14 p4:a0 p5:b0 p7:a1 p8:b1 p9:a2 p10:b2 p12:a3 p13:b3 <s3:Q7",
          "v12 s14 o10 v13 s15 # o11 o12 v14 w0 v15 o13 w1 o14 w2 o15 w3 w4", 25),
    _plan("xyABzCvs", 5, "<s0:q6",
          "v12 s14 q8 v13 s15 # o10 o11 o12 v14 o13 v15 o14 q9 o15 q10 q11", 22,
          "xAyBzCvs",
          "<s0:q12 <s1:q13 <s2:q14 p5:a0 p6:b0 p7:a1 p8:b1 p9:a2 p10:b2 p11:a3 p12:b3",
          "v12 s14 o10 v13 s15 # o11 o12 v14 o13 v15 o14 w0 o15 w1 w2 w3 w4", 24),
)


def _nt(a, b):
    return jax.lax.dot_general(a, b, (((1,), (1,)), ((), ())), preferred_element_type=F32)


def _nn(a, b):
    return jnp.dot(a, b, preferred_element_type=F32)


def _recip(x):
    r = pl.reciprocal(x, approx=True)
    return r * (2.0 - x * r)


def _kernel(ax_h, wqkv_h, woa_h, bx_h, mem0_h, wq_h, wk_h, wv_h, wo_h, out_h,
            ax_v, wqkv_v, woa_v, bx_v, xpre_v, mem0_v, wraw_v, wo_v,
            tmp_v, tmp2_v, wob_v, wqkvp_v, woap_v, slab_v, outa_v,
            wb_v, pre_v, qo_v, kvo_v, o8_v, mid_v, cap_v, outb_v,
            sem_in, sem_out):
    cp_xpre = [pltpu.make_async_copy(bx_h.at[pl.ds(a, n), pl.ds(0, PRE), :],
                                     xpre_v.at[pl.ds(a, n)], sem_in.at[s])
               for a, n, s in ((0, X_FIRST, 0), (X_FIRST, NIT - X_FIRST, 8 + len(U_HEAD) + U_N))]
    cp_wqkv = pltpu.make_async_copy(wqkv_h, wqkv_v, sem_in.at[1])
    cp_woa = pltpu.make_async_copy(woa_h, woa_v, sem_in.at[2])
    cp_mem = pltpu.make_async_copy(mem0_h, mem0_v, sem_in.at[3])
    cp_bx = pltpu.make_async_copy(bx_h, bx_v, sem_in.at[4])
    cp_ax = pltpu.make_async_copy(ax_h, ax_v, sem_in.at[5])
    cp_wo = pltpu.make_async_copy(wo_h, wo_v, sem_in.at[6])
    w_hs = (wq_h, wk_h, wv_h)
    groups = list(U_HEAD) + [U_BODY] * U_N + [U_TAIL]
    g_start = [sum(groups[:g]) for g in range(len(groups))]

    n_head = sum(U_HEAD)

    def unit(c, k):
        if c is not None and k < 2:
            return 3 * (2 * c + k) + 2, True
        if c is not None:
            e = n_head + (U_BODY - 2) * c + k - 2
        else:
            e = k if k < n_head else k - 2 * U_N
        return 3 * (e // 2) + e % 2, False

    def unit_at(p):
        in_loop = n_head <= p < g_start[-1]
        return unit(*divmod(p - n_head, U_BODY)) if in_loop else unit(None, p)

    assert sorted(unit_at(p)[0] for p in range(NU)) == list(range(NU))
    cp_xpre[0].start()
    for g, n in enumerate(groups):
        for p in range(g_start[g], g_start[g] + n):
            u = unit_at(p)[0]
            pltpu.make_async_copy(w_hs[u % 3].at[pl.ds(u // 3 * PAIR, PAIR)], wraw_v.at[p],
                                  sem_in.at[7 + g]).start()
        if g == 0:
            cp_xpre[1].start()
    cp_wo.start()
    cp_wqkv.start()
    cp_woa.start()
    cp_mem.start()
    cp_bx.start()
    cp_ax.start()

    def g_wait(g, p0, n):
        buf = wraw_v.at[pl.ds(p0, n)]
        pltpu.make_async_copy(buf, buf, sem_in.at[7 + g]).wait()

    n_dots = NIT * PRE // PRE_MB * (PAIR // 128)

    def b_pre(p, u, value, after=None, dots=(0, n_dots)):
        if value:
            blk = jnp.concatenate([wraw_v[p, r:r + 64, :] for r in ILV], axis=0)
        else:
            blk = wraw_v[p]
        if dots[0] == 0:
            wb_v[u] = pltpu.bitcast(blk.T, U32)
        nb = PRE_MB // PRE
        for k in range(*dots):
            mb, n = divmod(k, PAIR // 128)
            x = xpre_v[mb * nb:(mb + 1) * nb].reshape(PRE_MB, D)
            r = _nt(x, blk[n * 128:(n + 1) * 128])
            pre_v[u, mb * PRE_MB // 2:(mb + 1) * PRE_MB // 2, n * 128:(n + 1) * 128] = (
                pltpu.bitcast(r.astype(BF16), U32))
            if after is not None:
                after(r)

    cp_xpre[0].wait()
    g_wait(0, 0, 1)
    b_pre(0, *unit_at(0), dots=(0, 4))
    cp_xpre[1].wait()
    b_pre(0, *unit_at(0), dots=(4, n_dots))
    for g in range(1, len(U_HEAD)):
        g_wait(g, g_start[g], groups[g])
        for p in range(g_start[g], g_start[g] + groups[g]):
            b_pre(p, *unit_at(p))

    def pre_body(c, carry):
        p0 = n_head + c * U_BODY
        g_wait(len(U_HEAD) + c, p0, U_BODY)
        for k in range(U_BODY):
            b_pre(p0 + k, *unit(c, k))
        return carry + c

    off = jax.lax.fori_loop(0, U_N, pre_body, 0) < 0

    g_wait(len(groups) - 1, g_start[-1], U_TAIL)
    cp_wqkv.wait()
    cp_woa.wait()
    cp_wo.wait()
    tail_units = list(range(g_start[-1], NU))

    copies = [(woa_v, r, r, t, tmp2_v.at[t]) for t in range(LT) for r in range(0, D, 16)]
    copies += [(wo_v, j * PAIR + r + rr, j * PAIR + k * 64 + rr, t,
                wob_v.at[:, pl.ds(t * 128, 128)])
               for j in range(NPAIR) for k, r in enumerate(ILV) for t in range(LT)
               for rr in range(0, 64, 16)]

    def copy_some(res):
        for k in range(res.shape[0] // 8):
            tok = pltpu.bitcast(res[8 * k:8 * k + 8], U32)
            for _ in range(3):
                if copies:
                    src, r, rd, t, dst = copies.pop(0)
                    v = pltpu.bitcast(src[r:r + 16, t * 128:(t + 1) * 128], U32)
                    dst[rd // 2:rd // 2 + 8, :] = jnp.where(off, tok, v)

    def tail_pre(k):
        for p in tail_units[k * U_TAIL // 4:(k + 1) * U_TAIL // 4]:
            b_pre(p, *unit_at(p), copy_some)

    def regroup(src_v, t, base, g):
        parts = []
        for dp in (2 * g, 2 * g + 1):
            v = src_v[t, pl.ds(base + dp, A_H, stride=A_DH // 2), :]
            parts.append(pltpu.bitcast(v << 16, F32))
            parts.append(pltpu.bitcast(v & jnp.uint32(0xFFFF0000), F32))
        return jnp.concatenate(parts, axis=0).astype(BF16)

    def a_prep1(p):
        for b in range(p * LT, (p + 1) * LT):
            blk = pltpu.bitcast(wqkv_v[:, b * 128:(b + 1) * 128].T, U32)
            for t in range(LT):
                tmp_v[t, b * 64:(b + 1) * 64, :] = blk[:, t * 128:(t + 1) * 128]

    def a_prep2(p):
        for g in range(LT):
            blk = jnp.concatenate([regroup(tmp_v, t, p * D // 2, g) for t in range(LT)], axis=1)
            b = p * LT + g
            wqkvp_v[:, b * 128:(b + 1) * 128] = pltpu.bitcast(blk.T, U32)

    def a_prep3():
        for g in range(LT):
            for t in range(LT):
                woap_v[g * 64:(g + 1) * 64, t * 128:(t + 1) * 128] = pltpu.bitcast(
                    regroup(tmp2_v, t, 0, g), U32)

    a_prep1(0)
    a_prep1(1)
    tail_pre(0)
    a_prep1(2)
    a_prep2(0)
    tail_pre(1)
    a_prep2(1)
    tail_pre(2)
    a_prep2(2)
    a_prep3()
    tail_pre(3)
    for t in range(LT, 3 * LT):
        slab_v[0, t, 0:A_PAD, :] = jnp.zeros((A_PAD, 128), F32)
    assert not copies
    cp_mem.wait()
    cp_bx.wait()
    cp_ax.wait()

    a_scale = A_DH ** (-0.5)
    b_scale = B_DH ** (-0.5)
    qrow = jax.lax.broadcasted_iota(jnp.int32, (32, 128), 0)
    lane = jax.lax.broadcasted_iota(jnp.int32, (32, 128), 1)
    first = lane < B_L
    kcol = jnp.where(first, lane, lane - B_L)
    allowed = (qrow >= B_SEG - 8) | (kcol >= B_SEG) | (qrow + 8 >= kcol)
    cap = jnp.where(allowed, jnp.inf, NEG * LOG2E)
    cap_v[0] = jnp.where(first, cap, -jnp.inf)
    cap_v[1] = jnp.where(first | (lane >= 2 * B_L), -jnp.inf, cap)
    cap_v[2] = jnp.where(qrow % 8 >= qrow // 8, jnp.inf, NEG * LOG2E)
    cap_v[3] = jnp.where(qrow % 8 >= qrow // 8 + 4, jnp.inf, NEG * LOG2E)

    def blockdiag_k(t):
        n = t.shape[0]
        left = jax.lax.broadcasted_iota(jnp.int32, (n, 128), 1) < 64
        z = jnp.zeros((n, 128), F32)
        mid = t[:, 128:256]
        top = jnp.concatenate([t[:, 0:128], jnp.where(left, mid, 0.0), z], axis=1)
        bot = jnp.concatenate([z, jnp.where(left, 0.0, mid), t[:, 256:384]], axis=1)
        return jnp.concatenate([top, bot], axis=0).astype(BF16)

    def blockdiag_v(t):
        left = jax.lax.broadcasted_iota(jnp.int32, t.shape, 1) % 128 < 64
        return jnp.concatenate([jnp.where(left, t, 0.0), jnp.where(left, 0.0, t)],
                               axis=0).astype(BF16)

    def softmax(s):
        s = jnp.concatenate([s, jnp.zeros((32, 128 - 2 * B_L), F32)], axis=1) * (b_scale * LOG2E)
        sa, sb = jnp.minimum(s, cap_v[0]), jnp.minimum(s, cap_v[1])
        ma = jnp.max(sa, axis=1, keepdims=True)
        mb = jnp.max(sb, axis=1, keepdims=True)
        p = jnp.exp2(jnp.maximum(sa, sb) - jnp.where(first, ma, mb))
        la = jnp.sum(jnp.where(first, p, 0.0), axis=1, keepdims=True)
        lb = jnp.sum(p, axis=1, keepdims=True) - la
        p = p * pl.reciprocal(jnp.where(first, la, lb), approx=True)
        return p[:, :2 * B_L].astype(BF16)

    def bc(kv_x, kv_m, k, t):
        src = kv_x if k < 8 else kv_m
        return jnp.broadcast_to(src[k % 8:k % 8 + 1, t * 128:(t + 1) * 128], (8, 128))

    def first8_probs(q, kv_x, kv_m):
        left = jax.lax.broadcasted_iota(jnp.int32, (8, 128), 1) < 64
        q = q * (b_scale * LOG2E)
        q0, q2 = q[:, 0:128], q[:, 256:384]
        q1a, q1b = jnp.where(left, q[:, 128:256], 0.0), jnp.where(left, 0.0, q[:, 128:256])
        sc = []
        for k in range(16):
            k1 = bc(kv_x, kv_m, k, 1)
            xa = jnp.sum(q0 * bc(kv_x, kv_m, k, 0) + q1a * k1, axis=1, keepdims=True)
            xb = jnp.sum(q1b * k1 + q2 * bc(kv_x, kv_m, k, 2), axis=1, keepdims=True)
            x = jnp.where(left, xa, xb)
            if 0 < k < 8:
                x = jnp.minimum(x, cap_v[2 + k // 4, 8 * (k % 4):8 * (k % 4) + 8, :])
            sc.append(x)
        m = functools.reduce(jnp.maximum, sc)
        p = [jnp.exp2(x - m) for x in sc]
        return p, _recip(functools.reduce(jnp.add, p))

    def first8_values(p, inv, kv_x, kv_m):
        return [functools.reduce(jnp.add, [p[k] * bc(kv_x, kv_m, k, 3 + t) for k in range(16)])
                * inv for t in range(3)]

    def segment(i, sub, h, even, extra):
        order, dues = PLANS[sub][0 if even else 1]
        qkv, prob, att, q8, o8 = {}, {}, {}, {}, {}
        acc, acc16 = [None], [None]
        hh = [h]
        parts = []
        pins = extra['pins']

        def proj(j, part):
            cuts = sorted({3 * part, 3 * part + 3}
                          | {m for (jj, m) in dues if jj == j and m // 3 == part})
            for m, m2 in zip(cuts[:-1], cuts[1:]):
                due = [x for key in dues.get((j, m), ()) for x in pins.pop(key)]
                if due:
                    hh[0] = extra['pin'](hh[0], due)
                w = wb_v[3 * j + part, :, (m - 3 * part) * 128:(m2 - 3 * part) * 128]
                parts.append(_nn(hh[0], pltpu.bitcast(w, BF16)))
            if part < 2:
                return
            r = jnp.concatenate(parts, axis=1)
            parts.clear()
            if even:
                rows = pl.ds(pl.multiple_of(i * (PRE // 2), PRE // 2), PRE // 2)
                pre = jnp.concatenate([pre_v[3 * j + m, rows, :] for m in range(3)], axis=1)
                pre = pltpu.bitcast(pre, BF16).astype(F32)
                qo_v[j] = r[16:24, :PAIR]
                kvo_v[j] = r[16:24, PAIR:]
                q8[j] = (pre[0:8, :PAIR], pre[0:8, PAIR:], r[24:32, PAIR:])
                q = jnp.concatenate([pre[8:16, :PAIR], r[0:16, :PAIR], r[24:32, :PAIR]], axis=0)
                kv = jnp.concatenate([pre[:, PAIR:], r[0:16, PAIR:], r[24:32, PAIR:]], axis=0)
            else:
                q8[j] = (qo_v[j], kvo_v.at[j], r[24:32, PAIR:])
                q = r[:, :PAIR]
                kv = jnp.concatenate([kvo_v[j], r[:, PAIR:]], axis=0)
            qkv[j] = (q.astype(BF16), blockdiag_k(kv[:, :PAIR]), blockdiag_v(kv[:, PAIR:]))

        def vector(jj):
            j, second = jj // 2, jj % 2
            key = ('u' if even else 'U', jj)
            if not second:
                o8[j] = first8_probs(*q8[j])
                pins[key] = [pltpu.bitcast(o8[j][1], U32)]
                return
            o = first8_values(*o8[j], *q8[j][1:])
            pins[key] = [pltpu.bitcast(x, U32) for x in o]
            o = jnp.concatenate(o, axis=1)
            if even:
                o8_v[j] = o
            else:
                o8[j] = o

        def scores(j):
            prob[j] = softmax(_nt(qkv[j][0], qkv[j][1]))

        def values(j):
            att[j] = _nn(prob[j], qkv[j][2])

        def outp(j, t):
            lhs = att[j][:, t * 128:(t + 1) * 128]
            if even:
                wide = sub > 0 and t == MID
                if wide:
                    lhs = jnp.concatenate([lhs, mid_v[j]], axis=0)
            else:
                wide = sub == UNROLL - 1 or t != MID
                o16 = jnp.concatenate([o8_v[j, :, t * 128:(t + 1) * 128],
                                       o8[j][:, t * 128:(t + 1) * 128]], axis=0)
                if wide:
                    lhs = jnp.concatenate([lhs, o16], axis=0)
                else:
                    mid_v[j] = o16
            r = j * PAIR // 2 + t * 64
            d = _nn(lhs.astype(BF16), pltpu.bitcast(wob_v[r:r + 64, :], BF16))
            acc[0] = d[0:32] if acc[0] is None else acc[0] + d[0:32]
            if wide:
                acc16[0] = d[32:48] if acc16[0] is None else acc16[0] + d[32:48]

        fns = dict(extra, s=scores, v=values, u=vector)
        for t in range(3):
            fns['xyz'[t]] = functools.partial(proj, part=t)
            fns['ABC'[t]] = functools.partial(outp, t=t)
        for k, j in order:
            fns[k](j)
        return acc[0], acc16[0]

    def body(i, sub, mem, held):
        r0 = pl.multiple_of(i * BLK, BLK)

        slab = slab_v.at[sub]

        def a_qkv(b, ahead=0):
            x = ax_v[pl.ds(r0 + ahead * BLK, BLK), :]
            slab_v[sub + ahead, b, A_PAD:A_PAD + BLK, :] = _nn(
                x, pltpu.bitcast(wqkvp_v[:, b * 128:(b + 1) * 128], BF16))

        a_o, a_p = {}, {}
        never = i < 0
        pins = {}

        def a_logits(sb):
            base = A_PAD + sb * A_SUB
            q = [slab[t, base:base + A_SUB, :] for t in range(LT)]
            logits = []
            for w in range(A_W):
                lo = base - A_DIL * w
                acc = None
                for t in range(LT):
                    pr = q[t] * slab[LT + t, lo:lo + A_SUB, :]
                    acc = pr if acc is None else acc + pr
                acc = acc + pltpu.roll(acc, 64, 1)
                acc = acc + pltpu.roll(acc, 32, 1)
                acc = acc * a_scale
                if sb == 0 and w > 0:
                    row = jax.lax.broadcasted_iota(jnp.int32, (A_SUB, 128), 0) + r0
                    acc = jnp.where(row >= A_DIL * w, acc, NEG)
                logits.append(acc)
            m = logits[0]
            for w in range(1, A_W):
                m = jnp.maximum(m, logits[w])
            ps = [jnp.exp(l - m) for l in logits]
            den = ps[0]
            for w in range(1, A_W):
                den = den + ps[w]
            inv = _recip(den)
            a_p[sb] = (ps, inv)
            pins[('a', sb)] = [pltpu.bitcast(inv[8 * u:8 * u + 8], U32) for u in range(A_SUB // 8)]

        def a_values(sb):
            base = A_PAD + sb * A_SUB
            ps, inv = a_p[sb]
            o = []
            for t in range(LT):
                acc = None
                for w in range(A_W):
                    lo = base - A_DIL * w
                    pr = ps[w] * slab[2 * LT + t, lo:lo + A_SUB, :]
                    acc = pr if acc is None else acc + pr
                o.append(acc * inv)
            pins[('b', sb)] = [pltpu.bitcast(x[8 * u:8 * u + 8], U32) for x in o
                               for u in range(A_SUB // 8)]
            a_o[sb] = jnp.concatenate(o, axis=1)
            if sb == BLK // A_SUB - 1:
                for t in range(LT, 3 * LT):
                    slab_v[(sub + 1) % UNROLL, t, 0:A_PAD, :] = slab[t, BLK:BLK + A_PAD, :]

        def pin(h, due):
            u = pltpu.bitcast(h, U32)
            tiles = [u[8 * r:8 * r + 8, 128 * c:128 * c + 128]
                     for c in range(LT) for r in range(u.shape[0] // 8)]
            for k, x in enumerate(due):
                tiles[k % len(tiles)] = jnp.where(never, x, tiles[k % len(tiles)])
            n = u.shape[0] // 8
            cols = [jnp.concatenate(tiles[c * n:(c + 1) * n], axis=0) for c in range(LT)]
            return pltpu.bitcast(jnp.concatenate(cols, axis=1), BF16)

        def a_out(b):
            o = jnp.concatenate([a_o[sb] for sb in range(BLK // A_SUB)], axis=0).astype(BF16)
            res = _nn(o, pltpu.bitcast(woap_v[:, b * 128:(b + 1) * 128], BF16))
            outa_v[pl.ds(r0, BLK), b * 128:(b + 1) * 128] = res.astype(BF16)

        x = bx_v[i].astype(F32)
        extra = dict(q=a_qkv, Q=functools.partial(a_qkv, ahead=1), a=a_logits, b=a_values,
                     w=a_out, pin=pin, pins=pins)

        def emit(r, out_e, acc, acc16):
            out = jnp.concatenate([acc16[0:8], out_e, acc16[8:16], acc[0:24]], axis=0)
            outb_v[pl.ds(r, BLK), :] = out.astype(BF16)
            pltpu.make_async_copy(
                outb_v.at[pl.ds(r, BLK)], out_h.at[pl.ds(r, BLK), pl.ds(D, D)],
                sem_out.at[1]).start()

        acc, acc16 = segment(
            i, sub, jnp.concatenate([x[16:40], mem], axis=0).astype(BF16), True, extra)
        if held is not None:
            emit(held[0], held[1], held[2], held[3] + acc16)
        out_e = acc[0:24]
        mem = acc[24:32].astype(BF16).astype(F32)
        acc, acc16 = segment(
            i, sub, jnp.concatenate([x[40:64], mem], axis=0).astype(BF16), False, extra)
        held = (r0, out_e, acc, acc16)
        if sub == UNROLL - 1:
            emit(*held)
            held = None
        pltpu.make_async_copy(
            outa_v.at[pl.ds(r0, BLK)], out_h.at[pl.ds(r0, BLK), pl.ds(0, D)], sem_out.at[0]).start()
        return acc[24:32].astype(BF16).astype(F32), held

    def body_n(ii, mem):
        held = None
        for u in range(UNROLL):
            mem, held = body(ii * UNROLL + u, u, mem, held)
        return mem

    jax.lax.fori_loop(0, NIT // UNROLL, body_n, mem0_v[...].astype(F32))

    pltpu.make_async_copy(outa_v, out_h.at[:, pl.ds(0, D)], sem_out.at[0]).wait()
    pltpu.make_async_copy(outb_v, out_h.at[:, pl.ds(D, D)], sem_out.at[1]).wait()


@jax.jit
def _run(A_x, A_wqkv, A_wo, B_x, B_mem0, B_Wq, B_Wk, B_Wv, B_Wo):
    def feat_major(w):
        return jnp.transpose(w, (1, 2, 0)).reshape(B_F, D)

    any_spec = pl.BlockSpec(memory_space=pl.ANY)
    out = pl.pallas_call(
        _kernel,
        out_shape=jax.ShapeDtypeStruct((S, 2 * D), BF16),
        in_specs=[any_spec] * 9,
        out_specs=any_spec,
        scratch_shapes=[
            pltpu.VMEM((S, D), BF16),
            pltpu.VMEM((D, 3 * D), BF16),
            pltpu.VMEM((D, D), BF16),
            pltpu.VMEM((NIT, BLK, D), BF16),
            pltpu.VMEM((NIT, PRE, D), BF16),
            pltpu.VMEM((B_M, D), BF16),
            pltpu.VMEM((NU, PAIR, D), BF16),
            pltpu.VMEM((B_F, D), BF16),
            pltpu.VMEM((LT, 3 * D // 2, 128), U32),
            pltpu.VMEM((LT, D // 2, 128), U32),
            pltpu.VMEM((B_F // 2, D), U32),
            pltpu.VMEM((D // 2, 3 * D), U32),
            pltpu.VMEM((D // 2, D), U32),
            pltpu.VMEM((UNROLL, 3 * LT, A_PAD + BLK, 128), F32),
            pltpu.VMEM((S, D), BF16),
            pltpu.VMEM((NU, D // 2, PAIR), U32),
            pltpu.VMEM((NU, NIT * PRE // 2, PAIR), U32),
            pltpu.VMEM((NPAIR, 8, PAIR), F32),
            pltpu.VMEM((NPAIR, 8, 2 * PAIR), F32),
            pltpu.VMEM((NPAIR, 8, PAIR), F32),
            pltpu.VMEM((NPAIR, 16, 128), F32),
            pltpu.VMEM((4, 32, 128), F32),
            pltpu.VMEM((S, D), BF16),
            pltpu.SemaphoreType.DMA((9 + len(U_HEAD) + U_N,)),
            pltpu.SemaphoreType.DMA((2,)),
        ],
        compiler_params=pltpu.CompilerParams(vmem_limit_bytes=120 * 1024 * 1024,
                                             disable_bounds_checks=True),
    )(
        A_x.reshape(S, D), A_wqkv, A_wo, B_x.reshape(NIT, BLK, D), B_mem0.reshape(B_M, D),
        feat_major(B_Wq), feat_major(B_Wk), feat_major(B_Wv), B_Wo.reshape(B_F, D),
    )
    return out.reshape(1, S, 2 * D)


def pallas_concat_heads__sliding_local_dilated__memory_aug_recurrent_mem_tr__prompt_kernel(
    A_x: jax.Array,
    A_wqkv: jax.Array,
    A_wo: jax.Array,
    B_x: jax.Array,
    B_mem0: jax.Array,
    B_Wq: jax.Array,
    B_Wk: jax.Array,
    B_Wv: jax.Array,
    B_Wo: jax.Array,
    B_seg_len,
):
    assert A_x.shape == (1, S, D) and B_x.shape == (1, S, D) and B_mem0.shape == (1, B_M, D)
    assert B_Wq.shape == (D, B_H, B_DH) and B_Wo.shape == (B_H, B_DH, D)
    if isinstance(B_seg_len, int):
        assert B_seg_len == B_SEG
    return _run(A_x, A_wqkv, A_wo, B_x, B_mem0, B_Wq, B_Wk, B_Wv, B_Wo)
```

```python
import functools

import jax
import jax.numpy as jnp
import jax.experimental.pallas as pl
import jax.experimental.pallas.tpu as pltpu

F32 = jnp.float32
BF16 = jnp.bfloat16
U32 = jnp.uint32

S = 2048
D = 640
LT = D // 128
BLK = 64
NIT = S // BLK

A_H = 32
A_DH = 20
A_W = 8
A_DIL = 2
A_PAD = 16
A_SUB = 16

B_H = 32
B_DH = 192
B_F = B_H * B_DH
B_M = 8
B_SEG = 32
B_L = B_M + B_SEG
PAIR = 2 * B_DH
NPAIR = B_H // 2
NU = 3 * NPAIR
PRE = 16
PRE_MB = 128

NEG = -1000000000.0
LOG2E = 1.4426950408889634
ILV = [h * B_DH + t * 64 for t in range(3) for h in range(2)]
UNROLL = 2
U_HEAD = (1, 1, 2)
U_BODY = 5
U_N = 8
U_TAIL = NU - sum(U_HEAD) - U_BODY * U_N
X_FIRST = 16
MID = 1


def _schedule(order, lags, extra, tail):
    lag = dict(p=0, s=lags[0], v=lags[1], o=lags[2])
    kind = dict(x="p", y="p", z="p", A="o", B="o", C="o", s="s", v="v")
    hooks = {}
    for x in extra.split():
        key, val = x.split(":")
        hooks.setdefault(key, []).append((val[0], int(val[1:])))
    seq = []
    for t in range(NPAIR):
        for k in order:
            j = t - lag[kind[k]]
            if j >= 0:
                if k in "xAsv":
                    seq += hooks.get("<" + kind[k] + str(j), [])
                seq.append((k, j))
                if k in "zCsv":
                    seq += hooks.get(kind[k] + str(j), [])
            if t == NPAIR - 1 and k == "z":
                break
    for x in tail.split():
        seq += [(k, int(x[1:])) for k in ("ABC" if x[0] == "o" else x[0])
                if (k, int(x[1:])) not in seq]
    for k in "xyzABCsv":
        assert [j for kk, j in seq if kk == k] == list(range(NPAIR)), (k, seq)
    return seq


def _plan(order_e, lag_e, extra_e, tail_e, due_e, order_o, extra_o, tail_o, due_o):
    emit = " ".join(f"s{j}:u{2 * j} s{j}:u{2 * j + 1}" for j in range(NPAIR - 2))
    rest = " ".join(f"u{n}" for n in range(2 * NPAIR - 4, 2 * NPAIR))
    dues = ({}, {})
    for j in range(NPAIR):
        for e in range(2):
            d = 9 * j + due_e + e
            dues[d >= 9 * NPAIR].setdefault((d // 9 % NPAIR, d % 9), []).append(("u", 2 * j + e))
            d = 9 * j + due_o + e
            if d < 9 * NPAIR:
                dues[1].setdefault((d // 9, d % 9), []).append(("U", 2 * j + e))
    for key in dues[1]:
        dues[1][key].sort(key=lambda x: x[0] == "u")
    for x in extra_o.split():
        key, val = x.split(":")
        if val[0] in "ab":
            dues[1].setdefault((int(key[1:]) + 1, 0), []).append((val[0], int(val[1:])))
    return ((_schedule(order_e, (1, 3, lag_e), extra_e + " " + emit, tail_e.replace("#", rest)),
             dues[0]),
            (_schedule(order_o, (1, 3, 5), extra_o + " " + emit, tail_o.replace("#", rest)),
             dues[1]))


PLANS = (
    _plan("xyzBACvs", 4,
          "<s0:q0 <s1:q1 <s2:q2 <s3:Q0 <s4:Q1 <s5:q3 <s6:Q2 <s7:Q3 <s8:q4 <s9:Q4 <s10:q5 <s11:q6"
          " <s12:Q5 <s13:q7",
          "v12 s14 q8 v13 s15 # o11 o12 o13 v14 q9 v15 o14 o15 q10 q11", 25,
          "xAyzBCvs",
          "<s0:q12 <s1:q13 <s2:q14 <s3:Q7 p5:a0 p6:b0 p7:a1 p8:b1 p10:a2 p11:b2 p12:a3 p13:b3",
          "v12 s14 o10 v13 s15 # o11 o12 v14 w0 v15 o13 w1 o14 w2 o15 w3 w4", 25),
    _plan("xyABzCvs", 5, "<s0:q6",
          "v12 s14 q8 v13 s15 # o10 o11 o12 v14 o13 v15 o14 q9 o15 q10 q11", 22,
          "xAyBzCvs",
          "<s0:q12 <s1:q13 <s2:q14 p5:a0 p6:b0 p7:a1 p8:b1 p9:a2 p10:b2 p11:a3 p12:b3",
          "v12 s14 o10 v13 s15 # o11 o12 v14 o13 v15 o14 w0 o15 w1 w2 w3 w4", 24),
)


def _nt(a, b):
    return jax.lax.dot_general(a, b, (((1,), (1,)), ((), ())), preferred_element_type=F32)


def _nn(a, b):
    return jnp.dot(a, b, preferred_element_type=F32)


def _recip(x):
    r = pl.reciprocal(x, approx=True)
    return r * (2.0 - x * r)


def _kernel(ax_h, wqkv_h, woa_h, bx_h, mem0_h, wq_h, wk_h, wv_h, wo_h, out_h,
            ax_v, wqkv_v, woa_v, bx_v, xpre_v, mem0_v, wraw_v, wo_v,
            tmp_v, tmp2_v, wob_v, wqkvp_v, woap_v, slab_v, outa_v,
            wb_v, pre_v, qo_v, kvo_v, o8_v, mid_v, cap_v, outb_v,
            sem_in, sem_out):
    cp_xpre = [pltpu.make_async_copy(bx_h.at[pl.ds(a, n), pl.ds(0, PRE), :],
                                     xpre_v.at[pl.ds(a, n)], sem_in.at[s])
               for a, n, s in ((0, X_FIRST, 0), (X_FIRST, NIT - X_FIRST, 8 + len(U_HEAD) + U_N))]
    cp_wqkv = pltpu.make_async_copy(wqkv_h, wqkv_v, sem_in.at[1])
    cp_woa = pltpu.make_async_copy(woa_h, woa_v, sem_in.at[2])
    cp_mem = pltpu.make_async_copy(mem0_h, mem0_v, sem_in.at[3])
    cp_bx = pltpu.make_async_copy(bx_h, bx_v, sem_in.at[4])
    cp_ax = pltpu.make_async_copy(ax_h, ax_v, sem_in.at[5])
    cp_wo = pltpu.make_async_copy(wo_h, wo_v, sem_in.at[6])
    w_hs = (wq_h, wk_h, wv_h)
    groups = list(U_HEAD) + [U_BODY] * U_N + [U_TAIL]
    g_start = [sum(groups[:g]) for g in range(len(groups))]

    n_head = sum(U_HEAD)

    def unit(c, k):
        if c is not None and k < 2:
            return 3 * (2 * c + k) + 2, True
        if c is not None:
            e = n_head + (U_BODY - 2) * c + k - 2
        else:
            e = k if k < n_head else k - 2 * U_N
        return 3 * (e // 2) + e % 2, False

    def unit_at(p):
        in_loop = n_head <= p < g_start[-1]
        return unit(*divmod(p - n_head, U_BODY)) if in_loop else unit(None, p)

    assert sorted(unit_at(p)[0] for p in range(NU)) == list(range(NU))
    cp_xpre[0].start()
    for g, n in enumerate(groups):
        for p in range(g_start[g], g_start[g] + n):
            u = unit_at(p)[0]
            pltpu.make_async_copy(w_hs[u % 3].at[pl.ds(u // 3 * PAIR, PAIR)], wraw_v.at[p],
                                  sem_in.at[7 + g]).start()
        if g == 0:
            cp_xpre[1].start()
    cp_wo.start()
    cp_wqkv.start()
    cp_woa.start()
    cp_mem.start()
    cp_bx.start()
    cp_ax.start()

    def g_wait(g, p0, n):
        buf = wraw_v.at[pl.ds(p0, n)]
        pltpu.make_async_copy(buf, buf, sem_in.at[7 + g]).wait()

    n_dots = NIT * PRE // PRE_MB * (PAIR // 128)

    def b_pre(p, u, value, after=None, dots=(0, n_dots)):
        if value:
            blk = jnp.concatenate([wraw_v[p, r:r + 64, :] for r in ILV], axis=0)
        else:
            blk = wraw_v[p]
        if dots[0] == 0:
            wb_v[u] = pltpu.bitcast(blk.T, U32)
        nb = PRE_MB // PRE
        for k in range(*dots):
            mb, n = divmod(k, PAIR // 128)
            x = xpre_v[mb * nb:(mb + 1) * nb].reshape(PRE_MB, D)
            r = _nt(x, blk[n * 128:(n + 1) * 128])
            pre_v[u, mb * PRE_MB // 2:(mb + 1) * PRE_MB // 2, n * 128:(n + 1) * 128] = (
                pltpu.bitcast(r.astype(BF16), U32))
            if after is not None:
                after(r)

    cp_xpre[0].wait()
    g_wait(0, 0, 1)
    b_pre(0, *unit_at(0), dots=(0, 4))
    cp_xpre[1].wait()
    b_pre(0, *unit_at(0), dots=(4, n_dots))
    for g in range(1, len(U_HEAD)):
        g_wait(g, g_start[g], groups[g])
        for p in range(g_start[g], g_start[g] + groups[g]):
            b_pre(p, *unit_at(p))

    def pre_body(c, carry):
        p0 = n_head + c * U_BODY
        g_wait(len(U_HEAD) + c, p0, U_BODY)
        for k in range(U_BODY):
            b_pre(p0 + k, *unit(c, k))
        return carry + c

    off = jax.lax.fori_loop(0, U_N, pre_body, 0) < 0

    g_wait(len(groups) - 1, g_start[-1], U_TAIL)
    cp_wqkv.wait()
    cp_woa.wait()
    cp_wo.wait()

    copies = [(woa_v, r, r, t, tmp2_v.at[t]) for t in range(LT) for r in range(0, D, 16)]
    copies += [(wo_v, j * PAIR + r + rr, j * PAIR + k * 64 + rr, t,
                wob_v.at[:, pl.ds(t * 128, 128)])
               for j in range(NPAIR) for k, r in enumerate(ILV) for t in range(LT)
               for rr in range(0, 64, 16)]

    def copy_some(res, n):
        for k in range(res.shape[0] // 8):
            tok = pltpu.bitcast(res[8 * k:8 * k + 8], U32)
            for _ in range(n):
                if copies:
                    src, r, rd, t, dst = copies.pop(0)
                    v = pltpu.bitcast(src[r:r + 16, t * 128:(t + 1) * 128], U32)
                    dst[rd // 2:rd // 2 + 8, :] = jnp.where(off, tok, v)

    def tail_pre(k):
        p = g_start[-1] + k
        b_pre(p, *unit_at(p), functools.partial(copy_some, n=(2, 1, 3, 6)[k]))

    def regroup(src_v, t, base, g):
        parts = []
        for dp in (2 * g, 2 * g + 1):
            v = src_v[t, pl.ds(base + dp, A_H, stride=A_DH // 2), :]
            parts.append(pltpu.bitcast(v << 16, F32))
            parts.append(pltpu.bitcast(v & jnp.uint32(0xFFFF0000), F32))
        return jnp.concatenate(parts, axis=0).astype(BF16)

    def a_prep1(p):
        for b in range(p * LT, (p + 1) * LT):
            blk = pltpu.bitcast(wqkv_v[:, b * 128:(b + 1) * 128].T, U32)
            for t in range(LT):
                tmp_v[t, b * 64:(b + 1) * 64, :] = blk[:, t * 128:(t + 1) * 128]

    def a_prep2(p):
        for g in range(LT):
            blk = jnp.concatenate([regroup(tmp_v, t, p * D // 2, g) for t in range(LT)], axis=1)
            b = p * LT + g
            wqkvp_v[:, b * 128:(b + 1) * 128] = pltpu.bitcast(blk.T, U32)

    def a_prep3():
        for g in range(LT):
            for t in range(LT):
                woap_v[g * 64:(g + 1) * 64, t * 128:(t + 1) * 128] = pltpu.bitcast(
                    regroup(tmp2_v, t, 0, g), U32)

    a_prep1(0)
    a_prep1(1)
    tail_pre(0)
    a_prep1(2)
    a_prep2(0)
    tail_pre(1)
    a_prep2(1)
    tail_pre(2)
    a_prep2(2)
    a_prep3()
    tail_pre(3)
    for t in range(LT, 3 * LT):
        slab_v[0, t, 0:A_PAD, :] = jnp.zeros((A_PAD, 128), F32)
    assert not copies
    cp_mem.wait()
    cp_bx.wait()
    cp_ax.wait()

    a_scale = A_DH ** (-0.5)
    b_scale = B_DH ** (-0.5)
    qrow = jax.lax.broadcasted_iota(jnp.int32, (32, 128), 0)
    lane = jax.lax.broadcasted_iota(jnp.int32, (32, 128), 1)
    first = lane < B_L
    kcol = jnp.where(first, lane, lane - B_L)
    allowed = (qrow >= B_SEG - 8) | (kcol >= B_SEG) | (qrow + 8 >= kcol)
    cap = jnp.where(allowed, jnp.inf, NEG * LOG2E)
    cap_v[0] = jnp.where(first, cap, -jnp.inf)
    cap_v[1] = jnp.where(first | (lane >= 2 * B_L), -jnp.inf, cap)
    cap_v[2] = jnp.where(qrow % 8 >= qrow // 8, jnp.inf, NEG * LOG2E)
    cap_v[3] = jnp.where(qrow % 8 >= qrow // 8 + 4, jnp.inf, NEG * LOG2E)

    def blockdiag_k(t):
        n = t.shape[0]
        left = jax.lax.broadcasted_iota(jnp.int32, (n, 128), 1) < 64
        z = jnp.zeros((n, 128), F32)
        mid = t[:, 128:256]
        top = jnp.concatenate([t[:, 0:128], jnp.where(left, mid, 0.0), z], axis=1)
        bot = jnp.concatenate([z, jnp.where(left, 0.0, mid), t[:, 256:384]], axis=1)
        return jnp.concatenate([top, bot], axis=0).astype(BF16)

    def blockdiag_v(t):
        left = jax.lax.broadcasted_iota(jnp.int32, t.shape, 1) % 128 < 64
        return jnp.concatenate([jnp.where(left, t, 0.0), jnp.where(left, 0.0, t)],
                               axis=0).astype(BF16)

    def softmax(s):
        s = jnp.concatenate([s, jnp.zeros((32, 128 - 2 * B_L), F32)], axis=1) * (b_scale * LOG2E)
        sa, sb = jnp.minimum(s, cap_v[0]), jnp.minimum(s, cap_v[1])
        ma = jnp.max(sa, axis=1, keepdims=True)
        mb = jnp.max(sb, axis=1, keepdims=True)
        p = jnp.exp2(jnp.maximum(sa, sb) - jnp.where(first, ma, mb))
        la = jnp.sum(jnp.where(first, p, 0.0), axis=1, keepdims=True)
        lb = jnp.sum(p, axis=1, keepdims=True) - la
        p = p * pl.reciprocal(jnp.where(first, la, lb), approx=True)
        return p[:, :2 * B_L].astype(BF16)

    def bc(kv_x, kv_m, k, t):
        src = kv_x if k < 8 else kv_m
        return jnp.broadcast_to(src[k % 8:k % 8 + 1, t * 128:(t + 1) * 128], (8, 128))

    def first8_probs(q, kv_x, kv_m):
        left = jax.lax.broadcasted_iota(jnp.int32, (8, 128), 1) < 64
        q = q * (b_scale * LOG2E)
        q0, q2 = q[:, 0:128], q[:, 256:384]
        q1a, q1b = jnp.where(left, q[:, 128:256], 0.0), jnp.where(left, 0.0, q[:, 128:256])
        sc = []
        for k in range(16):
            k1 = bc(kv_x, kv_m, k, 1)
            xa = jnp.sum(q0 * bc(kv_x, kv_m, k, 0) + q1a * k1, axis=1, keepdims=True)
            xb = jnp.sum(q1b * k1 + q2 * bc(kv_x, kv_m, k, 2), axis=1, keepdims=True)
            x = jnp.where(left, xa, xb)
            if 0 < k < 8:
                x = jnp.minimum(x, cap_v[2 + k // 4, 8 * (k % 4):8 * (k % 4) + 8, :])
            sc.append(x)
        m = functools.reduce(jnp.maximum, sc)
        p = [jnp.exp2(x - m) for x in sc]
        return p, _recip(functools.reduce(jnp.add, p))

    def first8_values(p, inv, kv_x, kv_m):
        return [functools.reduce(jnp.add, [p[k] * bc(kv_x, kv_m, k, 3 + t) for k in range(16)])
                * inv for t in range(3)]

    def segment(i, sub, h, even, extra):
        order, dues = PLANS[sub][0 if even else 1]
        qkv, prob, att, q8, o8 = {}, {}, {}, {}, {}
        acc, acc16 = [None], [None]
        hh = [h]
        parts = []
        pins = extra['pins']

        def proj(j, part):
            cuts = sorted({3 * part, 3 * part + 3}
                          | {m for (jj, m) in dues if jj == j and m // 3 == part})
            for m, m2 in zip(cuts[:-1], cuts[1:]):
                due = [x for key in dues.get((j, m), ()) for x in pins.pop(key)]
                if due:
                    hh[0] = extra['pin'](hh[0], due)
                w = wb_v[3 * j + part, :, (m - 3 * part) * 128:(m2 - 3 * part) * 128]
                parts.append(_nn(hh[0], pltpu.bitcast(w, BF16)))
            if part < 2:
                return
            r = jnp.concatenate(parts, axis=1)
            parts.clear()
            if even:
                rows = pl.ds(pl.multiple_of(i * (PRE // 2), PRE // 2), PRE // 2)
                pre = jnp.concatenate([pre_v[3 * j + m, rows, :] for m in range(3)], axis=1)
                pre = pltpu.bitcast(pre, BF16).astype(F32)
                qo_v[j] = r[16:24, :PAIR]
                kvo_v[j] = r[16:24, PAIR:]
                q8[j] = (pre[0:8, :PAIR], pre[0:8, PAIR:], r[24:32, PAIR:])
                q = jnp.concatenate([pre[8:16, :PAIR], r[0:16, :PAIR], r[24:32, :PAIR]], axis=0)
                kv = jnp.concatenate([pre[:, PAIR:], r[0:16, PAIR:], r[24:32, PAIR:]], axis=0)
            else:
                q8[j] = (qo_v[j], kvo_v.at[j], r[24:32, PAIR:])
                q = r[:, :PAIR]
                kv = jnp.concatenate([kvo_v[j], r[:, PAIR:]], axis=0)
            qkv[j] = (q.astype(BF16), blockdiag_k(kv[:, :PAIR]), blockdiag_v(kv[:, PAIR:]))

        def vector(jj):
            j, second = jj // 2, jj % 2
            key = ('u' if even else 'U', jj)
            if not second:
                o8[j] = first8_probs(*q8[j])
                pins[key] = [pltpu.bitcast(o8[j][1], U32)]
                return
            o = first8_values(*o8[j], *q8[j][1:])
            pins[key] = [pltpu.bitcast(x, U32) for x in o]
            o = jnp.concatenate(o, axis=1)
            if even:
                o8_v[j] = o
            else:
                o8[j] = o

        def scores(j):
            prob[j] = softmax(_nt(qkv[j][0], qkv[j][1]))

        def values(j):
            att[j] = _nn(prob[j], qkv[j][2])

        def outp(j, t):
            lhs = att[j][:, t * 128:(t + 1) * 128]
            if even:
                wide = sub > 0 and t == MID
                if wide:
                    lhs = jnp.concatenate([lhs, mid_v[j]], axis=0)
            else:
                wide = sub == UNROLL - 1 or t != MID
                o16 = jnp.concatenate([o8_v[j, :, t * 128:(t + 1) * 128],
                                       o8[j][:, t * 128:(t + 1) * 128]], axis=0)
                if wide:
                    lhs = jnp.concatenate([lhs, o16], axis=0)
                else:
                    mid_v[j] = o16
            r = j * PAIR // 2 + t * 64
            d = _nn(lhs.astype(BF16), pltpu.bitcast(wob_v[r:r + 64, :], BF16))
            acc[0] = d[0:32] if acc[0] is None else acc[0] + d[0:32]
            if wide:
                acc16[0] = d[32:48] if acc16[0] is None else acc16[0] + d[32:48]

        fns = dict(extra, s=scores, v=values, u=vector)
        for t in range(3):
            fns['xyz'[t]] = functools.partial(proj, part=t)
            fns['ABC'[t]] = functools.partial(outp, t=t)
        for k, j in order:
            fns[k](j)
        return acc[0], acc16[0]

    def body(i, sub, mem, held):
        r0 = pl.multiple_of(i * BLK, BLK)

        slab = slab_v.at[sub]

        def a_qkv(b, ahead=0):
            x = ax_v[pl.ds(r0 + ahead * BLK, BLK), :]
            slab_v[sub + ahead, b, A_PAD:A_PAD + BLK, :] = _nn(
                x, pltpu.bitcast(wqkvp_v[:, b * 128:(b + 1) * 128], BF16))

        a_o, a_p = {}, {}
        never = i < 0
        pins = {}

        def a_logits(sb):
            base = A_PAD + sb * A_SUB
            q = [slab[t, base:base + A_SUB, :] for t in range(LT)]
            logits = []
            for w in range(A_W):
                lo = base - A_DIL * w
                acc = None
                for t in range(LT):
                    pr = q[t] * slab[LT + t, lo:lo + A_SUB, :]
                    acc = pr if acc is None else acc + pr
                acc = acc + pltpu.roll(acc, 64, 1)
                acc = acc + pltpu.roll(acc, 32, 1)
                acc = acc * a_scale
                if sb == 0 and w > 0:
                    row = jax.lax.broadcasted_iota(jnp.int32, (A_SUB, 128), 0) + r0
                    acc = jnp.where(row >= A_DIL * w, acc, NEG)
                logits.append(acc)
            m = logits[0]
            for w in range(1, A_W):
                m = jnp.maximum(m, logits[w])
            ps = [jnp.exp(l - m) for l in logits]
            den = ps[0]
            for w in range(1, A_W):
                den = den + ps[w]
            inv = _recip(den)
            a_p[sb] = (ps, inv)
            pins[('a', sb)] = [pltpu.bitcast(inv[8 * u:8 * u + 8], U32) for u in range(A_SUB // 8)]

        def a_values(sb):
            base = A_PAD + sb * A_SUB
            ps, inv = a_p[sb]
            o = []
            for t in range(LT):
                acc = None
                for w in range(A_W):
                    lo = base - A_DIL * w
                    pr = ps[w] * slab[2 * LT + t, lo:lo + A_SUB, :]
                    acc = pr if acc is None else acc + pr
                o.append(acc * inv)
            pins[('b', sb)] = [pltpu.bitcast(x[8 * u:8 * u + 8], U32) for x in o
                               for u in range(A_SUB // 8)]
            a_o[sb] = jnp.concatenate(o, axis=1)
            if sb == BLK // A_SUB - 1:
                for t in range(LT, 3 * LT):
                    slab_v[(sub + 1) % UNROLL, t, 0:A_PAD, :] = slab[t, BLK:BLK + A_PAD, :]

        def pin(h, due):
            u = pltpu.bitcast(h, U32)
            tiles = [u[8 * r:8 * r + 8, 128 * c:128 * c + 128]
                     for c in range(LT) for r in range(u.shape[0] // 8)]
            for k, x in enumerate(due):
                tiles[k % len(tiles)] = jnp.where(never, x, tiles[k % len(tiles)])
            n = u.shape[0] // 8
            cols = [jnp.concatenate(tiles[c * n:(c + 1) * n], axis=0) for c in range(LT)]
            return pltpu.bitcast(jnp.concatenate(cols, axis=1), BF16)

        def a_out(b):
            o = jnp.concatenate([a_o[sb] for sb in range(BLK // A_SUB)], axis=0).astype(BF16)
            res = _nn(o, pltpu.bitcast(woap_v[:, b * 128:(b + 1) * 128], BF16))
            outa_v[pl.ds(r0, BLK), b * 128:(b + 1) * 128] = res.astype(BF16)

        x = bx_v[i].astype(F32)
        extra = dict(q=a_qkv, Q=functools.partial(a_qkv, ahead=1), a=a_logits, b=a_values,
                     w=a_out, pin=pin, pins=pins)

        def emit(r, out_e, acc, acc16):
            out = jnp.concatenate([acc16[0:8], out_e, acc16[8:16], acc[0:24]], axis=0)
            outb_v[pl.ds(r, BLK), :] = out.astype(BF16)
            pltpu.make_async_copy(
                outb_v.at[pl.ds(r, BLK)], out_h.at[pl.ds(r, BLK), pl.ds(D, D)],
                sem_out.at[1]).start()

        acc, acc16 = segment(
            i, sub, jnp.concatenate([x[16:40], mem], axis=0).astype(BF16), True, extra)
        if held is not None:
            emit(held[0], held[1], held[2], held[3] + acc16)
        out_e = acc[0:24]
        mem = acc[24:32].astype(BF16).astype(F32)
        acc, acc16 = segment(
            i, sub, jnp.concatenate([x[40:64], mem], axis=0).astype(BF16), False, extra)
        held = (r0, out_e, acc, acc16)
        if sub == UNROLL - 1:
            emit(*held)
            held = None
        pltpu.make_async_copy(
            outa_v.at[pl.ds(r0, BLK)], out_h.at[pl.ds(r0, BLK), pl.ds(0, D)], sem_out.at[0]).start()
        return acc[24:32].astype(BF16).astype(F32), held

    def body_n(ii, mem):
        held = None
        for u in range(UNROLL):
            mem, held = body(ii * UNROLL + u, u, mem, held)
        return mem

    jax.lax.fori_loop(0, NIT // UNROLL, body_n, mem0_v[...].astype(F32))

    pltpu.make_async_copy(outa_v, out_h.at[:, pl.ds(0, D)], sem_out.at[0]).wait()
    pltpu.make_async_copy(outb_v, out_h.at[:, pl.ds(D, D)], sem_out.at[1]).wait()


@jax.jit
def _run(A_x, A_wqkv, A_wo, B_x, B_mem0, B_Wq, B_Wk, B_Wv, B_Wo):
    def feat_major(w):
        return jnp.transpose(w, (1, 2, 0)).reshape(B_F, D)

    any_spec = pl.BlockSpec(memory_space=pl.ANY)
    out = pl.pallas_call(
        _kernel,
        out_shape=jax.ShapeDtypeStruct((S, 2 * D), BF16),
        in_specs=[any_spec] * 9,
        out_specs=any_spec,
        scratch_shapes=[
            pltpu.VMEM((S, D), BF16),
            pltpu.VMEM((D, 3 * D), BF16),
            pltpu.VMEM((D, D), BF16),
            pltpu.VMEM((NIT, BLK, D), BF16),
            pltpu.VMEM((NIT, PRE, D), BF16),
            pltpu.VMEM((B_M, D), BF16),
            pltpu.VMEM((NU, PAIR, D), BF16),
            pltpu.VMEM((B_F, D), BF16),
            pltpu.VMEM((LT, 3 * D // 2 + 16, 128), U32),
            pltpu.VMEM((LT, D // 2 + 16, 128), U32),
            pltpu.VMEM((B_F // 2, D), U32),
            pltpu.VMEM((D // 2, 3 * D), U32),
            pltpu.VMEM((D // 2, D), U32),
            pltpu.VMEM((UNROLL, 3 * LT, A_PAD + BLK, 128), F32),
            pltpu.VMEM((S, D), BF16),
            pltpu.VMEM((NU, D // 2, PAIR), U32),
            pltpu.VMEM((NU, NIT * PRE // 2, PAIR), U32),
            pltpu.VMEM((NPAIR, 8, PAIR), F32),
            pltpu.VMEM((NPAIR, 8, 2 * PAIR), F32),
            pltpu.VMEM((NPAIR, 8, PAIR), F32),
            pltpu.VMEM((NPAIR, 16, 128), F32),
            pltpu.VMEM((4, 32, 128), F32),
            pltpu.VMEM((S, D), BF16),
            pltpu.SemaphoreType.DMA((9 + len(U_HEAD) + U_N,)),
            pltpu.SemaphoreType.DMA((2,)),
        ],
        compiler_params=pltpu.CompilerParams(vmem_limit_bytes=120 * 1024 * 1024,
                                             disable_bounds_checks=True),
    )(
        A_x.reshape(S, D), A_wqkv, A_wo, B_x.reshape(NIT, BLK, D), B_mem0.reshape(B_M, D),
        feat_major(B_Wq), feat_major(B_Wk), feat_major(B_Wv), B_Wo.reshape(B_F, D),
    )
    return out.reshape(1, S, 2 * D)


def pallas_concat_heads__sliding_local_dilated__memory_aug_recurrent_mem_tr__prompt_kernel(
    A_x: jax.Array,
    A_wqkv: jax.Array,
    A_wo: jax.Array,
    B_x: jax.Array,
    B_mem0: jax.Array,
    B_Wq: jax.Array,
    B_Wk: jax.Array,
    B_Wv: jax.Array,
    B_Wo: jax.Array,
    B_seg_len,
):
    assert A_x.shape == (1, S, D) and B_x.shape == (1, S, D) and B_mem0.shape == (1, B_M, D)
    assert B_Wq.shape == (D, B_H, B_DH) and B_Wo.shape == (B_H, B_DH, D)
    if isinstance(B_seg_len, int):
        assert B_seg_len == B_SEG
    return _run(A_x, A_wqkv, A_wo, B_x, B_mem0, B_Wq, B_Wk, B_Wv, B_Wo)
```

```python
import functools

import jax
import jax.numpy as jnp
import jax.experimental.pallas as pl
import jax.experimental.pallas.tpu as pltpu

F32 = jnp.float32
BF16 = jnp.bfloat16
U32 = jnp.uint32

S = 2048
D = 640
LT = D // 128
BLK = 64
NIT = S // BLK

A_H = 32
A_DH = 20
A_W = 8
A_DIL = 2
A_PAD = 16
A_SUB = 16

B_H = 32
B_DH = 192
B_F = B_H * B_DH
B_M = 8
B_SEG = 32
B_L = B_M + B_SEG
PAIR = 2 * B_DH
NPAIR = B_H // 2
NU = 3 * NPAIR
PRE = 16
PRE_MB = 128

NEG = -1000000000.0
LOG2E = 1.4426950408889634
ILV = [h * B_DH + t * 64 for t in range(3) for h in range(2)]
UNROLL = 2
U_HEAD = (1, 1, 2)
U_BODY = 5
U_N = 8
U_TAIL = NU - sum(U_HEAD) - U_BODY * U_N
X_FIRST = 16
MID = 1


def _schedule(order, lags, extra, tail):
    lag = dict(p=0, s=lags[0], v=lags[1], o=lags[2])
    kind = dict(x="p", y="p", z="p", A="o", B="o", C="o", s="s", v="v")
    hooks = {}
    for x in extra.split():
        key, val = x.split(":")
        hooks.setdefault(key, []).append((val[0], int(val[1:])))
    seq = []
    for t in range(NPAIR):
        for k in order:
            j = t - lag[kind[k]]
            if j >= 0:
                if k in "xAsv":
                    seq += hooks.get("<" + kind[k] + str(j), [])
                seq.append((k, j))
                if k in "zCsv":
                    seq += hooks.get(kind[k] + str(j), [])
            if t == NPAIR - 1 and k == "z":
                break
    for x in tail.split():
        seq += [(k, int(x[1:])) for k in ("ABC" if x[0] == "o" else x[0])
                if (k, int(x[1:])) not in seq]
    for k in "xyzABCsv":
        assert [j for kk, j in seq if kk == k] == list(range(NPAIR)), (k, seq)
    return seq


def _plan(order_e, lag_e, extra_e, tail_e, due_e, order_o, extra_o, tail_o, due_o, due_a):
    emit = " ".join(f"s{j}:u{2 * j} s{j}:u{2 * j + 1}" for j in range(NPAIR - 2))
    rest = " ".join(f"u{n}" for n in range(2 * NPAIR - 4, 2 * NPAIR))
    dues = ({}, {})
    for j in range(NPAIR):
        for e in range(2):
            d = 9 * j + due_e + e
            dues[d >= 9 * NPAIR].setdefault((d // 9 % NPAIR, d % 9), []).append(("u", 2 * j + e))
            d = 9 * j + due_o + e
            if d < 9 * NPAIR:
                dues[1].setdefault((d // 9, d % 9), []).append(("U", 2 * j + e))
    for key in dues[1]:
        dues[1][key].sort(key=lambda x: x[0] == "u")
    for x in extra_o.split():
        key, val = x.split(":")
        if val[0] in "ab":
            dues[1].setdefault((int(key[1:]) + 1, due_a), []).append((val[0], int(val[1:])))
    return ((_schedule(order_e, (1, 3, lag_e), extra_e + " " + emit, tail_e.replace("#", rest)),
             dues[0]),
            (_schedule(order_o, (1, 3, 5), extra_o + " " + emit, tail_o.replace("#", rest)),
             dues[1]))


PLANS = (
    _plan("xyzBACvs", 4,
          "<s0:q0 <s1:q1 <s2:q2 <s3:Q0 <s4:Q1 <s5:q3 <s6:Q2 <s7:Q3 <s8:q4 <s9:Q4 <s10:q5 <s11:q6"
          " <s12:Q5 <s13:q7",
          "v12 s14 q8 v13 s15 # o11 o12 o13 v14 q9 v15 o14 o15 q10 q11", 25,
          "xAyzBCvs",
          "<s0:q12 <s1:q13 <s2:q14 <s3:Q7 p5:a0 p6:b0 p7:a1 p8:b1 p10:a2 p11:b2 p12:a3 p13:b3",
          "v12 s14 o10 v13 s15 # o11 o12 v14 w0 v15 o13 w1 o14 w2 o15 w3 w4", 25, 0),
    _plan("xyABzCvs", 5, "<s0:q6",
          "v12 s14 q8 v13 s15 # o10 o11 o12 v14 o13 v15 o14 q9 o15 q10 q11", 22,
          "xAByzCvs",
          "<s0:q12 <s1:q13 <s2:q14 p5:a0 p6:b0 p7:a1 p8:b1 p9:a2 p10:b2 p11:a3 p12:b3",
          "v12 s14 o10 v13 s15 # o11 o12 v14 o13 v15 o14 w0 o15 w1 w2 w3 w4", 23, 2),
)
PIN_AT = ((8, 5), (1, 0))
_KEYS = list(range(16))
KEY_ORDER = (([k // 2 + 8 * (k % 2) for k in _KEYS], _KEYS), (_KEYS, _KEYS))


def _nt(a, b):
    return jax.lax.dot_general(a, b, (((1,), (1,)), ((), ())), preferred_element_type=F32)


def _nn(a, b):
    return jnp.dot(a, b, preferred_element_type=F32)


def _recip(x):
    r = pl.reciprocal(x, approx=True)
    return r * (2.0 - x * r)


def _kernel(ax_h, wqkv_h, woa_h, bx_h, mem0_h, wq_h, wk_h, wv_h, wo_h, out_h,
            ax_v, wqkv_v, woa_v, bx_v, xpre_v, mem0_v, wraw_v, wo_v,
            tmp_v, tmp2_v, wob_v, wqkvp_v, woap_v, slab_v, outa_v,
            wb_v, pre_v, qo_v, kvo_v, o8_v, mid_v, cap_v, outb_v,
            sem_in, sem_out):
    cp_xpre = [pltpu.make_async_copy(bx_h.at[pl.ds(a, n), pl.ds(0, PRE), :],
                                     xpre_v.at[pl.ds(a, n)], sem_in.at[s])
               for a, n, s in ((0, X_FIRST, 0), (X_FIRST, NIT - X_FIRST, 8 + len(U_HEAD) + U_N))]
    cp_wqkv = pltpu.make_async_copy(wqkv_h, wqkv_v, sem_in.at[1])
    cp_woa = pltpu.make_async_copy(woa_h, woa_v, sem_in.at[2])
    cp_mem = pltpu.make_async_copy(mem0_h, mem0_v, sem_in.at[3])
    cp_bx = pltpu.make_async_copy(bx_h, bx_v, sem_in.at[4])
    cp_ax = pltpu.make_async_copy(ax_h, ax_v, sem_in.at[5])
    cp_wo = pltpu.make_async_copy(wo_h, wo_v, sem_in.at[6])
    w_hs = (wq_h, wk_h, wv_h)
    groups = list(U_HEAD) + [U_BODY] * U_N + [U_TAIL]
    g_start = [sum(groups[:g]) for g in range(len(groups))]

    n_head = sum(U_HEAD)

    def unit(c, k):
        if c is not None and k < 2:
            return 3 * (2 * c + k) + 2, True
        if c is not None:
            e = n_head + (U_BODY - 2) * c + k - 2
        else:
            e = k if k < n_head else k - 2 * U_N
        return 3 * (e // 2) + e % 2, False

    def unit_at(p):
        in_loop = n_head <= p < g_start[-1]
        return unit(*divmod(p - n_head, U_BODY)) if in_loop else unit(None, p)

    assert sorted(unit_at(p)[0] for p in range(NU)) == list(range(NU))
    cp_xpre[0].start()
    for g, n in enumerate(groups):
        for p in range(g_start[g], g_start[g] + n):
            u = unit_at(p)[0]
            pltpu.make_async_copy(w_hs[u % 3].at[pl.ds(u // 3 * PAIR, PAIR)], wraw_v.at[p],
                                  sem_in.at[7 + g]).start()
        if g == 0:
            cp_xpre[1].start()
    cp_wo.start()
    cp_wqkv.start()
    cp_woa.start()
    cp_mem.start()
    cp_bx.start()
    cp_ax.start()

    def g_wait(g, p0, n):
        buf = wraw_v.at[pl.ds(p0, n)]
        pltpu.make_async_copy(buf, buf, sem_in.at[7 + g]).wait()

    n_dots = NIT * PRE // PRE_MB * (PAIR // 128)

    def b_pre(p, u, value, after=None, dots=(0, n_dots)):
        if value:
            blk = jnp.concatenate([wraw_v[p, r:r + 64, :] for r in ILV], axis=0)
        else:
            blk = wraw_v[p]
        if dots[0] == 0:
            wb_v[u] = pltpu.bitcast(blk.T, U32)
        nb = PRE_MB // PRE
        for k in range(*dots):
            mb, n = divmod(k, PAIR // 128)
            x = xpre_v[mb * nb:(mb + 1) * nb].reshape(PRE_MB, D)
            r = _nt(x, blk[n * 128:(n + 1) * 128])
            pre_v[u, mb * PRE_MB // 2:(mb + 1) * PRE_MB // 2, n * 128:(n + 1) * 128] = (
                pltpu.bitcast(r.astype(BF16), U32))
            if after is not None:
                after(r)

    cp_xpre[0].wait()
    g_wait(0, 0, 1)
    b_pre(0, *unit_at(0), dots=(0, 4))
    cp_xpre[1].wait()
    b_pre(0, *unit_at(0), dots=(4, n_dots))
    for g in range(1, len(U_HEAD)):
        g_wait(g, g_start[g], groups[g])
        for p in range(g_start[g], g_start[g] + groups[g]):
            b_pre(p, *unit_at(p))

    def pre_body(c, carry):
        p0 = n_head + c * U_BODY
        g_wait(len(U_HEAD) + c, p0, U_BODY)
        for k in range(U_BODY):
            b_pre(p0 + k, *unit(c, k))
        return carry + c

    off = jax.lax.fori_loop(0, U_N, pre_body, 0) < 0

    g_wait(len(groups) - 1, g_start[-1], U_TAIL)
    cp_wqkv.wait()
    cp_woa.wait()
    cp_wo.wait()

    copies = [(woa_v, r, r, t, tmp2_v.at[t]) for t in range(LT) for r in range(0, D, 16)]
    copies += [(wo_v, j * PAIR + r + rr, j * PAIR + k * 64 + rr, t,
                wob_v.at[:, pl.ds(t * 128, 128)])
               for j in range(NPAIR) for k, r in enumerate(ILV) for t in range(LT)
               for rr in range(0, 64, 16)]

    def copy_some(res, n):
        for k in range(res.shape[0] // 8):
            tok = pltpu.bitcast(res[8 * k:8 * k + 8], U32)
            for _ in range(n):
                if copies:
                    src, r, rd, t, dst = copies.pop(0)
                    v = pltpu.bitcast(src[r:r + 16, t * 128:(t + 1) * 128], U32)
                    dst[rd // 2:rd // 2 + 8, :] = jnp.where(off, tok, v)

    def tail_pre(k):
        p = g_start[-1] + k
        b_pre(p, *unit_at(p), functools.partial(copy_some, n=(2, 1, 3, 6)[k]))

    def regroup(src_v, t, base, g):
        parts = []
        for dp in (2 * g, 2 * g + 1):
            v = src_v[t, pl.ds(base + dp, A_H, stride=A_DH // 2), :]
            parts.append(pltpu.bitcast(v << 16, F32))
            parts.append(pltpu.bitcast(v & jnp.uint32(0xFFFF0000), F32))
        return jnp.concatenate(parts, axis=0).astype(BF16)

    def a_prep1(p):
        for b in range(p * LT, (p + 1) * LT):
            blk = pltpu.bitcast(wqkv_v[:, b * 128:(b + 1) * 128].T, U32)
            for t in range(LT):
                tmp_v[t, b * 64:(b + 1) * 64, :] = blk[:, t * 128:(t + 1) * 128]

    def a_prep2(p):
        for g in range(LT):
            blk = jnp.concatenate([regroup(tmp_v, t, p * D // 2, g) for t in range(LT)], axis=1)
            b = p * LT + g
            wqkvp_v[:, b * 128:(b + 1) * 128] = pltpu.bitcast(blk.T, U32)

    def a_prep3():
        for g in range(LT):
            for t in range(LT):
                woap_v[g * 64:(g + 1) * 64, t * 128:(t + 1) * 128] = pltpu.bitcast(
                    regroup(tmp2_v, t, 0, g), U32)

    a_prep1(0)
    a_prep1(1)
    tail_pre(0)
    a_prep1(2)
    a_prep2(0)
    tail_pre(1)
    a_prep2(1)
    tail_pre(2)
    a_prep2(2)
    a_prep3()
    tail_pre(3)
    for t in range(LT, 3 * LT):
        slab_v[0, t, 0:A_PAD, :] = jnp.zeros((A_PAD, 128), F32)
    assert not copies
    cp_mem.wait()
    cp_bx.wait()
    cp_ax.wait()

    a_scale = A_DH ** (-0.5)
    b_scale = B_DH ** (-0.5)
    qrow = jax.lax.broadcasted_iota(jnp.int32, (32, 128), 0)
    lane = jax.lax.broadcasted_iota(jnp.int32, (32, 128), 1)
    first = lane < B_L
    kcol = jnp.where(first, lane, lane - B_L)
    allowed = (qrow >= B_SEG - 8) | (kcol >= B_SEG) | (qrow + 8 >= kcol)
    cap = jnp.where(allowed, jnp.inf, NEG * LOG2E)
    cap_v[0] = jnp.where(first, cap, -jnp.inf)
    cap_v[1] = jnp.where(first | (lane >= 2 * B_L), -jnp.inf, cap)
    cap_v[2] = jnp.where(qrow % 8 >= qrow // 8, jnp.inf, NEG * LOG2E)
    cap_v[3] = jnp.where(qrow % 8 >= qrow // 8 + 4, jnp.inf, NEG * LOG2E)

    def blockdiag_k(t):
        n = t.shape[0]
        left = jax.lax.broadcasted_iota(jnp.int32, (n, 128), 1) < 64
        z = jnp.zeros((n, 128), F32)
        mid = t[:, 128:256]
        top = jnp.concatenate([t[:, 0:128], jnp.where(left, mid, 0.0), z], axis=1)
        bot = jnp.concatenate([z, jnp.where(left, 0.0, mid), t[:, 256:384]], axis=1)
        return jnp.concatenate([top, bot], axis=0).astype(BF16)

    def blockdiag_v(t):
        left = jax.lax.broadcasted_iota(jnp.int32, t.shape, 1) % 128 < 64
        return jnp.concatenate([jnp.where(left, t, 0.0), jnp.where(left, 0.0, t)],
                               axis=0).astype(BF16)

    def softmax(s):
        s = jnp.concatenate([s, jnp.zeros((32, 128 - 2 * B_L), F32)], axis=1) * (b_scale * LOG2E)
        sa, sb = jnp.minimum(s, cap_v[0]), jnp.minimum(s, cap_v[1])
        ma = jnp.max(sa, axis=1, keepdims=True)
        mb = jnp.max(sb, axis=1, keepdims=True)
        p = jnp.exp2(jnp.maximum(sa, sb) - jnp.where(first, ma, mb))
        la = jnp.sum(jnp.where(first, p, 0.0), axis=1, keepdims=True)
        lb = jnp.sum(p, axis=1, keepdims=True) - la
        p = p * pl.reciprocal(jnp.where(first, la, lb), approx=True)
        return p[:, :2 * B_L].astype(BF16)

    def bc(kv_x, kv_m, k, t):
        src = kv_x if k < 8 else kv_m
        return jnp.broadcast_to(src[k % 8:k % 8 + 1, t * 128:(t + 1) * 128], (8, 128))

    def first8_probs(q, kv_x, kv_m, keys):
        left = jax.lax.broadcasted_iota(jnp.int32, (8, 128), 1) < 64
        q = q * (b_scale * LOG2E)
        q0, q2 = q[:, 0:128], q[:, 256:384]
        q1a, q1b = jnp.where(left, q[:, 128:256], 0.0), jnp.where(left, 0.0, q[:, 128:256])
        sc = []
        for k in keys:
            k1 = bc(kv_x, kv_m, k, 1)
            xa = jnp.sum(q0 * bc(kv_x, kv_m, k, 0) + q1a * k1, axis=1, keepdims=True)
            xb = jnp.sum(q1b * k1 + q2 * bc(kv_x, kv_m, k, 2), axis=1, keepdims=True)
            x = jnp.where(left, xa, xb)
            if 0 < k < 8:
                x = jnp.minimum(x, cap_v[2 + k // 4, 8 * (k % 4):8 * (k % 4) + 8, :])
            sc.append(x)
        m = functools.reduce(jnp.maximum, sc)
        p = [jnp.exp2(x - m) for x in sc]
        return p, _recip(functools.reduce(jnp.add, p))

    def first8_values(p, inv, kv_x, kv_m, keys):
        return [functools.reduce(jnp.add, [x * bc(kv_x, kv_m, k, 3 + t) for x, k in zip(p, keys)])
                * inv for t in range(3)]

    def segment(i, sub, h, even, extra):
        order, dues = PLANS[sub][0 if even else 1]
        keys = KEY_ORDER[sub][0 if even else 1]
        qkv, prob, att, q8, o8 = {}, {}, {}, {}, {}
        acc, acc16 = [None], [None]
        hh = [h]
        parts = []
        pins = extra['pins']

        def proj(j, part):
            cuts = sorted({3 * part, 3 * part + 3}
                          | {m for (jj, m) in dues if jj == j and m // 3 == part})
            for m, m2 in zip(cuts[:-1], cuts[1:]):
                due = [x for key in dues.get((j, m), ()) for x in pins.pop(key)]
                if due:
                    hh[0] = extra['pin'](hh[0], due, PIN_AT[sub][0 if even else 1])
                w = wb_v[3 * j + part, :, (m - 3 * part) * 128:(m2 - 3 * part) * 128]
                parts.append(_nn(hh[0], pltpu.bitcast(w, BF16)))
            if part < 2:
                return
            r = jnp.concatenate(parts, axis=1)
            parts.clear()
            if even:
                rows = pl.ds(pl.multiple_of(i * (PRE // 2), PRE // 2), PRE // 2)
                pre = jnp.concatenate([pre_v[3 * j + m, rows, :] for m in range(3)], axis=1)
                pre = pltpu.bitcast(pre, BF16).astype(F32)
                qo_v[j] = r[16:24, :PAIR]
                kvo_v[j] = r[16:24, PAIR:]
                q8[j] = (pre[0:8, :PAIR], pre[0:8, PAIR:], r[24:32, PAIR:])
                q = jnp.concatenate([pre[8:16, :PAIR], r[0:16, :PAIR], r[24:32, :PAIR]], axis=0)
                kv = jnp.concatenate([pre[:, PAIR:], r[0:16, PAIR:], r[24:32, PAIR:]], axis=0)
            else:
                q8[j] = (qo_v[j], kvo_v.at[j], r[24:32, PAIR:])
                q = r[:, :PAIR]
                kv = jnp.concatenate([kvo_v[j], r[:, PAIR:]], axis=0)
            qkv[j] = (q.astype(BF16), blockdiag_k(kv[:, :PAIR]), blockdiag_v(kv[:, PAIR:]))

        def vector(jj):
            j, second = jj // 2, jj % 2
            key = ('u' if even else 'U', jj)
            if not second:
                o8[j] = first8_probs(*q8[j], keys)
                pins[key] = [pltpu.bitcast(o8[j][1], U32)]
                return
            o = first8_values(*o8[j], *q8[j][1:], keys)
            pins[key] = [pltpu.bitcast(x, U32) for x in o]
            o = jnp.concatenate(o, axis=1)
            if even:
                o8_v[j] = o
            else:
                o8[j] = o

        def scores(j):
            prob[j] = softmax(_nt(qkv[j][0], qkv[j][1]))

        def values(j):
            att[j] = _nn(prob[j], qkv[j][2])

        def outp(j, t):
            lhs = att[j][:, t * 128:(t + 1) * 128]
            if even:
                wide = sub > 0 and t == MID
                if wide:
                    lhs = jnp.concatenate([lhs, mid_v[j]], axis=0)
            else:
                wide = sub == UNROLL - 1 or t != MID
                o16 = jnp.concatenate([o8_v[j, :, t * 128:(t + 1) * 128],
                                       o8[j][:, t * 128:(t + 1) * 128]], axis=0)
                if wide:
                    lhs = jnp.concatenate([lhs, o16], axis=0)
                else:
                    mid_v[j] = o16
            r = j * PAIR // 2 + t * 64
            d = _nn(lhs.astype(BF16), pltpu.bitcast(wob_v[r:r + 64, :], BF16))
            acc[0] = d[0:32] if acc[0] is None else acc[0] + d[0:32]
            if wide:
                acc16[0] = d[32:48] if acc16[0] is None else acc16[0] + d[32:48]

        fns = dict(extra, s=scores, v=values, u=vector)
        for t in range(3):
            fns['xyz'[t]] = functools.partial(proj, part=t)
            fns['ABC'[t]] = functools.partial(outp, t=t)
        for k, j in order:
            fns[k](j)
        return acc[0], acc16[0]

    def body(i, sub, mem, held):
        r0 = pl.multiple_of(i * BLK, BLK)

        slab = slab_v.at[sub]

        def a_qkv(b, ahead=0):
            x = ax_v[pl.ds(r0 + ahead * BLK, BLK), :]
            slab_v[sub + ahead, b, A_PAD:A_PAD + BLK, :] = _nn(
                x, pltpu.bitcast(wqkvp_v[:, b * 128:(b + 1) * 128], BF16))

        a_o, a_p = {}, {}
        never = i < 0
        pins = {}

        def a_logits(sb):
            base = A_PAD + sb * A_SUB
            q = [slab[t, base:base + A_SUB, :] for t in range(LT)]
            logits = []
            for w in range(A_W):
                lo = base - A_DIL * w
                acc = None
                for t in range(LT):
                    pr = q[t] * slab[LT + t, lo:lo + A_SUB, :]
                    acc = pr if acc is None else acc + pr
                acc = acc + pltpu.roll(acc, 64, 1)
                acc = acc + pltpu.roll(acc, 32, 1)
                acc = acc * a_scale
                if sb == 0 and w > 0:
                    row = jax.lax.broadcasted_iota(jnp.int32, (A_SUB, 128), 0) + r0
                    acc = jnp.where(row >= A_DIL * w, acc, NEG)
                logits.append(acc)
            m = logits[0]
            for w in range(1, A_W):
                m = jnp.maximum(m, logits[w])
            ps = [jnp.exp(l - m) for l in logits]
            den = ps[0]
            for w in range(1, A_W):
                den = den + ps[w]
            inv = _recip(den)
            a_p[sb] = (ps, inv)
            pins[('a', sb)] = [pltpu.bitcast(inv[8 * u:8 * u + 8], U32) for u in range(A_SUB // 8)]

        def a_values(sb):
            base = A_PAD + sb * A_SUB
            ps, inv = a_p[sb]
            o = []
            for t in range(LT):
                acc = None
                for w in range(A_W):
                    lo = base - A_DIL * w
                    pr = ps[w] * slab[2 * LT + t, lo:lo + A_SUB, :]
                    acc = pr if acc is None else acc + pr
                o.append(acc * inv)
            pins[('b', sb)] = [pltpu.bitcast(x[8 * u:8 * u + 8], U32) for x in o
                               for u in range(A_SUB // 8)]
            a_o[sb] = jnp.concatenate(o, axis=1)
            if sb == BLK // A_SUB - 1:
                for t in range(LT, 3 * LT):
                    slab_v[(sub + 1) % UNROLL, t, 0:A_PAD, :] = slab[t, BLK:BLK + A_PAD, :]

        def pin(h, due, at):
            u = pltpu.bitcast(h, U32)
            tiles = [u[8 * r:8 * r + 8, 128 * c:128 * c + 128]
                     for c in range(LT) for r in range(u.shape[0] // 8)]
            for k, x in enumerate(due):
                k = (k + at) % len(tiles)
                tiles[k] = jnp.where(never, x, tiles[k])
            n = u.shape[0] // 8
            cols = [jnp.concatenate(tiles[c * n:(c + 1) * n], axis=0) for c in range(LT)]
            return pltpu.bitcast(jnp.concatenate(cols, axis=1), BF16)

        def a_out(b):
            o = jnp.concatenate([a_o[sb] for sb in range(BLK // A_SUB)], axis=0).astype(BF16)
            res = _nn(o, pltpu.bitcast(woap_v[:, b * 128:(b + 1) * 128], BF16))
            outa_v[pl.ds(r0, BLK), b * 128:(b + 1) * 128] = res.astype(BF16)

        x = bx_v[i].astype(F32)
        extra = dict(q=a_qkv, Q=functools.partial(a_qkv, ahead=1), a=a_logits, b=a_values,
                     w=a_out, pin=pin, pins=pins)

        def emit(r, out_e, acc, acc16):
            out = jnp.concatenate([acc16[0:8], out_e, acc16[8:16], acc[0:24]], axis=0)
            outb_v[pl.ds(r, BLK), :] = out.astype(BF16)
            pltpu.make_async_copy(
                outb_v.at[pl.ds(r, BLK)], out_h.at[pl.ds(r, BLK), pl.ds(D, D)],
                sem_out.at[1]).start()

        acc, acc16 = segment(
            i, sub, jnp.concatenate([x[16:40], mem], axis=0).astype(BF16), True, extra)
        if held is not None:
            emit(held[0], held[1], held[2], held[3] + acc16)
        out_e = acc[0:24]
        mem = acc[24:32].astype(BF16).astype(F32)
        acc, acc16 = segment(
            i, sub, jnp.concatenate([x[40:64], mem], axis=0).astype(BF16), False, extra)
        held = (r0, out_e, acc, acc16)
        if sub == UNROLL - 1:
            emit(*held)
            held = None
        pltpu.make_async_copy(
            outa_v.at[pl.ds(r0, BLK)], out_h.at[pl.ds(r0, BLK), pl.ds(0, D)], sem_out.at[0]).start()
        return acc[24:32].astype(BF16).astype(F32), held

    def body_n(ii, mem):
        held = None
        for u in range(UNROLL):
            mem, held = body(ii * UNROLL + u, u, mem, held)
        return mem

    jax.lax.fori_loop(0, NIT // UNROLL, body_n, mem0_v[...].astype(F32))

    pltpu.make_async_copy(outa_v, out_h.at[:, pl.ds(0, D)], sem_out.at[0]).wait()
    pltpu.make_async_copy(outb_v, out_h.at[:, pl.ds(D, D)], sem_out.at[1]).wait()


@jax.jit
def _run(A_x, A_wqkv, A_wo, B_x, B_mem0, B_Wq, B_Wk, B_Wv, B_Wo):
    def feat_major(w):
        return jnp.transpose(w, (1, 2, 0)).reshape(B_F, D)

    any_spec = pl.BlockSpec(memory_space=pl.ANY)
    out = pl.pallas_call(
        _kernel,
        out_shape=jax.ShapeDtypeStruct((S, 2 * D), BF16),
        in_specs=[any_spec] * 9,
        out_specs=any_spec,
        scratch_shapes=[
            pltpu.VMEM((S, D), BF16),
            pltpu.VMEM((D, 3 * D), BF16),
            pltpu.VMEM((D, D), BF16),
            pltpu.VMEM((NIT, BLK, D), BF16),
            pltpu.VMEM((NIT, PRE, D), BF16),
            pltpu.VMEM((B_M, D), BF16),
            pltpu.VMEM((NU, PAIR, D), BF16),
            pltpu.VMEM((B_F, D), BF16),
            pltpu.VMEM((LT, 3 * D // 2 + 16, 128), U32),
            pltpu.VMEM((LT, D // 2 + 16, 128), U32),
            pltpu.VMEM((B_F // 2, D), U32),
            pltpu.VMEM((D // 2, 3 * D), U32),
            pltpu.VMEM((D // 2, D), U32),
            pltpu.VMEM((UNROLL, 3 * LT, A_PAD + BLK, 128), F32),
            pltpu.VMEM((S, D), BF16),
            pltpu.VMEM((NU, D // 2, PAIR), U32),
            pltpu.VMEM((NU, NIT * PRE // 2, PAIR), U32),
            pltpu.VMEM((NPAIR, 8, PAIR), F32),
            pltpu.VMEM((NPAIR, 8, 2 * PAIR), F32),
            pltpu.VMEM((NPAIR, 8, PAIR), F32),
            pltpu.VMEM((NPAIR, 16, 128), F32),
            pltpu.VMEM((4, 32, 128), F32),
            pltpu.VMEM((S, D), BF16),
            pltpu.SemaphoreType.DMA((9 + len(U_HEAD) + U_N,)),
            pltpu.SemaphoreType.DMA((2,)),
        ],
        compiler_params=pltpu.CompilerParams(vmem_limit_bytes=120 * 1024 * 1024,
                                             disable_bounds_checks=True),
    )(
        A_x.reshape(S, D), A_wqkv, A_wo, B_x.reshape(NIT, BLK, D), B_mem0.reshape(B_M, D),
        feat_major(B_Wq), feat_major(B_Wk), feat_major(B_Wv), B_Wo.reshape(B_F, D),
    )
    return out.reshape(1, S, 2 * D)


def pallas_concat_heads__sliding_local_dilated__memory_aug_recurrent_mem_tr__prompt_kernel(
    A_x: jax.Array,
    A_wqkv: jax.Array,
    A_wo: jax.Array,
    B_x: jax.Array,
    B_mem0: jax.Array,
    B_Wq: jax.Array,
    B_Wk: jax.Array,
    B_Wv: jax.Array,
    B_Wo: jax.Array,
    B_seg_len,
):
    assert A_x.shape == (1, S, D) and B_x.shape == (1, S, D) and B_mem0.shape == (1, B_M, D)
    assert B_Wq.shape == (D, B_H, B_DH) and B_Wo.shape == (B_H, B_DH, D)
    if isinstance(B_seg_len, int):
        assert B_seg_len == B_SEG
    return _run(A_x, A_wqkv, A_wo, B_x, B_mem0, B_Wq, B_Wk, B_Wv, B_Wo)
```
